```python
import jax
import jax.numpy as jnp

def _softmax(x, axis=-1):
    return jax.nn.softmax(x, axis=axis)

def _gelu(x):
    return jax.nn.gelu(x, approximate=True)

def _silu(x):
    return jax.nn.silu(x)

def _sigmoid(x):
    return jax.nn.sigmoid(x)

def _layernorm(x, axis=-1, eps=1e-05):
    m = jnp.mean(x, axis=axis, keepdims=True)
    v = jnp.var(x, axis=axis, keepdims=True)
    return (x - m) / jnp.sqrt(v + eps)

def _scatter_add(tgt, idx, src, axis=0):
    return tgt.at[idx].add(src)

def _segment_sum(src, seg, n):
    return jax.ops.segment_sum(src, seg, n)

class _Rng:

    def __init__(self, key):
        self._k = key

    def _next(self):
        self._k, sub = jax.random.split(self._k)
        return sub

    def normal(self, shape):
        return jax.random.normal(self._next(), shape, dtype=jnp.bfloat16)

    def randint(self, lo, hi, shape):
        return jax.random.randint(self._next(), shape, lo, hi, dtype=jnp.int32)

    def uniform(self, shape, lo=0.0, hi=1.0):
        return jax.random.uniform(self._next(), shape, jnp.bfloat16, lo, hi)

    def permutation(self, n):
        return jax.random.permutation(self._next(), n)
kernel_name = 'adaLN_cond__ssm_conv_h3__glu_gated_bilinear__prompt'

def setup_inputs():
    _rng = _Rng(jax.random.key(int.from_bytes(__import__("os").urandom(4), "little")))
    _w = lambda a: (lambda t: t.astype(jnp.bfloat16) if jnp.issubdtype(t.dtype, jnp.floating) else t)(jnp.asarray(a))

    def _A_setup():
        B, S, D = (1, 2048, 640)
        ks = 4
        return {'q': _w((lambda *s: _rng.normal(s) * 0.05)(B, S, D)), 'k': _w((lambda *s: _rng.normal(s) * 0.05)(B, S, D)), 'v': _w((lambda *s: _rng.normal(s) * 0.05)(B, S, D)), 'shift_k': _w((lambda *s: _rng.normal(s) * 0.05)(D, ks) * 0.5), 'ssm_k': _w((lambda *s: _rng.normal(s) * 0.05)(D, S) * (1.0 / S ** 0.5)), 'ssm_D': _w((lambda *s: _rng.normal(s) * 0.05)(D))}
    _A_in = _A_setup()

    def _B_setup():
        B, S, D, F = (1, 2048, 640, 1536)
        return {'x': _w((lambda *s: _rng.normal(s) * 0.05)(B, S, D)), 'w_gate': _w((lambda *s: _rng.normal(s) * 0.05)(D, F) * D ** (-0.5)), 'w_up': _w((lambda *s: _rng.normal(s) * 0.05)(D, F) * D ** (-0.5)), 'w_down': _w((lambda *s: _rng.normal(s) * 0.05)(F, D) * F ** (-0.5))}
    _B_in = _B_setup()
    return {'A_q': _A_in['q'], 'A_k': _A_in['k'], 'A_v': _A_in['v'], 'A_shift_k': _A_in['shift_k'], 'A_ssm_k': _A_in['ssm_k'], 'A_ssm_D': _A_in['ssm_D'], 'B_x': _B_in['x'], 'B_w_gate': _B_in['w_gate'], 'B_w_up': _B_in['w_up'], 'B_w_down': _B_in['w_down'], 'c': _w((lambda *s: _rng.normal(s) * 0.05)(1, 640)), 'w_mod': _w((lambda *s: _rng.normal(s) * 0.05)(640, 6 * 640) * 640 ** (-0.5))}

def reference(A_q, A_k, A_v, A_shift_k, A_ssm_k, A_ssm_D, B_x, B_w_gate, B_w_up, B_w_down, c, w_mod):

    def _A_ref(q, k, v, shift_k, ssm_k, ssm_D):
        B, S, D = q.shape
        ks = shift_k.shape[-1]
        k_pad = jnp.pad(k, ((0, 0), (ks - 1, 0), (0, 0)))
        k_shift = jnp.zeros_like(k)
        for t in range(ks):
            k_shift = k_shift + k_pad[:, t:t + S, :] * shift_k[:, ks - 1 - t][None, None, :]
        kv = k_shift * v
        L = 2 * S
        kv_pad = jnp.pad(kv, ((0, 0), (0, S), (0, 0)))
        kf_pad = jnp.pad(ssm_k, ((0, 0), (0, S)))
        kv_f = (lambda x, axes=(-2, -1): jnp.fft.rfft2(x.astype(jnp.float32), axes=axes))(kv_pad[:, None, :, :], axes=(1, 2))
        kf_f = (lambda x, axes=(-2, -1): jnp.fft.rfft2(x.astype(jnp.float32), axes=axes))(kf_pad[:, None, :], axes=(1, 2))
        kf_f = (lambda x, *d: x.transpose(*d))(kf_f, 1, 2, 0)
        y_f = kv_f * kf_f[None, :, :, :]
        y = (lambda x, s, axes=(-2, -1): jnp.fft.irfft2(x, s=s, axes=axes).astype(jnp.bfloat16))(y_f, (1, L), axes=(1, 2))[:, 0, :S, :]
        y = y + kv * ssm_D[None, None, :]
        return q * y

    def _B_ref(x, w_gate, w_up, w_down):
        g = jnp.einsum('bsd,df->bsf', x, w_gate)
        u = jnp.einsum('bsd,df->bsf', x, w_up)
        h = g * u
        return jnp.einsum('bsf,fd->bsd', h, w_down)
    x = A_q
    mod = (_silu(c) @ w_mod).reshape(c.shape[0], 6, 1, -1)
    sa, ca, ga, sb, cb, gb = (mod[:, 0].copy(), mod[:, 1].copy(), mod[:, 2].copy(), mod[:, 3].copy(), mod[:, 4].copy(), mod[:, 5].copy())
    h = _layernorm(x, axis=-1) * (1 + ca) + sa
    x = x + ga * _A_ref(h, A_k, A_v, A_shift_k, A_ssm_k, A_ssm_D)
    h = _layernorm(x, axis=-1) * (1 + cb) + sb
    x = x + gb * _B_ref(h, B_w_gate, B_w_up, B_w_down)
    return x
```

```python
import functools

import numpy as np
import jax
import jax.numpy as jnp
from jax import lax
import jax.experimental.pallas as pl
import jax.experimental.pallas.tpu as pltpu

F32 = jnp.float32
BF16 = jnp.bfloat16
U32 = jnp.uint32

CB = 128
TM = 256
FC = 256
EPS = 1e-5
SCOPES = False
MAC_DIST = 2


def _dft_consts():
    k = np.arange(CB, dtype=np.float64)[:, None]
    n = np.arange(CB, dtype=np.float64)[None, :]
    th = np.pi * (4.0 * k + 1.0) * n / (2.0 * CB)
    fwd = np.concatenate([np.cos(th), np.sin(th)], axis=0)
    inv = fwd.T / CB
    return jnp.asarray(fwd, dtype=BF16), jnp.asarray(inv, dtype=BF16)


def _ln(x):
    m = jnp.mean(x, axis=-1, keepdims=True)
    xc = x - m
    v = jnp.mean(xc * xc, axis=-1, keepdims=True)
    return xc * lax.rsqrt(v + EPS)


def _pk(x):
    return pltpu.bitcast(x.astype(BF16), U32)


def _unpk(x):
    return pltpu.bitcast(x, BF16)


def _bc(x, row):
    return row


def _kernel(q_hbm, k_hbm, v_hbm, shk_hbm, ssmk_hbm, ssmd_hbm, wg_hbm, wu_hbm, wd_hbm,
            c_hbm, wmod_hbm, fwd_hbm, inv_hbm, o_hbm,
            u_ref, kk_ref, y_ref, x1_ref, q_ref, k_ref, v_ref, o_ref,
            x1s_ref, hp_ref, h2_ref, h2s_ref, hh_ref, kv_ref,
            wg2_ref, wu2_ref, wd2_ref,
            ssmk_ref, wmod_ref, wg_ref, wu_ref, wd_ref, fwd_ref, inv_ref,
            mod_ref, sh_ref, kbuf_ref, zm_ref, shk_ref, ssmd_ref, c_ref,
            sem,
            *, S, D, Fh):
    NB = S // CB
    NS = S // TM
    NL = D // 128
    NF = Fh // FC

    def scope(name):
        if SCOPES:
            return jax.named_scope(name)
        return functools.partial

    class _Sems:
        def __init__(self, base):
            self.base = base

        @property
        def at(self):
            return self

        def __getitem__(self, i):
            return sem.at[self.base + i]

    offs = np.cumsum([0, 5, NS, NS, NS, NL, 3, NF, NF, 1])
    sem_s, sem_q, sem_k, sem_v, sem_ssm, sem_mod, sem_g, sem_u, sem_d, sem_o = [_Sems(int(o)) for o in offs]

    def rows_cp(src, dst, sem, t):
        r = pl.ds(pl.multiple_of(t * TM, TM), TM) if not isinstance(t, int) else pl.ds(t * TM, TM)
        return pltpu.make_async_copy(src.at[r, :], dst.at[r, :], sem.at[t])

    q_cp = lambda t: rows_cp(q_hbm, q_ref, sem_q, t)
    k_cp = lambda t: rows_cp(k_hbm, k_ref, sem_k, t)
    v_cp = lambda t: rows_cp(v_hbm, v_ref, sem_v, t)
    o_cp = lambda t: rows_cp(o_ref, o_hbm, sem_o, t)
    small = [pltpu.make_async_copy(s, d, sem_s.at[i]) for i, (s, d) in enumerate(
        [(fwd_hbm, fwd_ref), (shk_hbm, shk_ref), (ssmd_hbm, ssmd_ref), (inv_hbm, inv_ref), (c_hbm, c_ref)])]
    ssm_cp = lambda i: pltpu.make_async_copy(
        ssmk_hbm.at[i * 128:(i + 1) * 128, :], ssmk_ref.at[i * 128:(i + 1) * 128, :], sem_ssm.at[i])
    mod_cols = [(0, 3 * D), (3 * D, 5 * D), (5 * D, 6 * D)]
    mod_cp = lambda i: pltpu.make_async_copy(
        wmod_hbm.at[:, mod_cols[i][0]:mod_cols[i][1]], wmod_ref.at[:, mod_cols[i][0]:mod_cols[i][1]],
        sem_mod.at[i])
    g_cp = lambda f: pltpu.make_async_copy(
        wg_hbm.at[:, f * FC:(f + 1) * FC], wg_ref.at[:, f * FC:(f + 1) * FC], sem_g.at[f])
    u_cp = lambda f: pltpu.make_async_copy(
        wu_hbm.at[:, f * FC:(f + 1) * FC], wu_ref.at[:, f * FC:(f + 1) * FC], sem_u.at[f])
    d_cp = pltpu.make_async_copy(wd_hbm, wd_ref, sem_d.at[0])

    order = [small[0], small[2], ssm_cp(0), small[1], small[3], small[4], ssm_cp(1), k_cp(0), v_cp(0),
             ssm_cp(2), k_cp(1), v_cp(1), ssm_cp(3), ssm_cp(4), q_cp(0), q_cp(1),
             mod_cp(0), mod_cp(1), g_cp(0), u_cp(0), k_cp(2), v_cp(2)]
    for f in range(1, NF):
        order += [g_cp(f), u_cp(f)]
    order += [q_cp(2), k_cp(3), v_cp(3), d_cp, mod_cp(2)]
    for t in range(3, NS):
        order += [q_cp(t)]
        if t + 1 < NS:
            order += [k_cp(t + 1), v_cp(t + 1)]
    for cp in order:
        cp.start()

    def rows_of(t, b=None):
        n = TM if b is None else CB
        off = 0 if b is None else b * CB
        if isinstance(t, int):
            return pl.ds(t * TM + off, n)
        return pl.ds(pl.multiple_of(t * TM + off, CB), n)

    def token(x):
        return pltpu.bitcast(pltpu.bitcast(x, jnp.int32) & zm_ref[...], F32)

    def modrow(i):
        return mod_ref[i, 0:1, :]

    def mod_chunk(i):
        c = c_ref[...].astype(F32)
        sc = jnp.broadcast_to((c * jax.nn.sigmoid(c)).astype(BF16), (16, D))
        lo, hi = mod_cols[i]
        m = jnp.dot(sc, wmod_ref[:, lo:hi], preferred_element_type=F32)[0:8]
        if i == 0:
            ga = m[:, 2 * D:3 * D]
            mod_ref[0] = (1.0 + m[:, D:2 * D]) * ga
            mod_ref[1] = m[:, 0:D] * ga
        elif i == 1:
            mod_ref[2] = 1.0 + m[:, D:2 * D]
            mod_ref[3] = m[:, 0:D]
        else:
            mod_ref[4] = m

    def k_fwd(i):
        ls = slice(i * 128, (i + 1) * 128)
        fwd = fwd_ref[...]
        prev = None
        for m in range(NB):
            kf = lax.dot_general(fwd, ssmk_ref[ls, m * CB:(m + 1) * CB], (((1,), (1,)), ((), ())),
                                 preferred_element_type=F32)
            if m == 0:
                c = kf[:CB] + ssmd_ref[...].astype(F32).reshape(1, D)[:, ls]
                d = kf[CB:]
            else:
                c = kf[:CB] + prev[CB:]
                d = kf[CB:] - prev[:CB]
            prev = kf
            kk_ref[m, 0:CB, ls] = c
            kk_ref[m, CB:2 * CB, ls] = d - c
            kk_ref[m, 2 * CB:3 * CB, ls] = c + d

    def pre_kv(t):
        r = rows_of(t)
        for i in range(NL):
            ls = slice(i * 128, (i + 1) * 128)
            kbuf_ref[i, 8:8 + TM, :] = k_ref[r, ls].astype(F32)
            ks = kbuf_ref[i, 8:8 + TM, :] * sh_ref[0:1, ls]
            for a in range(1, 4):
                ks = ks + kbuf_ref[i, 8 - a:8 - a + TM, :] * sh_ref[a:a + 1, ls]
            kv_ref[:, ls] = _pk(ks * v_ref[r, ls].astype(F32))
            kbuf_ref[i, 0:8, :] = kbuf_ref[i, TM:TM + 8, :]

    def pre_fwd(t):
        fwd = fwd_ref[...]
        for b in range(2):
            kv = _unpk(kv_ref[b * (CB // 2):(b + 1) * (CB // 2), :])
            uf = jnp.dot(fwd, kv, preferred_element_type=F32)
            a, bb = uf[:CB], uf[CB:]
            u_ref[t, b, 0:CB, :] = a + bb
            u_ref[t, b, CB:2 * CB, :] = a
            u_ref[t, b, 2 * CB:3 * CB, :] = bb

    def positions():
        for r0 in range(0, 3 * CB, 8):
            for l0 in range(0, D, 128):
                yield slice(r0, r0 + 8), slice(l0, l0 + 128)

    def y_init(s_lo, s_hi, n_u, dist=None):
        hist = []
        for rs, ls in positions():
            us = [u_ref[i // 2, i % 2, rs, ls] for i in range(n_u)]
            if dist is not None and len(hist) >= dist:
                tok = token(hist[-dist])
                us = [u + tok for u in us]
            ks = {}
            for s in range(s_lo, s_hi):
                acc = None
                for i in range(min(n_u, s + 1)):
                    m = s - i
                    if m not in ks:
                        ks[m] = kk_ref[m, rs, ls]
                    p = ks[m] * us[i]
                    acc = p if acc is None else acc + p
                y_ref[s // 2, s % 2, rs, ls] = acc
            hist.append(acc)

    def super_mac(J, I, dl, dist=None):
        diag = isinstance(dl, int) and dl == 0
        kview = kk_ref if diag else kk_ref.at[pl.ds(2 * dl - 1, 3)]
        hist = []
        for rs, ls in positions():
            u0 = u_ref[I, 0, rs, ls]
            u1 = u_ref[I, 1, rs, ls]
            if dist is not None and len(hist) >= dist:
                tok = token(hist[-dist])
                u0 = u0 + tok
                u1 = u1 + tok
            if diag:
                k0 = kview[0, rs, ls]
                y0 = k0 * u0
                y1 = kview[1, rs, ls] * u0 + k0 * u1
            else:
                k0 = kview[1, rs, ls]
                y0 = k0 * u0 + kview[0, rs, ls] * u1
                y1 = kview[2, rs, ls] * u0 + k0 * u1
            y1 = y1 + y_ref[J, 1, rs, ls]
            y_ref[J, 0, rs, ls] = y0 + y_ref[J, 0, rs, ls]
            y_ref[J, 1, rs, ls] = y1
            hist.append(y1)

    T0 = 3
    NLOOP = NS - T0

    def task(t, delta):
        p = t - delta
        left = p >= T0
        J = jnp.where(left, t, p + NLOOP)
        I = jnp.where(left, p, t)
        super_mac(J, I, J - I, MAC_DIST)

    def pre_ln1(t):
        for b in range(2):
            x = q_ref[rows_of(t, b), :].astype(F32)
            hp_ref[b * CB:(b + 1) * CB, :] = _ln(x) * modrow(0) + modrow(1)

    def pre_inv(t, x1_dst):
        inv = inv_ref[...]
        for b in range(2):
            k1 = y_ref[t, b, 0:CB, :]
            yre = (k1 - y_ref[t, b, 2 * CB:3 * CB, :]).astype(BF16)
            yim = (k1 + y_ref[t, b, CB:2 * CB, :]).astype(BF16)
            yy = jnp.concatenate([yre, yim], axis=0)
            y = jnp.dot(inv, yy, preferred_element_type=F32)
            rows = slice(b * CB, (b + 1) * CB)
            x1_dst[rows, :] = q_ref[rows_of(t, b), :].astype(F32) + hp_ref[rows, :] * y

    def pre_ln2(x1_src, h2_dst):
        G = 32
        for r0 in range(0, TM, G):
            x1 = x1_src[r0:r0 + G, :]
            h2_dst[r0 // 2:(r0 + G) // 2, :] = _pk(_ln(x1) * modrow(2) + modrow(3))

    def ffn_gu(f, h2_src, nrows, native):
        cols = slice(f * FC, (f + 1) * FC)
        h2 = _unpk(h2_src[...])
        if native:
            wg = wg_ref[:, cols]
            wu = wu_ref[:, cols]
            wg2_ref[:, cols] = pltpu.bitcast(wg, U32)
            wu2_ref[:, cols] = pltpu.bitcast(wu, U32)
        else:
            wg = _unpk(wg2_ref[:, cols])
            wu = _unpk(wu2_ref[:, cols])
        g = jnp.dot(h2, wg, preferred_element_type=F32)
        u = jnp.dot(h2, wu, preferred_element_type=F32)
        hh_ref[0:nrows // 2, cols] = _pk(g * u)

    def ffn_down(r0, nrows, x1_src, out_rows, native):
        if native:
            wd = wd_ref[...]
            wd2_ref[...] = pltpu.bitcast(wd, U32)
        else:
            wd = _unpk(wd2_ref[...])
        hh = _unpk(hh_ref[r0 // 2:(r0 + nrows) // 2, :])
        dn = jnp.dot(hh, wd, preferred_element_type=F32)
        o_ref[out_rows, :] = (x1_src[r0:r0 + nrows, :] + modrow(4) * dn).astype(o_ref.dtype)

    def prologue():
        small[0].wait()
        small[2].wait()
        ssm_cp(0).wait()
        k_fwd(0)
        small[1].wait()
        small[3].wait()
        small[4].wait()
        sh_ref[0:4, :] = shk_ref[...].astype(F32)
        zm_ref[...] = pltpu.bitcast(jnp.broadcast_to(inv_ref[0:1, CB:2 * CB].astype(F32), (8, 128)), jnp.int32)
        kbuf_ref[:, 0:8, :] = jnp.zeros((NL, 8, 128), F32)
        ssm_cp(1).wait()
        k_fwd(1)
        k_cp(0).wait()
        v_cp(0).wait()
        ssm_cp(2).wait()
        pre_kv(0)
        k_fwd(2)
        pre_fwd(0)
        k_cp(1).wait()
        v_cp(1).wait()
        ssm_cp(3).wait()
        pre_kv(1)
        k_fwd(3)
        pre_fwd(1)
        ssm_cp(4).wait()
        k_fwd(4)
        y_init(0, 4, 4)
        q_cp(0).wait()
        q_cp(1).wait()
        mod_cp(0).wait()
        mod_chunk(0)
        for t in range(2):
            pre_ln1(t)
            pre_inv(t, x1s_ref.at[t * TM:(t + 1) * TM])
        mod_cp(1).wait()
        mod_chunk(1)
        for t in range(2):
            pre_ln2(x1s_ref.at[t * TM:(t + 1) * TM], h2s_ref.at[t * (TM // 2):(t + 1) * (TM // 2)])

    def superstep():
        gu = lambda f: ffn_gu(f, h2s_ref, 2 * TM, True)
        g_cp(0).wait()
        u_cp(0).wait()
        gu(0)
        k_cp(2).wait()
        v_cp(2).wait()
        g_cp(1).wait()
        u_cp(1).wait()
        pre_kv(2)
        gu(1)
        pre_fwd(2)
        for f in range(2, 4):
            g_cp(f).wait()
            u_cp(f).wait()
        y_init(4, 8, 6, 1)
        gu(2)
        gu(3)
        for f in range(4, NF):
            g_cp(f).wait()
            u_cp(f).wait()
        q_cp(2).wait()
        k_cp(3).wait()
        v_cp(3).wait()
        y_init(8, 12, 6, 1)
        gu(4)
        pre_ln1(2)
        pre_kv(3)
        gu(5)
        d_cp.wait()
        mod_cp(2).wait()
        mod_chunk(2)
        pre_inv(2, x1_ref.at[0])
        pre_ln2(x1_ref.at[0], h2_ref)
        y_init(12, NB, 6, 1)
        ffn_down(0, 2 * TM, x1s_ref, pl.ds(0, 2 * TM), True)
        o_cp(0).start()
        o_cp(1).start()

    def step(t, carry):
        slot = lax.rem(t, 2)
        q_cp(t).wait()

        @pl.when(t + 1 < NS)
        def _():
            k_cp(t + 1).wait()
            v_cp(t + 1).wait()

        pre_fwd(t)
        ffn_gu(0, h2_ref, TM, False)
        super_mac(t, t, 0, MAC_DIST)
        ffn_gu(1, h2_ref, TM, False)
        task(t, 2)
        ffn_gu(2, h2_ref, TM, False)
        task(t, 1)
        ffn_gu(3, h2_ref, TM, False)
        pre_ln1(t)
        ffn_gu(4, h2_ref, TM, False)
        pre_kv(jnp.minimum(t + 1, NS - 1))
        ffn_gu(5, h2_ref, TM, False)
        pre_inv(t, x1_ref.at[slot])
        pre_ln2(x1_ref.at[slot], h2_ref)
        ffn_down(0, TM, x1_ref.at[1 - slot], rows_of(t - 1), False)
        o_cp(t - 1).start()
        return carry

    def epilogue():
        t = NS - 1
        for f in range(NF):
            ffn_gu(f, h2_ref, TM, False)
        x1 = x1_ref.at[t % 2]
        ffn_down(0, TM, x1, rows_of(t), False)
        o_cp(t).start()
        for i in range(NS):
            o_cp(i).wait()

    if SCOPES:
        jax.named_scope("prologue")(prologue)()
        jax.named_scope("superstep")(superstep)()
        lax.fori_loop(T0, NS, jax.named_scope("step")(step), 0)
        jax.named_scope("epilogue")(epilogue)()
    else:
        prologue()
        superstep()
        lax.fori_loop(T0, NS, step, 0)
        epilogue()


@jax.jit
def pallas_adaLN_cond__ssm_conv_h3__glu_gated_bilinear__prompt_kernel(
    A_q, A_k, A_v, A_shift_k, A_ssm_k, A_ssm_D, B_x, B_w_gate, B_w_up, B_w_down, c, w_mod,
):
    B, S, D = A_q.shape
    Fh = B_w_gate.shape[1]
    NB = S // CB
    NS = S // TM
    fwd, inv = _dft_consts()
    anyspec = pl.BlockSpec(memory_space=pl.ANY)
    V = pltpu.VMEM
    dma = pltpu.SemaphoreType.DMA
    out = pl.pallas_call(
        functools.partial(_kernel, S=S, D=D, Fh=Fh),
        in_specs=[anyspec] * 13,
        out_specs=anyspec,
        out_shape=jax.ShapeDtypeStruct((S, D), A_q.dtype),
        scratch_shapes=[
            V((NS, 2, 3 * CB, D), F32),
            V((NB, 3 * CB, D), F32),
            V((NS, 2, 3 * CB, D), F32),
            V((2, TM, D), F32),
            V((S, D), BF16), V((S, D), BF16), V((S, D), BF16), V((S, D), BF16),
            V((2 * TM, D), F32),
            V((TM, D), F32),
            V((TM // 2, D), U32),
            V((TM, D), U32),
            V((TM, Fh), U32),
            V((TM // 2, D), U32),
            V((D // 2, Fh), U32), V((D // 2, Fh), U32), V((Fh // 2, D), U32),
            V((D, S), BF16), V((D, 6 * D), BF16), V((D, Fh), BF16), V((D, Fh), BF16), V((Fh, D), BF16),
            V((2 * CB, CB), BF16), V((CB, 2 * CB), BF16),
            V((5, 8, D), F32), V((8, D), F32), V((D // 128, TM + 8, 128), F32), V((8, 128), jnp.int32),
            V((4, D), BF16), V((D,), BF16), V((1, D), BF16),
            dma((5 + 4 * NS + D // 128 + 3 + 2 * (Fh // FC) + 1,)),
        ],
        compiler_params=pltpu.CompilerParams(
            internal_scratch_in_bytes=48 * 1024,
            disable_semaphore_checks=True,
            vmem_limit_bytes=110 * 1024 * 1024),
        name="adaln_h3_glu",
    )(A_q.reshape(S, D), A_k.reshape(S, D), A_v.reshape(S, D), A_shift_k.T, A_ssm_k,
      A_ssm_D, B_w_gate, B_w_up, B_w_down, c, w_mod, fwd, inv)
    return out.reshape(B, S, D)
```

```python
import functools
import os

import numpy as np
import jax
import jax.numpy as jnp
from jax import lax
import jax.experimental.pallas as pl
import jax.experimental.pallas.tpu as pltpu

F32 = jnp.float32
BF16 = jnp.bfloat16
U32 = jnp.uint32
I32 = jnp.int32

CB = 128
HB = CB // 2
TM = 256
FC = 256
KS = 256
EPS = 1e-5
SCOPES = False
LNP = int(os.environ.get('LNP', 0))
JOIN = int(os.environ.get('JOIN', 0))
ONLY = os.environ.get('ONLY', '')
LV = os.environ.get('LV', 'b')
YSPLIT = 200
MAC_DIST = int(os.environ.get('MD', 3))
DIAG_DIST = int(os.environ.get('DD', 2))


def _dft_consts():
    k = np.arange(CB, dtype=np.float64)[:, None]
    n = np.arange(CB, dtype=np.float64)[None, :]
    th = np.pi * (4.0 * k + 1.0) * n / (2.0 * CB)
    fwd = np.concatenate([np.cos(th), np.sin(th)], axis=0)
    g = np.concatenate([np.cos(th[:HB]), np.sin(th[:HB])], axis=0).T / CB
    inv = np.concatenate([g[0::2], g[1::2], np.zeros((16, CB))], axis=0)
    return jnp.asarray(fwd, dtype=BF16), jnp.asarray(inv, dtype=BF16)


def _pk(x):
    return pltpu.bitcast(x.astype(BF16), U32)


def _unpk(x):
    return pltpu.bitcast(x, BF16)


def _dot(a, b):
    return jnp.dot(a, b, preferred_element_type=F32)


def _rep(r, n):
    return r if n == 8 else jnp.concatenate([r] * (n // 8), axis=0)


def _kernel(q_hbm, k_hbm, v_hbm, shk_hbm, ssmk_hbm, ssmd_hbm, wg_hbm, wu_hbm, wd_hbm,
            c_hbm, wmod_hbm, fwd_hbm, inv_hbm, o_hbm,
            u_ref, kk_ref, y_ref, x1_ref, q_ref, k_ref, v_ref, o_ref,
            x1s_ref, hp_ref, h2_ref, h2c_ref, hh_ref, hhc_ref, kv_ref, yb_ref,
            wgr_ref, wur_ref, wdr_ref, wgc_ref, wuc_ref, wdc_ref,
            ssmk_ref, wmod_ref, wg_ref, wu_ref, wd_ref, fwd_ref, inv_ref,
            mod_ref, sh_ref, kbuf_ref, zm_ref, tka_ref, tkb_ref, shk_ref, ssmd_ref, c_ref,
            sem, *, S, D, Fh):
    NB = S // CB
    NS = S // TM
    NL = D // 128
    NF = Fh // FC
    lanes = [slice(i * 128, (i + 1) * 128) for i in range(NL)]

    offs = [int(o) for o in np.cumsum([0, 5, NS, NS, NS, NL, 3, NF, NF, 1])]
    s_small, s_q, s_k, s_v, s_ssm, s_mod, s_g, s_u, s_d, s_o = offs

    def rows_of(t, b=None):
        n = TM if b is None else CB
        off = 0 if b is None else b * CB
        if isinstance(t, int):
            return pl.ds(t * TM + off, n)
        return pl.ds(pl.multiple_of(t * TM + off, CB), n)

    def rows_cp(src, dst, base, t):
        return pltpu.make_async_copy(src.at[rows_of(t), :], dst.at[rows_of(t), :], sem.at[base + t])

    def cols_cp(src, dst, lo, hi, si):
        return pltpu.make_async_copy(src.at[:, lo:hi], dst.at[:, lo:hi], sem.at[si])

    q_cp = lambda t: rows_cp(q_hbm, q_ref, s_q, t)
    k_cp = lambda t: rows_cp(k_hbm, k_ref, s_k, t)
    v_cp = lambda t: rows_cp(v_hbm, v_ref, s_v, t)
    o_cp = lambda t: rows_cp(o_ref, o_hbm, s_o, t)
    small = [pltpu.make_async_copy(s, d, sem.at[s_small + i]) for i, (s, d) in enumerate(
        [(fwd_hbm, fwd_ref), (shk_hbm, shk_ref), (ssmd_hbm, ssmd_ref), (inv_hbm, inv_ref), (c_hbm, c_ref)])]
    ssm_cp = lambda i: pltpu.make_async_copy(ssmk_hbm.at[lanes[i], :], ssmk_ref.at[lanes[i], :],
                                             sem.at[s_ssm + i])
    mod_cols = [(0, 3 * D), (3 * D, 5 * D), (5 * D, 6 * D)]
    mod_cp = lambda i: cols_cp(wmod_hbm, wmod_ref, mod_cols[i][0], mod_cols[i][1], s_mod + i)
    g_cp = lambda f: cols_cp(wg_hbm, wg_ref, f * FC, (f + 1) * FC, s_g + f)
    u_cp = lambda f: cols_cp(wu_hbm, wu_ref, f * FC, (f + 1) * FC, s_u + f)
    d_cp = pltpu.make_async_copy(wd_hbm, wd_ref, sem.at[s_d])

    order = [small[0], small[2], ssm_cp(0), small[1], small[3], small[4], ssm_cp(1), k_cp(0), v_cp(0),
             ssm_cp(2), k_cp(1), v_cp(1), ssm_cp(3), ssm_cp(4), q_cp(0), q_cp(1),
             mod_cp(0), mod_cp(1), g_cp(0), u_cp(0), k_cp(2), v_cp(2)]
    for f in range(1, NF):
        order += [g_cp(f), u_cp(f)]
    order += [d_cp, q_cp(2), mod_cp(2), k_cp(3), v_cp(3)]
    for t in range(3, NS):
        order += [q_cp(t)]
        if t + 1 < NS:
            order += [k_cp(t + 1), v_cp(t + 1)]
    for cp in order:
        cp.start()

    zs = []

    def token(x, extra=0):
        if x is None:
            return None
        tok = pltpu.bitcast(pltpu.bitcast(x, I32) & zm_ref[...], F32)
        for _ in range(extra):
            tok = tok + tok
        return tok

    def opaque(ref):
        return ref.at[pl.ds(pl.multiple_of(zs[0], 32), ref.shape[0])]

    def tokn(x):
        return _rep(token(x[0:8], LNP - 1), x.shape[0])

    def relay(ref, x=None):
        ref[...] = jnp.zeros((8, 128), F32) if x is None else x
        return opaque(ref)[...]

    def fold8(x):
        acc = x[0:8]
        for r in range(8, x.shape[0], 8):
            acc = acc + x[r:r + 8]
        return acc

    def mod_chunk(i):
        c = c_ref[...].astype(F32)
        sc = jnp.broadcast_to((c * jax.nn.sigmoid(c)).astype(BF16), (16, D))
        lo, hi = mod_cols[i]
        m = _dot(sc, wmod_ref[:, lo:hi])[0:8]
        if i == 0:
            ga = m[:, 2 * D:3 * D]
            mod_ref[0] = (1.0 + m[:, D:2 * D]) * ga
            mod_ref[1] = m[:, 0:D] * ga
        elif i == 1:
            mod_ref[2] = 1.0 + m[:, D:2 * D]
            mod_ref[3] = m[:, 0:D]
        else:
            mod_ref[4] = m

    def k_fwd(i):
        ls = lanes[i]
        fwd = fwd_ref[...]
        prev = None
        for m in range(NB):
            kf = lax.dot_general(fwd, ssmk_ref[ls, m * CB:(m + 1) * CB], (((1,), (1,)), ((), ())),
                                 preferred_element_type=F32)
            if m == 0:
                c = kf[:CB] + ssmd_ref[...].astype(F32).reshape(1, D)[:, ls]
                d = kf[CB:]
            else:
                c = kf[:CB] + prev[CB:]
                d = kf[CB:] - prev[:CB]
            prev = kf
            kk_ref[m, 0:CB, ls] = c
            kk_ref[m, CB:2 * CB, ls] = d - c
            kk_ref[m, 2 * CB:3 * CB, ls] = c + d

    def pre_kv(t, dep=None, paced=False):
        G = 32 if paced else 64
        for i, ls in enumerate(lanes):
            for r0 in range(0, TM, G):
                if isinstance(t, int):
                    r = pl.ds(t * TM + r0, G)
                else:
                    r = pl.ds(pl.multiple_of(t * TM + r0, G), G)
                kf = k_ref[r, ls].astype(F32)
                if dep is not None:
                    kf = kf + _rep(token(dep, 1), G)
                kbuf_ref[i, 8 + r0:8 + r0 + G, :] = kf
                ks = kf * _rep(sh_ref[0, :, ls], G)
                for a in range(1, 4):
                    ks = ks + kbuf_ref[i, 8 + r0 - a:8 + r0 - a + G, :] * _rep(sh_ref[a, :, ls], G)
                kv = ks * v_ref[r, ls].astype(F32)
                kv_ref[r0 // 2:(r0 + G) // 2, ls] = _pk(kv)
                if paced:
                    dep = kv[G - 8:G]
            kbuf_ref[i, 0:8, :] = kbuf_ref[i, TM:TM + 8, :]
        return dep

    def pre_fwd(t, staged=False):
        fwd = fwd_ref[...]
        kv = opaque(kv_ref) if staged else kv_ref
        for b in range(2):
            uf = _dot(fwd, _unpk(kv[b * HB:(b + 1) * HB, :]))
            a, bb = uf[:CB], uf[CB:]
            u_ref[t, b, 0:CB, :] = a + bb
            u_ref[t, b, CB:2 * CB, :] = a
            u_ref[t, b, 2 * CB:3 * CB, :] = bb
        return uf[2 * CB - 8:, D - 128:]

    def positions():
        for r0 in range(0, 3 * CB, 8):
            for ls in lanes:
                yield slice(r0, r0 + 8), ls

    def y_static(s_lo, s_hi, i_lo, i_hi, acc_in, dist=None, extra=0, dep=None, prange=None):
        hist = [] if dep is None else [dep] * dist
        pos = list(positions())
        if prange is not None:
            pos = pos[prange[0]:prange[1]]
        for rs, ls in pos:
            us = {i: u_ref[i // 2, i % 2, rs, ls] for i in range(i_lo, i_hi)}
            if dist is not None and len(hist) >= dist:
                tok = token(hist[-dist], extra)
                us = {i: u + tok for i, u in us.items()}
            ks = {}
            for s in range(s_lo, s_hi):
                acc = None
                for i in range(i_lo, min(i_hi, s + 1)):
                    m = s - i
                    if m not in ks:
                        ks[m] = kk_ref[m, rs, ls]
                    p = ks[m] * us[i]
                    acc = p if acc is None else acc + p
                if acc_in:
                    acc = acc + y_ref[s // 2, s % 2, rs, ls]
                y_ref[s // 2, s % 2, rs, ls] = acc
            hist.append(acc)
        return hist[-1]

    def super_mac(J, I, dl, dist):
        diag = isinstance(dl, int) and dl == 0
        kview = kk_ref if diag else kk_ref.at[pl.ds(2 * dl - 1, 3)]
        hist = []
        for rs, ls in positions():
            u0 = u_ref[I, 0, rs, ls]
            u1 = u_ref[I, 1, rs, ls]
            if len(hist) >= dist:
                tok = token(hist[-dist])
                u0 = u0 + tok
                u1 = u1 + tok
            if diag:
                k0 = kview[0, rs, ls]
                y0 = k0 * u0
                y1 = kview[1, rs, ls] * u0 + k0 * u1
            else:
                k0 = kview[1, rs, ls]
                y0 = k0 * u0 + kview[0, rs, ls] * u1
                y1 = kview[2, rs, ls] * u0 + k0 * u1
            y1 = y1 + y_ref[J, 1, rs, ls]
            y_ref[J, 0, rs, ls] = y0 + y_ref[J, 0, rs, ls]
            y_ref[J, 1, rs, ls] = y1
            hist.append(y1)
        return hist[-1]

    def diag_mac(t, I, dist, dep=None):
        kview = kk_ref.at[pl.ds(2 * (t - I) - 1, 3)]
        hist = [] if dep is None else [dep] * dist
        for rs, ls in positions():
            us = [u_ref[t, 0, rs, ls], u_ref[t, 1, rs, ls], u_ref[I, 0, rs, ls], u_ref[I, 1, rs, ls]]
            if len(hist) >= dist:
                tok = token(hist[-dist])
                us = [u + tok for u in us]
            k0 = kk_ref[0, rs, ls]
            kc = kview[1, rs, ls]
            y0 = (k0 * us[0] + y_ref[t, 0, rs, ls]) + (kc * us[2] + kview[0, rs, ls] * us[3])
            y1 = ((kk_ref[1, rs, ls] * us[0] + k0 * us[1]) + (kview[2, rs, ls] * us[2] + kc * us[3])
                  + y_ref[t, 1, rs, ls])
            y_ref[t, 0, rs, ls] = y0
            y_ref[t, 1, rs, ls] = y1
            hist.append(y1)
        return hist[-1]

    T0 = 3
    NLOOP = NS - T0

    def task(t, delta):
        p = t - delta
        left = p >= T0
        J = jnp.where(left, t, p + NLOOP)
        I = jnp.where(left, p, t)
        return super_mac(J, I, J - I, MAC_DIST)

    def pre_post(t, dep=None, paced=False):
        for b in range(2):
            for r0 in range(0, HB, 16):
                for ls in lanes:
                    def comp(c, off):
                        return y_ref[t, b, c * CB + off + r0:c * CB + off + r0 + 16, ls]
                    k1l, k1h = comp(0, 0), comp(0, HB)
                    if dep is not None:
                        tok = _rep(token(dep, 3), 16)
                        k1l = k1l + tok
                        k1h = k1h + tok
                    rel, reh = k1l - comp(2, 0), k1h - comp(2, HB)
                    iml, imh = k1l + comp(1, 0), k1h + comp(1, HB)
                    p0 = b * CB + r0 // 2
                    oim = iml - imh
                    yb_ref[p0:p0 + 8, ls] = _pk(rel + reh)
                    yb_ref[p0 + HB // 2:p0 + HB // 2 + 8, ls] = _pk(iml + imh)
                    yb_ref[p0 + HB:p0 + HB + 8, ls] = _pk(rel - reh)
                    yb_ref[p0 + HB + HB // 2:p0 + HB + HB // 2 + 8, ls] = _pk(oim)
                    if paced:
                        dep = oim[8:16]
        return dep

    def q_split(t, b, p0, n, ls):
        if isinstance(t, int):
            r = pl.ds(t * TM + b * CB + 2 * p0, 2 * n)
        else:
            r = pl.ds(pl.multiple_of(t * TM + b * CB + 2 * p0, 16), 2 * n)
        w = pltpu.bitcast(q_ref[r, ls], U32)
        return pltpu.bitcast(w << 16, F32), pltpu.bitcast(w & jnp.uint32(0xFFFF0000), F32)

    def ln_tiles(xs, tok):
        n = xs[0].shape[0]
        s = xs[0]
        for x in xs[1:]:
            s = s + x
        if tok is not None:
            s = s + _rep(tok, n)
        m = jnp.sum(s, axis=-1, keepdims=True) * (1.0 / D)
        xc = [x - m for x in xs]
        s2 = xc[0] * xc[0]
        for x in xc[1:]:
            s2 = s2 + x * x
        r = lax.rsqrt(jnp.sum(s2, axis=-1, keepdims=True) * (1.0 / D) + EPS)
        return xc, jnp.broadcast_to(r, (n, 128))

    def pre_ln1(t, dep=None, paced=False):
        G = 16
        for b in range(2):
            for p0 in range(0, HB, G):
                eo = [q_split(t, b, p0, G, ls) for ls in lanes]
                xs = [jnp.concatenate([e, o], axis=0) for e, o in eo]
                xc, r = ln_tiles(xs, token(dep))
                h = None
                for ls, x in zip(lanes, xc):
                    if paced and LNP and h is not None:
                        r = r + tokn(h)
                    h = (x * r) * _rep(mod_ref[0, :, ls], 2 * G) + _rep(mod_ref[1, :, ls], 2 * G)
                    hp_ref[b * CB + p0:b * CB + p0 + G, ls] = h[:G]
                    hp_ref[b * CB + HB + p0:b * CB + HB + p0 + G, ls] = h[G:]
                if paced:
                    dep = fold8(h)
        return dep

    def pre_inv(t, x1_dst):
        yb = opaque(yb_ref)
        hp = opaque(hp_ref)
        for b in range(2):
            ye = _dot(inv_ref[0:HB, :], _unpk(yb[b * CB:b * CB + HB, :]))
            yo = _dot(inv_ref[HB:CB, :], _unpk(yb[b * CB + HB:(b + 1) * CB, :]))
            for ls in lanes:
                qe, qo = q_split(t, b, 0, HB, ls)
                re, ro = slice(b * CB, b * CB + HB), slice(b * CB + HB, (b + 1) * CB)
                x1_dst[re, ls] = qe + hp[re, ls] * ye[:, ls]
                x1_dst[ro, ls] = qo + hp[ro, ls] * yo[:, ls]

    def a_combos(a11, a12, a21, a22):
        return [a11 + a22, a21 + a22, a11 + a12, a21 - a11, a12 - a22]

    def b_combos(b11, b12, b21, b22):
        return [b11 + b22, b12 - b22, b21 - b11, b11 + b12, b21 + b22]

    def pre_ln2(x1_src, unit, paced=False):
        G = 16
        dep = None
        x1_src = opaque(x1_src)
        h2_dst = h2_ref.at[unit * CB:(unit + 1) * CB]
        h2c_dst = h2c_ref.at[unit * 5 * HB:(unit + 1) * 5 * HB]
        for r0 in range(0, CB, G):
            xs = [jnp.concatenate([x1_src[r0:r0 + G, ls], x1_src[CB + r0:CB + r0 + G, ls]], axis=0)
                  for ls in lanes]
            xc, r = ln_tiles(xs, token(dep))
            pr = slice(r0 // 2, (r0 + G) // 2)
            pb = slice((CB + r0) // 2, (CB + r0 + G) // 2)
            nk = KS // 128
            hs = {}
            h = None
            for j in [x for jj in range(nk) for x in (jj, nk + jj)] + list(range(2 * nk, NL)):
                ls = lanes[j]
                if paced and LNP and h is not None:
                    r = r + tokn(h)
                h = (xc[j] * r) * _rep(mod_ref[2, :, ls], 2 * G) + _rep(mod_ref[3, :, ls], 2 * G)
                hs[j] = h
                h2_dst[pr, ls] = _pk(h[:G])
                h2_dst[pb, ls] = _pk(h[G:])
                if nk <= j < 2 * nk:
                    cs = a_combos(hs[j - nk][:G], h[:G], hs[j - nk][G:], h[G:])
                    for i, cmb in enumerate(cs):
                        h2c_dst[i * HB + r0 // 2:i * HB + (r0 + G) // 2, lanes[j - nk]] = _pk(cmb)
            if paced:
                dep = fold8(h)
        return dep

    def strassen(sa, a11, a22, tb, b11, b22, rem):
        if rem is None:
            m1 = _dot(sa[0], tb[0])
            m7 = _dot(sa[4], tb[4])
            m4 = _dot(a22, tb[2])
            m2 = _dot(sa[1], b11)
            c21 = m2 + m4
            m5 = _dot(sa[2], b22)
            c11 = m1 + m7 + m4 - m5
            m3 = _dot(a11, tb[1])
            c12 = m3 + m5
            m6 = _dot(sa[3], tb[3])
        else:
            at, ab, bl, br = rem
            cat = jnp.concatenate
            m1 = _dot(sa[0], tb[0])
            m7 = _dot(cat([sa[4], at], axis=1), cat([tb[4], bl], axis=0))
            m4 = _dot(a22, tb[2])
            m2 = _dot(sa[1], b11)
            c21 = m2 + m4 + _dot(ab, bl)
            m5 = _dot(sa[2], b22)
            c11 = m1 + m7 + m4 - m5
            m3 = _dot(a11, tb[1])
            c12 = m3 + m5 + _dot(at, br)
            m6 = _dot(cat([sa[3], ab], axis=1), cat([tb[3], br], axis=0))
        c22 = m1 - m2 + m3 + m6
        return c11, c12, c21, c22

    def w_combos_gu(f, dep=None):
        G = 16
        cl, cr = slice(f * FC, f * FC + 128), slice(f * FC + 128, (f + 1) * FC)
        for w_ref, wc_ref, wr_ref in ((wg_ref, wgc_ref, wgr_ref), (wu_ref, wuc_ref, wur_ref)):
            wr_ref[:, f * FC:(f + 1) * FC] = pltpu.bitcast(w_ref[2 * KS:D, f * FC:(f + 1) * FC], U32)
            for r0 in range(0, KS, G):
                b11 = w_ref[r0:r0 + G, cl].astype(F32)
                b22 = w_ref[KS + r0:KS + r0 + G, cr].astype(F32)
                if dep is not None:
                    tok = _rep(token(dep), G)
                    b11 = b11 + tok
                    b22 = b22 + tok
                cs = b_combos(b11, w_ref[r0:r0 + G, cr].astype(F32), w_ref[KS + r0:KS + r0 + G, cl].astype(F32), b22)
                for i, cmb in enumerate(cs + [b11, b22]):
                    wc_ref[(i * KS + r0) // 2:(i * KS + r0 + G) // 2, f * 128:(f + 1) * 128] = _pk(cmb)
                dep = opaque(wc_ref)[r0 // 2:r0 // 2 + 8, f * 128:(f + 1) * 128]
        return dep

    def w_combos_down(dep=None):
        G = 16
        for j in range(KS // 128):
            cl, cr = lanes[j], lanes[KS // 128 + j]
            for f in range(NF):
                for r0 in range(0, 128, G):
                    re = slice(f * FC + r0, f * FC + r0 + G)
                    ro = slice(f * FC + 128 + r0, f * FC + 128 + r0 + G)
                    b11 = wd_ref[re, cl].astype(F32)
                    b22 = wd_ref[ro, cr].astype(F32)
                    if dep is not None:
                        tok = _rep(token(dep), G)
                        b11 = b11 + tok
                        b22 = b22 + tok
                    cs = b_combos(b11, wd_ref[re, cr].astype(F32), wd_ref[ro, cl].astype(F32), b22)
                    for i, cmb in enumerate(cs + [b11, b22]):
                        p0 = i * (Fh // 4) + (f * 128 + r0) // 2
                        wdc_ref[p0:p0 + G // 2, cl] = _pk(cmb)
                    dep = opaque(wdc_ref)[p0:p0 + 8, cl]
        return dep

    def ffn_gu(f, unit, hunit, plain=False, staged=False):
        cl, cr = slice(f * FC, f * FC + 128), slice(f * FC + 128, (f + 1) * FC)
        h2 = h2_ref.at[unit * CB:(unit + 1) * CB]
        h2c = h2c_ref.at[unit * 5 * HB:(unit + 1) * 5 * HB]
        if plain:
            cols = slice(f * FC, (f + 1) * FC)
            x = _unpk(h2[...])
            p = _dot(x, wg_ref[:, cols]) * _dot(x, wu_ref[:, cols])
            p11, p12, p21, p22 = p[:CB, :128], p[:CB, 128:], p[CB:, :128], p[CB:, 128:]
        else:
            res = []
            for wr, wc in ((wgr_ref, wgc_ref), (wur_ref, wuc_ref)):
                if staged:
                    wr, wc = opaque(wr), opaque(wc)
                sa = [_unpk(h2c[i * HB:(i + 1) * HB, :]) for i in range(5)]
                a11 = _unpk(h2[0:HB, 0:KS])
                a22 = _unpk(h2[HB:CB, KS:2 * KS])
                at = _unpk(h2[0:HB, 2 * KS:D])
                ab = _unpk(h2[HB:CB, 2 * KS:D])
                tb = [_unpk(wc[i * KS // 2:(i + 1) * KS // 2, f * 128:(f + 1) * 128]) for i in range(7)]
                res.append(strassen(sa, a11, a22, tb, tb[5], tb[6], (at, ab, _unpk(wr[:, cl]), _unpk(wr[:, cr]))))
            p11, p12, p21, p22 = [g * u for g, u in zip(*res)]
        hh = hh_ref.at[hunit * CB:(hunit + 1) * CB]
        hhc = hhc_ref.at[hunit * 5 * HB:(hunit + 1) * 5 * HB]
        hh[0:HB, cl] = _pk(p11)
        hh[0:HB, cr] = _pk(p12)
        hh[HB:CB, cl] = _pk(p21)
        hh[HB:CB, cr] = _pk(p22)
        for i, cmb in enumerate(a_combos(p11, p12, p21, p22)):
            hhc[i * HB:(i + 1) * HB, f * 128:(f + 1) * 128] = _pk(cmb)

    def emit_out(dn, x1_src, r0, row0, ls):
        o = x1_src[r0:r0 + CB, ls] + _rep(mod_ref[4, :, ls], CB) * dn
        w = pltpu.pack_elementwise([o[:HB], o[HB:]], packed_dtype=BF16)
        o_ref[pl.ds(row0, CB), ls] = pltpu.bitcast(w, BF16)

    def out_row(t, b):
        return t * TM + b * CB if isinstance(t, int) else pl.multiple_of(t * TM + b * CB, CB)

    def ffn_down_rem(x1_src, t, hunit, native=False, keep=False, dep=None):
        ls = lanes[NL - 1]
        if native:
            wd = wd_ref[:, ls]
            if keep:
                wdr_ref[...] = pltpu.bitcast(wd, U32)
        elif dep is None:
            wd = _unpk(wdr_ref[...])
        else:
            j0 = JOIN * 64
            parts = [wdr_ref[0:j0, :], wdr_ref[j0:j0 + 8, :] | pltpu.bitcast(token(dep), U32), wdr_ref[j0 + 8:, :]]
            wd = _unpk(jnp.concatenate(parts, axis=0))
        dn = _dot(_unpk(hh_ref[hunit * CB:(hunit + 1) * CB, :]), wd)
        for b in range(2):
            emit_out(dn[b * CB:(b + 1) * CB], x1_src, b * CB, out_row(t, b), ls)

    def ffn_down_main(x1_src, t, hunit, j, staged=False):
        cat = jnp.concatenate
        nk = KS // 128
        hh = hh_ref.at[hunit * CB:(hunit + 1) * CB]
        hhc = hhc_ref.at[hunit * 5 * HB:(hunit + 1) * 5 * HB]
        wc = opaque(wdc_ref) if staged else wdc_ref
        cl, cr = lanes[j], lanes[nk + j]
        sa = [_unpk(hhc[i * HB:(i + 1) * HB, :]) for i in range(5)]
        a11 = cat([_unpk(hh[0:HB, f * FC:f * FC + 128]) for f in range(NF)], axis=1)
        a22 = cat([_unpk(hh[HB:CB, f * FC + 128:(f + 1) * FC]) for f in range(NF)], axis=1)
        tb = [_unpk(wc[i * (Fh // 4):(i + 1) * (Fh // 4), cl]) for i in range(7)]
        c11, c12, c21, c22 = strassen(sa, a11, a22, tb, tb[5], tb[6], None)
        emit_out(c21, x1_src, CB, out_row(t, 1), cl)
        emit_out(c11, x1_src, 0, out_row(t, 0), cl)
        emit_out(c12, x1_src, 0, out_row(t, 0), cr)
        emit_out(c22, x1_src, CB, out_row(t, 1), cr)

    def ffn_down(x1_src, t, hunit=0, dep=None):
        for j in range(KS // 128):
            ffn_down_main(x1_src, t, hunit, j)
        ffn_down_rem(x1_src, t, hunit, dep=dep)

    def prologue():
        small[0].wait()
        small[2].wait()
        ssm_cp(0).wait()
        k_fwd(0)
        small[1].wait()
        small[3].wait()
        small[4].wait()
        shk = shk_ref[...].astype(F32)
        for a in range(4):
            sh_ref[a] = jnp.broadcast_to(shk[a:a + 1, :], (8, D))
        zm_ref[...] = pltpu.bitcast(inv_ref[CB:CB + 16, :], I32)
        zs.append(zm_ref[0, 0])
        kbuf_ref[:, 0:8, :] = jnp.zeros((NL, 8, 128), F32)
        ssm_cp(1).wait()
        k_fwd(1)
        k_cp(0).wait()
        v_cp(0).wait()
        ssm_cp(2).wait()
        pre_kv(0)
        k_fwd(2)
        pre_fwd(0)
        k_cp(1).wait()
        v_cp(1).wait()
        ssm_cp(3).wait()
        pre_kv(1)
        k_fwd(3)
        pre_fwd(1)
        ssm_cp(4).wait()
        k_fwd(4)
        y_static(0, 12, 0, 4, False)
        q_cp(0).wait()
        q_cp(1).wait()
        mod_cp(0).wait()
        mod_chunk(0)
        for t in range(2):
            pre_post(t)
            pre_ln1(t)
            pre_inv(t, x1s_ref.at[t * TM:(t + 1) * TM])
        mod_cp(1).wait()
        mod_chunk(1)
        for t in range(2):
            pre_ln2(x1s_ref.at[t * TM:(t + 1) * TM], t)

    def superstep():
        plain = lambda f, r: ffn_gu(f, r, r, plain=True)
        fast = lambda f, r: ffn_gu(f, r, r, staged=True)
        x1s = [x1s_ref.at[r * TM:(r + 1) * TM] for r in range(2)]
        g_cp(0).wait()
        u_cp(0).wait()
        w_combos_gu(0)
        plain(0, 0)
        fast(0, 1)
        k_cp(2).wait()
        v_cp(2).wait()
        g_cp(1).wait()
        u_cp(1).wait()
        pre_kv(2, paced=True)
        w_combos_gu(1)
        plain(1, 0)
        fast(1, 1)
        for f in range(2, 4):
            g_cp(f).wait()
            u_cp(f).wait()
        dep = w_combos_gu(2)
        dep = w_combos_gu(3, dep)
        y_static(12, NB, 0, 4, False, 1, dep=dep, prange=(0, YSPLIT))
        pre_fwd(2)
        plain(2, 0)
        fast(2, 1)
        fast(3, 0)
        fast(3, 1)
        for f in range(4, NF):
            g_cp(f).wait()
            u_cp(f).wait()
        d_cp.wait()
        dep = w_combos_gu(4)
        dep = w_combos_gu(5, dep)
        dep = w_combos_down(dep)
        wdr_ref[...] = pltpu.bitcast(wd_ref[:, lanes[NL - 1]], U32)
        y_static(4, 6, 4, 6, True, 2, dep=dep)
        plain(4, 0)
        fast(4, 1)
        fast(5, 0)
        fast(5, 1)
        q_cp(2).wait()
        mod_cp(2).wait()
        k_cp(3).wait()
        v_cp(3).wait()
        pre_ln1(2, paced=True)
        dep = pre_post(2, paced=True)
        dep = y_static(12, NB, 0, 4, False, 1, dep=dep, prange=(YSPLIT, 240))
        pre_kv(3, dep, paced=True)
        mod_chunk(2)
        ffn_down(x1s[0], 0, 0)
        pre_inv(2, x1_ref.at[0])
        pre_ln2(x1_ref.at[0], 2, paced=True)
        ffn_down(x1s[1], 1, 1)
        o_cp(0).start()
        o_cp(1).start()

    def step(t, carry):
        slot = lax.rem(t, 2)
        q_cp(t).wait()

        @pl.when(t + 1 < NS)
        def _():
            k_cp(t + 1).wait()
            v_cp(t + 1).wait()

        tn = jnp.minimum(t + 1, NS - 1)
        dep0 = pre_fwd(t)
        if LV == 'a':
            diag_mac(t, T0 - 1, DIAG_DIST)
            task(t, 2)
            dep = task(t, 1)
            dep = pre_post(t, dep, paced=True)
            pre_ln1(t, dep0, paced=True)
            pre_kv(tn, dep, paced=True)
        elif LV == 'b':
            diag_mac(t, T0 - 1, DIAG_DIST)
            task(t, 2)
            dep = task(t, 1)
            dep = pre_post(t, dep, paced=True)
            pre_ln1(t, None, paced=True)
            pre_kv(tn, dep, paced=True)
        elif LV in ('c', 'd'):
            diag_mac(t, T0 - 1, DIAG_DIST)
            task(t, 2)
            dep = task(t, 1)
            dep = pre_post(t, dep, paced=True)
            pre_ln1(t, dep0 if LV == 'c' else None, paced=True)
        elif LV == 'e':
            depk = pre_kv(tn, relay(tka_ref, dep0), paced=True)
            diag_mac(t, T0 - 1, DIAG_DIST, depk)
            task(t, 2)
            dep = task(t, 1)
            dep = pre_post(t, dep, paced=True)
            pre_ln1(t, None, paced=True)
        for f in range(NF):
            ffn_gu(f, 2, 0)
        pre_inv(t, x1_ref.at[slot])
        depl = pre_ln2(x1_ref.at[slot], 2, paced=True)
        if LV in ('c', 'd'):
            pre_kv(tn, opaque(x1_ref.at[slot])[0:8, 0:128], paced=True)
        ffn_down(x1_ref.at[1 - slot], t - 1, dep=(relay(tkb_ref, depl) if JOIN else None))
        o_cp(t - 1).start()
        return carry

    def epilogue():
        t = NS - 1
        for f in range(NF):
            ffn_gu(f, 2, 0)
        ffn_down(x1_ref.at[t % 2], t)
        o_cp(t).start()
        for i in range(NS):
            o_cp(i).wait()

    if SCOPES:
        jax.named_scope("prologue")(prologue)()
        jax.named_scope("superstep")(superstep)()
        lax.fori_loop(T0, NS, jax.named_scope("step")(step), 0)
        jax.named_scope("epilogue")(epilogue)()
    elif ONLY == 'loop':
        zs.append(zm_ref[0, 0])
        lax.fori_loop(T0, NS, step, 0)
    elif ONLY == 'S':
        zs.append(zm_ref[0, 0])
        superstep()
        lax.fori_loop(T0, NS, step, 0)
    else:
        prologue()
        superstep()
        lax.fori_loop(T0, NS, step, 0)
        epilogue()


@jax.jit
def pallas_adaLN_cond__ssm_conv_h3__glu_gated_bilinear__prompt_kernel(
    A_q, A_k, A_v, A_shift_k, A_ssm_k, A_ssm_D, B_x, B_w_gate, B_w_up, B_w_down, c, w_mod,
):
    B, S, D = A_q.shape
    Fh = B_w_gate.shape[1]
    NB = S // CB
    NS = S // TM
    fwd, inv = _dft_consts()
    anyspec = pl.BlockSpec(memory_space=pl.ANY)
    V = pltpu.VMEM
    out = pl.pallas_call(
        functools.partial(_kernel, S=S, D=D, Fh=Fh),
        in_specs=[anyspec] * 13,
        out_specs=anyspec,
        out_shape=jax.ShapeDtypeStruct((S, D), A_q.dtype),
        scratch_shapes=[
            V((NS, 2, 3 * CB, D), F32),
            V((NB, 3 * CB, D), F32),
            V((NS, 2, 3 * CB, D), F32),
            V((2, TM, D), F32),
            V((S, D), BF16), V((S, D), BF16), V((S, D), BF16), V((S, D), BF16),
            V((2 * TM, D), F32),
            V((TM, D), F32),
            V((3 * CB, D), U32),
            V((3 * 5 * HB, KS), U32),
            V((2 * CB, Fh), U32),
            V((2 * 5 * HB, Fh // 2), U32),
            V((TM // 2, D), U32),
            V((2 * CB, D), U32),
            V(((D - 2 * KS) // 2, Fh), U32), V(((D - 2 * KS) // 2, Fh), U32), V((Fh // 2, D - 2 * KS), U32),
            V((7 * KS // 2, Fh // 2), U32), V((7 * KS // 2, Fh // 2), U32), V((7 * Fh // 4, KS), U32),
            V((D, S), BF16), V((D, 6 * D), BF16), V((D, Fh), BF16), V((D, Fh), BF16), V((Fh, D), BF16),
            V((2 * CB, CB), BF16), V((CB + 16, CB), BF16),
            V((5, 8, D), F32), V((4, 8, D), F32), V((D // 128, TM + 8, 128), F32), V((8, 128), I32),
            V((8, 128), F32), V((8, 128), F32),
            V((4, D), BF16), V((D,), BF16), V((1, D), BF16),
            pltpu.SemaphoreType.DMA((5 + 4 * NS + D // 128 + 3 + 2 * (Fh // FC) + 1,)),
        ],
        compiler_params=pltpu.CompilerParams(
            internal_scratch_in_bytes=48 * 1024,
            disable_semaphore_checks=True,
            vmem_limit_bytes=110 * 1024 * 1024),
        name="adaln_h3_glu",
    )(A_q.reshape(S, D), A_k.reshape(S, D), A_v.reshape(S, D), A_shift_k.T, A_ssm_k,
      A_ssm_D, B_w_gate, B_w_up, B_w_down, c, w_mod, fwd, inv)
    return out.reshape(B, S, D)
```

```python
import functools
import os

import numpy as np
import jax
import jax.numpy as jnp
from jax import lax
import jax.experimental.pallas as pl
import jax.experimental.pallas.tpu as pltpu

F32 = jnp.float32
BF16 = jnp.bfloat16
U32 = jnp.uint32
I32 = jnp.int32

CB = 128
HB = CB // 2
TM = 256
FC = 256
KS = 256
EPS = 1e-5
SCOPES = False
ONLY = os.environ.get('ONLY', '')


def _E(name, default):
    return int(os.environ.get(name, default))


def _dft_consts():
    k = np.arange(CB, dtype=np.float64)[:, None]
    n = np.arange(CB, dtype=np.float64)[None, :]
    th = np.pi * (4.0 * k + 1.0) * n / (2.0 * CB)
    fwd = np.concatenate([np.cos(th), np.sin(th)], axis=0)
    g = np.concatenate([np.cos(th[:HB]), np.sin(th[:HB])], axis=0).T / CB
    inv = np.concatenate([g[0::2], g[1::2], np.zeros((16, CB))], axis=0)
    return jnp.asarray(fwd, dtype=BF16), jnp.asarray(inv, dtype=BF16)


def _pk(x):
    return pltpu.bitcast(x.astype(BF16), U32)


def _unpk(x):
    return pltpu.bitcast(x, BF16)


def _rep(r, n):
    return r if n == 8 else jnp.concatenate([r] * (n // 8), axis=0)


def _add(x, tok):
    return x if tok is None else x + _rep(tok, x.shape[0])


def _group(pieces, n):
    def merged(ps):
        def run(tok):
            for p in ps:
                p(tok)
        return run
    return [merged(pieces[i:i + n]) for i in range(0, len(pieces), n)]


class _Sched:
    def __init__(self, token):
        self.token = token
        self.clock = 0.0
        self.q = []
        self.last = None

    def add(self, pieces, t0, t1):
        n = len(pieces)
        self.q += [(t0 + (t1 - t0) * i / n, len(self.q) + i, p) for i, p in enumerate(pieces)]
        self.q.sort(key=lambda e: e[:2])

    def note(self, m, dt):
        rows, cols = m.shape
        tiles = [(slice(r, r + 8), slice(c, c + 128)) for c in range(0, cols, 128) for r in range(0, rows, 8)]
        for i, tl in enumerate(tiles):
            tok = None
            while self.q and self.q[0][0] <= self.clock + dt * (i + 1) / len(tiles):
                if tok is None:
                    tok = self.token(m[tl])
                self.q.pop(0)[2](tok)
        self.clock += dt
        self.last = m[tiles[-1]]
        return m

    def dot(self, a, b):
        m = jnp.dot(a, b, preferred_element_type=F32)
        return self.note(m, max(a.shape[0], 32) * (a.shape[1] // 128) * (b.shape[1] // 128) / 4)

    def flush(self):
        tok = None if self.last is None or not self.q else self.token(self.last)
        while self.q:
            self.q.pop(0)[2](tok)
        self.clock = 0.0
        self.last = None


def _kernel(q_hbm, k_hbm, v_hbm, shk_hbm, ssmk_hbm, ssmd_hbm, wg_hbm, wu_hbm, wd_hbm,
            c_hbm, wmod_hbm, fwd_hbm, inv_hbm, o_hbm,
            u_ref, kk_ref, y_ref, x1_ref, q_ref, k_ref, v_ref, o_ref,
            x1s_ref, hp_ref, st_ref, h2_ref, h2c_ref, hh_ref, hhc_ref, kv_ref, yb_ref,
            wgr_ref, wur_ref, wdr_ref, wgc_ref, wuc_ref, wdc_ref,
            ssmk_ref, wmod_ref, wg_ref, wu_ref, wd_ref, fwd_ref, inv_ref,
            mod_ref, sh_ref, kbuf_ref, zm_ref, shk_ref, ssmd_ref, c_ref,
            sem, *, S, D, Fh):
    NB = S // CB
    NS = S // TM
    NL = D // 128
    NF = Fh // FC
    NK = KS // 128
    T0 = 3
    NLOOP = NS - T0
    lanes = [slice(i * 128, (i + 1) * 128) for i in range(NL)]
    cat = jnp.concatenate

    offs = [int(o) for o in np.cumsum([0, 5, NS, NS, NS, NL, 3, NF, NF, 1])]
    s_small, s_q, s_k, s_v, s_ssm, s_mod, s_g, s_u, s_d, s_o = offs

    def rows_of(t):
        return pl.ds(t * TM if isinstance(t, int) else pl.multiple_of(t * TM, TM), TM)

    def rows_cp(src, dst, base, t):
        return pltpu.make_async_copy(src.at[rows_of(t), :], dst.at[rows_of(t), :], sem.at[base + t])

    def cols_cp(src, dst, lo, hi, si):
        return pltpu.make_async_copy(src.at[:, lo:hi], dst.at[:, lo:hi], sem.at[si])

    q_cp = lambda t: rows_cp(q_hbm, q_ref, s_q, t)
    k_cp = lambda t: rows_cp(k_hbm, k_ref, s_k, t)
    v_cp = lambda t: rows_cp(v_hbm, v_ref, s_v, t)
    o_cp = lambda t: rows_cp(o_ref, o_hbm, s_o, t)
    small = [pltpu.make_async_copy(s, d, sem.at[s_small + i]) for i, (s, d) in enumerate(
        [(fwd_hbm, fwd_ref), (shk_hbm, shk_ref), (ssmd_hbm, ssmd_ref), (inv_hbm, inv_ref), (c_hbm, c_ref)])]
    ssm_cp = lambda i: pltpu.make_async_copy(ssmk_hbm.at[lanes[i], :], ssmk_ref.at[lanes[i], :],
                                             sem.at[s_ssm + i])
    mod_cols = [(0, 3 * D), (3 * D, 5 * D), (5 * D, 6 * D)]
    mod_cp = lambda i: cols_cp(wmod_hbm, wmod_ref, mod_cols[i][0], mod_cols[i][1], s_mod + i)
    g_cp = lambda f: cols_cp(wg_hbm, wg_ref, f * FC, (f + 1) * FC, s_g + f)
    u_cp = lambda f: cols_cp(wu_hbm, wu_ref, f * FC, (f + 1) * FC, s_u + f)
    d_cp = pltpu.make_async_copy(wd_hbm, wd_ref, sem.at[s_d])

    order = small + [ssm_cp(0), ssm_cp(1), k_cp(0), v_cp(0),
                     ssm_cp(2), k_cp(1), v_cp(1), ssm_cp(3), ssm_cp(4), q_cp(0), q_cp(1),
                     mod_cp(0), mod_cp(1), g_cp(0), u_cp(0), k_cp(2), v_cp(2)]
    for f in range(1, NF):
        order += [g_cp(f), u_cp(f)]
    order += [d_cp, q_cp(2), mod_cp(2), k_cp(3), v_cp(3)]
    for t in range(T0, NS):
        order += [q_cp(t)]
        if t + 1 < NS:
            order += [k_cp(t + 1), v_cp(t + 1)]
    for cp in order:
        cp.start()

    zs = []
    bg = _Sched(lambda x: pltpu.bitcast(pltpu.bitcast(x, I32) & zm_ref[...], F32))

    def opaque(ref):
        return ref.at[pl.ds(pl.multiple_of(zs[0], 32), ref.shape[0])]

    def chain(pieces, dist, extra=0, dep=None):
        hist = [] if dep is None else [dep] * dist
        for p in pieces:
            tok = None
            if len(hist) >= dist:
                tok = bg.token(hist[-dist])
                for _ in range(extra):
                    tok = tok + tok
            hist.append(p(tok))
        return hist[-1]

    def now(pieces):
        for p in pieces:
            p(None)

    def mod_chunk(i):
        c = c_ref[...].astype(F32)
        sc = jnp.broadcast_to((c * jax.nn.sigmoid(c)).astype(BF16), (16, D))
        lo, hi = mod_cols[i]
        m = bg.dot(sc, wmod_ref[:, lo:hi])[0:8]
        if i == 0:
            ga = m[:, 2 * D:3 * D]
            mod_ref[0] = (1.0 + m[:, D:2 * D]) * ga
            mod_ref[1] = m[:, 0:D] * ga
        elif i == 1:
            mod_ref[2] = 1.0 + m[:, D:2 * D]
            mod_ref[3] = m[:, 0:D]
        else:
            mod_ref[4] = m

    def k_fwd(i):
        ls = lanes[i]
        fwd = fwd_ref[...]
        prev = None
        for m in range(NB):
            kf = lax.dot_general(fwd, ssmk_ref[ls, m * CB:(m + 1) * CB], (((1,), (1,)), ((), ())),
                                 preferred_element_type=F32)
            if m == 0:
                c = kf[:CB] + ssmd_ref[...].astype(F32).reshape(1, D)[:, ls]
                d = kf[CB:]
            else:
                c = kf[:CB] + prev[CB:]
                d = kf[CB:] - prev[:CB]
            prev = kf
            kk_ref[m, 0:CB, ls] = c
            kk_ref[m, CB:2 * CB, ls] = d - c
            kk_ref[m, 2 * CB:3 * CB, ls] = c + d
            if m % 4 == 3:
                bg.note(kf, 2 * CB)

    def kv_pieces(t):
        G = 32
        kb, vb = k_ref.at[rows_of(t)], v_ref.at[rows_of(t)]

        def piece(i, r0):
            def run(tok):
                ls = lanes[i]
                kf = _add(kb[r0:r0 + G, ls].astype(F32), tok)
                kbuf_ref[i, 8 + r0:8 + r0 + G, :] = kf
                ks = kf * _rep(sh_ref[0, :, ls], G)
                for a in range(1, 4):
                    ks = ks + kbuf_ref[i, 8 + r0 - a:8 + r0 - a + G, :] * _rep(sh_ref[a, :, ls], G)
                kv_ref[r0 // 2:(r0 + G) // 2, ls] = _pk(ks * vb[r0:r0 + G, ls].astype(F32))
                if r0 + G == TM:
                    kbuf_ref[i, 0:8, :] = kf[G - 8:]
            return run
        return [piece(i, r0) for i in range(NL) for r0 in range(0, TM, G)]

    def u_fwd(t):
        fwd = fwd_ref[...]
        for b in range(2):
            uf = bg.dot(fwd, _unpk(kv_ref[b * HB:(b + 1) * HB, :]))
            a, bb = uf[:CB], uf[CB:]
            u_ref[t, b, 0:CB, :] = a + bb
            u_ref[t, b, CB:2 * CB, :] = a
            u_ref[t, b, 2 * CB:3 * CB, :] = bb

    positions = [(slice(r0, r0 + 8), ls) for r0 in range(0, 3 * CB, 8) for ls in lanes]

    def ystatic_pieces(s_lo, s_hi, i_lo, i_hi, acc_in, pos=None):
        def piece(rs, ls):
            def run(tok):
                us = {i: _add(u_ref[i // 2, i % 2, rs, ls], tok) for i in range(i_lo, i_hi)}
                ks = {}
                for s in range(s_lo, s_hi):
                    acc = None
                    for i in range(i_lo, min(i_hi, s + 1)):
                        m = s - i
                        if m not in ks:
                            ks[m] = kk_ref[m, rs, ls]
                        p = ks[m] * us[i]
                        acc = p if acc is None else acc + p
                    if acc_in:
                        acc = acc + y_ref[s // 2, s % 2, rs, ls]
                    y_ref[s // 2, s % 2, rs, ls] = acc
                return acc
            return run
        return [piece(*p) for p in (positions if pos is None else pos)]

    def task_pieces(t, delta):
        p = t - delta
        left = p >= T0
        J = jnp.where(left, t, p + NLOOP)
        I = jnp.where(left, p, t)
        kview = kk_ref.at[pl.ds(2 * (J - I) - 1, 3)]

        def piece(rs, ls):
            def run(tok):
                u0 = _add(u_ref[I, 0, rs, ls], tok)
                u1 = _add(u_ref[I, 1, rs, ls], tok)
                kc = kview[1, rs, ls]
                y_ref[J, 0, rs, ls] = (kc * u0 + kview[0, rs, ls] * u1) + y_ref[J, 0, rs, ls]
                y1 = (kview[2, rs, ls] * u0 + kc * u1) + y_ref[J, 1, rs, ls]
                y_ref[J, 1, rs, ls] = y1
                return y1
            return run
        return [piece(*p) for p in positions]

    def diag_pieces(t, I):
        kview = kk_ref.at[pl.ds(2 * (t - I) - 1, 3)]

        def piece(rs, ls):
            def run(tok):
                us = [_add(u_ref[a, b, rs, ls], tok) for a in (t, I) for b in range(2)]
                k0 = kk_ref[0, rs, ls]
                kc = kview[1, rs, ls]
                y_ref[t, 0, rs, ls] = ((k0 * us[0] + y_ref[t, 0, rs, ls])
                                       + (kc * us[2] + kview[0, rs, ls] * us[3]))
                y1 = ((kk_ref[1, rs, ls] * us[0] + k0 * us[1])
                      + (kview[2, rs, ls] * us[2] + kc * us[3]) + y_ref[t, 1, rs, ls])
                y_ref[t, 1, rs, ls] = y1
                return y1
            return run
        return [piece(*p) for p in positions]

    def post_pieces(t):
        def piece(b, r0, ls):
            def run(tok):
                comp = lambda c, off: y_ref[t, b, c * CB + off + r0:c * CB + off + r0 + 16, ls]
                k1l, k1h = _add(comp(0, 0), tok), _add(comp(0, HB), tok)
                rel, reh = k1l - comp(2, 0), k1h - comp(2, HB)
                iml, imh = k1l + comp(1, 0), k1h + comp(1, HB)
                p0 = b * CB + r0 // 2
                yb_ref[p0:p0 + 8, ls] = _pk(rel + reh)
                yb_ref[p0 + HB // 2:p0 + HB // 2 + 8, ls] = _pk(iml + imh)
                yb_ref[p0 + HB:p0 + HB + 8, ls] = _pk(rel - reh)
                oim = iml - imh
                yb_ref[p0 + HB + HB // 2:p0 + HB + HB // 2 + 8, ls] = _pk(oim)
                return oim[8:16]
            return run
        return [piece(b, r0, ls) for b in range(2) for r0 in range(0, HB, 16) for ls in lanes]

    def q_split(t, b, p0, n, ls):
        w = pltpu.bitcast(q_ref.at[rows_of(t)][b * CB + 2 * p0:b * CB + 2 * p0 + 2 * n, ls], U32)
        return pltpu.bitcast(w << 16, F32), pltpu.bitcast(w & jnp.uint32(0xFFFF0000), F32)

    def ln_tiles(xs, tok):
        n = xs[0].shape[0]
        s = _add(xs[0], tok)
        for x in xs[1:]:
            s = s + x
        m = jnp.sum(s, axis=-1, keepdims=True) * (1.0 / D)
        xc = [x - m for x in xs]
        s2 = xc[0] * xc[0]
        for x in xc[1:]:
            s2 = s2 + x * x
        r = lax.rsqrt(jnp.sum(s2, axis=-1, keepdims=True) * (1.0 / D) + EPS)
        return xc, jnp.broadcast_to(r, (n, 128)), jnp.broadcast_to(m, (n, 128))

    def ln1_pieces(t):
        G = _E('L1G', 8)

        def piece(b, p0):
            def run(tok):
                xc, r, _ = ln_tiles([cat(q_split(t, b, p0, G, ls), axis=0) for ls in lanes], tok)
                for ls, x in zip(lanes, xc):
                    h = (x * r) * _rep(mod_ref[0, :, ls], 2 * G) + _rep(mod_ref[1, :, ls], 2 * G)
                    hp_ref[b * CB + p0:b * CB + p0 + G, ls] = h[:G]
                    hp_ref[b * CB + HB + p0:b * CB + HB + p0 + G, ls] = h[G:]
                return functools.reduce(lambda a, c: a + c, [h[r:r + 8] for r in range(0, 2 * G, 8)])
            return run
        return [piece(b, p0) for b in range(2) for p0 in range(0, HB, G)]

    def y_inv(t, x1_dst):
        yb = opaque(yb_ref)
        hp = opaque(hp_ref)
        for b in range(2):
            ye = bg.dot(inv_ref[0:HB, :], _unpk(yb[b * CB:b * CB + HB, :]))
            yo = bg.dot(inv_ref[HB:CB, :], _unpk(yb[b * CB + HB:(b + 1) * CB, :]))
            for ls in lanes:
                qe, qo = q_split(t, b, 0, HB, ls)
                re, ro = slice(b * CB, b * CB + HB), slice(b * CB + HB, (b + 1) * CB)
                x1_dst[re, ls] = qe + hp[re, ls] * ye[:, ls]
                x1_dst[ro, ls] = qo + hp[ro, ls] * yo[:, ls]

    def a_combos(a11, a12, a21, a22):
        return [a11 + a22, a21 + a22, a11 + a12, a21 - a11, a12 - a22]

    def b_combos(b11, b12, b21, b22):
        return [b11 + b22, b12 - b22, b21 - b11, b11 + b12, b21 + b22, b11, b22]

    def ln2_stat_pieces(x1_src, st):
        x1o = opaque(x1_src)

        def piece(r0):
            def run(tok):
                _, r, m = ln_tiles([x1o[r0:r0 + 16, ls] for ls in lanes], tok)
                st[r0:r0 + 16, 0:128] = m
                st[r0:r0 + 16, 128:256] = r
            return run
        return [piece(h * CB + r0) for r0 in range(0, CB, 16) for h in range(2)]

    def ln2_apply_pieces(x1_src, st, unit):
        G = 16
        x1o = opaque(x1_src)
        h2_dst = h2_ref.at[unit * CB:(unit + 1) * CB]
        h2c_dst = h2c_ref.at[unit * 5 * HB:(unit + 1) * 5 * HB]

        def piece(r0, js):
            def run(tok):
                two = lambda ref, c: cat([ref[r0:r0 + G, c], ref[CB + r0:CB + r0 + G, c]], axis=0)
                m, r = _add(two(st, slice(0, 128)), tok), two(st, slice(128, 256))
                hs = {}
                for j in js:
                    ls = lanes[j]
                    h = ((two(x1o, ls) - m) * r) * _rep(mod_ref[2, :, ls], 2 * G) + _rep(mod_ref[3, :, ls], 2 * G)
                    hs[j] = h
                    h2_dst[r0 // 2:(r0 + G) // 2, ls] = _pk(h[:G])
                    h2_dst[(CB + r0) // 2:(CB + r0 + G) // 2, ls] = _pk(h[G:])
                    if NK <= j < 2 * NK:
                        cs = a_combos(hs[j - NK][:G], h[:G], hs[j - NK][G:], h[G:])
                        for i, cmb in enumerate(cs):
                            h2c_dst[i * HB + r0 // 2:i * HB + (r0 + G) // 2, lanes[j - NK]] = _pk(cmb)
            return run
        parts = [[j, NK + j] for j in range(NK)]
        parts[-1] += list(range(2 * NK, NL))
        return [piece(r0, js) for r0 in range(0, CB, G) for js in parts]

    def strassen(sa, a11, a22, tb, rem):
        dot = bg.dot
        m1 = dot(sa[0], tb[0])
        if rem is None:
            m7 = dot(sa[4], tb[4])
        else:
            m7 = dot(cat([sa[4], rem[0]], axis=1), cat([tb[4], rem[2]], axis=0))
        m4 = dot(a22, tb[2])
        m2 = dot(sa[1], tb[5])
        c21 = m2 + m4
        if rem is not None:
            c21 = c21 + dot(rem[1], rem[2])
        m5 = dot(sa[2], tb[6])
        c11 = m1 + m7 + m4 - m5
        m3 = dot(a11, tb[1])
        c12 = m3 + m5
        if rem is None:
            m6 = dot(sa[3], tb[3])
        else:
            c12 = c12 + dot(rem[0], rem[3])
            m6 = dot(cat([sa[3], rem[1]], axis=1), cat([tb[3], rem[3]], axis=0))
        c22 = m1 - m2 + m3 + m6
        return c11, c12, c21, c22

    def wgu_pieces(f):
        G = 16
        cl, cr = slice(f * FC, f * FC + 128), slice(f * FC + 128, (f + 1) * FC)

        def piece(w_ref, wc_ref, wr_ref, r0):
            def run(tok):
                b11 = _add(w_ref[r0:r0 + G, cl].astype(F32), tok)
                b22 = _add(w_ref[KS + r0:KS + r0 + G, cr].astype(F32), tok)
                cs = b_combos(b11, w_ref[r0:r0 + G, cr].astype(F32),
                              w_ref[KS + r0:KS + r0 + G, cl].astype(F32), b22)
                for i, cmb in enumerate(cs):
                    wc_ref[(i * KS + r0) // 2:(i * KS + r0 + G) // 2, f * 128:(f + 1) * 128] = _pk(cmb)
                if r0 < D - 2 * KS:
                    for c in (cl, cr):
                        w = pltpu.bitcast(w_ref[2 * KS + r0:2 * KS + r0 + G, c], U32)
                        wr_ref[r0 // 2:(r0 + G) // 2, c] = w if tok is None else w | pltpu.bitcast(tok, U32)
            return run
        return [piece(*refs, r0) for refs in ((wg_ref, wgc_ref, wgr_ref), (wu_ref, wuc_ref, wur_ref))
                for r0 in range(0, KS, G)]

    def wd_pieces():
        G = 16

        def piece(j, f, r0):
            def run(tok):
                cl, cr = lanes[j], lanes[NK + j]
                re = slice(f * FC + r0, f * FC + r0 + G)
                ro = slice(f * FC + 128 + r0, f * FC + 128 + r0 + G)
                b11 = _add(wd_ref[re, cl].astype(F32), tok)
                b22 = _add(wd_ref[ro, cr].astype(F32), tok)
                cs = b_combos(b11, wd_ref[re, cr].astype(F32), wd_ref[ro, cl].astype(F32), b22)
                for i, cmb in enumerate(cs):
                    p0 = i * (Fh // 4) + (f * 128 + r0) // 2
                    wdc_ref[p0:p0 + G // 2, cl] = _pk(cmb)
                rr = re if j == 0 else ro
                w = pltpu.bitcast(wd_ref[rr, lanes[NL - 1]], U32)
                wdr_ref[rr.start // 2:rr.stop // 2, :] = w if tok is None else w | pltpu.bitcast(tok, U32)
            return run
        return [piece(j, f, r0) for j in range(NK) for f in range(NF) for r0 in range(0, 128, G)]

    def ffn_gu(f, unit, plain=False):
        cl, cr = slice(f * FC, f * FC + 128), slice(f * FC + 128, (f + 1) * FC)
        h2 = h2_ref.at[unit * CB:(unit + 1) * CB]
        h2c = h2c_ref.at[unit * 5 * HB:(unit + 1) * 5 * HB]
        if plain:
            p11, p12, p21, p22 = [
                bg.dot(_unpk(h2[r:r + HB, :]), wg_ref[:, c]) * bg.dot(_unpk(h2[r:r + HB, :]), wu_ref[:, c])
                for r in (0, HB) for c in (cl, cr)]
        else:
            res = []
            for wr, wc in ((wgr_ref, wgc_ref), (wur_ref, wuc_ref)):
                sa = [_unpk(h2c[i * HB:(i + 1) * HB, :]) for i in range(5)]
                tb = [_unpk(wc[i * KS // 2:(i + 1) * KS // 2, f * 128:(f + 1) * 128]) for i in range(7)]
                rem = (_unpk(h2[0:HB, 2 * KS:D]), _unpk(h2[HB:CB, 2 * KS:D]), _unpk(wr[:, cl]), _unpk(wr[:, cr]))
                res.append(strassen(sa, _unpk(h2[0:HB, 0:KS]), _unpk(h2[HB:CB, KS:2 * KS]), tb, rem))
            p11, p12, p21, p22 = [g * u for g, u in zip(*res)]
        hh = hh_ref.at[unit * CB:(unit + 1) * CB]
        hhc = hhc_ref.at[unit * 5 * HB:(unit + 1) * 5 * HB]
        hh[0:HB, cl] = _pk(p11)
        hh[0:HB, cr] = _pk(p12)
        hh[HB:CB, cl] = _pk(p21)
        hh[HB:CB, cr] = _pk(p22)
        for i, cmb in enumerate(a_combos(p11, p12, p21, p22)):
            hhc[i * HB:(i + 1) * HB, f * 128:(f + 1) * 128] = _pk(cmb)

    def ffn_down(x1_src, t, unit):
        hh = hh_ref.at[unit * CB:(unit + 1) * CB]
        hhc = hhc_ref.at[unit * 5 * HB:(unit + 1) * 5 * HB]
        ob = o_ref.at[rows_of(t)]

        def emit(dn, b, ls):
            o = x1_src[b * CB:(b + 1) * CB, ls] + _rep(mod_ref[4, :, ls], CB) * dn
            w = pltpu.pack_elementwise([o[:HB], o[HB:]], packed_dtype=BF16)
            ob[b * CB:(b + 1) * CB, ls] = pltpu.bitcast(w, BF16)

        for b in range(2):
            emit(bg.dot(_unpk(hh[b * HB:(b + 1) * HB, :]), _unpk(wdr_ref[...])), b, lanes[NL - 1])
        for j in range(NK):
            cl, cr = lanes[j], lanes[NK + j]
            sa = [_unpk(hhc[i * HB:(i + 1) * HB, :]) for i in range(5)]
            a11 = cat([_unpk(hh[0:HB, f * FC:f * FC + 128]) for f in range(NF)], axis=1)
            a22 = cat([_unpk(hh[HB:CB, f * FC + 128:(f + 1) * FC]) for f in range(NF)], axis=1)
            tb = [_unpk(wdc_ref[i * (Fh // 4):(i + 1) * (Fh // 4), cl]) for i in range(7)]
            c11, c12, c21, c22 = strassen(sa, a11, a22, tb, None)
            emit(c21, 1, cl)
            emit(c11, 0, cl)
            emit(c12, 0, cr)
            emit(c22, 1, cr)

    x1s = [x1s_ref.at[r * TM:(r + 1) * TM] for r in range(2)]
    sts = [st_ref.at[r * TM:(r + 1) * TM] for r in range(2)]
    YP = _E('YP', 12)

    def prologue():
        for cp in small:
            cp.wait()
        shk = shk_ref[...].astype(F32)
        for a in range(4):
            sh_ref[a] = jnp.broadcast_to(shk[a:a + 1, :], (8, D))
        zm_ref[...] = pltpu.bitcast(inv_ref[CB:CB + 16, :], I32)
        zs.append(zm_ref[0, 0])
        kbuf_ref[:, 0:8, :] = jnp.zeros((NL, 8, 128), F32)
        ssm_cp(0).wait()
        k_fwd(0)
        ssm_cp(1).wait()
        k_fwd(1)
        for t in range(2):
            k_cp(t).wait()
            v_cp(t).wait()
            ssm_cp(2 + t).wait()
            now(kv_pieces(t))
            k_fwd(2 + t)
            u_fwd(t)
        ssm_cp(4).wait()
        bg.flush()
        pos = sorted(positions, key=lambda p: p[1].start)
        n0 = _E('PY0', 32)
        bg.add(ystatic_pieces(0, YP, 0, 4, False, pos[:n0]), 0, 1024)
        bg.add(ystatic_pieces(0, YP, 0, 4, False, pos[n0:n0 + 1]), 5000, 5001)
        k_fwd(4)
        bg.flush()
        q_cp(0).wait()
        now(ystatic_pieces(0, YP, 0, 4, False, pos[n0 + 1:]))
        q_cp(1).wait()
        mod_cp(0).wait()
        mod_chunk(0)
        for t in range(2):
            now(post_pieces(t))
            now(ln1_pieces(t))
            y_inv(t, x1s[t])
        for t in range(2):
            now(ln2_stat_pieces(x1s[t], sts[t]))
        mod_cp(1).wait()
        mod_chunk(1)
        for t in range(2):
            now(ln2_apply_pieces(x1s[t], sts[t], t))
        bg.flush()

    def superstep():
        yrest = ystatic_pieces(YP, NB, 0, 4, False)
        g_cp(0).wait()
        u_cp(0).wait()
        bg.add(wgu_pieces(0), 0, 900)
        bg.add(yrest[0:50], 1000, 2200)
        ffn_gu(0, 0, plain=True)
        ffn_gu(0, 1)
        bg.flush()
        k_cp(2).wait()
        v_cp(2).wait()
        g_cp(1).wait()
        u_cp(1).wait()
        bg.add(wgu_pieces(1), 0, 900)
        bg.add(kv_pieces(2), 1000, 2200)
        ffn_gu(1, 0, plain=True)
        ffn_gu(1, 1)
        bg.flush()
        for f in range(2, 4):
            g_cp(f).wait()
            u_cp(f).wait()
        bg.add(wgu_pieces(2), 0, 900)
        bg.add(wgu_pieces(3), 1900, 2700)
        bg.add(yrest[50:150], 2800, 5100)
        ffn_gu(2, 0, plain=True)
        u_fwd(2)
        ffn_gu(2, 1)
        ffn_gu(3, 0)
        ffn_gu(3, 1)
        bg.flush()
        for f in range(4, NF):
            g_cp(f).wait()
            u_cp(f).wait()
        d_cp.wait()
        bg.add(wgu_pieces(4), 0, 900)
        bg.add(wgu_pieces(5), 1000, 1900)
        bg.add(wd_pieces(), 2000, 4500)
        ffn_gu(4, 0, plain=True)
        ffn_gu(4, 1)
        ffn_gu(5, 0)
        ffn_gu(5, 1)
        bg.flush()
        q_cp(2).wait()
        mod_cp(2).wait()
        k_cp(3).wait()
        v_cp(3).wait()
        bg.add(_group(ystatic_pieces(4, 6, 4, 6, True), 4), 200, 2200)
        bg.add(ln1_pieces(2), 200, 2800)
        bg.add(_group(post_pieces(2), 2), 2300, 3200)
        t1 = 200 + 3456 + 320
        bg.add(ln2_stat_pieces(x1_ref.at[0], st_ref), t1 + 100, t1 + 1800)
        bg.add(ln2_apply_pieces(x1_ref.at[0], st_ref, 0), t1 + 1400, t1 + 3100)
        bg.add(kv_pieces(3), t1 + 100, t1 + 1500)
        bg.add(yrest[150:], t1 + 1500, t1 + 3200)
        mod_chunk(2)
        ffn_down(x1s[0], 0, 0)
        y_inv(2, x1_ref.at[0])
        ffn_down(x1s[1], 1, 1)
        bg.flush()
        o_cp(0).start()
        o_cp(1).start()
        for t in range(T0, NS):
            q_cp(t).wait()
            if t + 1 < NS:
                k_cp(t + 1).wait()
                v_cp(t + 1).wait()

    def step(t, carry):
        slot = lax.rem(t, 2)
        if _E('LA', 1):
            bg.add(ln1_pieces(t), _E('L0', 800), _E('L1', 6800))
        t1 = 640 + NF * 1152 + 320
        bg.add(ln2_stat_pieces(x1_ref.at[slot], st_ref), t1 + _E('S0', 100), t1 + _E('S1', 1800))
        bg.add(ln2_apply_pieces(x1_ref.at[slot], st_ref, 0), t1 + _E('P0', 1400), t1 + _E('P1', 3100))
        bg.add(kv_pieces(jnp.minimum(t + 1, NS - 1)), t1 + _E('K0', 100), t1 + _E('K1', 3100))
        u_fwd(t)
        chain(diag_pieces(t, T0 - 1), _E('DD', 2), _E('DE', 0))
        chain(task_pieces(t, 2), _E('MD', 2), _E('ME', 0))
        dep = chain(task_pieces(t, 1), _E('MD', 2), _E('ME', 0))
        chain(post_pieces(t), 1, 3, dep)
        if not _E('LA', 1):
            chain(ln1_pieces(t), 1)
        for f in range(NF):
            ffn_gu(f, 0)
        y_inv(t, x1_ref.at[slot])
        ffn_down(x1_ref.at[1 - slot], t - 1, 0)
        bg.flush()
        o_cp(t - 1).start()
        return carry

    def epilogue():
        t = NS - 1
        for f in range(NF):
            ffn_gu(f, 0)
        ffn_down(x1_ref.at[t % 2], t, 0)
        o_cp(t).start()
        for i in range(NS):
            o_cp(i).wait()

    if SCOPES:
        jax.named_scope("prologue")(prologue)()
        jax.named_scope("superstep")(superstep)()
        lax.fori_loop(T0, NS, jax.named_scope("step")(step), 0)
        jax.named_scope("epilogue")(epilogue)()
    elif ONLY == 'loop':
        zs.append(zm_ref[0, 0])
        lax.fori_loop(T0, NS, step, 0)
        epilogue()
    elif ONLY == 'S':
        zs.append(zm_ref[0, 0])
        superstep()
        lax.fori_loop(T0, NS, step, 0)
    else:
        prologue()
        superstep()
        lax.fori_loop(T0, NS, step, 0)
        epilogue()


@jax.jit
def pallas_adaLN_cond__ssm_conv_h3__glu_gated_bilinear__prompt_kernel(
    A_q, A_k, A_v, A_shift_k, A_ssm_k, A_ssm_D, B_x, B_w_gate, B_w_up, B_w_down, c, w_mod,
):
    B, S, D = A_q.shape
    Fh = B_w_gate.shape[1]
    NB = S // CB
    NS = S // TM
    fwd, inv = _dft_consts()
    anyspec = pl.BlockSpec(memory_space=pl.ANY)
    V = pltpu.VMEM
    out = pl.pallas_call(
        functools.partial(_kernel, S=S, D=D, Fh=Fh),
        in_specs=[anyspec] * 13,
        out_specs=anyspec,
        out_shape=jax.ShapeDtypeStruct((S, D), A_q.dtype),
        scratch_shapes=[
            V((NS, 2, 3 * CB, D), F32),
            V((NB, 3 * CB, D), F32),
            V((NS, 2, 3 * CB, D), F32),
            V((2, TM, D), F32),
            V((S, D), BF16), V((S, D), BF16), V((S, D), BF16), V((S, D), BF16),
            V((2 * TM, D), F32),
            V((TM, D), F32),
            V((2 * TM, 256), F32),
            V((2 * CB, D), U32),
            V((2 * 5 * HB, KS), U32),
            V((2 * CB, Fh), U32),
            V((2 * 5 * HB, Fh // 2), U32),
            V((TM // 2, D), U32),
            V((2 * CB, D), U32),
            V(((D - 2 * KS) // 2, Fh), U32), V(((D - 2 * KS) // 2, Fh), U32), V((Fh // 2, D - 2 * KS), U32),
            V((7 * KS // 2, Fh // 2), U32), V((7 * KS // 2, Fh // 2), U32), V((7 * Fh // 4, KS), U32),
            V((D, S), BF16), V((D, 6 * D), BF16), V((D, Fh), BF16), V((D, Fh), BF16), V((Fh, D), BF16),
            V((2 * CB, CB), BF16), V((CB + 16, CB), BF16),
            V((5, 8, D), F32), V((4, 8, D), F32), V((D // 128, TM + 8, 128), F32), V((8, 128), I32),
            V((4, D), BF16), V((D,), BF16), V((1, D), BF16),
            pltpu.SemaphoreType.DMA((5 + 4 * NS + D // 128 + 3 + 2 * (Fh // FC) + 1,)),
        ],
        compiler_params=pltpu.CompilerParams(
            internal_scratch_in_bytes=48 * 1024,
            disable_semaphore_checks=True,
            vmem_limit_bytes=110 * 1024 * 1024),
        name="adaln_h3_glu",
    )(A_q.reshape(S, D), A_k.reshape(S, D), A_v.reshape(S, D), A_shift_k.T, A_ssm_k,
      A_ssm_D, B_w_gate, B_w_up, B_w_down, c, w_mod, fwd, inv)
    return out.reshape(B, S, D)
```

```python
import functools
import os

import numpy as np
import jax
import jax.numpy as jnp
from jax import lax
import jax.experimental.pallas as pl
import jax.experimental.pallas.tpu as pltpu

F32 = jnp.float32
BF16 = jnp.bfloat16
U32 = jnp.uint32
I32 = jnp.int32

CB = 128
HB = CB // 2
TM = 256
FC = 256
KS = 256
EPS = 1e-5
SCOPES = False
ONLY = os.environ.get('ONLY', '')


def _E(name, default):
    return int(os.environ.get(name, default))


def _dft_consts():
    k = np.arange(CB, dtype=np.float64)[:, None]
    n = np.arange(CB, dtype=np.float64)[None, :]
    th = np.pi * (4.0 * k + 1.0) * n / (2.0 * CB)
    fwd = np.concatenate([np.cos(th), np.sin(th)], axis=0)
    g = np.concatenate([np.cos(th[:HB]), np.sin(th[:HB])], axis=0).T / CB
    inv = np.concatenate([g[0::2], g[1::2], np.zeros((16, CB))], axis=0)
    return jnp.asarray(fwd, dtype=BF16), jnp.asarray(inv, dtype=BF16)


def _pk(x):
    return pltpu.bitcast(x.astype(BF16), U32)


def _unpk(x):
    return pltpu.bitcast(x, BF16)


def _rep(r, n):
    return r if n == 8 else jnp.concatenate([r] * (n // 8), axis=0)


def _add(x, tok):
    return x if tok is None else x + _rep(tok, x.shape[0])


def _group(pieces, n):
    def merged(ps):
        def run(tok):
            for p in ps:
                p(tok)
        return run
    return [merged(pieces[i:i + n]) for i in range(0, len(pieces), n)]


class _Sched:
    def __init__(self, token):
        self.token = token
        self.clock = 0.0
        self.q = []
        self.last = None
        self.inj = []

    def add(self, pieces, t0, t1):
        n = len(pieces)
        self.q += [(t0 + (t1 - t0) * i / n, len(self.q) + i, p) for i, p in enumerate(pieces)]
        self.q.sort(key=lambda e: e[:2])

    def note(self, m, dt):
        rows, cols = m.shape
        tiles = [(slice(r, r + 8), slice(c, c + 128)) for c in range(0, cols, 128) for r in range(0, rows, 8)]
        for i, tl in enumerate(tiles):
            tok = None
            while self.q and self.q[0][0] <= self.clock + dt * (i + 1) / len(tiles):
                if tok is None:
                    tok = self.token(m[tl])
                self.q.pop(0)[2](tok)
        self.clock += dt
        self.last = m[tiles[-1]]
        return m

    def dot(self, a, b):
        if self.inj and self.clock >= self.inj[0][0]:
            self.inj.pop(0)[1]()
        m = jnp.dot(a, b, preferred_element_type=F32)
        return self.note(m, max(a.shape[0], 32) * (a.shape[1] // 128) * (b.shape[1] // 128) / 4)

    def flush(self):
        tok = None if self.last is None or not self.q else self.token(self.last)
        while self.q:
            self.q.pop(0)[2](tok)
        self.clock = 0.0
        self.last = None


def _kernel(q_hbm, k_hbm, v_hbm, shk_hbm, ssmk_hbm, ssmd_hbm, wg_hbm, wu_hbm, wd_hbm,
            c_hbm, wmod_hbm, fwd_hbm, inv_hbm, o_hbm,
            u_ref, kk_ref, y_ref, x1_ref, q_ref, k_ref, v_ref, o_ref,
            x1s_ref, hp_ref, st_ref, h2_ref, h2c_ref, hh_ref, hhc_ref, kv_ref, yb_ref,
            wgr_ref, wur_ref, wdr_ref, wgc_ref, wuc_ref, wdc_ref,
            ssmk_ref, wmod_ref, wg_ref, wu_ref, wd_ref, fwd_ref, inv_ref,
            mod_ref, sh_ref, kbuf_ref, zm_ref, shk_ref, ssmd_ref, c_ref,
            sem, *, S, D, Fh):
    NB = S // CB
    NS = S // TM
    NL = D // 128
    NF = Fh // FC
    NK = KS // 128
    T0 = 3
    NLOOP = NS - T0
    lanes = [slice(i * 128, (i + 1) * 128) for i in range(NL)]
    cat = jnp.concatenate

    offs = [int(o) for o in np.cumsum([0, 5, NS, NS, NS, NL, 3, NF, NF, 1])]
    s_small, s_q, s_k, s_v, s_ssm, s_mod, s_g, s_u, s_d, s_o = offs

    def rows_of(t):
        return pl.ds(t * TM if isinstance(t, int) else pl.multiple_of(t * TM, TM), TM)

    def rows_cp(src, dst, base, t):
        return pltpu.make_async_copy(src.at[rows_of(t), :], dst.at[rows_of(t), :], sem.at[base + t])

    def cols_cp(src, dst, lo, hi, si):
        return pltpu.make_async_copy(src.at[:, lo:hi], dst.at[:, lo:hi], sem.at[si])

    q_cp = lambda t: rows_cp(q_hbm, q_ref, s_q, t)
    k_cp = lambda t: rows_cp(k_hbm, k_ref, s_k, t)
    v_cp = lambda t: rows_cp(v_hbm, v_ref, s_v, t)
    o_cp = lambda t: rows_cp(o_ref, o_hbm, s_o, t)
    small = [pltpu.make_async_copy(s, d, sem.at[s_small + i]) for i, (s, d) in enumerate(
        [(fwd_hbm, fwd_ref), (shk_hbm, shk_ref), (ssmd_hbm, ssmd_ref), (inv_hbm, inv_ref), (c_hbm, c_ref)])]
    ssm_cp = lambda i: pltpu.make_async_copy(ssmk_hbm.at[lanes[i], :], ssmk_ref.at[lanes[i], :],
                                             sem.at[s_ssm + i])
    mod_cols = [(0, 3 * D), (3 * D, 5 * D), (5 * D, 6 * D)]
    mod_cp = lambda i: cols_cp(wmod_hbm, wmod_ref, mod_cols[i][0], mod_cols[i][1], s_mod + i)
    g_cp = lambda f: cols_cp(wg_hbm, wg_ref, f * FC, (f + 1) * FC, s_g + f)
    u_cp = lambda f: cols_cp(wu_hbm, wu_ref, f * FC, (f + 1) * FC, s_u + f)
    d_cp = pltpu.make_async_copy(wd_hbm, wd_ref, sem.at[s_d])

    order = small + [ssm_cp(0), ssm_cp(1), k_cp(0), v_cp(0),
                     ssm_cp(2), k_cp(1), v_cp(1), ssm_cp(3), ssm_cp(4), q_cp(0), q_cp(1),
                     mod_cp(0), mod_cp(1), g_cp(0), u_cp(0), k_cp(2), v_cp(2)]
    for f in range(1, NF):
        order += [g_cp(f), u_cp(f)]
    order += [q_cp(2), d_cp, mod_cp(2), k_cp(3), v_cp(3)]
    for t in range(T0, NS):
        order += [q_cp(t)]
        if t + 1 < NS:
            order += [k_cp(t + 1), v_cp(t + 1)]
    for cp in order:
        cp.start()

    zs = []
    bg = _Sched(lambda x: pltpu.bitcast(pltpu.bitcast(x, I32) & zm_ref[...], F32))

    def opaque(ref):
        return ref.at[pl.ds(pl.multiple_of(zs[0], 32), ref.shape[0])]

    def chain(pieces, dist, extra=0, dep=None):
        hist = [] if dep is None else [dep] * dist
        for p in pieces:
            tok = None
            if len(hist) >= dist:
                tok = bg.token(hist[-dist])
                for _ in range(extra):
                    tok = tok + tok
            hist.append(p(tok))
        return hist[-1]

    def linked(pieces, d):
        res = []

        def wrap(p):
            def run(tok):
                if d and len(res) >= d:
                    tok = tok + bg.token(res[-d])
                res.append(p(tok))
            return run
        return [wrap(p) for p in pieces]

    def now(pieces):
        for p in pieces:
            p(None)

    def mod_chunk(i):
        c = c_ref[...].astype(F32)
        sc = jnp.broadcast_to((c * jax.nn.sigmoid(c)).astype(BF16), (16, D))
        lo, hi = mod_cols[i]
        m = bg.dot(sc, wmod_ref[:, lo:hi])[0:8]
        if i == 0:
            ga = m[:, 2 * D:3 * D]
            mod_ref[0] = (1.0 + m[:, D:2 * D]) * ga
            mod_ref[1] = m[:, 0:D] * ga
        elif i == 1:
            mod_ref[2] = 1.0 + m[:, D:2 * D]
            mod_ref[3] = m[:, 0:D]
        else:
            mod_ref[4] = m

    def gb_tile(i):
        def run():
            c = c_ref[...].astype(F32)
            sc = jnp.broadcast_to((c * jax.nn.sigmoid(c)).astype(BF16), (16, D))
            w = wmod_ref[:, 5 * D + i * 128:5 * D + (i + 1) * 128]
            mod_ref[4, :, lanes[i]] = jnp.dot(sc, w, preferred_element_type=F32)[0:8]
        return run

    def k_fwd(i):
        ls = lanes[i]
        fwd = fwd_ref[...]
        prev = None
        for m in range(NB):
            kf = lax.dot_general(fwd, ssmk_ref[ls, m * CB:(m + 1) * CB], (((1,), (1,)), ((), ())),
                                 preferred_element_type=F32)
            if m == 0:
                c = kf[:CB] + ssmd_ref[...].astype(F32).reshape(1, D)[:, ls]
                d = kf[CB:]
            else:
                c = kf[:CB] + prev[CB:]
                d = kf[CB:] - prev[:CB]
            prev = kf
            kk_ref[m, 0:CB, ls] = c
            kk_ref[m, CB:2 * CB, ls] = d - c
            kk_ref[m, 2 * CB:3 * CB, ls] = c + d
            if m % 4 == 3:
                bg.note(kf, 2 * CB)

    def kv_pieces(t):
        G = 32
        kb, vb = k_ref.at[rows_of(t)], v_ref.at[rows_of(t)]

        def piece(i, r0):
            def run(tok):
                ls = lanes[i]
                kf = _add(kb[r0:r0 + G, ls].astype(F32), tok)
                kbuf_ref[i, 8 + r0:8 + r0 + G, :] = kf
                ks = kf * _rep(sh_ref[0, :, ls], G)
                for a in range(1, 4):
                    ks = ks + kbuf_ref[i, 8 + r0 - a:8 + r0 - a + G, :] * _rep(sh_ref[a, :, ls], G)
                kv_ref[r0 // 2:(r0 + G) // 2, ls] = _pk(ks * vb[r0:r0 + G, ls].astype(F32))
                if r0 + G == TM:
                    kbuf_ref[i, 0:8, :] = kf[G - 8:]
            return run
        return [piece(i, r0) for i in range(NL) for r0 in range(0, TM, G)]

    def u_fwd(t):
        fwd = fwd_ref[...]
        for b in range(2):
            uf = bg.dot(fwd, _unpk(kv_ref[b * HB:(b + 1) * HB, :]))
            a, bb = uf[:CB], uf[CB:]
            u_ref[t, b, 0:CB, :] = a + bb
            u_ref[t, b, CB:2 * CB, :] = a
            u_ref[t, b, 2 * CB:3 * CB, :] = bb

    positions = [(slice(r0, r0 + 8), ls) for r0 in range(0, 3 * CB, 8) for ls in lanes]

    def ystatic_pieces(s_lo, s_hi, i_lo, i_hi, acc_in, pos=None):
        def piece(rs, ls):
            def run(tok):
                us = {i: _add(u_ref[i // 2, i % 2, rs, ls], tok) for i in range(i_lo, i_hi)}
                ks = {}
                for s in range(s_lo, s_hi):
                    acc = None
                    for i in range(i_lo, min(i_hi, s + 1)):
                        m = s - i
                        if m not in ks:
                            ks[m] = kk_ref[m, rs, ls]
                        p = ks[m] * us[i]
                        acc = p if acc is None else acc + p
                    if acc_in:
                        acc = acc + y_ref[s // 2, s % 2, rs, ls]
                    y_ref[s // 2, s % 2, rs, ls] = acc
                return acc
            return run
        return [piece(*p) for p in (positions if pos is None else pos)]

    def task_pieces(t, delta):
        p = t - delta
        left = p >= T0
        J = jnp.where(left, t, p + NLOOP)
        I = jnp.where(left, p, t)
        kview = kk_ref.at[pl.ds(2 * (J - I) - 1, 3)]

        def piece(rs, ls):
            def run(tok):
                u0 = _add(u_ref[I, 0, rs, ls], tok)
                u1 = _add(u_ref[I, 1, rs, ls], tok)
                kc = kview[1, rs, ls]
                y_ref[J, 0, rs, ls] = (kc * u0 + kview[0, rs, ls] * u1) + y_ref[J, 0, rs, ls]
                y1 = (kview[2, rs, ls] * u0 + kc * u1) + y_ref[J, 1, rs, ls]
                y_ref[J, 1, rs, ls] = y1
                return y1
            return run
        return [piece(*p) for p in positions]

    def diag_pieces(t, I):
        kview = kk_ref.at[pl.ds(2 * (t - I) - 1, 3)]

        def piece(rs, ls):
            def run(tok):
                us = [_add(u_ref[a, b, rs, ls], tok) for a in (t, I) for b in range(2)]
                k0 = kk_ref[0, rs, ls]
                kc = kview[1, rs, ls]
                y_ref[t, 0, rs, ls] = ((k0 * us[0] + y_ref[t, 0, rs, ls])
                                       + (kc * us[2] + kview[0, rs, ls] * us[3]))
                y1 = ((kk_ref[1, rs, ls] * us[0] + k0 * us[1])
                      + (kview[2, rs, ls] * us[2] + kc * us[3]) + y_ref[t, 1, rs, ls])
                y_ref[t, 1, rs, ls] = y1
                return y1
            return run
        return [piece(*p) for p in positions]

    def post_pieces(t):
        def piece(b, r0, ls):
            def run(tok):
                comp = lambda c, off: y_ref[t, b, c * CB + off + r0:c * CB + off + r0 + 16, ls]
                k1l, k1h = _add(comp(0, 0), tok), _add(comp(0, HB), tok)
                rel, reh = k1l - comp(2, 0), k1h - comp(2, HB)
                iml, imh = k1l + comp(1, 0), k1h + comp(1, HB)
                p0 = b * CB + r0 // 2
                yb_ref[p0:p0 + 8, ls] = _pk(rel + reh)
                yb_ref[p0 + HB // 2:p0 + HB // 2 + 8, ls] = _pk(iml + imh)
                yb_ref[p0 + HB:p0 + HB + 8, ls] = _pk(rel - reh)
                oim = iml - imh
                yb_ref[p0 + HB + HB // 2:p0 + HB + HB // 2 + 8, ls] = _pk(oim)
                return oim[8:16]
            return run
        return [piece(b, r0, ls) for b in range(2) for r0 in range(0, HB, 16) for ls in lanes]

    def q_split(t, b, p0, n, ls):
        w = pltpu.bitcast(q_ref.at[rows_of(t)][b * CB + 2 * p0:b * CB + 2 * p0 + 2 * n, ls], U32)
        return pltpu.bitcast(w << 16, F32), pltpu.bitcast(w & jnp.uint32(0xFFFF0000), F32)

    def ln_tiles(xs, tok):
        n = xs[0].shape[0]
        s = _add(xs[0], tok)
        for x in xs[1:]:
            s = s + x
        m = jnp.sum(s, axis=-1, keepdims=True) * (1.0 / D)
        xc = [x - m for x in xs]
        s2 = xc[0] * xc[0]
        for x in xc[1:]:
            s2 = s2 + x * x
        r = lax.rsqrt(jnp.sum(s2, axis=-1, keepdims=True) * (1.0 / D) + EPS)
        return xc, jnp.broadcast_to(r, (n, 128)), jnp.broadcast_to(m, (n, 128))

    def ln1_pieces(t):
        G = _E('L1G', 8)

        def piece(b, p0):
            def run(tok):
                xc, r, _ = ln_tiles([cat(q_split(t, b, p0, G, ls), axis=0) for ls in lanes], tok)
                for ls, x in zip(lanes, xc):
                    h = (x * r) * _rep(mod_ref[0, :, ls], 2 * G) + _rep(mod_ref[1, :, ls], 2 * G)
                    hp_ref[b * CB + p0:b * CB + p0 + G, ls] = h[:G]
                    hp_ref[b * CB + HB + p0:b * CB + HB + p0 + G, ls] = h[G:]
                return functools.reduce(lambda a, c: a + c, [h[r:r + 8] for r in range(0, 2 * G, 8)])
            return run
        return [piece(b, p0) for b in range(2) for p0 in range(0, HB, G)]

    def y_inv(t, x1_dst):
        yb = opaque(yb_ref)
        hp = opaque(hp_ref)
        for b in range(2):
            ye = bg.dot(inv_ref[0:HB, :], _unpk(yb[b * CB:b * CB + HB, :]))
            yo = bg.dot(inv_ref[HB:CB, :], _unpk(yb[b * CB + HB:(b + 1) * CB, :]))
            for ls in lanes:
                qe, qo = q_split(t, b, 0, HB, ls)
                re, ro = slice(b * CB, b * CB + HB), slice(b * CB + HB, (b + 1) * CB)
                x1_dst[re, ls] = qe + hp[re, ls] * ye[:, ls]
                x1_dst[ro, ls] = qo + hp[ro, ls] * yo[:, ls]

    def a_combos(a11, a12, a21, a22):
        return [a11 + a22, a21 + a22, a11 + a12, a21 - a11, a12 - a22]

    def b_combos(b11, b12, b21, b22):
        return [b11 + b22, b12 - b22, b21 - b11, b11 + b12, b21 + b22, b11, b22]

    def ln2_stat_pieces(x1_src, st):
        x1o = opaque(x1_src)

        def piece(r0):
            def run(tok):
                _, r, m = ln_tiles([x1o[r0:r0 + 16, ls] for ls in lanes], tok)
                st[r0:r0 + 16, 0:128] = m
                st[r0:r0 + 16, 128:256] = r
                return r[0:8] + r[8:16]
            return run
        return [piece(h * CB + r0) for r0 in range(0, CB, 16) for h in range(2)]

    def ln2_apply_pieces(x1_src, st, unit):
        G = 16
        x1o = opaque(x1_src)
        h2_dst = h2_ref.at[unit * CB:(unit + 1) * CB]
        h2c_dst = h2c_ref.at[unit * 5 * HB:(unit + 1) * 5 * HB]

        def piece(r0, js):
            def run(tok):
                two = lambda ref, c: cat([ref[r0:r0 + G, c], ref[CB + r0:CB + r0 + G, c]], axis=0)
                m, r = _add(two(st, slice(0, 128)), tok), two(st, slice(128, 256))
                hs = {}
                for j in js:
                    ls = lanes[j]
                    h = ((two(x1o, ls) - m) * r) * _rep(mod_ref[2, :, ls], 2 * G) + _rep(mod_ref[3, :, ls], 2 * G)
                    hs[j] = h
                    h2_dst[r0 // 2:(r0 + G) // 2, ls] = _pk(h[:G])
                    h2_dst[(CB + r0) // 2:(CB + r0 + G) // 2, ls] = _pk(h[G:])
                    if NK <= j < 2 * NK:
                        cs = a_combos(hs[j - NK][:G], h[:G], hs[j - NK][G:], h[G:])
                        for i, cmb in enumerate(cs):
                            h2c_dst[i * HB + r0 // 2:i * HB + (r0 + G) // 2, lanes[j - NK]] = _pk(cmb)
            return run
        parts = [[j, NK + j] for j in range(NK)]
        parts[-1] += list(range(2 * NK, NL))
        return [piece(r0, js) for r0 in range(0, CB, G) for js in parts]

    def strassen(sa, a11, a22, tb, rem):
        dot = bg.dot
        m1 = dot(sa[0], tb[0])
        if rem is None:
            m7 = dot(sa[4], tb[4])
        else:
            m7 = dot(cat([sa[4], rem[0]], axis=1), cat([tb[4], rem[2]], axis=0))
        m4 = dot(a22, tb[2])
        m2 = dot(sa[1], tb[5])
        c21 = m2 + m4
        if rem is not None:
            c21 = c21 + dot(rem[1], rem[2])
        m5 = dot(sa[2], tb[6])
        c11 = m1 + m7 + m4 - m5
        m3 = dot(a11, tb[1])
        c12 = m3 + m5
        if rem is None:
            m6 = dot(sa[3], tb[3])
        else:
            c12 = c12 + dot(rem[0], rem[3])
            m6 = dot(cat([sa[3], rem[1]], axis=1), cat([tb[3], rem[3]], axis=0))
        c22 = m1 - m2 + m3 + m6
        return c11, c12, c21, c22

    def wgu_pieces(f):
        G = 16
        cl, cr = slice(f * FC, f * FC + 128), slice(f * FC + 128, (f + 1) * FC)

        def piece(w_ref, wc_ref, wr_ref, r0):
            def run(tok):
                b11 = _add(w_ref[r0:r0 + G, cl].astype(F32), tok)
                b22 = _add(w_ref[KS + r0:KS + r0 + G, cr].astype(F32), tok)
                cs = b_combos(b11, w_ref[r0:r0 + G, cr].astype(F32),
                              w_ref[KS + r0:KS + r0 + G, cl].astype(F32), b22)
                for i, cmb in enumerate(cs):
                    wc_ref[(i * KS + r0) // 2:(i * KS + r0 + G) // 2, f * 128:(f + 1) * 128] = _pk(cmb)
                if r0 < D - 2 * KS:
                    for c in (cl, cr):
                        w = pltpu.bitcast(w_ref[2 * KS + r0:2 * KS + r0 + G, c], U32)
                        wr_ref[r0 // 2:(r0 + G) // 2, c] = w if tok is None else w | pltpu.bitcast(tok, U32)
            return run
        return [piece(*refs, r0) for refs in ((wg_ref, wgc_ref, wgr_ref), (wu_ref, wuc_ref, wur_ref))
                for r0 in range(0, KS, G)]

    def wd_pieces():
        G = 16

        def piece(j, f, r0):
            def run(tok):
                cl, cr = lanes[j], lanes[NK + j]
                re = slice(f * FC + r0, f * FC + r0 + G)
                ro = slice(f * FC + 128 + r0, f * FC + 128 + r0 + G)
                b11 = _add(wd_ref[re, cl].astype(F32), tok)
                b22 = _add(wd_ref[ro, cr].astype(F32), tok)
                cs = b_combos(b11, wd_ref[re, cr].astype(F32), wd_ref[ro, cl].astype(F32), b22)
                for i, cmb in enumerate(cs):
                    p0 = i * (Fh // 4) + (f * 128 + r0) // 2
                    wdc_ref[p0:p0 + G // 2, cl] = _pk(cmb)
            return run
        return [piece(j, f, r0) for j in range(NK) for f in range(NF) for r0 in range(0, 128, G)]

    def wdr_pieces():
        G = 128

        def piece(r0):
            def run(tok):
                w = pltpu.bitcast(wd_ref[r0:r0 + G, lanes[NL - 1]], U32)
                wdr_ref[r0 // 2:(r0 + G) // 2, :] = w | _rep(pltpu.bitcast(tok, U32), G // 2)
            return run
        return [piece(r0) for r0 in range(0, Fh, G)]

    def ffn_gu(f, unit, plain=False):
        cl, cr = slice(f * FC, f * FC + 128), slice(f * FC + 128, (f + 1) * FC)
        h2 = h2_ref.at[unit * CB:(unit + 1) * CB]
        h2c = h2c_ref.at[unit * 5 * HB:(unit + 1) * 5 * HB]
        if plain:
            p11, p12, p21, p22 = [
                bg.dot(_unpk(h2[r:r + HB, :]), wg_ref[:, c]) * bg.dot(_unpk(h2[r:r + HB, :]), wu_ref[:, c])
                for r in (0, HB) for c in (cl, cr)]
        else:
            res = []
            for wr, wc in ((wgr_ref, wgc_ref), (wur_ref, wuc_ref)):
                sa = [_unpk(h2c[i * HB:(i + 1) * HB, :]) for i in range(5)]
                tb = [_unpk(wc[i * KS // 2:(i + 1) * KS // 2, f * 128:(f + 1) * 128]) for i in range(7)]
                rem = (_unpk(h2[0:HB, 2 * KS:D]), _unpk(h2[HB:CB, 2 * KS:D]), _unpk(wr[:, cl]), _unpk(wr[:, cr]))
                res.append(strassen(sa, _unpk(h2[0:HB, 0:KS]), _unpk(h2[HB:CB, KS:2 * KS]), tb, rem))
            p11, p12, p21, p22 = [g * u for g, u in zip(*res)]
        hh = hh_ref.at[unit * CB:(unit + 1) * CB]
        hhc = hhc_ref.at[unit * 5 * HB:(unit + 1) * 5 * HB]
        hh[0:HB, cl] = _pk(p11)
        hh[0:HB, cr] = _pk(p12)
        hh[HB:CB, cl] = _pk(p21)
        hh[HB:CB, cr] = _pk(p22)
        for i, cmb in enumerate(a_combos(p11, p12, p21, p22)):
            hhc[i * HB:(i + 1) * HB, f * 128:(f + 1) * 128] = _pk(cmb)

    def ffn_down(x1_src, t, unit):
        hh = hh_ref.at[unit * CB:(unit + 1) * CB]
        hhc = hhc_ref.at[unit * 5 * HB:(unit + 1) * 5 * HB]
        ob = o_ref.at[rows_of(t)]

        def emit(dn, b, ls):
            o = x1_src[b * CB:(b + 1) * CB, ls] + _rep(mod_ref[4, :, ls], CB) * dn
            w = pltpu.pack_elementwise([o[:HB], o[HB:]], packed_dtype=BF16)
            ob[b * CB:(b + 1) * CB, ls] = pltpu.bitcast(w, BF16)

        for b in range(2):
            KC = _E('KC', 512)
            ps = [bg.dot(_unpk(hh[b * HB:(b + 1) * HB, k0:k0 + KC]), _unpk(wdr_ref[k0 // 2:(k0 + KC) // 2, :]))
                  for k0 in range(0, Fh, KC)]
            emit(functools.reduce(lambda x, y: x + y, ps), b, lanes[NL - 1])
        for j in range(NK):
            cl, cr = lanes[j], lanes[NK + j]
            sa = [_unpk(hhc[i * HB:(i + 1) * HB, :]) for i in range(5)]
            a11 = cat([_unpk(hh[0:HB, f * FC:f * FC + 128]) for f in range(NF)], axis=1)
            a22 = cat([_unpk(hh[HB:CB, f * FC + 128:(f + 1) * FC]) for f in range(NF)], axis=1)
            tb = [_unpk(wdc_ref[i * (Fh // 4):(i + 1) * (Fh // 4), cl]) for i in range(7)]
            c11, c12, c21, c22 = strassen(sa, a11, a22, tb, None)
            emit(c21, 1, cl)
            emit(c11, 0, cl)
            emit(c12, 0, cr)
            emit(c22, 1, cr)

    x1s = [x1s_ref.at[r * TM:(r + 1) * TM] for r in range(2)]
    sts = [st_ref.at[r * TM:(r + 1) * TM] for r in range(2)]
    YP = _E('YP', 12)

    def prologue():
        for cp in small:
            cp.wait()
        shk = shk_ref[...].astype(F32)
        for a in range(4):
            sh_ref[a] = jnp.broadcast_to(shk[a:a + 1, :], (8, D))
        zm_ref[...] = pltpu.bitcast(inv_ref[CB:CB + 16, :], I32)
        zs.append(zm_ref[0, 0])
        kbuf_ref[:, 0:8, :] = jnp.zeros((NL, 8, 128), F32)
        ssm_cp(0).wait()
        k_fwd(0)
        ssm_cp(1).wait()
        k_fwd(1)
        for t in range(2):
            k_cp(t).wait()
            v_cp(t).wait()
            ssm_cp(2 + t).wait()
            now(kv_pieces(t))
            k_fwd(2 + t)
            u_fwd(t)
        ssm_cp(4).wait()
        bg.flush()
        pos = sorted(positions, key=lambda p: p[1].start)
        n0 = _E('PY0', 32)
        bg.add(ystatic_pieces(0, YP, 0, 4, False, pos[:n0]), 0, 1024)
        bg.add(ystatic_pieces(0, YP, 0, 4, False, pos[n0:n0 + 1]), 5000, 5001)
        k_fwd(4)
        bg.flush()
        q_cp(0).wait()
        now(ystatic_pieces(0, YP, 0, 4, False, pos[n0 + 1:]))
        q_cp(1).wait()
        mod_cp(0).wait()
        mod_chunk(0)
        for t in range(2):
            now(post_pieces(t))
            now(ln1_pieces(t))
            y_inv(t, x1s[t])
        for t in range(2):
            now(ln2_stat_pieces(x1s[t], sts[t]))
        mod_cp(1).wait()
        mod_chunk(1)
        for t in range(2):
            now(ln2_apply_pieces(x1s[t], sts[t], t))
        bg.flush()

    def superstep():
        yrest = ystatic_pieces(YP, NB, 0, 4, False)
        g_cp(0).wait()
        u_cp(0).wait()
        bg.add(wgu_pieces(0), 0, 900)
        bg.add(yrest[0:50], 1000, 2200)
        ffn_gu(0, 0, plain=True)
        ffn_gu(0, 1)
        bg.flush()
        k_cp(2).wait()
        v_cp(2).wait()
        g_cp(1).wait()
        u_cp(1).wait()
        bg.add(wgu_pieces(1), 0, 900)
        bg.add(kv_pieces(2), 1000, 2200)
        ffn_gu(1, 0, plain=True)
        ffn_gu(1, 1)
        bg.flush()
        for f in range(2, 4):
            g_cp(f).wait()
            u_cp(f).wait()
        bg.add(wgu_pieces(2), 0, 900)
        bg.add(wgu_pieces(3), 1900, 2700)
        bg.add(yrest[50:110], 2800, 4000)
        ffn_gu(2, 0, plain=True)
        u_fwd(2)
        ffn_gu(2, 1)
        ffn_gu(3, 0)
        bg.flush()
        for f in range(4, NF):
            g_cp(f).wait()
            u_cp(f).wait()
        q_cp(2).wait()
        bg.add(wgu_pieces(4), 0, 800)
        bg.add(wgu_pieces(5), 800, 1600)
        bg.add(_group(ystatic_pieces(4, 6, 4, 6, True), 3), 1600, 3000)
        bg.add(post_pieces(2), 3100, 3700)
        bg.add(yrest[110:140], 3700, 4400)
        bg.add(linked(ln1_pieces(2), _E('LK', 3)), 1600, 4000)
        ffn_gu(3, 1)
        ffn_gu(4, 0)
        ffn_gu(4, 1)
        ffn_gu(5, 0)
        bg.flush()
        d_cp.wait()
        mod_cp(2).wait()
        k_cp(3).wait()
        v_cp(3).wait()
        bg.add(wdr_pieces(), 0, 300)
        bg.add(wd_pieces(), 300, 3100)
        t1 = 1152 + 320
        bg.add(linked(ln2_stat_pieces(x1_ref.at[0], st_ref), _E('LK2', 3)), t1 + 1700, t1 + 3400)
        bg.add(ln2_apply_pieces(x1_ref.at[0], st_ref, 0), t1 + 3000, t1 + 4700)
        bg.add(kv_pieces(3), 3200, 5400)
        bg.add(yrest[140:], 5500, 8300)
        bg.inj = [(150 + 200 * i, gb_tile(i)) for i in range(NL)]
        ffn_gu(5, 1)
        y_inv(2, x1_ref.at[0])
        ffn_down(x1s[0], 0, 0)
        ffn_down(x1s[1], 1, 1)
        bg.flush()
        o_cp(0).start()
        o_cp(1).start()
        for t in range(T0, NS):
            q_cp(t).wait()
            if t + 1 < NS:
                k_cp(t + 1).wait()
                v_cp(t + 1).wait()

    def step(t, carry):
        slot = lax.rem(t, 2)
        if _E('LA', 1):
            bg.add(linked(ln1_pieces(t), _E('LK1', 2)), _E('L0', 800), _E('L1', 6800))
        t1 = 640 + NF * 1152 + 320
        bg.add(linked(ln2_stat_pieces(x1_ref.at[slot], st_ref), _E('LK2', 3)), t1 + _E('S0', 100), t1 + _E('S1', 1800))
        bg.add(ln2_apply_pieces(x1_ref.at[slot], st_ref, 0), t1 + _E('P0', 1400), t1 + _E('P1', 3100))
        bg.add(kv_pieces(jnp.minimum(t + 1, NS - 1)), t1 + _E('K0', 100), t1 + _E('K1', 3100))
        u_fwd(t)
        chain(diag_pieces(t, T0 - 1), _E('DD', 2), _E('DE', 0))
        chain(task_pieces(t, 2), _E('MD', 2), _E('ME', 0))
        dep = chain(task_pieces(t, 1), _E('MD', 2), _E('ME', 0))
        chain(post_pieces(t), 1, 3, dep)
        if not _E('LA', 1):
            chain(ln1_pieces(t), 1)
        for f in range(NF):
            ffn_gu(f, 0)
        y_inv(t, x1_ref.at[slot])
        ffn_down(x1_ref.at[1 - slot], t - 1, 0)
        bg.flush()
        o_cp(t - 1).start()
        return carry

    def epilogue():
        t = NS - 1
        for f in range(NF):
            ffn_gu(f, 0)
        ffn_down(x1_ref.at[t % 2], t, 0)
        o_cp(t).start()
        for i in range(NS):
            o_cp(i).wait()

    if SCOPES:
        jax.named_scope("prologue")(prologue)()
        jax.named_scope("superstep")(superstep)()
        lax.fori_loop(T0, NS, jax.named_scope("step")(step), 0)
        jax.named_scope("epilogue")(epilogue)()
    elif ONLY == 'loop':
        zs.append(zm_ref[0, 0])
        lax.fori_loop(T0, NS, step, 0)
        epilogue()
    elif ONLY == 'S':
        zs.append(zm_ref[0, 0])
        superstep()
        lax.fori_loop(T0, NS, step, 0)
    else:
        prologue()
        superstep()
        lax.fori_loop(T0, NS, step, 0)
        epilogue()


@jax.jit
def pallas_adaLN_cond__ssm_conv_h3__glu_gated_bilinear__prompt_kernel(
    A_q, A_k, A_v, A_shift_k, A_ssm_k, A_ssm_D, B_x, B_w_gate, B_w_up, B_w_down, c, w_mod,
):
    B, S, D = A_q.shape
    Fh = B_w_gate.shape[1]
    NB = S // CB
    NS = S // TM
    fwd, inv = _dft_consts()
    anyspec = pl.BlockSpec(memory_space=pl.ANY)
    V = pltpu.VMEM
    out = pl.pallas_call(
        functools.partial(_kernel, S=S, D=D, Fh=Fh),
        in_specs=[anyspec] * 13,
        out_specs=anyspec,
        out_shape=jax.ShapeDtypeStruct((S, D), A_q.dtype),
        scratch_shapes=[
            V((NS, 2, 3 * CB, D), F32),
            V((NB, 3 * CB, D), F32),
            V((NS, 2, 3 * CB, D), F32),
            V((2, TM, D), F32),
            V((S, D), BF16), V((S, D), BF16), V((S, D), BF16), V((S, D), BF16),
            V((2 * TM, D), F32),
            V((TM, D), F32),
            V((2 * TM, 256), F32),
            V((2 * CB, D), U32),
            V((2 * 5 * HB, KS), U32),
            V((2 * CB, Fh), U32),
            V((2 * 5 * HB, Fh // 2), U32),
            V((TM // 2, D), U32),
            V((2 * CB, D), U32),
            V(((D - 2 * KS) // 2, Fh), U32), V(((D - 2 * KS) // 2, Fh), U32), V((Fh // 2, D - 2 * KS), U32),
            V((7 * KS // 2, Fh // 2), U32), V((7 * KS // 2, Fh // 2), U32), V((7 * Fh // 4, KS), U32),
            V((D, S), BF16), V((D, 6 * D), BF16), V((D, Fh), BF16), V((D, Fh), BF16), V((Fh, D), BF16),
            V((2 * CB, CB), BF16), V((CB + 16, CB), BF16),
            V((5, 8, D), F32), V((4, 8, D), F32), V((D // 128, TM + 8, 128), F32), V((8, 128), I32),
            V((4, D), BF16), V((D,), BF16), V((1, D), BF16),
            pltpu.SemaphoreType.DMA((5 + 4 * NS + D // 128 + 3 + 2 * (Fh // FC) + 1,)),
        ],
        compiler_params=pltpu.CompilerParams(
            internal_scratch_in_bytes=48 * 1024,
            disable_semaphore_checks=True,
            vmem_limit_bytes=110 * 1024 * 1024),
        name="adaln_h3_glu",
    )(A_q.reshape(S, D), A_k.reshape(S, D), A_v.reshape(S, D), A_shift_k.T, A_ssm_k,
      A_ssm_D, B_w_gate, B_w_up, B_w_down, c, w_mod, fwd, inv)
    return out.reshape(B, S, D)
```

```python
import functools
import os

import numpy as np
import jax
import jax.numpy as jnp
from jax import lax
import jax.experimental.pallas as pl
import jax.experimental.pallas.tpu as pltpu

F32 = jnp.float32
BF16 = jnp.bfloat16
U32 = jnp.uint32
I32 = jnp.int32

CB = 128
HB = CB // 2
TM = 256
FC = 256
KS = 256
EPS = 1e-5
SCOPES = False
ONLY = os.environ.get('ONLY', '')


def _E(name, default):
    return int(os.environ.get(name, default))


def _dft_consts():
    k = np.arange(CB, dtype=np.float64)[:, None]
    n = np.arange(CB, dtype=np.float64)[None, :]
    th = np.pi * (4.0 * k + 1.0) * n / (2.0 * CB)
    fwd = np.concatenate([np.cos(th), np.sin(th)], axis=0)
    g = np.concatenate([np.cos(th[:HB]), np.sin(th[:HB])], axis=0).T / CB
    inv = np.concatenate([g[0::2], g[1::2], np.zeros((16, CB))], axis=0)
    return jnp.asarray(fwd, dtype=BF16), jnp.asarray(inv, dtype=BF16)


def _pk(x):
    return pltpu.bitcast(x.astype(BF16), U32)


def _unpk(x):
    return pltpu.bitcast(x, BF16)


def _rep(r, n):
    return r if n == 8 else jnp.concatenate([r] * (n // 8), axis=0)


def _add(x, tok):
    return x if tok is None else x + _rep(tok, x.shape[0])


def _group(pieces, n):
    def merged(ps):
        def run(tok):
            for p in ps:
                p(tok)
        return run
    return [merged(pieces[i:i + n]) for i in range(0, len(pieces), n)]


class _Sched:
    def __init__(self, token):
        self.token = token
        self.clock = 0.0
        self.q = []
        self.last = None
        self.inj = []

    def add(self, pieces, t0, t1):
        n = len(pieces)
        self.q += [(t0 + (t1 - t0) * i / n, len(self.q) + i, p) for i, p in enumerate(pieces)]
        self.q.sort(key=lambda e: e[:2])

    def note(self, m, dt):
        rows, cols = m.shape
        tiles = [(slice(r, r + 8), slice(c, c + 128)) for c in range(0, cols, 128) for r in range(0, rows, 8)]
        for i, tl in enumerate(tiles):
            tok = None
            while self.q and self.q[0][0] <= self.clock + dt * (i + 1) / len(tiles):
                if tok is None:
                    tok = self.token(m[tl])
                self.q.pop(0)[2](tok)
        self.clock += dt
        self.last = m[tiles[-1]]
        return m

    def dot(self, a, b):
        if self.inj and self.clock >= self.inj[0][0]:
            self.inj.pop(0)[1]()
        m = jnp.dot(a, b, preferred_element_type=F32)
        return self.note(m, max(a.shape[0], 32) * (a.shape[1] // 128) * (b.shape[1] // 128) / 4)

    def flush(self):
        tok = None if self.last is None or not self.q else self.token(self.last)
        while self.q:
            self.q.pop(0)[2](tok)
        self.clock = 0.0
        self.last = None


def _kernel(q_hbm, k_hbm, v_hbm, shk_hbm, ssmk_hbm, ssmd_hbm, wg_hbm, wu_hbm, wd_hbm,
            c_hbm, wmod_hbm, fwd_hbm, inv_hbm, o_hbm,
            u_ref, kk_ref, y_ref, x1_ref, q_ref, k_ref, v_ref, o_ref,
            x1s_ref, hp_ref, st_ref, h2_ref, h2c_ref, hh_ref, hhc_ref, kv_ref, yb_ref,
            wgr_ref, wur_ref, wdr_ref, wgc_ref, wuc_ref, wdc_ref,
            ssmk_ref, wmod_ref, wg_ref, wu_ref, wd_ref, fwd_ref, inv_ref,
            mod_ref, sh_ref, zm_ref, shk_ref, ssmd_ref, c_ref,
            sem, *, S, D, Fh):
    NB = S // CB
    NS = S // TM
    NL = D // 128
    NF = Fh // FC
    NK = KS // 128
    T0 = 3
    NLOOP = NS - T0
    lanes = [slice(i * 128, (i + 1) * 128) for i in range(NL)]
    cat = jnp.concatenate

    offs = [int(o) for o in np.cumsum([0, 5, NS, NS, NS, NL, 3, NF, NF, 1])]
    s_small, s_q, s_k, s_v, s_ssm, s_mod, s_g, s_u, s_d, s_o = offs

    def rows_of(t):
        return pl.ds(t * TM if isinstance(t, int) else pl.multiple_of(t * TM, TM), TM)

    def rows_cp(src, dst, base, t):
        return pltpu.make_async_copy(src.at[rows_of(t), :], dst.at[rows_of(t), :], sem.at[base + t])

    def cols_cp(src, dst, lo, hi, si):
        return pltpu.make_async_copy(src.at[:, lo:hi], dst.at[:, lo:hi], sem.at[si])

    q_cp = lambda t: rows_cp(q_hbm, q_ref, s_q, t)
    k_cp = lambda t: rows_cp(k_hbm, k_ref, s_k, t)
    v_cp = lambda t: rows_cp(v_hbm, v_ref, s_v, t)
    o_cp = lambda t: rows_cp(o_ref, o_hbm, s_o, t)
    small = [pltpu.make_async_copy(s, d, sem.at[s_small + i]) for i, (s, d) in enumerate(
        [(fwd_hbm, fwd_ref), (shk_hbm, shk_ref), (ssmd_hbm, ssmd_ref), (inv_hbm, inv_ref), (c_hbm, c_ref)])]
    ssm_cp = lambda i: pltpu.make_async_copy(ssmk_hbm.at[lanes[i], :], ssmk_ref.at[lanes[i], :],
                                             sem.at[s_ssm + i])
    mod_cols = [(0, 3 * D), (3 * D, 5 * D), (5 * D, 6 * D)]
    mod_cp = lambda i: cols_cp(wmod_hbm, wmod_ref, mod_cols[i][0], mod_cols[i][1], s_mod + i)
    g_cp = lambda f: cols_cp(wg_hbm, wg_ref, f * FC, (f + 1) * FC, s_g + f)
    u_cp = lambda f: cols_cp(wu_hbm, wu_ref, f * FC, (f + 1) * FC, s_u + f)
    d_cp = pltpu.make_async_copy(wd_hbm, wd_ref, sem.at[s_d])

    order = small + [ssm_cp(0), ssm_cp(1), k_cp(0), v_cp(0),
                     ssm_cp(2), k_cp(1), v_cp(1), ssm_cp(3), ssm_cp(4), q_cp(0), q_cp(1),
                     mod_cp(0), mod_cp(1), g_cp(0), u_cp(0), k_cp(2), v_cp(2)]
    for f in range(1, NF):
        order += [g_cp(f), u_cp(f)]
    order += [q_cp(2), d_cp, mod_cp(2), k_cp(3), v_cp(3)]
    for t in range(T0, NS):
        order += [q_cp(t)]
        if t + 1 < NS:
            order += [k_cp(t + 1), v_cp(t + 1)]
    for cp in order:
        cp.start()

    zs = []
    bg = _Sched(lambda x: pltpu.bitcast(pltpu.bitcast(x, I32) & zm_ref[...], F32))

    def opaque(ref):
        return ref.at[pl.ds(pl.multiple_of(zs[0], 32), ref.shape[0])]

    def chain(pieces, dist, extra=0, dep=None):
        hist = [] if dep is None else [dep] * dist
        for p in pieces:
            tok = None
            if len(hist) >= dist:
                tok = bg.token(hist[-dist])
                for _ in range(extra):
                    tok = tok + tok
            hist.append(p(tok))
        return hist[-1]

    def linked(pieces, d):
        res = []

        def wrap(p):
            def run(tok):
                if d and len(res) >= d:
                    tok = tok + bg.token(res[-d])
                res.append(p(tok))
            return run
        return [wrap(p) for p in pieces]

    def now(pieces):
        for p in pieces:
            p(None)

    def mod_chunk(i):
        c = c_ref[...].astype(F32)
        sc = jnp.broadcast_to((c * jax.nn.sigmoid(c)).astype(BF16), (16, D))
        lo, hi = mod_cols[i]
        m = bg.dot(sc, wmod_ref[:, lo:hi])[0:8]
        if i == 0:
            ga = m[:, 2 * D:3 * D]
            mod_ref[0] = (1.0 + m[:, D:2 * D]) * ga
            mod_ref[1] = m[:, 0:D] * ga
        elif i == 1:
            mod_ref[2] = 1.0 + m[:, D:2 * D]
            mod_ref[3] = m[:, 0:D]
        else:
            mod_ref[4] = m

    def gb_tile(i):
        def run():
            c = c_ref[...].astype(F32)
            sc = jnp.broadcast_to((c * jax.nn.sigmoid(c)).astype(BF16), (16, D))
            w = wmod_ref[:, 5 * D + i * 128:5 * D + (i + 1) * 128]
            mod_ref[4, :, lanes[i]] = jnp.dot(sc, w, preferred_element_type=F32)[0:8]
        return run

    def k_fwd(i):
        ls = lanes[i]
        fwd = fwd_ref[...]
        prev = None
        for m in range(NB):
            kf = lax.dot_general(fwd, ssmk_ref[ls, m * CB:(m + 1) * CB], (((1,), (1,)), ((), ())),
                                 preferred_element_type=F32)
            if m == 0:
                c = kf[:CB] + ssmd_ref[...].astype(F32).reshape(1, D)[:, ls]
                d = kf[CB:]
            else:
                c = kf[:CB] + prev[CB:]
                d = kf[CB:] - prev[:CB]
            prev = kf
            kk_ref[m, 0:CB, ls] = c
            kk_ref[m, CB:2 * CB, ls] = d - c
            kk_ref[m, 2 * CB:3 * CB, ls] = c + d
            if m % 4 == 3:
                bg.note(kf, 2 * CB)

    def lo_hi(w):
        return pltpu.bitcast(w << 16, F32), pltpu.bitcast(w & jnp.uint32(0xFFFF0000), F32)

    def kv_pieces(t):
        G = _E('KG', 32)
        n = G // 2
        kb, vb = k_ref.at[rows_of(t)], v_ref.at[rows_of(t)]

        def piece(ls, r0):
            def run(tok):
                if r0 > 0:
                    w = pltpu.bitcast(kb[r0 - 16:r0 + G, ls], U32)
                else:
                    if isinstance(t, int) and t == 0:
                        halo = jnp.zeros((8, 128), U32)
                    else:
                        halo = pltpu.bitcast(k_ref.at[rows_of(t - 1)][TM - 16:TM, ls], U32)
                    w = cat([halo, pltpu.bitcast(kb[0:G, ls], U32)], axis=0)
                if tok is not None:
                    w = w | _rep(pltpu.bitcast(tok, U32), n + 8)
                ke, ko = lo_hi(w[8:])
                ke1, ko1 = lo_hi(pltpu.roll(w, 1, 0)[8:])
                _, ko2 = lo_hi(pltpu.roll(w, 2, 0)[8:])
                s0, s1, s2, s3 = [_rep(sh_ref[a, :, ls], n) for a in range(4)]
                ve, vo = lo_hi(pltpu.bitcast(vb[r0:r0 + G, ls], U32))
                kve = ((ke * s0 + ko1 * s1) + (ke1 * s2 + ko2 * s3)) * ve
                kvo = ((ko * s0 + ke * s1) + (ko1 * s2 + ke1 * s3)) * vo
                kv_ref[r0 // 2:(r0 + G) // 2, ls] = pltpu.bitcast(
                    pltpu.pack_elementwise([kve, kvo], packed_dtype=BF16), U32)
            return run
        return [piece(ls, r0) for ls in lanes for r0 in range(0, TM, G)]

    def u_fwd(t):
        fwd = fwd_ref[...]
        for b in range(2):
            uf = bg.dot(fwd, _unpk(kv_ref[b * HB:(b + 1) * HB, :]))
            a, bb = uf[:CB], uf[CB:]
            u_ref[t, b, 0:CB, :] = a + bb
            u_ref[t, b, CB:2 * CB, :] = a
            u_ref[t, b, 2 * CB:3 * CB, :] = bb

    positions = [(slice(r0, r0 + 8), ls) for r0 in range(0, 3 * CB, 8) for ls in lanes]

    def ystatic_pieces(s_lo, s_hi, i_lo, i_hi, acc_in, pos=None):
        def piece(rs, ls):
            def run(tok):
                us = {i: _add(u_ref[i // 2, i % 2, rs, ls], tok) for i in range(i_lo, i_hi)}
                ks = {}
                for s in range(s_lo, s_hi):
                    acc = None
                    for i in range(i_lo, min(i_hi, s + 1)):
                        m = s - i
                        if m not in ks:
                            ks[m] = kk_ref[m, rs, ls]
                        p = ks[m] * us[i]
                        acc = p if acc is None else acc + p
                    if acc_in:
                        acc = acc + y_ref[s // 2, s % 2, rs, ls]
                    y_ref[s // 2, s % 2, rs, ls] = acc
                return acc
            return run
        return [piece(*p) for p in (positions if pos is None else pos)]

    def task_pieces(t, delta):
        p = t - delta
        left = p >= T0
        J = jnp.where(left, t, p + NLOOP)
        I = jnp.where(left, p, t)
        kview = kk_ref.at[pl.ds(2 * (J - I) - 1, 3)]

        def piece(rs, ls):
            def run(tok):
                u0 = _add(u_ref[I, 0, rs, ls], tok)
                u1 = _add(u_ref[I, 1, rs, ls], tok)
                kc = kview[1, rs, ls]
                y_ref[J, 0, rs, ls] = (kc * u0 + kview[0, rs, ls] * u1) + y_ref[J, 0, rs, ls]
                y1 = (kview[2, rs, ls] * u0 + kc * u1) + y_ref[J, 1, rs, ls]
                y_ref[J, 1, rs, ls] = y1
                return y1
            return run
        return [piece(*p) for p in positions]

    def diag_pieces(t, I):
        kview = kk_ref.at[pl.ds(2 * (t - I) - 1, 3)]

        def piece(rs, ls):
            def run(tok):
                us = [_add(u_ref[a, b, rs, ls], tok) for a in (t, I) for b in range(2)]
                k0 = kk_ref[0, rs, ls]
                kc = kview[1, rs, ls]
                y_ref[t, 0, rs, ls] = ((k0 * us[0] + y_ref[t, 0, rs, ls])
                                       + (kc * us[2] + kview[0, rs, ls] * us[3]))
                y1 = ((kk_ref[1, rs, ls] * us[0] + k0 * us[1])
                      + (kview[2, rs, ls] * us[2] + kc * us[3]) + y_ref[t, 1, rs, ls])
                y_ref[t, 1, rs, ls] = y1
                return y1
            return run
        return [piece(*p) for p in positions]

    def post_pieces(t):
        def piece(b, r0, ls):
            def run(tok):
                comp = lambda c, off: y_ref[t, b, c * CB + off + r0:c * CB + off + r0 + 16, ls]
                k1l, k1h = _add(comp(0, 0), tok), _add(comp(0, HB), tok)
                rel, reh = k1l - comp(2, 0), k1h - comp(2, HB)
                iml, imh = k1l + comp(1, 0), k1h + comp(1, HB)
                p0 = b * CB + r0 // 2
                yb_ref[p0:p0 + 8, ls] = _pk(rel + reh)
                yb_ref[p0 + HB // 2:p0 + HB // 2 + 8, ls] = _pk(iml + imh)
                yb_ref[p0 + HB:p0 + HB + 8, ls] = _pk(rel - reh)
                oim = iml - imh
                yb_ref[p0 + HB + HB // 2:p0 + HB + HB // 2 + 8, ls] = _pk(oim)
                return oim[8:16]
            return run
        return [piece(b, r0, ls) for b in range(2) for r0 in range(0, HB, 16) for ls in lanes]

    def q_split(t, b, p0, n, ls):
        w = pltpu.bitcast(q_ref.at[rows_of(t)][b * CB + 2 * p0:b * CB + 2 * p0 + 2 * n, ls], U32)
        return lo_hi(w)

    def ln_tiles(xs, tok):
        n = xs[0].shape[0]
        s = _add(xs[0], tok)
        for x in xs[1:]:
            s = s + x
        m = jnp.sum(s, axis=-1, keepdims=True) * (1.0 / D)
        xc = [x - m for x in xs]
        s2 = xc[0] * xc[0]
        for x in xc[1:]:
            s2 = s2 + x * x
        r = lax.rsqrt(jnp.sum(s2, axis=-1, keepdims=True) * (1.0 / D) + EPS)
        return xc, jnp.broadcast_to(r, (n, 128)), jnp.broadcast_to(m, (n, 128))

    def ln1_pieces(t):
        G = _E('L1G', 8)

        def piece(b, p0):
            def run(tok):
                xc, r, _ = ln_tiles([cat(q_split(t, b, p0, G, ls), axis=0) for ls in lanes], tok)
                for ls, x in zip(lanes, xc):
                    h = (x * r) * _rep(mod_ref[0, :, ls], 2 * G) + _rep(mod_ref[1, :, ls], 2 * G)
                    hp_ref[b * CB + p0:b * CB + p0 + G, ls] = h[:G]
                    hp_ref[b * CB + HB + p0:b * CB + HB + p0 + G, ls] = h[G:]
                return functools.reduce(lambda a, c: a + c, [h[r:r + 8] for r in range(0, 2 * G, 8)])
            return run
        return [piece(b, p0) for b in range(2) for p0 in range(0, HB, G)]

    def y_inv(t, x1_dst):
        yb = opaque(yb_ref)
        hp = opaque(hp_ref)
        for b in range(2):
            ye = bg.dot(inv_ref[0:HB, :], _unpk(yb[b * CB:b * CB + HB, :]))
            yo = bg.dot(inv_ref[HB:CB, :], _unpk(yb[b * CB + HB:(b + 1) * CB, :]))
            for ls in lanes:
                qe, qo = q_split(t, b, 0, HB, ls)
                re, ro = slice(b * CB, b * CB + HB), slice(b * CB + HB, (b + 1) * CB)
                x1_dst[re, ls] = qe + hp[re, ls] * ye[:, ls]
                x1_dst[ro, ls] = qo + hp[ro, ls] * yo[:, ls]

    def a_combos(a11, a12, a21, a22):
        return [a11 + a22, a21 + a22, a11 + a12, a21 - a11, a12 - a22]

    def b_combos(b11, b12, b21, b22):
        return [b11 + b22, b12 - b22, b21 - b11, b11 + b12, b21 + b22, b11, b22]

    def ln2_stat_pieces(x1_src, st):
        x1o = opaque(x1_src)

        def piece(r0):
            def run(tok):
                _, r, m = ln_tiles([x1o[r0:r0 + 16, ls] for ls in lanes], tok)
                st[r0:r0 + 16, 0:128] = m
                st[r0:r0 + 16, 128:256] = r
                return r[0:8] + r[8:16]
            return run
        return [piece(h * CB + r0) for r0 in range(0, CB, 16) for h in range(2)]

    def ln2_apply_pieces(x1_src, st, unit):
        G = 16
        x1o = opaque(x1_src)
        h2_dst = h2_ref.at[unit * CB:(unit + 1) * CB]
        h2c_dst = h2c_ref.at[unit * 5 * HB:(unit + 1) * 5 * HB]

        def piece(r0, js):
            def run(tok):
                two = lambda ref, c: cat([ref[r0:r0 + G, c], ref[CB + r0:CB + r0 + G, c]], axis=0)
                m, r = _add(two(st, slice(0, 128)), tok), two(st, slice(128, 256))
                hs = {}
                for j in js:
                    ls = lanes[j]
                    h = ((two(x1o, ls) - m) * r) * _rep(mod_ref[2, :, ls], 2 * G) + _rep(mod_ref[3, :, ls], 2 * G)
                    hs[j] = h
                    h2_dst[r0 // 2:(r0 + G) // 2, ls] = _pk(h[:G])
                    h2_dst[(CB + r0) // 2:(CB + r0 + G) // 2, ls] = _pk(h[G:])
                    if NK <= j < 2 * NK:
                        cs = a_combos(hs[j - NK][:G], h[:G], hs[j - NK][G:], h[G:])
                        for i, cmb in enumerate(cs):
                            h2c_dst[i * HB + r0 // 2:i * HB + (r0 + G) // 2, lanes[j - NK]] = _pk(cmb)
            return run
        parts = [[j, NK + j] for j in range(NK)]
        parts[-1] += list(range(2 * NK, NL))
        return [piece(r0, js) for r0 in range(0, CB, G) for js in parts]

    def strassen(sa, a11, a22, tb, rem):
        dot = bg.dot
        m1 = dot(sa[0], tb[0])
        if rem is None:
            m7 = dot(sa[4], tb[4])
        else:
            m7 = dot(cat([sa[4], rem[0]], axis=1), cat([tb[4], rem[2]], axis=0))
        m4 = dot(a22, tb[2])
        m2 = dot(sa[1], tb[5])
        c21 = m2 + m4
        if rem is not None:
            c21 = c21 + dot(rem[1], rem[2])
        m5 = dot(sa[2], tb[6])
        c11 = m1 + m7 + m4 - m5
        m3 = dot(a11, tb[1])
        c12 = m3 + m5
        if rem is None:
            m6 = dot(sa[3], tb[3])
        else:
            c12 = c12 + dot(rem[0], rem[3])
            m6 = dot(cat([sa[3], rem[1]], axis=1), cat([tb[3], rem[3]], axis=0))
        c22 = m1 - m2 + m3 + m6
        return c11, c12, c21, c22

    def wgu_pieces(f):
        G = 16
        cl, cr = slice(f * FC, f * FC + 128), slice(f * FC + 128, (f + 1) * FC)

        def piece(w_ref, wc_ref, wr_ref, r0):
            def run(tok):
                b11 = _add(w_ref[r0:r0 + G, cl].astype(F32), tok)
                b22 = _add(w_ref[KS + r0:KS + r0 + G, cr].astype(F32), tok)
                cs = b_combos(b11, w_ref[r0:r0 + G, cr].astype(F32),
                              w_ref[KS + r0:KS + r0 + G, cl].astype(F32), b22)
                for i, cmb in enumerate(cs):
                    wc_ref[(i * KS + r0) // 2:(i * KS + r0 + G) // 2, f * 128:(f + 1) * 128] = _pk(cmb)
                if r0 < D - 2 * KS:
                    for c in (cl, cr):
                        w = pltpu.bitcast(w_ref[2 * KS + r0:2 * KS + r0 + G, c], U32)
                        wr_ref[r0 // 2:(r0 + G) // 2, c] = w if tok is None else w | pltpu.bitcast(tok, U32)
            return run
        return [piece(*refs, r0) for refs in ((wg_ref, wgc_ref, wgr_ref), (wu_ref, wuc_ref, wur_ref))
                for r0 in range(0, KS, G)]

    def wd_pieces():
        G = 16

        def piece(j, f, r0):
            def run(tok):
                cl, cr = lanes[j], lanes[NK + j]
                re = slice(f * FC + r0, f * FC + r0 + G)
                ro = slice(f * FC + 128 + r0, f * FC + 128 + r0 + G)
                b11 = _add(wd_ref[re, cl].astype(F32), tok)
                b22 = _add(wd_ref[ro, cr].astype(F32), tok)
                cs = b_combos(b11, wd_ref[re, cr].astype(F32), wd_ref[ro, cl].astype(F32), b22)
                for i, cmb in enumerate(cs):
                    p0 = i * (Fh // 4) + (f * 128 + r0) // 2
                    wdc_ref[p0:p0 + G // 2, cl] = _pk(cmb)
            return run
        return [piece(j, f, r0) for j in range(NK) for f in range(NF) for r0 in range(0, 128, G)]

    def wdr_pieces():
        G = 128

        def piece(r0):
            def run(tok):
                w = pltpu.bitcast(wd_ref[r0:r0 + G, lanes[NL - 1]], U32)
                wdr_ref[r0 // 2:(r0 + G) // 2, :] = w | _rep(pltpu.bitcast(tok, U32), G // 2)
            return run
        return [piece(r0) for r0 in range(0, Fh, G)]

    def ffn_gu(f, unit, plain=False):
        cl, cr = slice(f * FC, f * FC + 128), slice(f * FC + 128, (f + 1) * FC)
        h2 = h2_ref.at[unit * CB:(unit + 1) * CB]
        h2c = h2c_ref.at[unit * 5 * HB:(unit + 1) * 5 * HB]
        if plain:
            p11, p12, p21, p22 = [
                bg.dot(_unpk(h2[r:r + HB, :]), wg_ref[:, c]) * bg.dot(_unpk(h2[r:r + HB, :]), wu_ref[:, c])
                for r in (0, HB) for c in (cl, cr)]
        else:
            res = []
            for wr, wc in ((wgr_ref, wgc_ref), (wur_ref, wuc_ref)):
                sa = [_unpk(h2c[i * HB:(i + 1) * HB, :]) for i in range(5)]
                tb = [_unpk(wc[i * KS // 2:(i + 1) * KS // 2, f * 128:(f + 1) * 128]) for i in range(7)]
                rem = (_unpk(h2[0:HB, 2 * KS:D]), _unpk(h2[HB:CB, 2 * KS:D]), _unpk(wr[:, cl]), _unpk(wr[:, cr]))
                res.append(strassen(sa, _unpk(h2[0:HB, 0:KS]), _unpk(h2[HB:CB, KS:2 * KS]), tb, rem))
            p11, p12, p21, p22 = [g * u for g, u in zip(*res)]
        hh = hh_ref.at[unit * CB:(unit + 1) * CB]
        hhc = hhc_ref.at[unit * 5 * HB:(unit + 1) * 5 * HB]
        hh[0:HB, cl] = _pk(p11)
        hh[0:HB, cr] = _pk(p12)
        hh[HB:CB, cl] = _pk(p21)
        hh[HB:CB, cr] = _pk(p22)
        for i, cmb in enumerate(a_combos(p11, p12, p21, p22)):
            hhc[i * HB:(i + 1) * HB, f * 128:(f + 1) * 128] = _pk(cmb)

    def ffn_down(x1_src, t, unit):
        hh = hh_ref.at[unit * CB:(unit + 1) * CB]
        hhc = hhc_ref.at[unit * 5 * HB:(unit + 1) * 5 * HB]
        ob = o_ref.at[rows_of(t)]

        def emit(dn, b, ls):
            o = x1_src[b * CB:(b + 1) * CB, ls] + _rep(mod_ref[4, :, ls], CB) * dn
            w = pltpu.pack_elementwise([o[:HB], o[HB:]], packed_dtype=BF16)
            ob[b * CB:(b + 1) * CB, ls] = pltpu.bitcast(w, BF16)

        for b in range(2):
            KC = _E('KC', 512)
            ps = [bg.dot(_unpk(hh[b * HB:(b + 1) * HB, k0:k0 + KC]), _unpk(wdr_ref[k0 // 2:(k0 + KC) // 2, :]))
                  for k0 in range(0, Fh, KC)]
            emit(functools.reduce(lambda x, y: x + y, ps), b, lanes[NL - 1])
        for j in range(NK):
            cl, cr = lanes[j], lanes[NK + j]
            sa = [_unpk(hhc[i * HB:(i + 1) * HB, :]) for i in range(5)]
            a11 = cat([_unpk(hh[0:HB, f * FC:f * FC + 128]) for f in range(NF)], axis=1)
            a22 = cat([_unpk(hh[HB:CB, f * FC + 128:(f + 1) * FC]) for f in range(NF)], axis=1)
            tb = [_unpk(wdc_ref[i * (Fh // 4):(i + 1) * (Fh // 4), cl]) for i in range(7)]
            c11, c12, c21, c22 = strassen(sa, a11, a22, tb, None)
            emit(c21, 1, cl)
            emit(c11, 0, cl)
            emit(c12, 0, cr)
            emit(c22, 1, cr)

    x1s = [x1s_ref.at[r * TM:(r + 1) * TM] for r in range(2)]
    sts = [st_ref.at[r * TM:(r + 1) * TM] for r in range(2)]
    YP = _E('YP', 12)

    def prologue():
        for cp in small:
            cp.wait()
        shk = shk_ref[...].astype(F32)
        for a in range(4):
            sh_ref[a] = jnp.broadcast_to(shk[a:a + 1, :], (8, D))
        zm_ref[...] = pltpu.bitcast(inv_ref[CB:CB + 16, :], I32)
        zs.append(zm_ref[0, 0])
        ssm_cp(0).wait()
        k_fwd(0)
        ssm_cp(1).wait()
        k_fwd(1)
        for t in range(2):
            k_cp(t).wait()
            v_cp(t).wait()
            ssm_cp(2 + t).wait()
            now(kv_pieces(t))
            k_fwd(2 + t)
            u_fwd(t)
        ssm_cp(4).wait()
        bg.flush()
        pos = sorted(positions, key=lambda p: p[1].start)
        n0 = _E('PY0', 32)
        bg.add(ystatic_pieces(0, YP, 0, 4, False, pos[:n0]), 0, 1024)
        bg.add(ystatic_pieces(0, YP, 0, 4, False, pos[n0:n0 + 1]), 5000, 5001)
        k_fwd(4)
        bg.flush()
        q_cp(0).wait()
        now(ystatic_pieces(0, YP, 0, 4, False, pos[n0 + 1:]))
        q_cp(1).wait()
        mod_cp(0).wait()
        mod_chunk(0)
        for t in range(2):
            now(post_pieces(t))
            now(ln1_pieces(t))
            y_inv(t, x1s[t])
        for t in range(2):
            now(ln2_stat_pieces(x1s[t], sts[t]))
        mod_cp(1).wait()
        mod_chunk(1)
        for t in range(2):
            now(ln2_apply_pieces(x1s[t], sts[t], t))
        bg.flush()

    def superstep():
        yrest = ystatic_pieces(YP, NB, 0, 4, False)
        g_cp(0).wait()
        u_cp(0).wait()
        bg.add(wgu_pieces(0), 0, 900)
        bg.add(yrest[0:50], 1000, 2200)
        ffn_gu(0, 0, plain=True)
        ffn_gu(0, 1)
        bg.flush()
        k_cp(2).wait()
        v_cp(2).wait()
        g_cp(1).wait()
        u_cp(1).wait()
        bg.add(wgu_pieces(1), 0, 900)
        bg.add(kv_pieces(2), 1000, 2200)
        ffn_gu(1, 0, plain=True)
        ffn_gu(1, 1)
        bg.flush()
        for f in range(2, 4):
            g_cp(f).wait()
            u_cp(f).wait()
        bg.add(wgu_pieces(2), 0, 900)
        bg.add(wgu_pieces(3), 1900, 2700)
        bg.add(yrest[50:110], 2800, 4000)
        ffn_gu(2, 0, plain=True)
        u_fwd(2)
        ffn_gu(2, 1)
        ffn_gu(3, 0)
        bg.flush()
        for f in range(4, NF):
            g_cp(f).wait()
            u_cp(f).wait()
        q_cp(2).wait()
        bg.add(wgu_pieces(4), 0, 800)
        bg.add(wgu_pieces(5), 800, 1600)
        bg.add(_group(ystatic_pieces(4, 6, 4, 6, True), 3), 1600, 3000)
        bg.add(post_pieces(2), 3100, 3700)
        bg.add(yrest[110:140], 3700, 4400)
        bg.add(linked(ln1_pieces(2), _E('LK', 3)), 1600, 4000)
        ffn_gu(3, 1)
        ffn_gu(4, 0)
        ffn_gu(4, 1)
        ffn_gu(5, 0)
        bg.flush()
        d_cp.wait()
        mod_cp(2).wait()
        k_cp(3).wait()
        v_cp(3).wait()
        bg.add(wdr_pieces(), 0, 300)
        bg.add(wd_pieces(), 300, 3100)
        t1 = 1152 + 320
        bg.add(linked(ln2_stat_pieces(x1_ref.at[0], st_ref), _E('LK2', 3)), t1 + 1700, t1 + 3400)
        bg.add(ln2_apply_pieces(x1_ref.at[0], st_ref, 0), t1 + 3000, t1 + 4700)
        bg.add(kv_pieces(3), 3200, 5400)
        bg.add(yrest[140:], 5500, 8300)
        bg.inj = [(150 + 200 * i, gb_tile(i)) for i in range(NL)]
        ffn_gu(5, 1)
        y_inv(2, x1_ref.at[0])
        ffn_down(x1s[0], 0, 0)
        ffn_down(x1s[1], 1, 1)
        bg.flush()
        o_cp(0).start()
        o_cp(1).start()
        for t in range(T0, NS):
            q_cp(t).wait()
            if t + 1 < NS:
                k_cp(t + 1).wait()
                v_cp(t + 1).wait()

    def step(t, carry):
        slot = lax.rem(t, 2)
        if _E('LA', 1):
            bg.add(linked(ln1_pieces(t), _E('LK1', 2)), _E('L0', 800), _E('L1', 6800))
        t1 = 640 + NF * 1152 + 320
        bg.add(linked(ln2_stat_pieces(x1_ref.at[slot], st_ref), _E('LK2', 3)), t1 + _E('S0', 100), t1 + _E('S1', 1800))
        bg.add(ln2_apply_pieces(x1_ref.at[slot], st_ref, 0), t1 + _E('P0', 1400), t1 + _E('P1', 3100))
        bg.add(kv_pieces(jnp.minimum(t + 1, NS - 1)), t1 + _E('K0', 100), t1 + _E('K1', 3100))
        u_fwd(t)
        chain(diag_pieces(t, T0 - 1), _E('DD', 2), _E('DE', 0))
        chain(task_pieces(t, 2), _E('MD', 2), _E('ME', 0))
        dep = chain(task_pieces(t, 1), _E('MD', 2), _E('ME', 0))
        chain(post_pieces(t), 1, 3, dep)
        if not _E('LA', 1):
            chain(ln1_pieces(t), 1)
        for f in range(NF):
            ffn_gu(f, 0)
        y_inv(t, x1_ref.at[slot])
        ffn_down(x1_ref.at[1 - slot], t - 1, 0)
        bg.flush()
        o_cp(t - 1).start()
        return carry

    def epilogue():
        t = NS - 1
        for f in range(NF):
            ffn_gu(f, 0)
        ffn_down(x1_ref.at[t % 2], t, 0)
        o_cp(t).start()
        for i in range(NS):
            o_cp(i).wait()

    if SCOPES:
        jax.named_scope("prologue")(prologue)()
        jax.named_scope("superstep")(superstep)()
        lax.fori_loop(T0, NS, jax.named_scope("step")(step), 0)
        jax.named_scope("epilogue")(epilogue)()
    elif ONLY == 'loop':
        zs.append(zm_ref[0, 0])
        lax.fori_loop(T0, NS, step, 0)
        epilogue()
    elif ONLY == 'S':
        zs.append(zm_ref[0, 0])
        superstep()
        lax.fori_loop(T0, NS, step, 0)
    else:
        prologue()
        superstep()
        lax.fori_loop(T0, NS, step, 0)
        epilogue()


@jax.jit
def pallas_adaLN_cond__ssm_conv_h3__glu_gated_bilinear__prompt_kernel(
    A_q, A_k, A_v, A_shift_k, A_ssm_k, A_ssm_D, B_x, B_w_gate, B_w_up, B_w_down, c, w_mod,
):
    B, S, D = A_q.shape
    Fh = B_w_gate.shape[1]
    NB = S // CB
    NS = S // TM
    fwd, inv = _dft_consts()
    anyspec = pl.BlockSpec(memory_space=pl.ANY)
    V = pltpu.VMEM
    out = pl.pallas_call(
        functools.partial(_kernel, S=S, D=D, Fh=Fh),
        in_specs=[anyspec] * 13,
        out_specs=anyspec,
        out_shape=jax.ShapeDtypeStruct((S, D), A_q.dtype),
        scratch_shapes=[
            V((NS, 2, 3 * CB, D), F32),
            V((NB, 3 * CB, D), F32),
            V((NS, 2, 3 * CB, D), F32),
            V((2, TM, D), F32),
            V((S, D), BF16), V((S, D), BF16), V((S, D), BF16), V((S, D), BF16),
            V((2 * TM, D), F32),
            V((TM, D), F32),
            V((2 * TM, 256), F32),
            V((2 * CB, D), U32),
            V((2 * 5 * HB, KS), U32),
            V((2 * CB, Fh), U32),
            V((2 * 5 * HB, Fh // 2), U32),
            V((TM // 2, D), U32),
            V((2 * CB, D), U32),
            V(((D - 2 * KS) // 2, Fh), U32), V(((D - 2 * KS) // 2, Fh), U32), V((Fh // 2, D - 2 * KS), U32),
            V((7 * KS // 2, Fh // 2), U32), V((7 * KS // 2, Fh // 2), U32), V((7 * Fh // 4, KS), U32),
            V((D, S), BF16), V((D, 6 * D), BF16), V((D, Fh), BF16), V((D, Fh), BF16), V((Fh, D), BF16),
            V((2 * CB, CB), BF16), V((CB + 16, CB), BF16),
            V((5, 8, D), F32), V((4, 8, D), F32), V((8, 128), I32),
            V((4, D), BF16), V((D,), BF16), V((1, D), BF16),
            pltpu.SemaphoreType.DMA((5 + 4 * NS + D // 128 + 3 + 2 * (Fh // FC) + 1,)),
        ],
        compiler_params=pltpu.CompilerParams(
            internal_scratch_in_bytes=48 * 1024,
            disable_semaphore_checks=True,
            vmem_limit_bytes=110 * 1024 * 1024),
        name="adaln_h3_glu",
    )(A_q.reshape(S, D), A_k.reshape(S, D), A_v.reshape(S, D), A_shift_k.T, A_ssm_k,
      A_ssm_D, B_w_gate, B_w_up, B_w_down, c, w_mod, fwd, inv)
    return out.reshape(B, S, D)
```

```python
import functools
import os

import numpy as np
import jax
import jax.numpy as jnp
from jax import lax
import jax.experimental.pallas as pl
import jax.experimental.pallas.tpu as pltpu

F32 = jnp.float32
BF16 = jnp.bfloat16
U32 = jnp.uint32
I32 = jnp.int32

CB = 128
HB = CB // 2
TM = 256
FC = 256
KS = 256
EPS = 1e-5
SCOPES = False
ONLY = os.environ.get('ONLY', '')


def _E(name, default):
    return int(os.environ.get(name, default))


def _dft_consts():
    k = np.arange(CB, dtype=np.float64)[:, None]
    n = np.arange(CB, dtype=np.float64)[None, :]
    th = np.pi * (4.0 * k + 1.0) * n / (2.0 * CB)
    fwd = np.concatenate([np.cos(th), np.sin(th)], axis=0)
    g = np.concatenate([np.cos(th[:HB]), np.sin(th[:HB])], axis=0).T / CB
    inv = np.concatenate([g[0::2], g[1::2], np.zeros((16, CB))], axis=0)
    return jnp.asarray(fwd, dtype=BF16), jnp.asarray(inv, dtype=BF16)


def _pk(x):
    return pltpu.bitcast(x.astype(BF16), U32)


def _unpk(x):
    return pltpu.bitcast(x, BF16)


def _rep(r, n):
    return r if n == 8 else jnp.concatenate([r] * (n // 8), axis=0)


def _add(x, tok):
    return x if tok is None else x + _rep(tok, x.shape[0])


def _group(pieces, n):
    def merged(ps):
        def run(tok):
            for p in ps:
                p(tok)
        return run
    return [merged(pieces[i:i + n]) for i in range(0, len(pieces), n)]


class _Sched:
    def __init__(self, token):
        self.token = token
        self.clock = 0.0
        self.q = []
        self.last = None
        self.inj = []

    def add(self, pieces, t0, t1):
        n = len(pieces)
        self.q += [(t0 + (t1 - t0) * i / n, len(self.q) + i, p) for i, p in enumerate(pieces)]
        self.q.sort(key=lambda e: e[:2])

    def note(self, m, dt):
        rows, cols = m.shape
        tiles = [(slice(r, r + 8), slice(c, c + 128)) for c in range(0, cols, 128) for r in range(0, rows, 8)]
        for i, tl in enumerate(tiles):
            tok = None
            while self.q and self.q[0][0] <= self.clock + dt * (i + 1) / len(tiles):
                if tok is None:
                    tok = self.token(m[tl])
                self.q.pop(0)[2](tok)
        self.clock += dt
        self.last = m[tiles[-1]]
        return m

    def dot(self, a, b):
        if self.inj and self.clock >= self.inj[0][0]:
            self.inj.pop(0)[1]()
        m = jnp.dot(a, b, preferred_element_type=F32)
        return self.note(m, max(a.shape[0], 32) * (a.shape[1] // 128) * (b.shape[1] // 128) / 4)

    def flush(self):
        tok = None if self.last is None or not self.q else self.token(self.last)
        while self.q:
            self.q.pop(0)[2](tok)
        self.clock = 0.0
        self.last = None


def _kernel(q_hbm, k_hbm, v_hbm, shk_hbm, ssmk_hbm, ssmd_hbm, wg_hbm, wu_hbm, wd_hbm,
            c_hbm, wmod_hbm, fwd_hbm, inv_hbm, o_hbm,
            u_ref, kk_ref, y_ref, x1_ref, q_ref, k_ref, v_ref, o_ref,
            x1s_ref, hp_ref, st_ref, h2_ref, h2c_ref, hh_ref, hhc_ref, kv_ref, yb_ref,
            wgr_ref, wur_ref, wdr_ref, wgc_ref, wuc_ref, wdc_ref,
            ssmk_ref, wmod_ref, wg_ref, wu_ref, wd_ref, fwd_ref, inv_ref,
            mod_ref, sh_ref, zm_ref, shk_ref, ssmd_ref, c_ref,
            sem, *, S, D, Fh):
    NB = S // CB
    NS = S // TM
    NL = D // 128
    NF = Fh // FC
    NK = KS // 128
    T0 = 3
    NLOOP = NS - T0
    lanes = [slice(i * 128, (i + 1) * 128) for i in range(NL)]
    cat = jnp.concatenate

    offs = [int(o) for o in np.cumsum([0, 5, NS, NS, NS, NL, 3, NF, NF, 1])]
    s_small, s_q, s_k, s_v, s_ssm, s_mod, s_g, s_u, s_d, s_o = offs

    def rows_of(t):
        return pl.ds(t * TM if isinstance(t, int) else pl.multiple_of(t * TM, TM), TM)

    def rows_cp(src, dst, base, t):
        return pltpu.make_async_copy(src.at[rows_of(t), :], dst.at[rows_of(t), :], sem.at[base + t])

    def cols_cp(src, dst, lo, hi, si):
        return pltpu.make_async_copy(src.at[:, lo:hi], dst.at[:, lo:hi], sem.at[si])

    q_cp = lambda t: rows_cp(q_hbm, q_ref, s_q, t)
    k_cp = lambda t: rows_cp(k_hbm, k_ref, s_k, t)
    v_cp = lambda t: rows_cp(v_hbm, v_ref, s_v, t)
    o_cp = lambda t: rows_cp(o_ref, o_hbm, s_o, t)
    small = [pltpu.make_async_copy(s, d, sem.at[s_small + i]) for i, (s, d) in enumerate(
        [(fwd_hbm, fwd_ref), (shk_hbm, shk_ref), (ssmd_hbm, ssmd_ref), (inv_hbm, inv_ref), (c_hbm, c_ref)])]
    ssm_cp = lambda i: pltpu.make_async_copy(ssmk_hbm.at[lanes[i], :], ssmk_ref.at[lanes[i], :],
                                             sem.at[s_ssm + i])
    mod_cols = [(0, 3 * D), (3 * D, 5 * D), (5 * D, 6 * D)]
    mod_cp = lambda i: cols_cp(wmod_hbm, wmod_ref, mod_cols[i][0], mod_cols[i][1], s_mod + i)
    g_cp = lambda f: cols_cp(wg_hbm, wg_ref, f * FC, (f + 1) * FC, s_g + f)
    u_cp = lambda f: cols_cp(wu_hbm, wu_ref, f * FC, (f + 1) * FC, s_u + f)
    d_cp = pltpu.make_async_copy(wd_hbm, wd_ref, sem.at[s_d])

    order = small + [ssm_cp(0), ssm_cp(1), k_cp(0), v_cp(0),
                     ssm_cp(2), k_cp(1), v_cp(1), ssm_cp(3), ssm_cp(4), q_cp(0), q_cp(1),
                     mod_cp(0), mod_cp(1), g_cp(0), u_cp(0), k_cp(2), v_cp(2)]
    for f in range(1, NF):
        order += [g_cp(f), u_cp(f)]
    order += [q_cp(2), d_cp, mod_cp(2), k_cp(3), v_cp(3)]
    for t in range(T0, NS):
        order += [q_cp(t)]
        if t + 1 < NS:
            order += [k_cp(t + 1), v_cp(t + 1)]
    for cp in order:
        cp.start()

    zs = []
    bg = _Sched(lambda x: pltpu.bitcast(pltpu.bitcast(x, I32) & zm_ref[...], F32))

    def opaque(ref):
        return ref.at[pl.ds(pl.multiple_of(zs[0], 32), ref.shape[0])]

    def chain(pieces, dist, extra=0, dep=None):
        hist = [] if dep is None else [dep] * dist
        for p in pieces:
            tok = None
            if len(hist) >= dist:
                tok = bg.token(hist[-dist])
                for _ in range(extra):
                    tok = tok + tok
            hist.append(p(tok))
        return hist[-1]

    def linked(pieces, d):
        res = []

        def wrap(p):
            def run(tok):
                if d and len(res) >= d:
                    tok = tok + bg.token(res[-d])
                res.append(p(tok))
            return run
        return [wrap(p) for p in pieces]

    def now(pieces):
        for p in pieces:
            p(None)

    def mod_chunk(i):
        c = c_ref[...].astype(F32)
        sc = jnp.broadcast_to((c * jax.nn.sigmoid(c)).astype(BF16), (16, D))
        lo, hi = mod_cols[i]
        m = bg.dot(sc, wmod_ref[:, lo:hi])[0:8]
        if i == 0:
            ga = m[:, 2 * D:3 * D]
            mod_ref[0] = (1.0 + m[:, D:2 * D]) * ga
            mod_ref[1] = m[:, 0:D] * ga
        elif i == 1:
            mod_ref[2] = 1.0 + m[:, D:2 * D]
            mod_ref[3] = m[:, 0:D]
        else:
            mod_ref[4] = m

    def gb_tile(i):
        def run():
            c = c_ref[...].astype(F32)
            sc = jnp.broadcast_to((c * jax.nn.sigmoid(c)).astype(BF16), (16, D))
            w = wmod_ref[:, 5 * D + i * 128:5 * D + (i + 1) * 128]
            mod_ref[4, :, lanes[i]] = jnp.dot(sc, w, preferred_element_type=F32)[0:8]
        return run

    def k_fwd(i):
        ls = lanes[i]
        fwd = fwd_ref[...]
        prev = None
        for m in range(NB):
            kf = lax.dot_general(fwd, ssmk_ref[ls, m * CB:(m + 1) * CB], (((1,), (1,)), ((), ())),
                                 preferred_element_type=F32)
            if m == 0:
                c = kf[:CB] + ssmd_ref[...].astype(F32).reshape(1, D)[:, ls]
                d = kf[CB:]
            else:
                c = kf[:CB] + prev[CB:]
                d = kf[CB:] - prev[:CB]
            prev = kf
            kk_ref[m, 0:CB, ls] = c
            kk_ref[m, CB:2 * CB, ls] = d - c
            kk_ref[m, 2 * CB:3 * CB, ls] = c + d
            if m % 4 == 3:
                bg.note(kf, 2 * CB)

    def lo_hi(w):
        return pltpu.bitcast(w << 16, F32), pltpu.bitcast(w & jnp.uint32(0xFFFF0000), F32)

    def kv_pieces(t, G=32):
        n = G // 2
        kb, vb = k_ref.at[rows_of(t)], v_ref.at[rows_of(t)]

        def piece(ls, r0):
            def run(tok):
                if r0 > 0:
                    w = pltpu.bitcast(kb[r0 - 16:r0 + G, ls], U32)
                else:
                    if isinstance(t, int) and t == 0:
                        halo = jnp.zeros((8, 128), U32)
                    else:
                        halo = pltpu.bitcast(k_ref.at[rows_of(t - 1)][TM - 16:TM, ls], U32)
                    w = cat([halo, pltpu.bitcast(kb[0:G, ls], U32)], axis=0)
                if tok is not None:
                    w = w | _rep(pltpu.bitcast(tok, U32), n + 8)
                ke, ko = lo_hi(w[8:])
                ke1, ko1 = lo_hi(pltpu.roll(w, 1, 0)[8:])
                _, ko2 = lo_hi(pltpu.roll(w, 2, 0)[8:])
                s0, s1, s2, s3 = [_rep(sh_ref[a, :, ls], n) for a in range(4)]
                ve, vo = lo_hi(pltpu.bitcast(vb[r0:r0 + G, ls], U32))
                kve = ((ke * s0 + ko1 * s1) + (ke1 * s2 + ko2 * s3)) * ve
                kvo = ((ko * s0 + ke * s1) + (ko1 * s2 + ke1 * s3)) * vo
                kv_ref[r0 // 2:(r0 + G) // 2, ls] = pltpu.bitcast(
                    pltpu.pack_elementwise([kve, kvo], packed_dtype=BF16), U32)
            return run
        return [piece(ls, r0) for ls in lanes for r0 in range(0, TM, G)]

    def u_fwd(t):
        fwd = fwd_ref[...]
        for b in range(2):
            uf = bg.dot(fwd, _unpk(kv_ref[b * HB:(b + 1) * HB, :]))
            a, bb = uf[:CB], uf[CB:]
            u_ref[t, b, 0:CB, :] = a + bb
            u_ref[t, b, CB:2 * CB, :] = a
            u_ref[t, b, 2 * CB:3 * CB, :] = bb

    positions = [(slice(r0, r0 + 8), ls) for r0 in range(0, 3 * CB, 8) for ls in lanes]

    def ystatic_pieces(s_lo, s_hi, i_lo, i_hi, acc_in, pos=None):
        def piece(rs, ls):
            def run(tok):
                us = {i: _add(u_ref[i // 2, i % 2, rs, ls], tok) for i in range(i_lo, i_hi)}
                ks = {}
                for s in range(s_lo, s_hi):
                    acc = None
                    for i in range(i_lo, min(i_hi, s + 1)):
                        m = s - i
                        if m not in ks:
                            ks[m] = kk_ref[m, rs, ls]
                        p = ks[m] * us[i]
                        acc = p if acc is None else acc + p
                    if acc_in:
                        acc = acc + y_ref[s // 2, s % 2, rs, ls]
                    y_ref[s // 2, s % 2, rs, ls] = acc
                return acc
            return run
        return [piece(*p) for p in (positions if pos is None else pos)]

    def task_pieces(t, delta):
        p = t - delta
        left = p >= T0
        J = jnp.where(left, t, p + NLOOP)
        I = jnp.where(left, p, t)
        kview = kk_ref.at[pl.ds(2 * (J - I) - 1, 3)]

        def piece(rs, ls):
            def run(tok):
                u0 = _add(u_ref[I, 0, rs, ls], tok)
                u1 = _add(u_ref[I, 1, rs, ls], tok)
                kc = kview[1, rs, ls]
                y_ref[J, 0, rs, ls] = (kc * u0 + kview[0, rs, ls] * u1) + y_ref[J, 0, rs, ls]
                y1 = (kview[2, rs, ls] * u0 + kc * u1) + y_ref[J, 1, rs, ls]
                y_ref[J, 1, rs, ls] = y1
                return y1
            return run
        return [piece(*p) for p in positions]

    def diag_pieces(t, I):
        kview = kk_ref.at[pl.ds(2 * (t - I) - 1, 3)]

        def piece(rs, ls):
            def run(tok):
                us = [_add(u_ref[a, b, rs, ls], tok) for a in (t, I) for b in range(2)]
                k0 = kk_ref[0, rs, ls]
                kc = kview[1, rs, ls]
                y_ref[t, 0, rs, ls] = ((k0 * us[0] + y_ref[t, 0, rs, ls])
                                       + (kc * us[2] + kview[0, rs, ls] * us[3]))
                y1 = ((kk_ref[1, rs, ls] * us[0] + k0 * us[1])
                      + (kview[2, rs, ls] * us[2] + kc * us[3]) + y_ref[t, 1, rs, ls])
                y_ref[t, 1, rs, ls] = y1
                return y1
            return run
        return [piece(*p) for p in positions]

    def post_pieces(t):
        def piece(b, r0, ls):
            def run(tok):
                comp = lambda c, off: y_ref[t, b, c * CB + off + r0:c * CB + off + r0 + 16, ls]
                k1l, k1h = _add(comp(0, 0), tok), _add(comp(0, HB), tok)
                rel, reh = k1l - comp(2, 0), k1h - comp(2, HB)
                iml, imh = k1l + comp(1, 0), k1h + comp(1, HB)
                p0 = b * CB + r0 // 2
                yb_ref[p0:p0 + 8, ls] = _pk(rel + reh)
                yb_ref[p0 + HB // 2:p0 + HB // 2 + 8, ls] = _pk(iml + imh)
                yb_ref[p0 + HB:p0 + HB + 8, ls] = _pk(rel - reh)
                oim = iml - imh
                yb_ref[p0 + HB + HB // 2:p0 + HB + HB // 2 + 8, ls] = _pk(oim)
                return oim[8:16]
            return run
        return [piece(b, r0, ls) for b in range(2) for r0 in range(0, HB, 16) for ls in lanes]

    def q_split(t, b, p0, n, ls):
        w = pltpu.bitcast(q_ref.at[rows_of(t)][b * CB + 2 * p0:b * CB + 2 * p0 + 2 * n, ls], U32)
        return lo_hi(w)

    def ln_tiles(xs, tok):
        n = xs[0].shape[0]
        s = _add(xs[0], tok)
        for x in xs[1:]:
            s = s + x
        m = jnp.sum(s, axis=-1, keepdims=True) * (1.0 / D)
        xc = [x - m for x in xs]
        s2 = xc[0] * xc[0]
        for x in xc[1:]:
            s2 = s2 + x * x
        r = lax.rsqrt(jnp.sum(s2, axis=-1, keepdims=True) * (1.0 / D) + EPS)
        return xc, jnp.broadcast_to(r, (n, 128)), jnp.broadcast_to(m, (n, 128))

    def ln1_pieces(t):
        G = _E('L1G', 8)

        def piece(b, p0):
            def run(tok):
                xc, r, _ = ln_tiles([cat(q_split(t, b, p0, G, ls), axis=0) for ls in lanes], tok)
                for ls, x in zip(lanes, xc):
                    h = (x * r) * _rep(mod_ref[0, :, ls], 2 * G) + _rep(mod_ref[1, :, ls], 2 * G)
                    hp_ref[b * CB + p0:b * CB + p0 + G, ls] = h[:G]
                    hp_ref[b * CB + HB + p0:b * CB + HB + p0 + G, ls] = h[G:]
                return functools.reduce(lambda a, c: a + c, [h[r:r + 8] for r in range(0, 2 * G, 8)])
            return run
        return [piece(b, p0) for b in range(2) for p0 in range(0, HB, G)]

    def y_inv(t, x1_dst):
        yb = opaque(yb_ref)
        hp = opaque(hp_ref)
        for b in range(2):
            ye = bg.dot(inv_ref[0:HB, :], _unpk(yb[b * CB:b * CB + HB, :]))
            yo = bg.dot(inv_ref[HB:CB, :], _unpk(yb[b * CB + HB:(b + 1) * CB, :]))
            for ls in lanes:
                qe, qo = q_split(t, b, 0, HB, ls)
                re, ro = slice(b * CB, b * CB + HB), slice(b * CB + HB, (b + 1) * CB)
                x1_dst[re, ls] = qe + hp[re, ls] * ye[:, ls]
                x1_dst[ro, ls] = qo + hp[ro, ls] * yo[:, ls]

    def a_combos(a11, a12, a21, a22):
        return [a11 + a22, a21 + a22, a11 + a12, a21 - a11, a12 - a22]

    def b_combos(b11, b12, b21, b22):
        return [b11 + b22, b12 - b22, b21 - b11, b11 + b12, b21 + b22, b11, b22]

    def ln2_stat_pieces(x1_src, st):
        x1o = opaque(x1_src)

        def piece(r0):
            def run(tok):
                _, r, m = ln_tiles([x1o[r0:r0 + 16, ls] for ls in lanes], tok)
                st[r0:r0 + 16, 0:128] = m
                st[r0:r0 + 16, 128:256] = r
                return r[0:8] + r[8:16]
            return run
        return [piece(h * CB + r0) for r0 in range(0, CB, 16) for h in range(2)]

    def ln2_apply_pieces(x1_src, st, unit):
        G = 16
        x1o = opaque(x1_src)
        h2_dst = h2_ref.at[unit * CB:(unit + 1) * CB]
        h2c_dst = h2c_ref.at[unit * 5 * HB:(unit + 1) * 5 * HB]

        def piece(r0, js):
            def run(tok):
                two = lambda ref, c: cat([ref[r0:r0 + G, c], ref[CB + r0:CB + r0 + G, c]], axis=0)
                m, r = _add(two(st, slice(0, 128)), tok), two(st, slice(128, 256))
                hs = {}
                for j in js:
                    ls = lanes[j]
                    h = ((two(x1o, ls) - m) * r) * _rep(mod_ref[2, :, ls], 2 * G) + _rep(mod_ref[3, :, ls], 2 * G)
                    hs[j] = h
                    h2_dst[r0 // 2:(r0 + G) // 2, ls] = _pk(h[:G])
                    h2_dst[(CB + r0) // 2:(CB + r0 + G) // 2, ls] = _pk(h[G:])
                    if NK <= j < 2 * NK:
                        cs = a_combos(hs[j - NK][:G], h[:G], hs[j - NK][G:], h[G:])
                        for i, cmb in enumerate(cs):
                            h2c_dst[i * HB + r0 // 2:i * HB + (r0 + G) // 2, lanes[j - NK]] = _pk(cmb)
            return run
        parts = [[j, NK + j] for j in range(NK)]
        parts[-1] += list(range(2 * NK, NL))
        return [piece(r0, js) for r0 in range(0, CB, G) for js in parts]

    def strassen(sa, a11, a22, tb, rem):
        dot = bg.dot
        m1 = dot(sa[0], tb[0])
        if rem is None:
            m7 = dot(sa[4], tb[4])
        else:
            m7 = dot(cat([sa[4], rem[0]], axis=1), cat([tb[4], rem[2]], axis=0))
        m4 = dot(a22, tb[2])
        m2 = dot(sa[1], tb[5])
        c21 = m2 + m4
        if rem is not None:
            c21 = c21 + dot(rem[1], rem[2])
        m5 = dot(sa[2], tb[6])
        c11 = m1 + m7 + m4 - m5
        m3 = dot(a11, tb[1])
        c12 = m3 + m5
        if rem is None:
            m6 = dot(sa[3], tb[3])
        else:
            c12 = c12 + dot(rem[0], rem[3])
            m6 = dot(cat([sa[3], rem[1]], axis=1), cat([tb[3], rem[3]], axis=0))
        c22 = m1 - m2 + m3 + m6
        return c11, c12, c21, c22

    def wgu_pieces(f):
        G = 16
        cl, cr = slice(f * FC, f * FC + 128), slice(f * FC + 128, (f + 1) * FC)

        def piece(w_ref, wc_ref, wr_ref, r0):
            def run(tok):
                b11 = _add(w_ref[r0:r0 + G, cl].astype(F32), tok)
                b22 = _add(w_ref[KS + r0:KS + r0 + G, cr].astype(F32), tok)
                cs = b_combos(b11, w_ref[r0:r0 + G, cr].astype(F32),
                              w_ref[KS + r0:KS + r0 + G, cl].astype(F32), b22)
                for i, cmb in enumerate(cs):
                    wc_ref[(i * KS + r0) // 2:(i * KS + r0 + G) // 2, f * 128:(f + 1) * 128] = _pk(cmb)
                if r0 < D - 2 * KS:
                    for c in (cl, cr):
                        w = pltpu.bitcast(w_ref[2 * KS + r0:2 * KS + r0 + G, c], U32)
                        wr_ref[r0 // 2:(r0 + G) // 2, c] = w if tok is None else w | pltpu.bitcast(tok, U32)
            return run
        return [piece(*refs, r0) for refs in ((wg_ref, wgc_ref, wgr_ref), (wu_ref, wuc_ref, wur_ref))
                for r0 in range(0, KS, G)]

    def wd_pieces():
        G = 16

        def piece(j, f, r0):
            def run(tok):
                cl, cr = lanes[j], lanes[NK + j]
                re = slice(f * FC + r0, f * FC + r0 + G)
                ro = slice(f * FC + 128 + r0, f * FC + 128 + r0 + G)
                b11 = _add(wd_ref[re, cl].astype(F32), tok)
                b22 = _add(wd_ref[ro, cr].astype(F32), tok)
                cs = b_combos(b11, wd_ref[re, cr].astype(F32), wd_ref[ro, cl].astype(F32), b22)
                for i, cmb in enumerate(cs):
                    p0 = i * (Fh // 4) + (f * 128 + r0) // 2
                    wdc_ref[p0:p0 + G // 2, cl] = _pk(cmb)
            return run
        return [piece(j, f, r0) for j in range(NK) for f in range(NF) for r0 in range(0, 128, G)]

    def wdr_pieces():
        G = 128

        def piece(r0):
            def run(tok):
                w = pltpu.bitcast(wd_ref[r0:r0 + G, lanes[NL - 1]], U32)
                wdr_ref[r0 // 2:(r0 + G) // 2, :] = w | _rep(pltpu.bitcast(tok, U32), G // 2)
            return run
        return [piece(r0) for r0 in range(0, Fh, G)]

    def ffn_gu(f, unit, plain=False, n=HB):
        cl, cr = slice(f * FC, f * FC + 128), slice(f * FC + 128, (f + 1) * FC)
        h2 = h2_ref.at[unit * CB:(unit + 1) * CB]
        h2c = h2c_ref.at[unit * 5 * HB:(unit + 1) * 5 * HB]
        hh = hh_ref.at[unit * CB:(unit + 1) * CB]
        hhc = hhc_ref.at[unit * 5 * HB:(unit + 1) * 5 * HB]

        def store(p0, n, p11, p12, p21, p22):
            hh[p0:p0 + n, cl] = _pk(p11)
            hh[p0:p0 + n, cr] = _pk(p12)
            hh[HB + p0:HB + p0 + n, cl] = _pk(p21)
            hh[HB + p0:HB + p0 + n, cr] = _pk(p22)
            for i, cmb in enumerate(a_combos(p11, p12, p21, p22)):
                hhc[i * HB + p0:i * HB + p0 + n, f * 128:(f + 1) * 128] = _pk(cmb)

        if plain:
            p11, p12, p21, p22 = [
                bg.dot(_unpk(h2[r:r + HB, :]), wg_ref[:, c]) * bg.dot(_unpk(h2[r:r + HB, :]), wu_ref[:, c])
                for r in (0, HB) for c in (cl, cr)]
            store(0, HB, p11, p12, p21, p22)
        else:
            for p0 in range(0, HB, n):
                res = []
                top, bot = slice(p0, p0 + n), slice(HB + p0, HB + p0 + n)
                for wr, wc in ((wgr_ref, wgc_ref), (wur_ref, wuc_ref)):
                    sa = [_unpk(h2c[i * HB + p0:i * HB + p0 + n, :]) for i in range(5)]
                    tb = [_unpk(wc[i * KS // 2:(i + 1) * KS // 2, f * 128:(f + 1) * 128]) for i in range(7)]
                    rem = (_unpk(h2[top, 2 * KS:D]), _unpk(h2[bot, 2 * KS:D]), _unpk(wr[:, cl]), _unpk(wr[:, cr]))
                    res.append(strassen(sa, _unpk(h2[top, 0:KS]), _unpk(h2[bot, KS:2 * KS]), tb, rem))
                store(p0, n, *[g * u for g, u in zip(*res)])

    def ffn_down(x1_src, t, unit):
        hh = hh_ref.at[unit * CB:(unit + 1) * CB]
        hhc = hhc_ref.at[unit * 5 * HB:(unit + 1) * 5 * HB]
        ob = o_ref.at[rows_of(t)]

        def emit(dn, b, ls):
            o = x1_src[b * CB:(b + 1) * CB, ls] + _rep(mod_ref[4, :, ls], CB) * dn
            w = pltpu.pack_elementwise([o[:HB], o[HB:]], packed_dtype=BF16)
            ob[b * CB:(b + 1) * CB, ls] = pltpu.bitcast(w, BF16)

        for b in range(2):
            KC = _E('KC', 512)
            ps = [bg.dot(_unpk(hh[b * HB:(b + 1) * HB, k0:k0 + KC]), _unpk(wdr_ref[k0 // 2:(k0 + KC) // 2, :]))
                  for k0 in range(0, Fh, KC)]
            emit(functools.reduce(lambda x, y: x + y, ps), b, lanes[NL - 1])
        for j in range(NK):
            cl, cr = lanes[j], lanes[NK + j]
            sa = [_unpk(hhc[i * HB:(i + 1) * HB, :]) for i in range(5)]
            a11 = cat([_unpk(hh[0:HB, f * FC:f * FC + 128]) for f in range(NF)], axis=1)
            a22 = cat([_unpk(hh[HB:CB, f * FC + 128:(f + 1) * FC]) for f in range(NF)], axis=1)
            tb = [_unpk(wdc_ref[i * (Fh // 4):(i + 1) * (Fh // 4), cl]) for i in range(7)]
            c11, c12, c21, c22 = strassen(sa, a11, a22, tb, None)
            emit(c21, 1, cl)
            emit(c11, 0, cl)
            emit(c12, 0, cr)
            emit(c22, 1, cr)

    x1s = [x1s_ref.at[r * TM:(r + 1) * TM] for r in range(2)]
    sts = [st_ref.at[r * TM:(r + 1) * TM] for r in range(2)]
    YP = _E('YP', 11)

    def prologue():
        for cp in small:
            cp.wait()
        shk = shk_ref[...].astype(F32)
        for a in range(4):
            sh_ref[a] = jnp.broadcast_to(shk[a:a + 1, :], (8, D))
        zm_ref[...] = pltpu.bitcast(inv_ref[CB:CB + 16, :], I32)
        zs.append(zm_ref[0, 0])
        ssm_cp(0).wait()
        k_fwd(0)
        ssm_cp(1).wait()
        k_fwd(1)
        for t in range(2):
            k_cp(t).wait()
            v_cp(t).wait()
            ssm_cp(2 + t).wait()
            now(kv_pieces(t, 64))
            k_fwd(2 + t)
            u_fwd(t)
        ssm_cp(4).wait()
        bg.flush()
        pos = sorted(positions, key=lambda p: p[1].start)
        n0 = _E('PY0', 32)
        bg.add(ystatic_pieces(0, YP, 0, 4, False, pos[:n0]), 0, 1024)
        bg.add(ystatic_pieces(0, YP, 0, 4, False, pos[n0:n0 + 1]), 5000, 5001)
        k_fwd(4)
        bg.flush()
        q_cp(0).wait()
        now(ystatic_pieces(0, YP, 0, 4, False, pos[n0 + 1:]))
        q_cp(1).wait()
        mod_cp(0).wait()
        mod_chunk(0)
        for t in range(2):
            now(post_pieces(t))
            now(ln1_pieces(t))
            y_inv(t, x1s[t])
        for t in range(2):
            now(ln2_stat_pieces(x1s[t], sts[t]))
        bg.flush()

    def superstep():
        yrest = ystatic_pieces(YP, NB, 0, 4, False)
        mod_cp(1).wait()
        mod_chunk(1)
        now(ln2_apply_pieces(x1s[0], sts[0], 0))
        bg.flush()
        g_cp(0).wait()
        u_cp(0).wait()
        bg.add(ln2_apply_pieces(x1s[1], sts[1], 1), 0, 850)
        bg.add(wgu_pieces(0), 0, 950)
        bg.add(yrest[0:_E('Y1', 40)], 1050, 2250)
        ffn_gu(0, 0, plain=True)
        ffn_gu(0, 1)
        bg.flush()
        k_cp(2).wait()
        v_cp(2).wait()
        g_cp(1).wait()
        u_cp(1).wait()
        bg.add(wgu_pieces(1), 0, 900)
        bg.add(kv_pieces(2), 1000, 2200)
        ffn_gu(1, 0, plain=True)
        ffn_gu(1, 1)
        bg.flush()
        for f in range(2, 4):
            g_cp(f).wait()
            u_cp(f).wait()
        bg.add(wgu_pieces(2), 0, 900)
        bg.add(wgu_pieces(3), 1900, 2700)
        bg.add(_group(ystatic_pieces(4, 6, 4, 6, True), 2), 2750, 4050)
        ffn_gu(2, 0, plain=True)
        u_fwd(2)
        ffn_gu(2, 1)
        ffn_gu(3, 0)
        bg.flush()
        for f in range(4, NF):
            g_cp(f).wait()
            u_cp(f).wait()
        q_cp(2).wait()
        y1, y2 = _E('Y1', 40), _E('Y2', 130)
        bg.add(wgu_pieces(4), 0, 800)
        bg.add(post_pieces(2), 850, 1600)
        bg.add(wgu_pieces(5), 1650, 2500)
        bg.add(linked(ln1_pieces(2), _E('LK', 3)), _E('W3', 300), _E('W4', 2900))
        bg.add(yrest[y1:y2], 2600, 4750)
        ffn_gu(3, 1)
        ffn_gu(4, 0)
        ffn_gu(4, 1)
        y_inv(2, x1_ref.at[0])
        ffn_gu(5, 0)
        bg.flush()
        d_cp.wait()
        mod_cp(2).wait()
        k_cp(3).wait()
        v_cp(3).wait()
        bg.add(wdr_pieces(), 0, 300)
        bg.add(wd_pieces(), 300, 2800)
        bg.add(linked(ln2_stat_pieces(x1_ref.at[0], st_ref), _E('LK2', 3)), 1200, 3000)
        bg.add(ln2_apply_pieces(x1_ref.at[0], st_ref, 0), 2900, 4000)
        bg.add(kv_pieces(3), _E('W1', 3900), _E('W2', 5400))
        bg.add(yrest[y2:], _E('W2', 5400), 7850)
        bg.inj = [(150 + 200 * i, gb_tile(i)) for i in range(NL)]
        ffn_gu(5, 1)
        ffn_down(x1s[0], 0, 0)
        ffn_down(x1s[1], 1, 1)
        bg.flush()
        o_cp(0).start()
        o_cp(1).start()

    def run_super(fn):
        if _E('SL', 1):
            def body(i, carry):
                fn()
                return carry
            lax.fori_loop(0, zs[0] + 1, body, 0)
        else:
            fn()

    def late_waits():
        for t in range(T0, NS):
            q_cp(t).wait()
            if t + 1 < NS:
                k_cp(t + 1).wait()
                v_cp(t + 1).wait()

    def step(t, carry):
        slot = lax.rem(t, 2)
        if _E('LA', 1):
            bg.add(linked(ln1_pieces(t), _E('LK1', 2)), _E('L0', 800), _E('L1', 6800))
        t1 = 640 + NF * 1152 + 320
        bg.add(linked(ln2_stat_pieces(x1_ref.at[slot], st_ref), _E('LK2', 3)), t1 + _E('S0', 100), t1 + _E('S1', 1800))
        bg.add(ln2_apply_pieces(x1_ref.at[slot], st_ref, 0), t1 + _E('P0', 1400), t1 + _E('P1', 3100))
        bg.add(kv_pieces(jnp.minimum(t + 1, NS - 1), 16), t1 + _E('K0', 100), t1 + _E('K1', 3100))
        u_fwd(t)
        chain(diag_pieces(t, T0 - 1), _E('DD', 2), _E('DE', 0))
        chain(task_pieces(t, 2), _E('MD', 2), _E('ME', 0))
        dep = chain(task_pieces(t, 1), _E('MD', 2), _E('ME', 0))
        chain(post_pieces(t), 1, 3, dep)
        if not _E('LA', 1):
            chain(ln1_pieces(t), 1)
        for f in range(NF):
            ffn_gu(f, 0, n=HB // 2)
        y_inv(t, x1_ref.at[slot])
        ffn_down(x1_ref.at[1 - slot], t - 1, 0)
        bg.flush()
        o_cp(t - 1).start()
        return carry

    def epilogue():
        t = NS - 1
        for f in range(NF):
            ffn_gu(f, 0, n=HB // 2)
        ffn_down(x1_ref.at[t % 2], t, 0)
        o_cp(t).start()
        for i in range(NS):
            o_cp(i).wait()

    if SCOPES:
        jax.named_scope("prologue")(prologue)()
        run_super(jax.named_scope("superstep")(superstep))
        late_waits()
        lax.fori_loop(T0, NS, jax.named_scope("step")(step), 0)
        jax.named_scope("epilogue")(epilogue)()
    elif ONLY == 'loop':
        zs.append(zm_ref[0, 0])
        lax.fori_loop(T0, NS, step, 0)
        epilogue()
    elif ONLY == 'S':
        zs.append(zm_ref[0, 0])
        run_super(superstep)
        lax.fori_loop(T0, NS, step, 0)
    else:
        prologue()
        run_super(superstep)
        late_waits()
        lax.fori_loop(T0, NS, step, 0)
        epilogue()


@jax.jit
def pallas_adaLN_cond__ssm_conv_h3__glu_gated_bilinear__prompt_kernel(
    A_q, A_k, A_v, A_shift_k, A_ssm_k, A_ssm_D, B_x, B_w_gate, B_w_up, B_w_down, c, w_mod,
):
    B, S, D = A_q.shape
    Fh = B_w_gate.shape[1]
    NB = S // CB
    NS = S // TM
    fwd, inv = _dft_consts()
    anyspec = pl.BlockSpec(memory_space=pl.ANY)
    V = pltpu.VMEM
    out = pl.pallas_call(
        functools.partial(_kernel, S=S, D=D, Fh=Fh),
        in_specs=[anyspec] * 13,
        out_specs=anyspec,
        out_shape=jax.ShapeDtypeStruct((S, D), A_q.dtype),
        scratch_shapes=[
            V((NS, 2, 3 * CB, D), F32),
            V((NB, 3 * CB, D), F32),
            V((NS, 2, 3 * CB, D), F32),
            V((2, TM, D), F32),
            V((S, D), BF16), V((S, D), BF16), V((S, D), BF16), V((S, D), BF16),
            V((2 * TM, D), F32),
            V((TM, D), F32),
            V((2 * TM, 256), F32),
            V((2 * CB, D), U32),
            V((2 * 5 * HB, KS), U32),
            V((2 * CB, Fh), U32),
            V((2 * 5 * HB, Fh // 2), U32),
            V((TM // 2, D), U32),
            V((2 * CB, D), U32),
            V(((D - 2 * KS) // 2, Fh), U32), V(((D - 2 * KS) // 2, Fh), U32), V((Fh // 2, D - 2 * KS), U32),
            V((7 * KS // 2, Fh // 2), U32), V((7 * KS // 2, Fh // 2), U32), V((7 * Fh // 4, KS), U32),
            V((D, S), BF16), V((D, 6 * D), BF16), V((D, Fh), BF16), V((D, Fh), BF16), V((Fh, D), BF16),
            V((2 * CB, CB), BF16), V((CB + 16, CB), BF16),
            V((5, 8, D), F32), V((4, 8, D), F32), V((8, 128), I32),
            V((4, D), BF16), V((D,), BF16), V((1, D), BF16),
            pltpu.SemaphoreType.DMA((5 + 4 * NS + D // 128 + 3 + 2 * (Fh // FC) + 1,)),
        ],
        compiler_params=pltpu.CompilerParams(
            internal_scratch_in_bytes=48 * 1024,
            disable_semaphore_checks=True,
            disable_bounds_checks=True,
            vmem_limit_bytes=110 * 1024 * 1024),
        name="adaln_h3_glu",
    )(A_q.reshape(S, D), A_k.reshape(S, D), A_v.reshape(S, D), A_shift_k.T, A_ssm_k,
      A_ssm_D, B_w_gate, B_w_up, B_w_down, c, w_mod, fwd, inv)
    return out.reshape(B, S, D)
```

```python
import functools
import os

import numpy as np
import jax
import jax.numpy as jnp
from jax import lax
import jax.experimental.pallas as pl
import jax.experimental.pallas.tpu as pltpu

F32 = jnp.float32
BF16 = jnp.bfloat16
U32 = jnp.uint32
I32 = jnp.int32

CB = 128
HB = CB // 2
TM = 256
FC = 256
KS = 256
EPS = 1e-5
SCOPES = False
ONLY = os.environ.get('ONLY', '')


def _E(name, default):
    return int(os.environ.get(name, default))


def _dft_consts():
    k = np.arange(CB, dtype=np.float64)[:, None]
    n = np.arange(CB, dtype=np.float64)[None, :]
    th = np.pi * (4.0 * k + 1.0) * n / (2.0 * CB)
    fwd = np.concatenate([np.cos(th), np.sin(th)], axis=0)
    g = np.concatenate([np.cos(th[:HB]), np.sin(th[:HB])], axis=0).T / CB
    inv = np.concatenate([g[0::2], g[1::2], np.zeros((16, CB))], axis=0)
    return jnp.asarray(fwd, dtype=BF16), jnp.asarray(inv, dtype=BF16)


def _pk(x):
    return pltpu.bitcast(x.astype(BF16), U32)


def _unpk(x):
    return pltpu.bitcast(x, BF16)


def _rep(r, n):
    return r if n == 8 else jnp.concatenate([r] * (n // 8), axis=0)


def _add(x, tok):
    return x if tok is None else x + _rep(tok, x.shape[0])


def _group(pieces, n):
    def merged(ps):
        def run(tok):
            for p in ps:
                p(tok)
        return run
    return [merged(pieces[i:i + n]) for i in range(0, len(pieces), n)]


class _Sched:
    def __init__(self, token):
        self.token = token
        self.clock = 0.0
        self.q = []
        self.last = None
        self.inj = []

    def add(self, pieces, t0, t1):
        n = len(pieces)
        self.q += [(t0 + (t1 - t0) * i / n, len(self.q) + i, p) for i, p in enumerate(pieces)]
        self.q.sort(key=lambda e: e[:2])

    def note(self, m, dt):
        rows, cols = m.shape
        tiles = [(slice(r, r + 8), slice(c, c + 128)) for c in range(0, cols, 128) for r in range(0, rows, 8)]
        for i, tl in enumerate(tiles):
            tok = None
            while self.q and self.q[0][0] <= self.clock + dt * (i + 1) / len(tiles):
                if tok is None:
                    tok = self.token(m[tl])
                self.q.pop(0)[2](tok)
        self.clock += dt
        self.last = m[tiles[-1]]
        return m

    def dot(self, a, b):
        if self.inj and self.clock >= self.inj[0][0]:
            self.inj.pop(0)[1]()
        m = jnp.dot(a, b, preferred_element_type=F32)
        return self.note(m, max(a.shape[0], 32) * (a.shape[1] // 128) * (b.shape[1] // 128) / 4)

    def flush(self):
        tok = None if self.last is None or not self.q else self.token(self.last)
        while self.q:
            self.q.pop(0)[2](tok)
        self.clock = 0.0
        self.last = None


def _kernel(q_hbm, k_hbm, v_hbm, shk_hbm, ssmk_hbm, ssmd_hbm, wg_hbm, wu_hbm, wd_hbm,
            c_hbm, wmod_hbm, fwd_hbm, inv_hbm, o_hbm,
            u_ref, kk_ref, y_ref, x1_ref, q_ref, k_ref, v_ref, o_ref,
            x1s_ref, hp_ref, st_ref, h2_ref, h2c_ref, hh_ref, hhc_ref, kv_ref, yb_ref,
            wgr_ref, wur_ref, wdr_ref, wgc_ref, wuc_ref, wdc_ref,
            ssmk_ref, wmod_ref, wg_ref, wu_ref, wd_ref, fwd_ref, inv_ref,
            mod_ref, sh_ref, zm_ref, shk_ref, ssmd_ref, c_ref,
            sem, *, S, D, Fh):
    NB = S // CB
    NS = S // TM
    NL = D // 128
    NF = Fh // FC
    NK = KS // 128
    T0 = 3
    NLOOP = NS - T0
    lanes = [slice(i * 128, (i + 1) * 128) for i in range(NL)]
    cat = jnp.concatenate

    offs = [int(o) for o in np.cumsum([0, 5, NS, NS, NS, NL, 3, NF, NF, 1])]
    s_small, s_q, s_k, s_v, s_ssm, s_mod, s_g, s_u, s_d, s_o = offs

    def rows_of(t):
        return pl.ds(t * TM if isinstance(t, int) else pl.multiple_of(t * TM, TM), TM)

    def rows_cp(src, dst, base, t):
        return pltpu.make_async_copy(src.at[rows_of(t), :], dst.at[rows_of(t), :], sem.at[base + t])

    def cols_cp(src, dst, lo, hi, si):
        return pltpu.make_async_copy(src.at[:, lo:hi], dst.at[:, lo:hi], sem.at[si])

    q_cp = lambda t: rows_cp(q_hbm, q_ref, s_q, t)
    k_cp = lambda t: rows_cp(k_hbm, k_ref, s_k, t)
    v_cp = lambda t: rows_cp(v_hbm, v_ref, s_v, t)
    o_cp = lambda t: rows_cp(o_ref, o_hbm, s_o, t)
    small = [pltpu.make_async_copy(s, d, sem.at[s_small + i]) for i, (s, d) in enumerate(
        [(fwd_hbm, fwd_ref), (shk_hbm, shk_ref), (ssmd_hbm, ssmd_ref), (inv_hbm, inv_ref), (c_hbm, c_ref)])]
    ssm_cp = lambda i: pltpu.make_async_copy(ssmk_hbm.at[lanes[i], :], ssmk_ref.at[lanes[i], :],
                                             sem.at[s_ssm + i])
    mod_cols = [(0, 3 * D), (3 * D, 5 * D), (5 * D, 6 * D)]
    mod_cp = lambda i: cols_cp(wmod_hbm, wmod_ref, mod_cols[i][0], mod_cols[i][1], s_mod + i)
    g_cp = lambda f: cols_cp(wg_hbm, wg_ref, f * FC, (f + 1) * FC, s_g + f)
    u_cp = lambda f: cols_cp(wu_hbm, wu_ref, f * FC, (f + 1) * FC, s_u + f)
    d_cp = pltpu.make_async_copy(wd_hbm, wd_ref, sem.at[s_d])

    order = small + [ssm_cp(0), ssm_cp(1), k_cp(0), v_cp(0),
                     ssm_cp(2), k_cp(1), v_cp(1), ssm_cp(3), ssm_cp(4), q_cp(0), q_cp(1),
                     mod_cp(0), mod_cp(1), g_cp(0), u_cp(0), k_cp(2), v_cp(2)]
    for f in range(1, NF):
        order += [g_cp(f), u_cp(f)]
    order += [q_cp(2), d_cp, mod_cp(2), k_cp(3), v_cp(3)]
    for t in range(T0, NS):
        order += [q_cp(t)]
        if t + 1 < NS:
            order += [k_cp(t + 1), v_cp(t + 1)]
    for cp in order:
        cp.start()

    zs = []
    bg = _Sched(lambda x: pltpu.bitcast(pltpu.bitcast(x, I32) & zm_ref[...], F32))

    def opaque(ref):
        return ref.at[pl.ds(pl.multiple_of(zs[0], 32), ref.shape[0])]

    def chain(pieces, dist, extra=0, dep=None):
        hist = [] if dep is None else [dep] * dist
        for p in pieces:
            tok = None
            if len(hist) >= dist:
                tok = bg.token(hist[-dist])
                for _ in range(extra):
                    tok = tok + tok
            hist.append(p(tok))
        return hist[-1]

    def linked(pieces, d):
        res = []

        def wrap(p):
            def run(tok):
                if d and len(res) >= d:
                    tok = tok + bg.token(res[-d])
                res.append(p(tok))
            return run
        return [wrap(p) for p in pieces]

    def now(pieces):
        for p in pieces:
            p(None)

    def mod_chunk(i):
        c = c_ref[...].astype(F32)
        sc = jnp.broadcast_to((c * jax.nn.sigmoid(c)).astype(BF16), (16, D))
        lo, hi = mod_cols[i]
        m = bg.dot(sc, wmod_ref[:, lo:hi])[0:8]
        if i == 0:
            ga = m[:, 2 * D:3 * D]
            mod_ref[0] = (1.0 + m[:, D:2 * D]) * ga
            mod_ref[1] = m[:, 0:D] * ga
        elif i == 1:
            mod_ref[2] = 1.0 + m[:, D:2 * D]
            mod_ref[3] = m[:, 0:D]
        else:
            mod_ref[4] = m

    def gb_tile(i):
        def run():
            c = c_ref[...].astype(F32)
            sc = jnp.broadcast_to((c * jax.nn.sigmoid(c)).astype(BF16), (16, D))
            w = wmod_ref[:, 5 * D + i * 128:5 * D + (i + 1) * 128]
            mod_ref[4, :, lanes[i]] = jnp.dot(sc, w, preferred_element_type=F32)[0:8]
        return run

    def k_fwd(i):
        ls = lanes[i]
        fwd = fwd_ref[...]
        prev = None
        for m in range(NB):
            kf = lax.dot_general(fwd, ssmk_ref[ls, m * CB:(m + 1) * CB], (((1,), (1,)), ((), ())),
                                 preferred_element_type=F32)
            if m == 0:
                c = kf[:CB] + ssmd_ref[...].astype(F32).reshape(1, D)[:, ls]
                d = kf[CB:]
            else:
                c = kf[:CB] + prev[CB:]
                d = kf[CB:] - prev[:CB]
            prev = kf
            kk_ref[m, 0:CB, ls] = c
            kk_ref[m, CB:2 * CB, ls] = d - c
            kk_ref[m, 2 * CB:3 * CB, ls] = c + d
            if m % 4 == 3:
                bg.note(kf, 2 * CB)

    def lo_hi(w):
        return pltpu.bitcast(w << 16, F32), pltpu.bitcast(w & jnp.uint32(0xFFFF0000), F32)

    def kv_pieces(t, G=32):
        n = G // 2
        kb, vb = k_ref.at[rows_of(t)], v_ref.at[rows_of(t)]

        def piece(ls, r0):
            def run(tok):
                if r0 > 0:
                    w = pltpu.bitcast(kb[r0 - 16:r0 + G, ls], U32)
                else:
                    if isinstance(t, int) and t == 0:
                        halo = jnp.zeros((8, 128), U32)
                    else:
                        halo = pltpu.bitcast(k_ref.at[rows_of(t - 1)][TM - 16:TM, ls], U32)
                    w = cat([halo, pltpu.bitcast(kb[0:G, ls], U32)], axis=0)
                if tok is not None:
                    w = w | _rep(pltpu.bitcast(tok, U32), n + 8)
                ke, ko = lo_hi(w[8:])
                ke1, ko1 = lo_hi(pltpu.roll(w, 1, 0)[8:])
                _, ko2 = lo_hi(pltpu.roll(w, 2, 0)[8:])
                s0, s1, s2, s3 = [_rep(sh_ref[a, :, ls], n) for a in range(4)]
                ve, vo = lo_hi(pltpu.bitcast(vb[r0:r0 + G, ls], U32))
                kve = ((ke * s0 + ko1 * s1) + (ke1 * s2 + ko2 * s3)) * ve
                kvo = ((ko * s0 + ke * s1) + (ko1 * s2 + ke1 * s3)) * vo
                kv_ref[r0 // 2:(r0 + G) // 2, ls] = pltpu.bitcast(
                    pltpu.pack_elementwise([kve, kvo], packed_dtype=BF16), U32)
            return run
        return [piece(ls, r0) for ls in lanes for r0 in range(0, TM, G)]

    def u_fwd(t):
        fwd = fwd_ref[...]
        for b in range(2):
            uf = bg.dot(fwd, _unpk(kv_ref[b * HB:(b + 1) * HB, :]))
            a, bb = uf[:CB], uf[CB:]
            u_ref[t, b, 0:CB, :] = a + bb
            u_ref[t, b, CB:2 * CB, :] = a
            u_ref[t, b, 2 * CB:3 * CB, :] = bb

    positions = [(slice(r0, r0 + 8), ls) for r0 in range(0, 3 * CB, 8) for ls in lanes]

    def ystatic_pieces(s_lo, s_hi, i_lo, i_hi, acc_in, pos=None):
        def piece(rs, ls):
            def run(tok):
                us = {i: _add(u_ref[i // 2, i % 2, rs, ls], tok) for i in range(i_lo, i_hi)}
                ks = {}
                for s in range(s_lo, s_hi):
                    acc = None
                    for i in range(i_lo, min(i_hi, s + 1)):
                        m = s - i
                        if m not in ks:
                            ks[m] = kk_ref[m, rs, ls]
                        p = ks[m] * us[i]
                        acc = p if acc is None else acc + p
                    if acc_in:
                        acc = acc + y_ref[s // 2, s % 2, rs, ls]
                    y_ref[s // 2, s % 2, rs, ls] = acc
                return acc
            return run
        return [piece(*p) for p in (positions if pos is None else pos)]

    def task_pieces(t, delta):
        p = t - delta
        left = p >= T0
        J = jnp.where(left, t, p + NLOOP)
        I = jnp.where(left, p, t)
        kview = kk_ref.at[pl.ds(2 * (J - I) - 1, 3)]

        def piece(rs, ls):
            def run(tok):
                u0 = _add(u_ref[I, 0, rs, ls], tok)
                u1 = _add(u_ref[I, 1, rs, ls], tok)
                kc = kview[1, rs, ls]
                y_ref[J, 0, rs, ls] = (kc * u0 + kview[0, rs, ls] * u1) + y_ref[J, 0, rs, ls]
                y1 = (kview[2, rs, ls] * u0 + kc * u1) + y_ref[J, 1, rs, ls]
                y_ref[J, 1, rs, ls] = y1
                return y1
            return run
        return [piece(*p) for p in positions]

    def diag_pieces(t, I):
        kview = kk_ref.at[pl.ds(2 * (t - I) - 1, 3)]

        def piece(rs, ls):
            def run(tok):
                us = [_add(u_ref[a, b, rs, ls], tok) for a in (t, I) for b in range(2)]
                k0 = kk_ref[0, rs, ls]
                kc = kview[1, rs, ls]
                y_ref[t, 0, rs, ls] = ((k0 * us[0] + y_ref[t, 0, rs, ls])
                                       + (kc * us[2] + kview[0, rs, ls] * us[3]))
                y1 = ((kk_ref[1, rs, ls] * us[0] + k0 * us[1])
                      + (kview[2, rs, ls] * us[2] + kc * us[3]) + y_ref[t, 1, rs, ls])
                y_ref[t, 1, rs, ls] = y1
                return y1
            return run
        return [piece(*p) for p in positions]

    def post_pieces(t):
        def piece(b, r0, ls):
            def run(tok):
                comp = lambda c, off: y_ref[t, b, c * CB + off + r0:c * CB + off + r0 + 16, ls]
                k1l, k1h = _add(comp(0, 0), tok), _add(comp(0, HB), tok)
                rel, reh = k1l - comp(2, 0), k1h - comp(2, HB)
                iml, imh = k1l + comp(1, 0), k1h + comp(1, HB)
                p0 = b * CB + r0 // 2
                yb_ref[p0:p0 + 8, ls] = _pk(rel + reh)
                yb_ref[p0 + HB // 2:p0 + HB // 2 + 8, ls] = _pk(iml + imh)
                yb_ref[p0 + HB:p0 + HB + 8, ls] = _pk(rel - reh)
                oim = iml - imh
                yb_ref[p0 + HB + HB // 2:p0 + HB + HB // 2 + 8, ls] = _pk(oim)
                return oim[8:16]
            return run
        return [piece(b, r0, ls) for b in range(2) for r0 in range(0, HB, 16) for ls in lanes]

    def q_split(t, b, p0, n, ls):
        w = pltpu.bitcast(q_ref.at[rows_of(t)][b * CB + 2 * p0:b * CB + 2 * p0 + 2 * n, ls], U32)
        return lo_hi(w)

    def ln_tiles(xs, tok):
        n = xs[0].shape[0]
        s = _add(xs[0], tok)
        for x in xs[1:]:
            s = s + x
        m = jnp.sum(s, axis=-1, keepdims=True) * (1.0 / D)
        xc = [x - m for x in xs]
        s2 = xc[0] * xc[0]
        for x in xc[1:]:
            s2 = s2 + x * x
        r = lax.rsqrt(jnp.sum(s2, axis=-1, keepdims=True) * (1.0 / D) + EPS)
        return xc, jnp.broadcast_to(r, (n, 128)), jnp.broadcast_to(m, (n, 128))

    def ln1_pieces(t):
        G = _E('L1G', 8)

        def piece(b, p0):
            def run(tok):
                xc, r, _ = ln_tiles([cat(q_split(t, b, p0, G, ls), axis=0) for ls in lanes], tok)
                for ls, x in zip(lanes, xc):
                    h = (x * r) * _rep(mod_ref[0, :, ls], 2 * G) + _rep(mod_ref[1, :, ls], 2 * G)
                    hp_ref[b * CB + p0:b * CB + p0 + G, ls] = h[:G]
                    hp_ref[b * CB + HB + p0:b * CB + HB + p0 + G, ls] = h[G:]
                return functools.reduce(lambda a, c: a + c, [h[r:r + 8] for r in range(0, 2 * G, 8)])
            return run
        return [piece(b, p0) for b in range(2) for p0 in range(0, HB, G)]

    def y_inv(t, x1_dst):
        yb = opaque(yb_ref)
        hp = opaque(hp_ref)
        for b in range(2):
            ye = bg.dot(inv_ref[0:HB, :], _unpk(yb[b * CB:b * CB + HB, :]))
            yo = bg.dot(inv_ref[HB:CB, :], _unpk(yb[b * CB + HB:(b + 1) * CB, :]))
            for ls in lanes:
                qe, qo = q_split(t, b, 0, HB, ls)
                re, ro = slice(b * CB, b * CB + HB), slice(b * CB + HB, (b + 1) * CB)
                x1_dst[re, ls] = qe + hp[re, ls] * ye[:, ls]
                x1_dst[ro, ls] = qo + hp[ro, ls] * yo[:, ls]

    def a_combos(a11, a12, a21, a22):
        return [a11 + a22, a21 + a22, a11 + a12, a21 - a11, a12 - a22]

    def b_combos(b11, b12, b21, b22):
        return [b11 + b22, b12 - b22, b21 - b11, b11 + b12, b21 + b22, b11, b22]

    def ln2_stat_pieces(x1_src, st):
        x1o = opaque(x1_src)

        def piece(r0):
            def run(tok):
                _, r, m = ln_tiles([x1o[r0:r0 + 16, ls] for ls in lanes], tok)
                st[r0:r0 + 16, 0:128] = m
                st[r0:r0 + 16, 128:256] = r
                return r[0:8] + r[8:16]
            return run
        return [piece(h * CB + r0) for r0 in range(0, CB, 16) for h in range(2)]

    def ln2_apply_pieces(x1_src, st, unit):
        G = 16
        x1o = opaque(x1_src)
        h2_dst = h2_ref.at[unit * CB:(unit + 1) * CB]
        h2c_dst = h2c_ref.at[unit * 5 * HB:(unit + 1) * 5 * HB]

        def piece(r0, js):
            def run(tok):
                two = lambda ref, c: cat([ref[r0:r0 + G, c], ref[CB + r0:CB + r0 + G, c]], axis=0)
                m, r = _add(two(st, slice(0, 128)), tok), two(st, slice(128, 256))
                hs = {}
                for j in js:
                    ls = lanes[j]
                    h = ((two(x1o, ls) - m) * r) * _rep(mod_ref[2, :, ls], 2 * G) + _rep(mod_ref[3, :, ls], 2 * G)
                    hs[j] = h
                    h2_dst[r0 // 2:(r0 + G) // 2, ls] = _pk(h[:G])
                    h2_dst[(CB + r0) // 2:(CB + r0 + G) // 2, ls] = _pk(h[G:])
                    if NK <= j < 2 * NK:
                        cs = a_combos(hs[j - NK][:G], h[:G], hs[j - NK][G:], h[G:])
                        for i, cmb in enumerate(cs):
                            h2c_dst[i * HB + r0 // 2:i * HB + (r0 + G) // 2, lanes[j - NK]] = _pk(cmb)
            return run
        parts = [[j, NK + j] for j in range(NK)]
        parts[-1] += list(range(2 * NK, NL))
        return [piece(r0, js) for r0 in range(0, CB, G) for js in parts]

    def strassen(sa, a11, a22, tb, rem):
        dot = bg.dot
        m1 = dot(sa[0], tb[0])
        if rem is None:
            m7 = dot(sa[4], tb[4])
        else:
            m7 = dot(cat([sa[4], rem[0]], axis=1), cat([tb[4], rem[2]], axis=0))
        m4 = dot(a22, tb[2])
        m2 = dot(sa[1], tb[5])
        c21 = m2 + m4
        if rem is not None:
            c21 = c21 + dot(rem[1], rem[2])
        m5 = dot(sa[2], tb[6])
        c11 = m1 + m7 + m4 - m5
        m3 = dot(a11, tb[1])
        c12 = m3 + m5
        if rem is None:
            m6 = dot(sa[3], tb[3])
        else:
            c12 = c12 + dot(rem[0], rem[3])
            m6 = dot(cat([sa[3], rem[1]], axis=1), cat([tb[3], rem[3]], axis=0))
        c22 = m1 - m2 + m3 + m6
        return c11, c12, c21, c22

    def wgu_pieces(f):
        G = 16
        cl, cr = slice(f * FC, f * FC + 128), slice(f * FC + 128, (f + 1) * FC)

        def piece(w_ref, wc_ref, wr_ref, r0):
            def run(tok):
                b11 = _add(w_ref[r0:r0 + G, cl].astype(F32), tok)
                b22 = _add(w_ref[KS + r0:KS + r0 + G, cr].astype(F32), tok)
                cs = b_combos(b11, w_ref[r0:r0 + G, cr].astype(F32),
                              w_ref[KS + r0:KS + r0 + G, cl].astype(F32), b22)
                for i, cmb in enumerate(cs):
                    wc_ref[(i * KS + r0) // 2:(i * KS + r0 + G) // 2, f * 128:(f + 1) * 128] = _pk(cmb)
                if r0 < D - 2 * KS:
                    for c in (cl, cr):
                        w = pltpu.bitcast(w_ref[2 * KS + r0:2 * KS + r0 + G, c], U32)
                        wr_ref[r0 // 2:(r0 + G) // 2, c] = w if tok is None else w | pltpu.bitcast(tok, U32)
            return run
        return [piece(*refs, r0) for refs in ((wg_ref, wgc_ref, wgr_ref), (wu_ref, wuc_ref, wur_ref))
                for r0 in range(0, KS, G)]

    def wd_pieces():
        G = 16

        def piece(j, f, r0):
            def run(tok):
                cl, cr = lanes[j], lanes[NK + j]
                re = slice(f * FC + r0, f * FC + r0 + G)
                ro = slice(f * FC + 128 + r0, f * FC + 128 + r0 + G)
                b11 = _add(wd_ref[re, cl].astype(F32), tok)
                b22 = _add(wd_ref[ro, cr].astype(F32), tok)
                cs = b_combos(b11, wd_ref[re, cr].astype(F32), wd_ref[ro, cl].astype(F32), b22)
                for i, cmb in enumerate(cs):
                    p0 = i * (Fh // 4) + (f * 128 + r0) // 2
                    wdc_ref[p0:p0 + G // 2, cl] = _pk(cmb)
            return run
        return [piece(j, f, r0) for j in range(NK) for f in range(NF) for r0 in range(0, 128, G)]

    def wdr_pieces():
        G = 128

        def piece(r0):
            def run(tok):
                w = pltpu.bitcast(wd_ref[r0:r0 + G, lanes[NL - 1]], U32)
                wdr_ref[r0 // 2:(r0 + G) // 2, :] = w | _rep(pltpu.bitcast(tok, U32), G // 2)
            return run
        return [piece(r0) for r0 in range(0, Fh, G)]

    def ffn_gu(f, unit, plain=False, n=HB):
        cl, cr = slice(f * FC, f * FC + 128), slice(f * FC + 128, (f + 1) * FC)
        h2 = h2_ref.at[unit * CB:(unit + 1) * CB]
        h2c = h2c_ref.at[unit * 5 * HB:(unit + 1) * 5 * HB]
        hh = hh_ref.at[unit * CB:(unit + 1) * CB]
        hhc = hhc_ref.at[unit * 5 * HB:(unit + 1) * 5 * HB]

        def store(p0, n, p11, p12, p21, p22):
            hh[p0:p0 + n, cl] = _pk(p11)
            hh[p0:p0 + n, cr] = _pk(p12)
            hh[HB + p0:HB + p0 + n, cl] = _pk(p21)
            hh[HB + p0:HB + p0 + n, cr] = _pk(p22)
            for i, cmb in enumerate(a_combos(p11, p12, p21, p22)):
                hhc[i * HB + p0:i * HB + p0 + n, f * 128:(f + 1) * 128] = _pk(cmb)

        if plain:
            p11, p12, p21, p22 = [
                bg.dot(_unpk(h2[r:r + HB, :]), wg_ref[:, c]) * bg.dot(_unpk(h2[r:r + HB, :]), wu_ref[:, c])
                for r in (0, HB) for c in (cl, cr)]
            store(0, HB, p11, p12, p21, p22)
        else:
            for p0 in range(0, HB, n):
                res = []
                top, bot = slice(p0, p0 + n), slice(HB + p0, HB + p0 + n)
                for wr, wc in ((wgr_ref, wgc_ref), (wur_ref, wuc_ref)):
                    sa = [_unpk(h2c[i * HB + p0:i * HB + p0 + n, :]) for i in range(5)]
                    tb = [_unpk(wc[i * KS // 2:(i + 1) * KS // 2, f * 128:(f + 1) * 128]) for i in range(7)]
                    rem = (_unpk(h2[top, 2 * KS:D]), _unpk(h2[bot, 2 * KS:D]), _unpk(wr[:, cl]), _unpk(wr[:, cr]))
                    res.append(strassen(sa, _unpk(h2[top, 0:KS]), _unpk(h2[bot, KS:2 * KS]), tb, rem))
                store(p0, n, *[g * u for g, u in zip(*res)])

    def ffn_down(x1_src, t, unit):
        hh = hh_ref.at[unit * CB:(unit + 1) * CB]
        hhc = hhc_ref.at[unit * 5 * HB:(unit + 1) * 5 * HB]
        ob = o_ref.at[rows_of(t)]

        def emit(dn, b, ls):
            o = x1_src[b * CB:(b + 1) * CB, ls] + _rep(mod_ref[4, :, ls], CB) * dn
            w = pltpu.pack_elementwise([o[:HB], o[HB:]], packed_dtype=BF16)
            ob[b * CB:(b + 1) * CB, ls] = pltpu.bitcast(w, BF16)

        for b in range(2):
            KC = _E('KC', 512)
            ps = [bg.dot(_unpk(hh[b * HB:(b + 1) * HB, k0:k0 + KC]), _unpk(wdr_ref[k0 // 2:(k0 + KC) // 2, :]))
                  for k0 in range(0, Fh, KC)]
            emit(functools.reduce(lambda x, y: x + y, ps), b, lanes[NL - 1])
        for j in range(NK):
            cl, cr = lanes[j], lanes[NK + j]
            sa = [_unpk(hhc[i * HB:(i + 1) * HB, :]) for i in range(5)]
            a11 = cat([_unpk(hh[0:HB, f * FC:f * FC + 128]) for f in range(NF)], axis=1)
            a22 = cat([_unpk(hh[HB:CB, f * FC + 128:(f + 1) * FC]) for f in range(NF)], axis=1)
            tb = [_unpk(wdc_ref[i * (Fh // 4):(i + 1) * (Fh // 4), cl]) for i in range(7)]
            c11, c12, c21, c22 = strassen(sa, a11, a22, tb, None)
            emit(c21, 1, cl)
            emit(c11, 0, cl)
            emit(c12, 0, cr)
            emit(c22, 1, cr)

    x1s = [x1s_ref.at[r * TM:(r + 1) * TM] for r in range(2)]
    sts = [st_ref.at[r * TM:(r + 1) * TM] for r in range(2)]
    YP = _E('YP', 11)

    def setup():
        for cp in small:
            cp.wait()
        shk = shk_ref[...].astype(F32)
        for a in range(4):
            sh_ref[a] = jnp.broadcast_to(shk[a:a + 1, :], (8, D))
        zm_ref[...] = pltpu.bitcast(inv_ref[CB:CB + 16, :], I32)
        zs.append(zm_ref[0, 0])

    def prologue():
        ssm_cp(0).wait()
        k_fwd(0)
        ssm_cp(1).wait()
        k_fwd(1)
        for t in range(2):
            k_cp(t).wait()
            v_cp(t).wait()
            ssm_cp(2 + t).wait()
            now(kv_pieces(t, 64))
            k_fwd(2 + t)
            u_fwd(t)
        ssm_cp(4).wait()
        bg.flush()
        pos = sorted(positions, key=lambda p: p[1].start)
        n0 = _E('PY0', 32)
        bg.add(ystatic_pieces(0, YP, 0, 4, False, pos[:n0]), 0, 1024)
        bg.add(ystatic_pieces(0, YP, 0, 4, False, pos[n0:n0 + 1]), 5000, 5001)
        k_fwd(4)
        bg.flush()
        q_cp(0).wait()
        now(ystatic_pieces(0, YP, 0, 4, False, pos[n0 + 1:]))
        q_cp(1).wait()
        mod_cp(0).wait()
        mod_chunk(0)
        for t in range(2):
            now(post_pieces(t))
            now(ln1_pieces(t))
            y_inv(t, x1s[t])
        for t in range(2):
            now(ln2_stat_pieces(x1s[t], sts[t]))
        bg.flush()

    def superstep():
        yrest = ystatic_pieces(YP, NB, 0, 4, False)
        mod_cp(1).wait()
        mod_chunk(1)
        now(ln2_apply_pieces(x1s[0], sts[0], 0))
        bg.flush()
        g_cp(0).wait()
        u_cp(0).wait()
        bg.add(ln2_apply_pieces(x1s[1], sts[1], 1), 0, 850)
        bg.add(wgu_pieces(0), 0, 950)
        bg.add(yrest[0:_E('Y1', 40)], 1050, 2250)
        ffn_gu(0, 0, plain=True)
        ffn_gu(0, 1)
        bg.flush()
        k_cp(2).wait()
        v_cp(2).wait()
        g_cp(1).wait()
        u_cp(1).wait()
        bg.add(wgu_pieces(1), 0, 900)
        bg.add(kv_pieces(2), 1000, 2200)
        ffn_gu(1, 0, plain=True)
        ffn_gu(1, 1)
        bg.flush()
        for f in range(2, 4):
            g_cp(f).wait()
            u_cp(f).wait()
        bg.add(wgu_pieces(2), 0, 900)
        bg.add(wgu_pieces(3), 1900, 2700)
        bg.add(_group(ystatic_pieces(4, 6, 4, 6, True), 2), 2750, 4050)
        ffn_gu(2, 0, plain=True)
        u_fwd(2)
        ffn_gu(2, 1)
        ffn_gu(3, 0)
        bg.flush()
        for f in range(4, NF):
            g_cp(f).wait()
            u_cp(f).wait()
        q_cp(2).wait()
        y1, y2 = _E('Y1', 40), _E('Y2', 130)
        bg.add(wgu_pieces(4), 0, 800)
        bg.add(post_pieces(2), 850, 1600)
        bg.add(wgu_pieces(5), 1650, 2500)
        bg.add(linked(ln1_pieces(2), _E('LK', 3)), _E('W3', 300), _E('W4', 2900))
        bg.add(yrest[y1:y2], 2600, 4750)
        ffn_gu(3, 1)
        ffn_gu(4, 0)
        ffn_gu(4, 1)
        y_inv(2, x1_ref.at[0])
        ffn_gu(5, 0)
        bg.flush()
        d_cp.wait()
        mod_cp(2).wait()
        k_cp(3).wait()
        v_cp(3).wait()
        bg.add(wdr_pieces(), 0, 300)
        bg.add(wd_pieces(), 300, 2800)
        bg.add(linked(ln2_stat_pieces(x1_ref.at[0], st_ref), _E('LK2', 3)), 1200, 3000)
        bg.add(ln2_apply_pieces(x1_ref.at[0], st_ref, 0), 2900, 4000)
        bg.add(kv_pieces(3), _E('W1', 3900), _E('W2', 5400))
        bg.add(yrest[y2:], _E('W2', 5400), 7850)
        bg.inj = [(150 + 200 * i, gb_tile(i)) for i in range(NL)]
        ffn_gu(5, 1)
        ffn_down(x1s[0], 0, 0)
        ffn_down(x1s[1], 1, 1)
        bg.flush()
        o_cp(0).start()
        o_cp(1).start()

    def run_super(fn):
        if _E('SL', 1):
            def body(i, carry):
                fn()
                return carry
            lax.fori_loop(0, zs[0] + 1, body, 0)
        else:
            fn()

    def late_waits():
        for t in range(T0, NS):
            q_cp(t).wait()
            if t + 1 < NS:
                k_cp(t + 1).wait()
                v_cp(t + 1).wait()

    def step(t, carry):
        slot = lax.rem(t, 2)
        if _E('LA', 1):
            bg.add(linked(ln1_pieces(t), _E('LK1', 2)), _E('L0', 800), _E('L1', 6800))
        t1 = 640 + NF * 1152 + 320
        bg.add(linked(ln2_stat_pieces(x1_ref.at[slot], st_ref), _E('LK2', 3)), t1 + _E('S0', 100), t1 + _E('S1', 1800))
        bg.add(ln2_apply_pieces(x1_ref.at[slot], st_ref, 0), t1 + _E('P0', 1400), t1 + _E('P1', 3100))
        bg.add(kv_pieces(jnp.minimum(t + 1, NS - 1), 16), t1 + _E('K0', 100), t1 + _E('K1', 3100))
        u_fwd(t)
        chain(diag_pieces(t, T0 - 1), _E('DD', 2), _E('DE', 0))
        chain(task_pieces(t, 2), _E('MD', 2), _E('ME', 0))
        dep = chain(task_pieces(t, 1), _E('MD', 2), _E('ME', 0))
        chain(post_pieces(t), 1, 3, dep)
        if not _E('LA', 1):
            chain(ln1_pieces(t), 1)
        for f in range(NF):
            ffn_gu(f, 0, n=HB // 2)
        y_inv(t, x1_ref.at[slot])
        ffn_down(x1_ref.at[1 - slot], t - 1, 0)
        bg.flush()
        o_cp(t - 1).start()
        return carry

    def epilogue():
        t = NS - 1
        for f in range(NF):
            ffn_gu(f, 0, n=HB // 2)
        ffn_down(x1_ref.at[t % 2], t, 0)
        o_cp(t).start()
        for i in range(NS):
            o_cp(i).wait()

    sc = jax.named_scope if SCOPES else (lambda name: (lambda f: f))

    def rest():
        sc("superstep")(superstep)()
        late_waits()
        lax.fori_loop(T0, NS, sc("step")(step), 0)
        sc("epilogue")(epilogue)()

    if ONLY == 'loop':
        zs.append(zm_ref[0, 0])
        lax.fori_loop(T0, NS, step, 0)
        epilogue()
    elif ONLY == 'S':
        zs.append(zm_ref[0, 0])
        run_super(superstep)
        lax.fori_loop(T0, NS, step, 0)
    elif _E('NEST', 3) == 3:
        setup()

        def everything():
            sc("prologue")(prologue)()
            rest()
        run_super(everything)
    else:
        setup()
        sc("prologue")(prologue)()
        run_super(rest)


@jax.jit
def pallas_adaLN_cond__ssm_conv_h3__glu_gated_bilinear__prompt_kernel(
    A_q, A_k, A_v, A_shift_k, A_ssm_k, A_ssm_D, B_x, B_w_gate, B_w_up, B_w_down, c, w_mod,
):
    B, S, D = A_q.shape
    Fh = B_w_gate.shape[1]
    NB = S // CB
    NS = S // TM
    fwd, inv = _dft_consts()
    anyspec = pl.BlockSpec(memory_space=pl.ANY)
    V = pltpu.VMEM
    out = pl.pallas_call(
        functools.partial(_kernel, S=S, D=D, Fh=Fh),
        in_specs=[anyspec] * 13,
        out_specs=anyspec,
        out_shape=jax.ShapeDtypeStruct((S, D), A_q.dtype),
        scratch_shapes=[
            V((NS, 2, 3 * CB, D), F32),
            V((NB, 3 * CB, D), F32),
            V((NS, 2, 3 * CB, D), F32),
            V((2, TM, D), F32),
            V((S, D), BF16), V((S, D), BF16), V((S, D), BF16), V((S, D), BF16),
            V((2 * TM, D), F32),
            V((TM, D), F32),
            V((2 * TM, 256), F32),
            V((2 * CB, D), U32),
            V((2 * 5 * HB, KS), U32),
            V((2 * CB, Fh), U32),
            V((2 * 5 * HB, Fh // 2), U32),
            V((TM // 2, D), U32),
            V((2 * CB, D), U32),
            V(((D - 2 * KS) // 2, Fh), U32), V(((D - 2 * KS) // 2, Fh), U32), V((Fh // 2, D - 2 * KS), U32),
            V((7 * KS // 2, Fh // 2), U32), V((7 * KS // 2, Fh // 2), U32), V((7 * Fh // 4, KS), U32),
            V((D, S), BF16), V((D, 6 * D), BF16), V((D, Fh), BF16), V((D, Fh), BF16), V((Fh, D), BF16),
            V((2 * CB, CB), BF16), V((CB + 16, CB), BF16),
            V((5, 8, D), F32), V((4, 8, D), F32), V((8, 128), I32),
            V((4, D), BF16), V((D,), BF16), V((1, D), BF16),
            pltpu.SemaphoreType.DMA((5 + 4 * NS + D // 128 + 3 + 2 * (Fh // FC) + 1,)),
        ],
        compiler_params=pltpu.CompilerParams(
            internal_scratch_in_bytes=48 * 1024,
            disable_semaphore_checks=True,
            disable_bounds_checks=True,
            vmem_limit_bytes=110 * 1024 * 1024),
        name="adaln_h3_glu",
    )(A_q.reshape(S, D), A_k.reshape(S, D), A_v.reshape(S, D), A_shift_k.T, A_ssm_k,
      A_ssm_D, B_w_gate, B_w_up, B_w_down, c, w_mod, fwd, inv)
    return out.reshape(B, S, D)
```

```python
import functools
import os

import numpy as np
import jax
import jax.numpy as jnp
from jax import lax
import jax.experimental.pallas as pl
import jax.experimental.pallas.tpu as pltpu

F32 = jnp.float32
BF16 = jnp.bfloat16
U32 = jnp.uint32
I32 = jnp.int32

CB = 128
HB = CB // 2
TM = 256
FC = 256
KS = 256
EPS = 1e-5
SCOPES = False
ONLY = os.environ.get('ONLY', '')


def _E(name, default):
    return int(os.environ.get(name, default))


def _dft_consts():
    k = np.arange(CB, dtype=np.float64)[:, None]
    n = np.arange(CB, dtype=np.float64)[None, :]
    th = np.pi * (4.0 * k + 1.0) * n / (2.0 * CB)
    fwd = np.concatenate([np.cos(th), np.sin(th)], axis=0)
    g = np.concatenate([np.cos(th[:HB]), np.sin(th[:HB])], axis=0).T / CB
    inv = np.concatenate([g[0::2], g[1::2], np.zeros((16, CB))], axis=0)
    return jnp.asarray(fwd, dtype=BF16), jnp.asarray(inv, dtype=BF16)


def _pk(x):
    return pltpu.bitcast(x.astype(BF16), U32)


def _unpk(x):
    return pltpu.bitcast(x, BF16)


def _rep(r, n):
    return r if n == 8 else jnp.concatenate([r] * (n // 8), axis=0)


def _add(x, tok):
    return x if tok is None else x + _rep(tok, x.shape[0])


def _group(pieces, n):
    def merged(ps):
        def run(tok):
            for p in ps:
                p(tok)
        return run
    return [merged(pieces[i:i + n]) for i in range(0, len(pieces), n)]


class _Sched:
    def __init__(self, token):
        self.token = token
        self.clock = 0.0
        self.q = []
        self.last = None
        self.inj = []

    def add(self, pieces, t0, t1):
        n = len(pieces)
        self.q += [(t0 + (t1 - t0) * i / n, len(self.q) + i, p) for i, p in enumerate(pieces)]
        self.q.sort(key=lambda e: e[:2])

    def note(self, m, dt):
        rows, cols = m.shape
        tiles = [(slice(r, r + 8), slice(c, c + 128)) for c in range(0, cols, 128) for r in range(0, rows, 8)]
        for i, tl in enumerate(tiles):
            tok = None
            while self.q and self.q[0][0] <= self.clock + dt * (i + 1) / len(tiles):
                if tok is None:
                    tok = self.token(m[tl])
                self.q.pop(0)[2](tok)
        self.clock += dt
        self.last = m[tiles[-1]]
        return m

    def dot(self, a, b):
        if self.inj and self.clock >= self.inj[0][0]:
            self.inj.pop(0)[1]()
        m = jnp.dot(a, b, preferred_element_type=F32)
        return self.note(m, max(a.shape[0], 32) * (a.shape[1] // 128) * (b.shape[1] // 128) / 4)

    def flush(self):
        tok = None if self.last is None or not self.q else self.token(self.last)
        while self.q:
            self.q.pop(0)[2](tok)
        self.clock = 0.0
        self.last = None


def _kernel(q_hbm, k_hbm, v_hbm, shk_hbm, ssmk_hbm, ssmd_hbm, wg_hbm, wu_hbm, wd_hbm,
            c_hbm, wmod_hbm, fwd_hbm, inv_hbm, o_hbm,
            u_ref, kk_ref, y_ref, x1_ref, q_ref, k_ref, v_ref, o_ref,
            x1s_ref, hp_ref, st_ref, h2_ref, h2c_ref, hh_ref, hhc_ref, kv_ref, yb_ref,
            wgr_ref, wur_ref, wdr_ref, wgc_ref, wuc_ref, wdc_ref,
            ssmk_ref, wmod_ref, wg_ref, wu_ref, wd_ref, fwd_ref, inv_ref,
            mod_ref, sh_ref, zm_ref, shk_ref, ssmd_ref, c_ref,
            sem, *, S, D, Fh):
    NB = S // CB
    NS = S // TM
    NL = D // 128
    NF = Fh // FC
    NK = KS // 128
    T0 = 3
    NLOOP = NS - T0
    lanes = [slice(i * 128, (i + 1) * 128) for i in range(NL)]
    cat = jnp.concatenate

    offs = [int(o) for o in np.cumsum([0, 5, NS, NS, NS, NL, 3, NF, NF, 1])]
    s_small, s_q, s_k, s_v, s_ssm, s_mod, s_g, s_u, s_d, s_o = offs

    def rows_of(t):
        return pl.ds(t * TM if isinstance(t, int) else pl.multiple_of(t * TM, TM), TM)

    def rows_cp(src, dst, base, t):
        return pltpu.make_async_copy(src.at[rows_of(t), :], dst.at[rows_of(t), :], sem.at[base + t])

    def cols_cp(src, dst, lo, hi, si):
        return pltpu.make_async_copy(src.at[:, lo:hi], dst.at[:, lo:hi], sem.at[si])

    q_cp = lambda t: rows_cp(q_hbm, q_ref, s_q, t)
    k_cp = lambda t: rows_cp(k_hbm, k_ref, s_k, t)
    v_cp = lambda t: rows_cp(v_hbm, v_ref, s_v, t)
    o_cp = lambda t: rows_cp(o_ref, o_hbm, s_o, t)
    small = [pltpu.make_async_copy(s, d, sem.at[s_small + i]) for i, (s, d) in enumerate(
        [(fwd_hbm, fwd_ref), (shk_hbm, shk_ref), (ssmd_hbm, ssmd_ref), (inv_hbm, inv_ref), (c_hbm, c_ref)])]
    ssm_cp = lambda i: pltpu.make_async_copy(ssmk_hbm.at[lanes[i], :], ssmk_ref.at[lanes[i], :],
                                             sem.at[s_ssm + i])
    mod_cols = [(0, 3 * D), (3 * D, 5 * D), (5 * D, 6 * D)]
    mod_cp = lambda i: cols_cp(wmod_hbm, wmod_ref, mod_cols[i][0], mod_cols[i][1], s_mod + i)
    g_cp = lambda f: cols_cp(wg_hbm, wg_ref, f * FC, (f + 1) * FC, s_g + f)
    u_cp = lambda f: cols_cp(wu_hbm, wu_ref, f * FC, (f + 1) * FC, s_u + f)
    d_cp = pltpu.make_async_copy(wd_hbm, wd_ref, sem.at[s_d])

    order = small + [ssm_cp(0), ssm_cp(1), k_cp(0), v_cp(0),
                     ssm_cp(2), k_cp(1), v_cp(1), ssm_cp(3), ssm_cp(4), q_cp(0), q_cp(1),
                     mod_cp(0), mod_cp(1), g_cp(0), u_cp(0), k_cp(2), v_cp(2)]
    for f in range(1, NF):
        order += [g_cp(f), u_cp(f)]
    order += [q_cp(2), d_cp, mod_cp(2), k_cp(3), v_cp(3)]
    for t in range(T0, NS):
        order += [q_cp(t)]
        if t + 1 < NS:
            order += [k_cp(t + 1), v_cp(t + 1)]
    for cp in order:
        cp.start()

    zs = []
    bg = _Sched(lambda x: pltpu.bitcast(pltpu.bitcast(x, I32) & zm_ref[...], F32))

    def opaque(ref):
        return ref.at[pl.ds(pl.multiple_of(zs[0], 32), ref.shape[0])]

    def chain(pieces, dist, extra=0, dep=None):
        hist = [] if dep is None else [dep] * dist
        for p in pieces:
            tok = None
            if len(hist) >= dist:
                tok = bg.token(hist[-dist])
                for _ in range(extra):
                    tok = tok + tok
            hist.append(p(tok))
        return hist[-1]

    def linked(pieces, d):
        res = []

        def wrap(p):
            def run(tok):
                if d and len(res) >= d:
                    tok = tok + bg.token(res[-d])
                res.append(p(tok))
            return run
        return [wrap(p) for p in pieces]

    def now(pieces):
        for p in pieces:
            p(None)

    def mod_chunk(i):
        c = c_ref[...].astype(F32)
        sc = jnp.broadcast_to((c * jax.nn.sigmoid(c)).astype(BF16), (16, D))
        lo, hi = mod_cols[i]
        m = bg.dot(sc, wmod_ref[:, lo:hi])[0:8]
        if i == 0:
            ga = m[:, 2 * D:3 * D]
            mod_ref[0] = (1.0 + m[:, D:2 * D]) * ga
            mod_ref[1] = m[:, 0:D] * ga
        elif i == 1:
            mod_ref[2] = 1.0 + m[:, D:2 * D]
            mod_ref[3] = m[:, 0:D]
        else:
            mod_ref[4] = m

    def gb_tile(i):
        def run():
            c = c_ref[...].astype(F32)
            sc = jnp.broadcast_to((c * jax.nn.sigmoid(c)).astype(BF16), (16, D))
            w = wmod_ref[:, 5 * D + i * 128:5 * D + (i + 1) * 128]
            mod_ref[4, :, lanes[i]] = jnp.dot(sc, w, preferred_element_type=F32)[0:8]
        return run

    def k_fwd(i):
        ls = lanes[i]
        fwd = fwd_ref[...]
        prev = None
        for m in range(NB):
            kf = lax.dot_general(fwd, ssmk_ref[ls, m * CB:(m + 1) * CB], (((1,), (1,)), ((), ())),
                                 preferred_element_type=F32)
            if m == 0:
                c = kf[:CB] + ssmd_ref[...].astype(F32).reshape(1, D)[:, ls]
                d = kf[CB:]
            else:
                c = kf[:CB] + prev[CB:]
                d = kf[CB:] - prev[:CB]
            prev = kf
            kk_ref[m, 0:CB, ls] = c
            kk_ref[m, CB:2 * CB, ls] = d - c
            kk_ref[m, 2 * CB:3 * CB, ls] = c + d
            if m % 4 == 3:
                bg.note(kf, 2 * CB)

    def lo_hi(w):
        return pltpu.bitcast(w << 16, F32), pltpu.bitcast(w & jnp.uint32(0xFFFF0000), F32)

    def kv_pieces(t, G=32):
        n = G // 2
        kb, vb = k_ref.at[rows_of(t)], v_ref.at[rows_of(t)]

        def piece(ls, r0):
            def run(tok):
                if r0 > 0:
                    w = pltpu.bitcast(kb[r0 - 16:r0 + G, ls], U32)
                else:
                    if isinstance(t, int) and t == 0:
                        halo = jnp.zeros((8, 128), U32)
                    else:
                        halo = pltpu.bitcast(k_ref.at[rows_of(t - 1)][TM - 16:TM, ls], U32)
                    w = cat([halo, pltpu.bitcast(kb[0:G, ls], U32)], axis=0)
                if tok is not None:
                    w = w | _rep(pltpu.bitcast(tok, U32), n + 8)
                ke, ko = lo_hi(w[8:])
                ke1, ko1 = lo_hi(pltpu.roll(w, 1, 0)[8:])
                _, ko2 = lo_hi(pltpu.roll(w, 2, 0)[8:])
                s0, s1, s2, s3 = [_rep(sh_ref[a, :, ls], n) for a in range(4)]
                ve, vo = lo_hi(pltpu.bitcast(vb[r0:r0 + G, ls], U32))
                kve = ((ke * s0 + ko1 * s1) + (ke1 * s2 + ko2 * s3)) * ve
                kvo = ((ko * s0 + ke * s1) + (ko1 * s2 + ke1 * s3)) * vo
                kv_ref[r0 // 2:(r0 + G) // 2, ls] = pltpu.bitcast(
                    pltpu.pack_elementwise([kve, kvo], packed_dtype=BF16), U32)
            return run
        return [piece(ls, r0) for ls in lanes for r0 in range(0, TM, G)]

    def u_fwd(t):
        fwd = fwd_ref[...]
        for b in range(2):
            uf = bg.dot(fwd, _unpk(kv_ref[b * HB:(b + 1) * HB, :]))
            a, bb = uf[:CB], uf[CB:]
            u_ref[t, b, 0:CB, :] = a + bb
            u_ref[t, b, CB:2 * CB, :] = a
            u_ref[t, b, 2 * CB:3 * CB, :] = bb

    positions = [(slice(r0, r0 + 8), ls) for r0 in range(0, 3 * CB, 8) for ls in lanes]

    def ystatic_pieces(s_lo, s_hi, i_lo, i_hi, acc_in, pos=None):
        def piece(rs, ls):
            def run(tok):
                us = {i: _add(u_ref[i // 2, i % 2, rs, ls], tok) for i in range(i_lo, i_hi)}
                ks = {}
                for s in range(s_lo, s_hi):
                    acc = None
                    for i in range(i_lo, min(i_hi, s + 1)):
                        m = s - i
                        if m not in ks:
                            ks[m] = kk_ref[m, rs, ls]
                        p = ks[m] * us[i]
                        acc = p if acc is None else acc + p
                    if acc_in:
                        acc = acc + y_ref[s // 2, s % 2, rs, ls]
                    y_ref[s // 2, s % 2, rs, ls] = acc
                return acc
            return run
        return [piece(*p) for p in (positions if pos is None else pos)]

    def task_pieces(t, delta):
        p = t - delta
        left = p >= T0
        J = jnp.where(left, t, p + NLOOP)
        I = jnp.where(left, p, t)
        kview = kk_ref.at[pl.ds(2 * (J - I) - 1, 3)]

        def piece(rs, ls):
            def run(tok):
                u0 = _add(u_ref[I, 0, rs, ls], tok)
                u1 = _add(u_ref[I, 1, rs, ls], tok)
                kc = kview[1, rs, ls]
                y_ref[J, 0, rs, ls] = (kc * u0 + kview[0, rs, ls] * u1) + y_ref[J, 0, rs, ls]
                y1 = (kview[2, rs, ls] * u0 + kc * u1) + y_ref[J, 1, rs, ls]
                y_ref[J, 1, rs, ls] = y1
                return y1
            return run
        return [piece(*p) for p in positions]

    def diag_pieces(t, I):
        kview = kk_ref.at[pl.ds(2 * (t - I) - 1, 3)]

        def piece(rs, ls):
            def run(tok):
                us = [_add(u_ref[a, b, rs, ls], tok) for a in (t, I) for b in range(2)]
                k0 = kk_ref[0, rs, ls]
                kc = kview[1, rs, ls]
                y_ref[t, 0, rs, ls] = ((k0 * us[0] + y_ref[t, 0, rs, ls])
                                       + (kc * us[2] + kview[0, rs, ls] * us[3]))
                y1 = ((kk_ref[1, rs, ls] * us[0] + k0 * us[1])
                      + (kview[2, rs, ls] * us[2] + kc * us[3]) + y_ref[t, 1, rs, ls])
                y_ref[t, 1, rs, ls] = y1
                return y1
            return run
        return [piece(*p) for p in positions]

    def post_pieces(t):
        def piece(b, r0, ls):
            def run(tok):
                comp = lambda c, off: y_ref[t, b, c * CB + off + r0:c * CB + off + r0 + 16, ls]
                k1l, k1h = _add(comp(0, 0), tok), _add(comp(0, HB), tok)
                rel, reh = k1l - comp(2, 0), k1h - comp(2, HB)
                iml, imh = k1l + comp(1, 0), k1h + comp(1, HB)
                p0 = b * CB + r0 // 2
                yb_ref[p0:p0 + 8, ls] = _pk(rel + reh)
                yb_ref[p0 + HB // 2:p0 + HB // 2 + 8, ls] = _pk(iml + imh)
                yb_ref[p0 + HB:p0 + HB + 8, ls] = _pk(rel - reh)
                oim = iml - imh
                yb_ref[p0 + HB + HB // 2:p0 + HB + HB // 2 + 8, ls] = _pk(oim)
                return oim[8:16]
            return run
        return [piece(b, r0, ls) for b in range(2) for r0 in range(0, HB, 16) for ls in lanes]

    def q_split(t, b, p0, n, ls):
        w = pltpu.bitcast(q_ref.at[rows_of(t)][b * CB + 2 * p0:b * CB + 2 * p0 + 2 * n, ls], U32)
        return lo_hi(w)

    def ln_tiles(xs, tok):
        n = xs[0].shape[0]
        s = _add(xs[0], tok)
        for x in xs[1:]:
            s = s + x
        m = jnp.sum(s, axis=-1, keepdims=True) * (1.0 / D)
        xc = [x - m for x in xs]
        s2 = xc[0] * xc[0]
        for x in xc[1:]:
            s2 = s2 + x * x
        r = lax.rsqrt(jnp.sum(s2, axis=-1, keepdims=True) * (1.0 / D) + EPS)
        return xc, jnp.broadcast_to(r, (n, 128)), jnp.broadcast_to(m, (n, 128))

    def ln1_pieces(t):
        G = _E('L1G', 8)

        def piece(b, p0):
            def run(tok):
                xc, r, _ = ln_tiles([cat(q_split(t, b, p0, G, ls), axis=0) for ls in lanes], tok)
                for ls, x in zip(lanes, xc):
                    h = (x * r) * _rep(mod_ref[0, :, ls], 2 * G) + _rep(mod_ref[1, :, ls], 2 * G)
                    hp_ref[b * CB + p0:b * CB + p0 + G, ls] = h[:G]
                    hp_ref[b * CB + HB + p0:b * CB + HB + p0 + G, ls] = h[G:]
                return functools.reduce(lambda a, c: a + c, [h[r:r + 8] for r in range(0, 2 * G, 8)])
            return run
        return [piece(b, p0) for b in range(2) for p0 in range(0, HB, G)]

    def y_inv(t, x1_dst):
        yb = opaque(yb_ref)
        hp = opaque(hp_ref)
        for b in range(2):
            ye = bg.dot(inv_ref[0:HB, :], _unpk(yb[b * CB:b * CB + HB, :]))
            yo = bg.dot(inv_ref[HB:CB, :], _unpk(yb[b * CB + HB:(b + 1) * CB, :]))
            for ls in lanes:
                qe, qo = q_split(t, b, 0, HB, ls)
                re, ro = slice(b * CB, b * CB + HB), slice(b * CB + HB, (b + 1) * CB)
                x1_dst[re, ls] = qe + hp[re, ls] * ye[:, ls]
                x1_dst[ro, ls] = qo + hp[ro, ls] * yo[:, ls]

    def a_combos(a11, a12, a21, a22):
        return [a11 + a22, a21 + a22, a11 + a12, a21 - a11, a12 - a22]

    def b_combos(b11, b12, b21, b22):
        return [b11 + b22, b12 - b22, b21 - b11, b11 + b12, b21 + b22, b11, b22]

    def ln2_stat_pieces(x1_src, st):
        x1o = opaque(x1_src)

        def piece(r0):
            def run(tok):
                _, r, m = ln_tiles([x1o[r0:r0 + 16, ls] for ls in lanes], tok)
                st[r0:r0 + 16, 0:128] = m
                st[r0:r0 + 16, 128:256] = r
                return r[0:8] + r[8:16]
            return run
        return [piece(h * CB + r0) for r0 in range(0, CB, 16) for h in range(2)]

    def ln2_apply_pieces(x1_src, st, unit):
        G = 16
        x1o = opaque(x1_src)
        h2_dst = h2_ref.at[unit * CB:(unit + 1) * CB]
        h2c_dst = h2c_ref.at[unit * 5 * HB:(unit + 1) * 5 * HB]

        def piece(r0, js):
            def run(tok):
                two = lambda ref, c: cat([ref[r0:r0 + G, c], ref[CB + r0:CB + r0 + G, c]], axis=0)
                m, r = _add(two(st, slice(0, 128)), tok), two(st, slice(128, 256))
                hs = {}
                for j in js:
                    ls = lanes[j]
                    h = ((two(x1o, ls) - m) * r) * _rep(mod_ref[2, :, ls], 2 * G) + _rep(mod_ref[3, :, ls], 2 * G)
                    hs[j] = h
                    h2_dst[r0 // 2:(r0 + G) // 2, ls] = _pk(h[:G])
                    h2_dst[(CB + r0) // 2:(CB + r0 + G) // 2, ls] = _pk(h[G:])
                    if NK <= j < 2 * NK:
                        cs = a_combos(hs[j - NK][:G], h[:G], hs[j - NK][G:], h[G:])
                        for i, cmb in enumerate(cs):
                            h2c_dst[i * HB + r0 // 2:i * HB + (r0 + G) // 2, lanes[j - NK]] = _pk(cmb)
            return run
        parts = [[j, NK + j] for j in range(NK)]
        parts[-1] += list(range(2 * NK, NL))
        return [piece(r0, js) for r0 in range(0, CB, G) for js in parts]

    def strassen(sa, a11, a22, tb, rem):
        dot = bg.dot
        m1 = dot(sa[0], tb[0])
        if rem is None:
            m7 = dot(sa[4], tb[4])
        else:
            m7 = dot(cat([sa[4], rem[0]], axis=1), cat([tb[4], rem[2]], axis=0))
        m4 = dot(a22, tb[2])
        m2 = dot(sa[1], tb[5])
        c21 = m2 + m4
        if rem is not None:
            c21 = c21 + dot(rem[1], rem[2])
        m5 = dot(sa[2], tb[6])
        c11 = m1 + m7 + m4 - m5
        m3 = dot(a11, tb[1])
        c12 = m3 + m5
        if rem is None:
            m6 = dot(sa[3], tb[3])
        else:
            c12 = c12 + dot(rem[0], rem[3])
            m6 = dot(cat([sa[3], rem[1]], axis=1), cat([tb[3], rem[3]], axis=0))
        c22 = m1 - m2 + m3 + m6
        return c11, c12, c21, c22

    def wgu_pieces(f):
        G = 16
        cl, cr = slice(f * FC, f * FC + 128), slice(f * FC + 128, (f + 1) * FC)

        def piece(w_ref, wc_ref, wr_ref, r0):
            def run(tok):
                b11 = _add(w_ref[r0:r0 + G, cl].astype(F32), tok)
                b22 = _add(w_ref[KS + r0:KS + r0 + G, cr].astype(F32), tok)
                cs = b_combos(b11, w_ref[r0:r0 + G, cr].astype(F32),
                              w_ref[KS + r0:KS + r0 + G, cl].astype(F32), b22)
                for i, cmb in enumerate(cs):
                    wc_ref[(i * KS + r0) // 2:(i * KS + r0 + G) // 2, f * 128:(f + 1) * 128] = _pk(cmb)
                if r0 < D - 2 * KS:
                    for c in (cl, cr):
                        w = pltpu.bitcast(w_ref[2 * KS + r0:2 * KS + r0 + G, c], U32)
                        wr_ref[r0 // 2:(r0 + G) // 2, c] = w if tok is None else w | pltpu.bitcast(tok, U32)
            return run
        return [piece(*refs, r0) for refs in ((wg_ref, wgc_ref, wgr_ref), (wu_ref, wuc_ref, wur_ref))
                for r0 in range(0, KS, G)]

    def wd_pieces():
        G = 16

        def piece(j, f, r0):
            def run(tok):
                cl, cr = lanes[j], lanes[NK + j]
                re = slice(f * FC + r0, f * FC + r0 + G)
                ro = slice(f * FC + 128 + r0, f * FC + 128 + r0 + G)
                b11 = _add(wd_ref[re, cl].astype(F32), tok)
                b22 = _add(wd_ref[ro, cr].astype(F32), tok)
                cs = b_combos(b11, wd_ref[re, cr].astype(F32), wd_ref[ro, cl].astype(F32), b22)
                for i, cmb in enumerate(cs):
                    p0 = i * (Fh // 4) + (f * 128 + r0) // 2
                    wdc_ref[p0:p0 + G // 2, cl] = _pk(cmb)
            return run
        return [piece(j, f, r0) for j in range(NK) for f in range(NF) for r0 in range(0, 128, G)]

    def wdr_pieces():
        G = 128

        def piece(r0):
            def run(tok):
                w = pltpu.bitcast(wd_ref[r0:r0 + G, lanes[NL - 1]], U32)
                wdr_ref[r0 // 2:(r0 + G) // 2, :] = w | _rep(pltpu.bitcast(tok, U32), G // 2)
            return run
        return [piece(r0) for r0 in range(0, Fh, G)]

    def ffn_gu(f, unit, plain=False, n=HB):
        cl, cr = slice(f * FC, f * FC + 128), slice(f * FC + 128, (f + 1) * FC)
        h2 = h2_ref.at[unit * CB:(unit + 1) * CB]
        h2c = h2c_ref.at[unit * 5 * HB:(unit + 1) * 5 * HB]
        hh = hh_ref.at[unit * CB:(unit + 1) * CB]
        hhc = hhc_ref.at[unit * 5 * HB:(unit + 1) * 5 * HB]

        def store(p0, n, p11, p12, p21, p22):
            hh[p0:p0 + n, cl] = _pk(p11)
            hh[p0:p0 + n, cr] = _pk(p12)
            hh[HB + p0:HB + p0 + n, cl] = _pk(p21)
            hh[HB + p0:HB + p0 + n, cr] = _pk(p22)
            for i, cmb in enumerate(a_combos(p11, p12, p21, p22)):
                hhc[i * HB + p0:i * HB + p0 + n, f * 128:(f + 1) * 128] = _pk(cmb)

        if plain:
            p11, p12, p21, p22 = [
                bg.dot(_unpk(h2[r:r + HB, :]), wg_ref[:, c]) * bg.dot(_unpk(h2[r:r + HB, :]), wu_ref[:, c])
                for r in (0, HB) for c in (cl, cr)]
            store(0, HB, p11, p12, p21, p22)
        else:
            for p0 in range(0, HB, n):
                res = []
                top, bot = slice(p0, p0 + n), slice(HB + p0, HB + p0 + n)
                for wr, wc in ((wgr_ref, wgc_ref), (wur_ref, wuc_ref)):
                    sa = [_unpk(h2c[i * HB + p0:i * HB + p0 + n, :]) for i in range(5)]
                    tb = [_unpk(wc[i * KS // 2:(i + 1) * KS // 2, f * 128:(f + 1) * 128]) for i in range(7)]
                    rem = (_unpk(h2[top, 2 * KS:D]), _unpk(h2[bot, 2 * KS:D]), _unpk(wr[:, cl]), _unpk(wr[:, cr]))
                    res.append(strassen(sa, _unpk(h2[top, 0:KS]), _unpk(h2[bot, KS:2 * KS]), tb, rem))
                store(p0, n, *[g * u for g, u in zip(*res)])

    def ffn_down(x1_src, t, unit, mid=None):
        hh = hh_ref.at[unit * CB:(unit + 1) * CB]
        hhc = hhc_ref.at[unit * 5 * HB:(unit + 1) * 5 * HB]
        ob = o_ref.at[rows_of(t)]

        def emit(dn, b, ls):
            o = x1_src[b * CB:(b + 1) * CB, ls] + _rep(mod_ref[4, :, ls], CB) * dn
            w = pltpu.pack_elementwise([o[:HB], o[HB:]], packed_dtype=BF16)
            ob[b * CB:(b + 1) * CB, ls] = pltpu.bitcast(w, BF16)

        def rem():
            KC = 512
            for b in range(2):
                ps = [bg.dot(_unpk(hh[b * HB:(b + 1) * HB, k0:k0 + KC]), _unpk(wdr_ref[k0 // 2:(k0 + KC) // 2, :]))
                      for k0 in range(0, Fh, KC)]
                emit(functools.reduce(lambda x, y: x + y, ps), b, lanes[NL - 1])

        if mid is None:
            rem()
        for j in range(NK):
            cl, cr = lanes[j], lanes[NK + j]
            sa = [_unpk(hhc[i * HB:(i + 1) * HB, :]) for i in range(5)]
            a11 = cat([_unpk(hh[0:HB, f * FC:f * FC + 128]) for f in range(NF)], axis=1)
            a22 = cat([_unpk(hh[HB:CB, f * FC + 128:(f + 1) * FC]) for f in range(NF)], axis=1)
            tb = [_unpk(wdc_ref[i * (Fh // 4):(i + 1) * (Fh // 4), cl]) for i in range(7)]
            c11, c12, c21, c22 = strassen(sa, a11, a22, tb, None)
            emit(c21, 1, cl)
            emit(c11, 0, cl)
            emit(c12, 0, cr)
            emit(c22, 1, cr)
        if mid is not None:
            mid()
            rem()

    x1s = [x1s_ref.at[r * TM:(r + 1) * TM] for r in range(2)]
    sts = [st_ref.at[r * TM:(r + 1) * TM] for r in range(2)]
    YP = _E('YP', 11)

    def setup():
        for cp in small:
            cp.wait()
        shk = shk_ref[...].astype(F32)
        for a in range(4):
            sh_ref[a] = jnp.broadcast_to(shk[a:a + 1, :], (8, D))
        zm_ref[...] = pltpu.bitcast(inv_ref[CB:CB + 16, :], I32)
        zs.append(zm_ref[0, 0])

    def prologue():
        ssm_cp(0).wait()
        k_fwd(0)
        ssm_cp(1).wait()
        k_fwd(1)
        for t in range(2):
            k_cp(t).wait()
            v_cp(t).wait()
            ssm_cp(2 + t).wait()
            now(kv_pieces(t, 64))
            k_fwd(2 + t)
            u_fwd(t)
        ssm_cp(4).wait()
        bg.flush()
        pos = sorted(positions, key=lambda p: p[1].start)
        n0 = _E('PY0', 32)
        bg.add(ystatic_pieces(0, YP, 0, 4, False, pos[:n0]), 0, 1024)
        bg.add(ystatic_pieces(0, YP, 0, 4, False, pos[n0:n0 + 1]), 5000, 5001)
        k_fwd(4)
        bg.flush()
        q_cp(0).wait()
        now(ystatic_pieces(0, YP, 0, 4, False, pos[n0 + 1:]))
        q_cp(1).wait()
        mod_cp(0).wait()
        mod_chunk(0)
        for t in range(2):
            now(post_pieces(t))
            now(ln1_pieces(t))
            y_inv(t, x1s[t])
        for t in range(2):
            now(ln2_stat_pieces(x1s[t], sts[t]))
        bg.flush()

    def superstep():
        yrest = ystatic_pieces(YP, NB, 0, 4, False)
        mod_cp(1).wait()
        mod_chunk(1)
        now(ln2_apply_pieces(x1s[0], sts[0], 0))
        bg.flush()
        g_cp(0).wait()
        u_cp(0).wait()
        bg.add(ln2_apply_pieces(x1s[1], sts[1], 1), 0, 850)
        bg.add(wgu_pieces(0), 0, 950)
        bg.add(yrest[0:_E('Y1', 40)], 1050, 2250)
        ffn_gu(0, 0, plain=True)
        ffn_gu(0, 1)
        bg.flush()
        k_cp(2).wait()
        v_cp(2).wait()
        g_cp(1).wait()
        u_cp(1).wait()
        bg.add(wgu_pieces(1), 0, 900)
        bg.add(kv_pieces(2), 1000, 2200)
        ffn_gu(1, 0, plain=True)
        ffn_gu(1, 1)
        bg.flush()
        for f in range(2, 4):
            g_cp(f).wait()
            u_cp(f).wait()
        bg.add(wgu_pieces(2), 0, 900)
        bg.add(wgu_pieces(3), 1900, 2700)
        bg.add(_group(ystatic_pieces(4, 6, 4, 6, True), 2), 2750, 4050)
        ffn_gu(2, 0, plain=True)
        u_fwd(2)
        ffn_gu(2, 1)
        ffn_gu(3, 0)
        bg.flush()
        for f in range(4, NF):
            g_cp(f).wait()
            u_cp(f).wait()
        q_cp(2).wait()
        y1, y2 = _E('Y1', 40), _E('Y2', 130)
        bg.add(wgu_pieces(4), 0, 800)
        bg.add(post_pieces(2), 850, 1600)
        bg.add(wgu_pieces(5), 1650, 2500)
        bg.add(linked(ln1_pieces(2), _E('LK', 3)), _E('W3', 300), _E('W4', 2900))
        bg.add(yrest[y1:y2], 2600, 4750)
        ffn_gu(3, 1)
        ffn_gu(4, 0)
        ffn_gu(4, 1)
        y_inv(2, x1_ref.at[0])
        ffn_gu(5, 0)
        bg.flush()
        d_cp.wait()
        mod_cp(2).wait()
        k_cp(3).wait()
        v_cp(3).wait()
        bg.add(wdr_pieces(), 0, 300)
        bg.add(wd_pieces(), 300, 2800)
        bg.add(linked(ln2_stat_pieces(x1_ref.at[0], st_ref), _E('LK2', 3)), 1200, 3000)
        bg.add(ln2_apply_pieces(x1_ref.at[0], st_ref, 0), 2900, 4000)
        bg.add(kv_pieces(3), _E('W1', 3900), _E('W2', 5400))
        bg.add(yrest[y2:], _E('W2', 5400), 7850)
        bg.inj = [(150 + 200 * i, gb_tile(i)) for i in range(NL)]
        ffn_gu(5, 1)
        ffn_down(x1s[0], 0, 0)
        ffn_down(x1s[1], 1, 1)
        bg.flush()
        o_cp(0).start()
        o_cp(1).start()

    def run_super(fn):
        if _E('SL', 1):
            def body(i, carry):
                fn()
                return carry
            lax.fori_loop(0, zs[0] + 1, body, 0)
        else:
            fn()

    def late_waits():
        for t in range(T0, NS):
            q_cp(t).wait()
            if t + 1 < NS:
                k_cp(t + 1).wait()
                v_cp(t + 1).wait()

    def step(t, carry):
        slot = lax.rem(t, 2)
        if _E('LA', 1):
            bg.add(linked(ln1_pieces(t), _E('LK1', 2)), _E('L0', 800), _E('L1', 6800))
        t1 = 640 + NF * 1152 + 320
        bg.add(linked(ln2_stat_pieces(x1_ref.at[slot], st_ref), _E('LK2', 3)), t1 + _E('S0', 100), t1 + _E('S1', 1800))
        bg.add(ln2_apply_pieces(x1_ref.at[slot], st_ref, 0), t1 + _E('P0', 1400), t1 + _E('P1', 3100))
        bg.add(kv_pieces(jnp.minimum(t + 1, NS - 1), 16), t1 + _E('K0', 100), t1 + _E('K1', 3100))
        u_fwd(t)
        chain(diag_pieces(t, T0 - 1), _E('DD', 2), _E('DE', 0))
        chain(task_pieces(t, 2), _E('MD', 2), _E('ME', 0))
        dep = chain(task_pieces(t, 1), _E('MD', 2), _E('ME', 0))
        chain(post_pieces(t), 1, 3, dep)
        if not _E('LA', 1):
            chain(ln1_pieces(t), 1)
        for f in range(NF):
            ffn_gu(f, 0, n=HB // 2)
        y_inv(t, x1_ref.at[slot])
        ffn_down(x1_ref.at[1 - slot], t - 1, 0)
        bg.flush()
        o_cp(t - 1).start()
        return carry

    def epilogue():
        t = NS - 1
        for f in range(NF):
            ffn_gu(f, 0, n=HB // 2)
        last = [pltpu.make_async_copy(o_ref.at[rows_of(t), lo:hi], o_hbm.at[rows_of(t), lo:hi], sem.at[s_o + t + i])
                for i, (lo, hi) in enumerate([(0, 2 * KS), (2 * KS, D)])]
        ffn_down(x1_ref.at[t % 2], t, 0, mid=last[0].start)
        last[1].start()
        for i in range(NS - 1):
            o_cp(i).wait()
        for cp in last:
            cp.wait()

    sc = jax.named_scope if SCOPES else (lambda name: (lambda f: f))

    def rest():
        sc("superstep")(superstep)()
        late_waits()
        lax.fori_loop(T0, NS, sc("step")(step), 0)
        sc("epilogue")(epilogue)()

    if ONLY == 'loop':
        zs.append(zm_ref[0, 0])
        lax.fori_loop(T0, NS, step, 0)
        epilogue()
    elif ONLY == 'S':
        zs.append(zm_ref[0, 0])
        run_super(superstep)
        lax.fori_loop(T0, NS, step, 0)
    elif _E('NEST', 3) == 3:
        setup()

        def everything():
            sc("prologue")(prologue)()
            rest()
        run_super(everything)
    else:
        setup()
        sc("prologue")(prologue)()
        run_super(rest)


@jax.jit
def pallas_adaLN_cond__ssm_conv_h3__glu_gated_bilinear__prompt_kernel(
    A_q, A_k, A_v, A_shift_k, A_ssm_k, A_ssm_D, B_x, B_w_gate, B_w_up, B_w_down, c, w_mod,
):
    B, S, D = A_q.shape
    Fh = B_w_gate.shape[1]
    NB = S // CB
    NS = S // TM
    fwd, inv = _dft_consts()
    anyspec = pl.BlockSpec(memory_space=pl.ANY)
    V = pltpu.VMEM
    out = pl.pallas_call(
        functools.partial(_kernel, S=S, D=D, Fh=Fh),
        in_specs=[anyspec] * 13,
        out_specs=anyspec,
        out_shape=jax.ShapeDtypeStruct((S, D), A_q.dtype),
        scratch_shapes=[
            V((NS, 2, 3 * CB, D), F32),
            V((NB, 3 * CB, D), F32),
            V((NS, 2, 3 * CB, D), F32),
            V((2, TM, D), F32),
            V((S, D), BF16), V((S, D), BF16), V((S, D), BF16), V((S, D), BF16),
            V((2 * TM, D), F32),
            V((TM, D), F32),
            V((2 * TM, 256), F32),
            V((2 * CB, D), U32),
            V((2 * 5 * HB, KS), U32),
            V((2 * CB, Fh), U32),
            V((2 * 5 * HB, Fh // 2), U32),
            V((TM // 2, D), U32),
            V((2 * CB, D), U32),
            V(((D - 2 * KS) // 2, Fh), U32), V(((D - 2 * KS) // 2, Fh), U32), V((Fh // 2, D - 2 * KS), U32),
            V((7 * KS // 2, Fh // 2), U32), V((7 * KS // 2, Fh // 2), U32), V((7 * Fh // 4, KS), U32),
            V((D, S), BF16), V((D, 6 * D), BF16), V((D, Fh), BF16), V((D, Fh), BF16), V((Fh, D), BF16),
            V((2 * CB, CB), BF16), V((CB + 16, CB), BF16),
            V((5, 8, D), F32), V((4, 8, D), F32), V((8, 128), I32),
            V((4, D), BF16), V((D,), BF16), V((1, D), BF16),
            pltpu.SemaphoreType.DMA((5 + 4 * NS + D // 128 + 3 + 2 * (Fh // FC) + 2,)),
        ],
        compiler_params=pltpu.CompilerParams(
            internal_scratch_in_bytes=48 * 1024,
            disable_semaphore_checks=True,
            disable_bounds_checks=True,
            vmem_limit_bytes=110 * 1024 * 1024),
        name="adaln_h3_glu",
    )(A_q.reshape(S, D), A_k.reshape(S, D), A_v.reshape(S, D), A_shift_k.T, A_ssm_k,
      A_ssm_D, B_w_gate, B_w_up, B_w_down, c, w_mod, fwd, inv)
    return out.reshape(B, S, D)
```

```python
import functools
import os

import numpy as np
import jax
import jax.numpy as jnp
from jax import lax
import jax.experimental.pallas as pl
import jax.experimental.pallas.tpu as pltpu

F32 = jnp.float32
BF16 = jnp.bfloat16
U32 = jnp.uint32
I32 = jnp.int32

CB = 128
HB = CB // 2
TM = 256
FC = 256
KS = 256
EPS = 1e-5
SCOPES = False
ONLY = os.environ.get('ONLY', '')


def _E(name, default):
    return int(os.environ.get(name, default))


def _dft_consts():
    k = np.arange(CB, dtype=np.float64)[:, None]
    n = np.arange(CB, dtype=np.float64)[None, :]
    th = np.pi * (4.0 * k + 1.0) * n / (2.0 * CB)
    fwd = np.concatenate([np.cos(th), np.sin(th)], axis=0)
    g = np.concatenate([np.cos(th[:HB]), np.sin(th[:HB])], axis=0).T / CB
    inv = np.concatenate([g[0::2], g[1::2], np.zeros((16, CB))], axis=0)
    return jnp.asarray(fwd, dtype=BF16), jnp.asarray(inv, dtype=BF16)


def _pk(x):
    return pltpu.bitcast(x.astype(BF16), U32)


def _unpk(x):
    return pltpu.bitcast(x, BF16)


def _rep(r, n):
    return r if n == 8 else jnp.concatenate([r] * (n // 8), axis=0)


def _add(x, tok):
    return x if tok is None else x + _rep(tok, x.shape[0])


def _group(pieces, n):
    def merged(ps):
        def run(tok):
            for p in ps:
                p(tok)
        return run
    return [merged(pieces[i:i + n]) for i in range(0, len(pieces), n)]


def _a2(x, y):
    return [x[0] + y[1], y[0] + y[1], x[0] + x[1], y[0] - x[0], x[1] - y[1], x[0], y[1]]


def _b2(b):
    return [b[0][0] + b[1][1], b[0][0], b[1][1], b[0][0] + b[0][1], b[1][0] + b[1][1],
            b[0][1] - b[1][1], b[1][0] - b[0][0]]


def _c2(m):
    m1, m7, m4, m2 = m(0), m(4), m(6), m(1)
    q0 = m2 + m4
    m5 = m(2)
    p0 = m1 + m7 + m4 - m5
    m3 = m(5)
    p1 = m3 + m5
    q1 = m1 - m2 + m3 + m(3)
    return [p0, p1], [q0, q1]


def _a3(x, y):
    w = [a + b for a, b in zip(x, y)]
    return [x[0], y[0], x[1], w[1], y[2], w[2], x[1] + y[2], x[2] - x[1], y[1] - y[2],
            w[1] - y[0], y[0] - y[1], w[0] - w[1], w[2] - x[0], x[0] - x[2], w[0] - w[2]]


def _b3(b):
    return [b[0][0] - b[0][1] + b[2][0], b[0][0] - b[0][2] + b[1][0], b[1][1] - b[1][0] + b[2][1],
            b[0][1] + b[1][1] - b[1][2], b[1][2] - b[2][0] + b[2][2], b[0][2] - b[2][1] + b[2][2],
            b[1][2] + b[2][1], b[2][1], b[1][2], b[0][1] + b[1][0], b[1][0], b[0][1],
            b[0][2] + b[2][0], b[2][0], b[0][2]]


_C3 = [(7, "+p1 +p2"), (8, "+q1 +q2"), (6, "+q1 +p2"), (14, "+q0 +q2"), (11, "+p0 +p1"), (5, "+p2"),
       (4, "-p2 +q2"), (12, "+q0 -p2 +q2"), (13, "-p0 +q0 -p2 +q2"), (3, "+q1"), (2, "+p1 -q1"),
       (9, "+p0 +p1 -q1"), (10, "+p0 -q0 +p1 -q1"), (1, "+q0"), (0, "+p0")]


def _c3(m, p=None, q=None, pad=0):
    v = {"p": [None] * 3 if p is None else list(p), "q": [None] * 3 if q is None else list(q)}
    for i, terms in _C3:
        x = m(i)
        for sg, h, n in terms.split():
            cur = v[h][int(n)]
            v[h][int(n)] = x if cur is None else (cur + x if sg == "+" else cur - x)
    return v["p"], v["q"]


def _c3cse(m, p=None, q=None, pad=0):
    p = [None] * 3 if p is None else list(p)
    q = [None] * 3 if q is None else list(q)

    def acc(v, n, x, neg=False):
        v[n] = (-x if neg else x) if v[n] is None else (v[n] - x if neg else v[n] + x)

    singles = [(5, p, 2), (3, q, 1), (1, q, 0), (0, p, 0)]
    for i, v, n in singles[:pad]:
        acc(v, n, m(i))
    m6, m7, m8 = m(6), m(7), m(8)
    if pad < 4:
        i, v, n = singles[pad]
        acc(v, n, m(i))
    acc(p, 1, m7), acc(q, 2, m8), acc(q, 1, m6 + m8), acc(p, 2, m6 + m7)
    m12, m13, m4, m14 = m(12), m(13), m(4), m(14)
    s2 = m12 + m13
    t2 = m4 + s2
    acc(q, 2, t2 + m14), acc(q, 0, s2 + m14), acc(p, 2, t2, True)
    m9, m10, m2, m11 = m(9), m(10), m(2), m(11)
    s1 = m9 + m10
    t1 = m2 + s1
    if p[0] is None:
        p[0] = (s1 + m11) - m13
    else:
        p[0] = (p[0] - m13) + (s1 + m11)
    acc(p, 1, t1 + m11), acc(q, 1, t1, True), acc(q, 0, m10, True)
    for i, v, n in singles[pad + 1:]:
        acc(v, n, m(i))
    return p, q


def _c3d(m, p=None, q=None, pad=0):
    p = [None] * 3 if p is None else list(p)
    q = [None] * 3 if q is None else list(q)

    def acc(v, n, x, neg=False):
        v[n] = x if v[n] is None else (v[n] - x if neg else v[n] + x)

    for i, a, b in ((7, (p, 1), (p, 2)), (8, (q, 1), (q, 2)), (6, (q, 1), (p, 2)), (14, (q, 0), (q, 2)),
                    (11, (p, 0), (p, 1))):
        x = m(i)
        acc(*a, x), acc(*b, x)
    m13 = m(13)
    m12 = m(12)
    acc(q, 0, m12)
    d2 = (m13 + m12) + m(4)
    acc(q, 2, d2), acc(p, 2, d2, True)
    acc(p, 2, m(5))
    m10 = m(10)
    d0 = m10 - m13
    acc(p, 0, d0), acc(q, 0, d0, True)
    m9 = m(9)
    acc(p, 0, m9)
    d1 = (m10 + m9) + m(2)
    acc(p, 1, d1), acc(q, 1, d1, True)
    acc(q, 1, m(3)), acc(q, 0, m(1)), acc(p, 0, m(0))
    return p, q


class _Sched:
    def __init__(self, token):
        self.token = token
        self.clock = 0.0
        self.q = []
        self.last = None
        self.inj = []

    def add(self, pieces, t0, t1):
        n = len(pieces)
        self.q += [(t0 + (t1 - t0) * i / n, len(self.q) + i, p) for i, p in enumerate(pieces)]
        self.q.sort(key=lambda e: e[:2])

    def note(self, m, dt):
        rows, cols = m.shape
        tiles = [(slice(r, r + 8), slice(c, c + 128)) for c in range(0, cols, 128) for r in range(0, rows, 8)]
        for i, tl in enumerate(tiles):
            tok = None
            while self.q and self.q[0][0] <= self.clock + dt * (i + 1) / len(tiles):
                if tok is None:
                    tok = self.token(m[tl])
                self.q.pop(0)[2](tok)
        self.clock += dt
        self.last = m[tiles[-1]]
        return m

    def dot(self, a, b):
        if self.inj and self.clock >= self.inj[0][0]:
            self.inj.pop(0)[1]()
        m = jnp.dot(a, b, preferred_element_type=F32)
        return self.note(m, max(a.shape[0], 32) * (a.shape[1] // 128) * (b.shape[1] // 128) / 4)

    def flush(self):
        tok = None if self.last is None or not self.q else self.token(self.last)
        while self.q:
            self.q.pop(0)[2](tok)
        self.clock = 0.0
        self.last = None


def _kernel(q_hbm, k_hbm, v_hbm, shk_hbm, ssmk_hbm, ssmd_hbm, wg_hbm, wu_hbm, wd_hbm,
            c_hbm, wmod_hbm, fwd_hbm, inv_hbm, o_hbm,
            u_ref, kk_ref, y_ref, x1_ref, q_ref, k_ref, v_ref, o_ref,
            hp_ref, st_ref, pp_ref, h2_ref, hf_ref, ha_ref, hs_ref, kv_ref, yb_ref,
            wga_ref, wua_ref, wdf_ref, wgs_ref, wus_ref,
            ssmk_ref, wmod_ref, wg_ref, wu_ref, wd_ref, fwd_ref, inv_ref,
            mod_ref, sh_ref, zm_ref, shk_ref, ssmd_ref, c_ref,
            sem, *, S, D, Fh):
    NB = S // CB
    NS = S // TM
    NL = D // 128
    NF = Fh // FC
    NT = Fh // 128
    T0 = 3
    NLOOP = NS - T0
    lanes = [slice(i * 128, (i + 1) * 128) for i in range(NL)]
    cat = jnp.concatenate

    offs = [int(o) for o in np.cumsum([0, 5, NS, NS, NS, NL, 3, NF, NF, 1])]
    s_small, s_q, s_k, s_v, s_ssm, s_mod, s_g, s_u, s_d, s_o = offs

    def rows_of(t):
        return pl.ds(t * TM if isinstance(t, int) else pl.multiple_of(t * TM, TM), TM)

    def rows_cp(src, dst, base, t):
        return pltpu.make_async_copy(src.at[rows_of(t), :], dst.at[rows_of(t), :], sem.at[base + t])

    def cols_cp(src, dst, lo, hi, si):
        return pltpu.make_async_copy(src.at[:, lo:hi], dst.at[:, lo:hi], sem.at[si])

    q_cp = lambda t: rows_cp(q_hbm, q_ref, s_q, t)
    k_cp = lambda t: rows_cp(k_hbm, k_ref, s_k, t)
    v_cp = lambda t: rows_cp(v_hbm, v_ref, s_v, t)
    o_cp = lambda t: rows_cp(o_ref, o_hbm, s_o, t)
    small = [pltpu.make_async_copy(s, d, sem.at[s_small + i]) for i, (s, d) in enumerate(
        [(fwd_hbm, fwd_ref), (shk_hbm, shk_ref), (ssmd_hbm, ssmd_ref), (inv_hbm, inv_ref), (c_hbm, c_ref)])]
    ssm_cp = lambda i: pltpu.make_async_copy(ssmk_hbm.at[lanes[i], :], ssmk_ref.at[lanes[i], :],
                                             sem.at[s_ssm + i])
    mod_cols = [(0, 3 * D), (3 * D, 5 * D), (5 * D, 6 * D)]
    mod_cp = lambda i: cols_cp(wmod_hbm, wmod_ref, mod_cols[i][0], mod_cols[i][1], s_mod + i)
    g_cp = lambda f: cols_cp(wg_hbm, wg_ref, f * FC, (f + 1) * FC, s_g + f)
    u_cp = lambda f: cols_cp(wu_hbm, wu_ref, f * FC, (f + 1) * FC, s_u + f)
    d_cp = pltpu.make_async_copy(wd_hbm, wd_ref, sem.at[s_d])

    order = small + [ssm_cp(0), k_cp(0), v_cp(0), k_cp(1), v_cp(1),
                     ssm_cp(1), ssm_cp(2), ssm_cp(3), ssm_cp(4), q_cp(0), q_cp(1),
                     mod_cp(0), mod_cp(1), g_cp(0), u_cp(0), k_cp(2), v_cp(2)]
    for f in range(1, NF):
        order += [g_cp(f), u_cp(f)]
    order += [q_cp(2), d_cp, mod_cp(2), k_cp(3), v_cp(3)]
    for t in range(T0, NS):
        order += [q_cp(t)]
        if t + 1 < NS:
            order += [k_cp(t + 1), v_cp(t + 1)]
    for cp in order:
        cp.start()

    zs = []
    bg = _Sched(lambda x: pltpu.bitcast(pltpu.bitcast(x, I32) & zm_ref[...], F32))

    def opaque(ref):
        return ref.at[pl.ds(pl.multiple_of(zs[0], 32), ref.shape[0])]

    def chain(pieces, dist, extra=0, dep=None):
        hist = [] if dep is None else [dep] * dist
        for p in pieces:
            tok = None
            if len(hist) >= dist:
                tok = bg.token(hist[-dist])
                for _ in range(extra):
                    tok = tok + tok
            hist.append(p(tok))
        return hist[-1]

    def linked(pieces, d):
        res = []

        def wrap(p):
            def run(tok):
                if d and len(res) >= d:
                    tok = tok + bg.token(res[-d])
                res.append(p(tok))
            return run
        return [wrap(p) for p in pieces]

    def now(pieces):
        for p in pieces:
            p(None)

    def mod_chunk(i):
        c = c_ref[...].astype(F32)
        sc = jnp.broadcast_to((c * jax.nn.sigmoid(c)).astype(BF16), (16, D))
        lo, hi = mod_cols[i]
        m = bg.dot(sc, wmod_ref[:, lo:hi])[0:8]
        if i == 0:
            ga = m[:, 2 * D:3 * D]
            mod_ref[0] = (1.0 + m[:, D:2 * D]) * ga
            mod_ref[1] = m[:, 0:D] * ga
        elif i == 1:
            mod_ref[2] = 1.0 + m[:, D:2 * D]
            mod_ref[3] = m[:, 0:D]
        else:
            mod_ref[4] = m

    def gb_tile(i):
        def run():
            c = c_ref[...].astype(F32)
            sc = jnp.broadcast_to((c * jax.nn.sigmoid(c)).astype(BF16), (16, D))
            w = wmod_ref[:, 5 * D + i * 128:5 * D + (i + 1) * 128]
            mod_ref[4, :, lanes[i]] = jnp.dot(sc, w, preferred_element_type=F32)[0:8]
        return run

    def k_fwd(i):
        ls = lanes[i]
        fwd = fwd_ref[...]
        prev = None
        for m in range(NB):
            kf = lax.dot_general(fwd, ssmk_ref[ls, m * CB:(m + 1) * CB], (((1,), (1,)), ((), ())),
                                 preferred_element_type=F32)
            if m == 0:
                c = kf[:CB] + ssmd_ref[...].astype(F32).reshape(1, D)[:, ls]
                d = kf[CB:]
            else:
                c = kf[:CB] + prev[CB:]
                d = kf[CB:] - prev[:CB]
            prev = kf
            kk_ref[m, 0:CB, ls] = c
            kk_ref[m, CB:2 * CB, ls] = d - c
            kk_ref[m, 2 * CB:3 * CB, ls] = c + d
            if m % 4 == 3:
                bg.note(kf, 2 * CB)

    def lo_hi(w):
        return pltpu.bitcast(w << 16, F32), pltpu.bitcast(w & jnp.uint32(0xFFFF0000), F32)

    def kv_pieces(t, G=32):
        n = G // 2
        kb, vb = k_ref.at[rows_of(t)], v_ref.at[rows_of(t)]

        def piece(ls, r0):
            def run(tok):
                if r0 > 0:
                    w = pltpu.bitcast(kb[r0 - 16:r0 + G, ls], U32)
                else:
                    if isinstance(t, int) and t == 0:
                        halo = jnp.zeros((8, 128), U32)
                    else:
                        halo = pltpu.bitcast(k_ref.at[rows_of(t - 1)][TM - 16:TM, ls], U32)
                    w = cat([halo, pltpu.bitcast(kb[0:G, ls], U32)], axis=0)
                if tok is not None:
                    w = w | _rep(pltpu.bitcast(tok, U32), n + 8)
                ke, ko = lo_hi(w[8:])
                ke1, ko1 = lo_hi(pltpu.roll(w, 1, 0)[8:])
                _, ko2 = lo_hi(pltpu.roll(w, 2, 0)[8:])
                s0, s1, s2, s3 = [_rep(sh_ref[a, :, ls], n) for a in range(4)]
                ve, vo = lo_hi(pltpu.bitcast(vb[r0:r0 + G, ls], U32))
                kve = ((ke * s0 + ko1 * s1) + (ke1 * s2 + ko2 * s3)) * ve
                kvo = ((ko * s0 + ke * s1) + (ko1 * s2 + ke1 * s3)) * vo
                kv_ref[r0 // 2:(r0 + G) // 2, ls] = pltpu.bitcast(
                    pltpu.pack_elementwise([kve, kvo], packed_dtype=BF16), U32)
            return run
        return [piece(ls, r0) for ls in lanes for r0 in range(0, TM, G)]

    def u_fwd(t):
        for b in range(2):
            for ls in lanes:
                kv = lambda: _unpk(kv_ref[b * HB:(b + 1) * HB, ls])
                a = bg.dot(fwd_ref[0:CB, :], kv())
                bb = bg.dot(fwd_ref[CB:2 * CB, :], kv())
                u_ref[t, b, 0:CB, ls] = a + bb
                u_ref[t, b, CB:2 * CB, ls] = a
                u_ref[t, b, 2 * CB:3 * CB, ls] = bb

    positions = [(slice(r0, r0 + 8), ls) for r0 in range(0, 3 * CB, 8) for ls in lanes]

    def ystatic_pieces(blocks, acc_in, pos=None):
        def piece(rs, ls):
            def run(tok):
                us, ks = {}, {}
                for s, lo, hi in blocks:
                    acc = None
                    for i in range(lo, min(hi, s + 1)):
                        if i not in us:
                            us[i] = _add(u_ref[i // 2, i % 2, rs, ls], tok)
                        if s - i not in ks:
                            ks[s - i] = kk_ref[s - i, rs, ls]
                        p = ks[s - i] * us[i]
                        acc = p if acc is None else acc + p
                    if acc_in:
                        acc = acc + y_ref[s // 2, s % 2, rs, ls]
                    y_ref[s // 2, s % 2, rs, ls] = acc
                return acc
            return run
        return [piece(*p) for p in (positions if pos is None else pos)]

    y_first = [(s, 0, 2 if s in (8, 9) else 4) for s in range(NB)]

    def mac_pieces(J, I, diag):
        kview = kk_ref if diag else kk_ref.at[pl.ds(2 * (J - I) - 3, 5)]
        uview = u_ref.at[pl.ds(I, 2)]

        def piece(rs, ls):
            def run(tok):
                one = _E('TK', 0)
                us = [_add(uview[a, b, rs, ls], None if one else tok) for a in range(2) for b in range(2)]
                ks = ([None] + [kview[i, rs, ls] for i in range(4)]) if diag else [kview[i, rs, ls] for i in range(5)]
                if one:
                    ks[2] = _add(ks[2], tok)
                    if one == 2:
                        ks[1], ks[3] = _add(ks[1], tok), _add(ks[3], tok)
                y0 = (ks[3] * us[0] + ks[2] * us[1]) + (ks[1] * us[2] + y_ref[J, 0, rs, ls])
                if not diag:
                    y0 = y0 + ks[0] * us[3]
                y1 = ((ks[4] * us[0] + ks[3] * us[1]) + (ks[2] * us[2] + ks[1] * us[3])) + y_ref[J, 1, rs, ls]
                y_ref[J, 0, rs, ls] = y0
                y_ref[J, 1, rs, ls] = y1
                return y1
            return run
        return [piece(*p) for p in positions]

    def post_pieces(t):
        def piece(b, r0, ls):
            def run(tok):
                comp = lambda c, off: y_ref[t, b, c * CB + off + r0:c * CB + off + r0 + 16, ls]
                k1l, k1h = _add(comp(0, 0), tok), _add(comp(0, HB), tok)
                rel, reh = k1l - comp(2, 0), k1h - comp(2, HB)
                iml, imh = k1l + comp(1, 0), k1h + comp(1, HB)
                p0 = b * CB + r0 // 2
                yb_ref[p0:p0 + 8, ls] = _pk(rel + reh)
                yb_ref[p0 + HB // 2:p0 + HB // 2 + 8, ls] = _pk(iml + imh)
                yb_ref[p0 + HB:p0 + HB + 8, ls] = _pk(rel - reh)
                oim = iml - imh
                yb_ref[p0 + HB + HB // 2:p0 + HB + HB // 2 + 8, ls] = _pk(oim)
                return oim[8:16]
            return run
        return [piece(b, r0, ls) for b in range(2) for r0 in range(0, HB, 16) for ls in lanes]

    def q_split(t, b, p0, n, ls):
        w = pltpu.bitcast(q_ref.at[rows_of(t)][b * CB + 2 * p0:b * CB + 2 * p0 + 2 * n, ls], U32)
        return lo_hi(w)

    def ln_tiles(xs, tok):
        n = xs[0].shape[0]
        s = _add(xs[0], tok)
        for x in xs[1:]:
            s = s + x
        m = jnp.sum(s, axis=-1, keepdims=True) * (1.0 / D)
        xc = [x - m for x in xs]
        s2 = xc[0] * xc[0]
        for x in xc[1:]:
            s2 = s2 + x * x
        r = lax.rsqrt(jnp.sum(s2, axis=-1, keepdims=True) * (1.0 / D) + EPS)
        return xc, jnp.broadcast_to(r, (n, 128)), jnp.broadcast_to(m, (n, 128))

    def ln1_pieces(t):
        G = _E('L1G', 8)

        def piece(b, p0):
            def run(tok):
                xc, r, _ = ln_tiles([cat(q_split(t, b, p0, G, ls), axis=0) for ls in lanes], tok)
                for ls, x in zip(lanes, xc):
                    h = (x * r) * _rep(mod_ref[0, :, ls], 2 * G) + _rep(mod_ref[1, :, ls], 2 * G)
                    hp_ref[b * CB + p0:b * CB + p0 + G, ls] = h[:G]
                    hp_ref[b * CB + HB + p0:b * CB + HB + p0 + G, ls] = h[G:]
                return functools.reduce(lambda a, c: a + c, [h[r:r + 8] for r in range(0, 2 * G, 8)])
            return run
        return [piece(b, p0) for b in range(2) for p0 in range(0, HB, G)]

    def y_inv(t, x1_dst):
        yb = opaque(yb_ref)
        hp = opaque(hp_ref)
        for b in range(2):
            ye = bg.dot(inv_ref[0:HB, :], _unpk(yb[b * CB:b * CB + HB, :]))
            yo = bg.dot(inv_ref[HB:CB, :], _unpk(yb[b * CB + HB:(b + 1) * CB, :]))
            for ls in lanes:
                qe, qo = q_split(t, b, 0, HB, ls)
                re, ro = slice(b * CB, b * CB + HB), slice(b * CB + HB, (b + 1) * CB)
                x1_dst[re, ls] = qe + hp[re, ls] * ye[:, ls]
                x1_dst[ro, ls] = qo + hp[ro, ls] * yo[:, ls]

    def ln2_stat_pieces(x1_src, st):
        x1o = opaque(x1_src)

        def piece(r0):
            def run(tok):
                _, r, m = ln_tiles([x1o[r0:r0 + 16, ls] for ls in lanes], tok)
                st[r0:r0 + 16, 0:128] = m
                st[r0:r0 + 16, 128:256] = r
                return r[0:8] + r[8:16]
            return run
        return [piece(h * CB + r0) for r0 in range(0, CB, 16) for h in range(2)]

    done = set()

    def ln2_apply_pieces(x1_src, st, unit, plain=False, link=False):
        G = 16
        x1o = opaque(x1_src)

        def piece(r0, js):
            def run(tok):
                two = lambda ref, c: cat([ref[r0:r0 + G, c], ref[CB + r0:CB + r0 + G, c]], axis=0)
                m, r = _add(two(st, slice(0, 128)), tok), two(st, slice(128, 256))
                hs = [((two(x1o, lanes[j]) - m) * r) * _rep(mod_ref[2, :, lanes[j]], 2 * G)
                      + _rep(mod_ref[3, :, lanes[j]], 2 * G) for j in js]
                if plain:
                    for j, h in zip(js, hs):
                        p0 = unit * CB + r0 // 2
                        h2_ref[p0:p0 + G // 2, lanes[j]] = _pk(h[:G])
                        h2_ref[p0 + HB:p0 + HB + G // 2, lanes[j]] = _pk(h[G:])
                else:
                    fs = (_a3 if len(js) == 3 else _a2)([h[:G] for h in hs], [h[G:] for h in hs])
                    for i, fm in enumerate(fs):
                        p0 = (i + (0 if len(js) == 3 else 15)) * HB + r0 // 2
                        hf_ref[p0:p0 + G // 2, lanes[unit]] = _pk(fm)
                if isinstance(unit, int):
                    done.add(('h2' if plain else 'hf', unit, r0, js[0]))

            return run
        return [piece(r0, js) for r0 in range(0, CB, G) for js in ([0, 1, 2], [3, 4])]

    def need(*key, rows=range(0, CB, 16)):
        for r0 in rows:
            assert key[:2] + (r0,) + key[2:] in done, key

    tile = lambda j: slice(j * 128, (j + 1) * 128)
    gu_refs = ((wg_ref, wga_ref, wgs_ref), (wu_ref, wua_ref, wus_ref))

    def w_pieces(w, n, g):
        G = 16

        def piece(r0):
            def run(tok):
                off = 0 if n == 3 else 3
                if w < 2:
                    ld = lambda k, j: gu_refs[w][0][(off + k) * 128 + r0:(off + k) * 128 + r0 + G, tile(n * g + j)]
                else:
                    ld = lambda k, j: wd_ref[(n * g + k) * 128 + r0:(n * g + k) * 128 + r0 + G, tile(off + j)]
                pin = (lambda k, j: k != j) if n == 3 else (lambda k, j: k == j)
                bb = [[_add(ld(k, j).astype(F32), tok if pin(k, j) else None) for j in range(n)] for k in range(n)]
                for i, fm in enumerate((_b3 if n == 3 else _b2)(bb)):
                    if w < 2:
                        gu_refs[w][1 if n == 3 else 2][i * HB + r0 // 2:i * HB + (r0 + G) // 2, tile(g)] = _pk(fm)
                    else:
                        p0 = (i * (NT // n) + g) * HB + r0 // 2
                        wdf_ref[p0:p0 + G // 2, tile(3 - n)] = _pk(fm)
                done.add(('w', w, r0, n, g))
            return run
        return [piece(r0) for r0 in range(0, CB, G)]

    def put_forms(unit, n, g, p0, x, y):
        rows = x[0].shape[0] // 2
        dst, nf = (ha_ref, 15) if n == 3 else (hs_ref, 7)
        for i, fm in enumerate((_a3 if n == 3 else _a2)(x, y)):
            dst[(unit * nf + i) * HB + p0:(unit * nf + i) * HB + p0 + rows, tile(g)] = _pk(fm)
        for r0 in range(2 * p0, 2 * (p0 + rows), 16):
            done.add(('hh', unit, r0, n, g))

    def gu_plain(j, unit):
        need('h2', unit, 0)
        need('h2', unit, 3)
        for h in range(2):
            x = lambda: _unpk(h2_ref[unit * CB + h * HB:unit * CB + (h + 1) * HB, :])
            p = bg.dot(x(), wg_ref[:, tile(j)]) * bg.dot(x(), wu_ref[:, tile(j)])
            pp_ref[unit * TM + h * CB:unit * TM + (h + 1) * CB, tile(j)] = p
        done.add(('pp', unit, j))

    def pp_pieces(unit, n, g, rows=range(0, CB, 16), chk=True):
        G = 16

        def piece(r0):
            def run(tok):
                assert not chk or all(('pp', unit, n * g + j) in done for j in range(n))
                ld = lambda h, j: _add((opaque(pp_ref) if chk or _E('PO', 0) else pp_ref)[unit * TM + h * CB + r0:unit * TM + h * CB + r0 + G,
                                                      tile(n * g + j)], tok)
                put_forms(unit, n, g, r0 // 2, [ld(0, j) for j in range(n)], [ld(1, j) for j in range(n)])
            return run
        return [piece(r0) for r0 in rows]

    def gu_fast(sc, unit, n, stage=False, src=None, mid=None):
        if src is None:
            need('hf', unit, 0)
            need('hf', unit, 3)
        subs = [(p0, min(n, HB - p0)) for p0 in range(0, HB, n)]
        cnt = [2 * sc * len(subs)]
        for p0, n in subs:
            if mid is not None and p0 > 0:
                mid()
            lhs = lambda i: _unpk(hf_ref[i * HB + p0:i * HB + p0 + n, lanes[unit]])

            def m3(w, g, p, q):
                need('w', w, 3, g)
                pad = (-cnt[0]) % 4 if _E('PAD', 1) else 0
                cnt[0] += 15
                return [_c3, _c3cse, _c3d][_E('CSE', 2)](lambda i: bg.dot(lhs(i), _unpk(gu_refs[w][1][i * HB:(i + 1) * HB, tile(g)])), p, q, pad)

            def m2(w, g):
                need('w', w, 2, g)
                cnt[0] += 7
                return _c2(lambda i: bg.dot(lhs(15 + i), _unpk(gu_refs[w][2][i * HB:(i + 1) * HB, tile(g)])))

            res, carry = [], []
            for w in range(2):
                c, b = m2(w, 3 * sc + 1), m2(w, 3 * sc)
                res.append(m3(w, 2 * sc, b[0] + c[0][:1], b[1] + c[1][:1]))
                carry.append([c[h][1] for h in range(2)])
            lo = [[g * u for g, u in zip(res[0][h], res[1][h])] for h in range(2)]
            rows = range(2 * p0, 2 * (p0 + n), 16)

            def staged(pr, j0, groups):
                for h in range(2):
                    for j, x in enumerate(pr[h]):
                        r = unit * TM + h * CB + 2 * p0
                        pp_ref[r:r + 2 * n, tile(j0 + j)] = x
                ps = [p for nn, g in groups for p in pp_pieces(unit, nn, g, rows, False)]
                bg.add(ps, bg.clock + _E('F0', 100), bg.clock + _E('F1', 700))

            if stage:
                staged(lo, 6 * sc, [(2, 3 * sc), (3, 2 * sc)])
            else:
                put_forms(unit, 2, 3 * sc, p0, lo[0][:2], lo[1][:2])
                put_forms(unit, 3, 2 * sc, p0, lo[0], lo[1])
            res = []
            for w in range(2):
                b = m2(w, 3 * sc + 2)
                res.append(m3(w, 2 * sc + 1, [carry[w][0]] + b[0], [carry[w][1]] + b[1]))
            hi = [[g * u for g, u in zip(res[0][h], res[1][h])] for h in range(2)]
            if stage and not (sc == NT // 6 - 1 and p0 + n == HB):
                staged(hi, 6 * sc + 3, [(2, 3 * sc + 1), (2, 3 * sc + 2), (3, 2 * sc + 1)])
            else:
                put_forms(unit, 2, 3 * sc + 1, p0, [lo[0][2], hi[0][0]], [lo[1][2], hi[1][0]])
                put_forms(unit, 2, 3 * sc + 2, p0, hi[0][1:], hi[1][1:])
                put_forms(unit, 3, 2 * sc + 1, p0, hi[0], hi[1])

    def ffn_down(x1_src, t, unit, mid=None, flip=False):
        ob = o_ref.at[rows_of(t)]

        def emit(dn, b, ls):
            o = x1_src[b * CB:(b + 1) * CB, ls] + _rep(mod_ref[4, :, ls], CB) * dn
            w = pltpu.pack_elementwise([o[:HB], o[HB:]], packed_dtype=BF16)
            ob[b * CB:(b + 1) * CB, ls] = pltpu.bitcast(w, BF16)

        parts = [(3, 15, ha_ref, [_c3, _c3cse, _c3d][_E('CSD', 0)], 0), (2, 7, hs_ref, _c2, 3)]
        for n, nf, h_ref, comb, off in (parts[::-1] if flip else parts):
            for g in range(NT // n):
                need('w', 2, n, g)
                need('hh', unit, n, g)
            kr = (NT // n) * HB
            if _E('OH', 0):
                h_ref = opaque(h_ref)
            def prod(i):
                base = (unit * nf + i) * HB
                w = lambda: _unpk(wdf_ref[i * kr:(i + 1) * kr, tile(3 - n)])
                if n == 2 and i == 3:
                    return cat([bg.dot(_unpk(h_ref[base + r:base + r + HB // 2, :]), w()) for r in (0, HB // 2)],
                               axis=0)
                return bg.dot(_unpk(h_ref[base:base + HB, :]), w())
            res = comb(prod)
            for j in range(n):
                for b in range(2):
                    emit(res[b][j], b, lanes[off + j])
            if n == (2 if flip else 3) and mid is not None:
                mid()

    x1s = [x1_ref.at[r] for r in range(NS)]
    sts = [st_ref.at[r * TM:(r + 1) * TM] for r in range(2)]
    YP = _E('YP', 12)

    def setup():
        for cp in small:
            cp.wait()
        shk = shk_ref[...].astype(F32)
        for a in range(4):
            sh_ref[a] = jnp.broadcast_to(shk[a:a + 1, :], (8, D))
        zm_ref[...] = pltpu.bitcast(inv_ref[CB:CB + 16, :], I32)
        zs.append(zm_ref[0, 0])

    def prologue():
        ytile = lambda i: ystatic_pieces(y_first, False, [p for p in positions if p[1] == lanes[i]])
        ssm_cp(0).wait()
        k_fwd(0)
        for t in range(2):
            k_cp(t).wait()
            v_cp(t).wait()
            now(kv_pieces(t, 64))
            u_fwd(t)
        bg.flush()
        for i in range(1, NL):
            if i != 3:
                ssm_cp(i).wait()
            if i == 2:
                ssm_cp(3).wait()
            bg.add(ytile(i - 1), 0, 1024)
            k_fwd(i)
            bg.flush()
        q_cp(0).wait()
        now(ytile(NL - 1))
        q_cp(1).wait()
        mod_cp(0).wait()
        mod_chunk(0)
        for t in range(2):
            now(post_pieces(t))
            now(ln1_pieces(t))
            y_inv(t, x1s[t])
        for t in range(2):
            now(ln2_stat_pieces(x1s[t], sts[t]))
        bg.flush()

    def superstep():
        wp = lambda n, g: w_pieces(0, n, g) + w_pieces(1, n, g)
        pp = lambda n, g: pp_pieces(0, n, g) + pp_pieces(1, n, g)
        mod_cp(1).wait()
        mod_chunk(1)
        now(ln2_apply_pieces(x1s[0], sts[0], 0, plain=True))
        bg.flush()
        g_cp(0).wait()
        u_cp(0).wait()
        bg.add(ln2_apply_pieces(x1s[1], sts[1], 1, plain=True), 0, 800)
        bg.add(ln2_apply_pieces(x1s[0], sts[0], 0) + ln2_apply_pieces(x1s[1], sts[1], 1) + wp(2, 0), 800, 2450)
        for u in range(2):
            gu_plain(0, u)
            gu_plain(1, u)
        bg.flush()
        k_cp(2).wait()
        v_cp(2).wait()
        g_cp(1).wait()
        u_cp(1).wait()
        bg.add(kv_pieces(2), 0, 1250)
        bg.add(wp(3, 0) + wp(2, 1) + pp(2, 0), 1250, 2450)
        for u in range(2):
            gu_plain(2, u)
            gu_plain(3, u)
        bg.flush()
        for f in range(2, 4):
            g_cp(f).wait()
            u_cp(f).wait()
        ymid = ystatic_pieces([(s, 4, 6) for s in (4, 5, 12, 13)], True)
        bg.add(wp(2, 3) + wp(3, 1) + wp(2, 2) + pp(3, 0) + pp(2, 1), 660, 2450)
        u_fwd(2)
        gu_plain(4, 0)
        gu_plain(5, 0)
        gu_plain(4, 1)
        bg.flush()
        for f in range(4, NF):
            g_cp(f).wait()
            u_cp(f).wait()
        q_cp(2).wait()
        bg.add(w_pieces(0, 2, 4) + w_pieces(0, 3, 2), 0, 500)
        bg.add(w_pieces(1, 2, 4) + w_pieces(1, 3, 2), 500, 1300)
        bg.add(w_pieces(0, 2, 5) + w_pieces(0, 3, 3) + w_pieces(1, 2, 5) + w_pieces(1, 3, 3), 1300, 2700)
        bg.add(linked(ln1_pieces(2), 3), 1000, 3500)
        gu_plain(5, 1)
        gu_fast(1, 0, HB)
        bg.flush()
        d_cp.wait()
        wdp = [p for g in range(NT // 3) for p in w_pieces(2, 3, g)]
        bg.add(pp(3, 1) + wdp, 0, 3100)
        bg.add(ymid[:_E('YM', 120)], 0, 3100)
        gu_fast(1, 1, HB // 2, True)
        bg.flush()
        mod_cp(2).wait()
        k_cp(3).wait()
        v_cp(3).wait()
        wdp = [p for g in range(NT // 2) for p in w_pieces(2, 2, g)]
        bg.add(ymid[_E('YM', 120):] + post_pieces(2), 0, 1600)
        bg.add(wdp + pp(2, 2), 0, 1900)
        bg.add(kv_pieces(3), 2300, 3450)
        bg.add(ln2_stat_pieces(x1s[2], st_ref), 2300, 3100)
        bg.inj = [(100 + 200 * i, gb_tile(i)) for i in range(NL)]
        ffn_down(x1s[0], 0, 0, mid=lambda: y_inv(2, x1s[2]))
        bg.flush()
        o_cp(0).start()

    def run_super(fn):
        if _E('SL', 1):
            def body(i, carry):
                fn()
                return carry
            lax.fori_loop(0, zs[0] + 1, body, 0)
        else:
            fn()

    def step(t, carry):
        q_cp(t).wait()

        @pl.when(t + 1 < NS)
        def _():
            k_cp(t + 1).wait()
            v_cp(t + 1).wait()

        x1v = x1_ref.at[pl.ds(t - 2, 3)]
        x1 = x1v.at[2]
        iv = _E('IV', 2)
        t1 = 640 + 3264 + iv * 1632 + 320
        end = 10752
        bg.add(linked(ln1_pieces(t), _E('LK1', 2)), _E('L0', 3400), t1 - _E('L1', 800))
        bg.add(linked(ln2_stat_pieces(x1, st_ref), _E('LK2', 3)), t1 + _E('S0', 100), t1 + _E('S1', 2600))
        la = _E('LKA', 0)
        bg.add(linked(ln2_apply_pieces(x1v.at[1], st_ref, 1, link=bool(la)), la), _E('P0', 700), _E('P1', 3300))
        bg.add(kv_pieces(jnp.minimum(t + 1, NS - 1), 16), t1 + _E('K0', 100), t1 + _E('K1', 2900))
        u_fwd(t)
        J = jnp.minimum(t + 1, NS - 1)
        I = jnp.where(t == NS - 2, 2, jnp.minimum(t - 2, 4))
        chain(mac_pieces(t, t - 1, True), _E('DD', 2), _E('DE', 0))
        dep = chain(mac_pieces(J, I, False), _E('MD', 2), _E('ME', 0))
        chain(post_pieces(t), 1, 3, dep)
        ffn_down(x1v.at[0], t - 2, 1)
        if _E('OMID', 0):
            o_cp(t - 2).start()
        inv = lambda: y_inv(t, x1)
        stg = bool(_E('STG', 1))
        gu_fast(0, 1, HB // 2, stg, None, inv if iv == 1 else None)
        if iv == 2:
            inv()
        gu_fast(1, 1, HB // 2, stg, None, inv if iv == 3 else None)
        bg.flush()
        if not _E('OMID', 0):
            o_cp(t - 2).start()
        return carry

    def epilogue():
        t = NS - 1
        bg.add(ln2_apply_pieces(x1s[t], st_ref, 1), 100, 2700)
        ffn_down(x1s[t - 1], t - 1, 1)
        o_cp(t - 1).start()
        for sc6 in range(NT // 6):
            gu_fast(sc6, 1, HB // 2, True)
        last = [pltpu.make_async_copy(o_ref.at[rows_of(t), lo:hi], o_hbm.at[rows_of(t), lo:hi], sem.at[s_o + t + i])
                for i, (lo, hi) in enumerate([(0, 384), (384, D)])]
        ffn_down(x1s[t], t, 1, mid=last[0].start)
        last[1].start()
        for i in range(NS - 1):
            o_cp(i).wait()
        for cp in last:
            cp.wait()

    sc = jax.named_scope if SCOPES else (lambda name: (lambda f: f))

    def rest():
        sc("superstep")(superstep)()
        lax.fori_loop(T0, NS, sc("step")(step), 0)
        sc("epilogue")(epilogue)()

    if ONLY == 'loop':
        need = lambda *a, **k: None
        zs.append(zm_ref[0, 0])
        lax.fori_loop(T0, NS, step, 0)
        epilogue()
    elif ONLY == 'S':
        zs.append(zm_ref[0, 0])
        run_super(superstep)
        lax.fori_loop(T0, NS, step, 0)
    elif _E('NEST', 3) == 3:
        setup()

        def everything():
            sc("prologue")(prologue)()
            rest()
        run_super(everything)
    else:
        setup()
        sc("prologue")(prologue)()
        run_super(rest)


@jax.jit
def pallas_adaLN_cond__ssm_conv_h3__glu_gated_bilinear__prompt_kernel(
    A_q, A_k, A_v, A_shift_k, A_ssm_k, A_ssm_D, B_x, B_w_gate, B_w_up, B_w_down, c, w_mod,
):
    B, S, D = A_q.shape
    Fh = B_w_gate.shape[1]
    NB = S // CB
    NS = S // TM
    fwd, inv = _dft_consts()
    anyspec = pl.BlockSpec(memory_space=pl.ANY)
    V = pltpu.VMEM
    out = pl.pallas_call(
        functools.partial(_kernel, S=S, D=D, Fh=Fh),
        in_specs=[anyspec] * 13,
        out_specs=anyspec,
        out_shape=jax.ShapeDtypeStruct((S, D), A_q.dtype),
        scratch_shapes=[
            V((NS, 2, 3 * CB, D), F32),
            V((NB, 3 * CB, D), F32),
            V((NS, 2, 3 * CB, D), F32),
            V((NS, TM, D), F32),
            V((S, D), BF16), V((S, D), BF16), V((S, D), BF16), V((S, D), BF16),
            V((TM, D), F32),
            V((2 * TM, 256), F32),
            V((2 * TM, Fh), F32),
            V((2 * CB, D), U32),
            V((22 * HB, 256), U32),
            V((2 * 15 * HB, Fh // 3), U32),
            V((2 * 7 * HB, Fh // 2), U32),
            V((TM // 2, D), U32),
            V((2 * CB, D), U32),
            V((15 * HB, Fh // 3), U32), V((15 * HB, Fh // 3), U32), V((15 * Fh // 6, 256), U32),
            V((7 * HB, Fh // 2), U32), V((7 * HB, Fh // 2), U32),
            V((D, S), BF16), V((D, 6 * D), BF16), V((D, Fh), BF16), V((D, Fh), BF16), V((Fh, D), BF16),
            V((2 * CB, CB), BF16), V((CB + 16, CB), BF16),
            V((5, 8, D), F32), V((4, 8, D), F32), V((8, 128), I32),
            V((4, D), BF16), V((D,), BF16), V((1, D), BF16),
            pltpu.SemaphoreType.DMA((5 + 4 * NS + D // 128 + 3 + 2 * (Fh // FC) + 2,)),
        ],
        compiler_params=pltpu.CompilerParams(
            internal_scratch_in_bytes=48 * 1024,
            disable_semaphore_checks=True,
            disable_bounds_checks=True,
            vmem_limit_bytes=110 * 1024 * 1024),
        name="adaln_h3_glu",
    )(A_q.reshape(S, D), A_k.reshape(S, D), A_v.reshape(S, D), A_shift_k.T, A_ssm_k,
      A_ssm_D, B_w_gate, B_w_up, B_w_down, c, w_mod, fwd, inv)
    return out.reshape(B, S, D)
```

```python
import functools
import os

import numpy as np
import jax
import jax.numpy as jnp
from jax import lax
import jax.experimental.pallas as pl
import jax.experimental.pallas.tpu as pltpu

F32 = jnp.float32
BF16 = jnp.bfloat16
U32 = jnp.uint32
I32 = jnp.int32

CB = 128
HB = CB // 2
TM = 256
FC = 256
KS = 256
EPS = 1e-5
SCOPES = False
ONLY = os.environ.get('ONLY', '')


def _E(name, default):
    return int(os.environ.get(name, default))


def _dft_consts():
    k = np.arange(CB, dtype=np.float64)[:, None]
    n = np.arange(CB, dtype=np.float64)[None, :]
    th = np.pi * (4.0 * k + 1.0) * n / (2.0 * CB)
    fwd = np.concatenate([np.cos(th), np.sin(th)], axis=0)
    g = np.concatenate([np.cos(th[:HB]), np.sin(th[:HB])], axis=0).T / CB
    inv = np.concatenate([g[0::2], g[1::2], np.zeros((16, CB))], axis=0)
    return jnp.asarray(fwd, dtype=BF16), jnp.asarray(inv, dtype=BF16)


def _pk(x):
    return pltpu.bitcast(x.astype(BF16), U32)


def _unpk(x):
    return pltpu.bitcast(x, BF16)


def _rep(r, n):
    return r if n == 8 else jnp.concatenate([r] * (n // 8), axis=0)


def _add(x, tok):
    return x if tok is None else x + _rep(tok, x.shape[0])


def _costed(pieces, cost):
    for p in pieces:
        p.cost = cost
    return pieces


def _group(pieces, n):
    def merged(ps):
        def run(tok):
            for p in ps:
                p(tok)
        return run
    return [merged(pieces[i:i + n]) for i in range(0, len(pieces), n)]


def _a2(x, y):
    return [x[0] + y[1], y[0] + y[1], x[0] + x[1], y[0] - x[0], x[1] - y[1], x[0], y[1]]


def _b2(b):
    return [b[0][0] + b[1][1], b[0][0], b[1][1], b[0][0] + b[0][1], b[1][0] + b[1][1],
            b[0][1] - b[1][1], b[1][0] - b[0][0]]


def _c2(m):
    m1, m7, m4, m2 = m(0), m(4), m(6), m(1)
    q0 = m2 + m4
    m5 = m(2)
    p0 = m1 + m7 + m4 - m5
    m3 = m(5)
    p1 = m3 + m5
    q1 = m1 - m2 + m3 + m(3)
    return [p0, p1], [q0, q1]


def _a3(x, y):
    w = [a + b for a, b in zip(x, y)]
    return [x[0], y[0], x[1], w[1], y[2], w[2], x[1] + y[2], x[2] - x[1], y[1] - y[2],
            w[1] - y[0], y[0] - y[1], w[0] - w[1], w[2] - x[0], x[0] - x[2], w[0] - w[2]]


def _b3(b):
    return [b[0][0] - b[0][1] + b[2][0], b[0][0] - b[0][2] + b[1][0], b[1][1] - b[1][0] + b[2][1],
            b[0][1] + b[1][1] - b[1][2], b[1][2] - b[2][0] + b[2][2], b[0][2] - b[2][1] + b[2][2],
            b[1][2] + b[2][1], b[2][1], b[1][2], b[0][1] + b[1][0], b[1][0], b[0][1],
            b[0][2] + b[2][0], b[2][0], b[0][2]]


_C3 = [(7, "+p1 +p2"), (8, "+q1 +q2"), (6, "+q1 +p2"), (14, "+q0 +q2"), (11, "+p0 +p1"), (5, "+p2"),
       (4, "-p2 +q2"), (12, "+q0 -p2 +q2"), (13, "-p0 +q0 -p2 +q2"), (3, "+q1"), (2, "+p1 -q1"),
       (9, "+p0 +p1 -q1"), (10, "+p0 -q0 +p1 -q1"), (1, "+q0"), (0, "+p0")]


def _c3(m, p=None, q=None, pad=0):
    v = {"p": [None] * 3 if p is None else list(p), "q": [None] * 3 if q is None else list(q)}
    for i, terms in _C3:
        x = m(i)
        for sg, h, n in terms.split():
            cur = v[h][int(n)]
            v[h][int(n)] = x if cur is None else (cur + x if sg == "+" else cur - x)
    return v["p"], v["q"]


def _c3cse(m, p=None, q=None, pad=0):
    p = [None] * 3 if p is None else list(p)
    q = [None] * 3 if q is None else list(q)

    def acc(v, n, x, neg=False):
        v[n] = (-x if neg else x) if v[n] is None else (v[n] - x if neg else v[n] + x)

    singles = [(5, p, 2), (3, q, 1), (1, q, 0), (0, p, 0)]
    for i, v, n in singles[:pad]:
        acc(v, n, m(i))
    m6, m7, m8 = m(6), m(7), m(8)
    if pad < 4:
        i, v, n = singles[pad]
        acc(v, n, m(i))
    acc(p, 1, m7), acc(q, 2, m8), acc(q, 1, m6 + m8), acc(p, 2, m6 + m7)
    m12, m13, m4, m14 = m(12), m(13), m(4), m(14)
    s2 = m12 + m13
    t2 = m4 + s2
    acc(q, 2, t2 + m14), acc(q, 0, s2 + m14), acc(p, 2, t2, True)
    m9, m10, m2, m11 = m(9), m(10), m(2), m(11)
    s1 = m9 + m10
    t1 = m2 + s1
    if p[0] is None:
        p[0] = (s1 + m11) - m13
    else:
        p[0] = (p[0] - m13) + (s1 + m11)
    acc(p, 1, t1 + m11), acc(q, 1, t1, True), acc(q, 0, m10, True)
    for i, v, n in singles[pad + 1:]:
        acc(v, n, m(i))
    return p, q


def _c3d(m, p=None, q=None, pad=0):
    p = [None] * 3 if p is None else list(p)
    q = [None] * 3 if q is None else list(q)

    def acc(v, n, x, neg=False):
        v[n] = x if v[n] is None else (v[n] - x if neg else v[n] + x)

    for i, a, b in ((7, (p, 1), (p, 2)), (8, (q, 1), (q, 2)), (6, (q, 1), (p, 2)), (14, (q, 0), (q, 2)),
                    (11, (p, 0), (p, 1))):
        x = m(i)
        acc(*a, x), acc(*b, x)
    m13 = m(13)
    m12 = m(12)
    acc(q, 0, m12)
    d2 = (m13 + m12) + m(4)
    acc(q, 2, d2), acc(p, 2, d2, True)
    acc(p, 2, m(5))
    m10 = m(10)
    d0 = m10 - m13
    acc(p, 0, d0), acc(q, 0, d0, True)
    m9 = m(9)
    acc(p, 0, m9)
    d1 = (m10 + m9) + m(2)
    acc(p, 1, d1), acc(q, 1, d1, True)
    acc(q, 1, m(3)), acc(q, 0, m(1)), acc(p, 0, m(0))
    return p, q


class _Sched:
    def __init__(self, token):
        self.token = token
        self.clock = 0.0
        self.q = []
        self.last = None
        self.inj = []

    def add(self, pieces, t0, t1):
        cum = np.cumsum([0.0] + [getattr(p, "cost", 1.0) for p in pieces])
        self.q += [(t0 + (t1 - t0) * cum[i] / cum[-1], i, p) for i, p in enumerate(pieces)]
        self.q.sort(key=lambda e: e[:2])

    def note(self, m, dt):
        rows, cols = m.shape
        tiles = [(slice(r, r + 8), slice(c, c + 128)) for c in range(0, cols, 128) for r in range(0, rows, 8)]
        for i, tl in enumerate(tiles):
            tok = None
            while self.q and self.q[0][0] <= self.clock + dt * (i + 1) / len(tiles):
                if tok is None:
                    tok = self.token(m[tl])
                self.q.pop(0)[2](tok)
        self.clock += dt
        self.last = m[tiles[-1]]
        return m

    def dot(self, a, b):
        if self.inj and self.clock >= self.inj[0][0]:
            self.inj.pop(0)[1]()
        m = jnp.dot(a, b, preferred_element_type=F32)
        return self.note(m, max(a.shape[0], 32) * (a.shape[1] // 128) * (b.shape[1] // 128) / 4)

    def flush(self):
        tok = None if self.last is None or not self.q else self.token(self.last)
        while self.q:
            self.q.pop(0)[2](tok)
        self.clock = 0.0
        self.last = None


def _kernel(q_hbm, k_hbm, v_hbm, shk_hbm, ssmk_hbm, ssmd_hbm, wg_hbm, wu_hbm, wd_hbm,
            c_hbm, wmod_hbm, fwd_hbm, inv_hbm, o_hbm,
            u_ref, kk_ref, y_ref, x1_ref, q_ref, k_ref, v_ref, o_ref,
            hp_ref, st_ref, pp_ref, h2_ref, hf_ref, ha_ref, hs_ref, kv_ref, yb_ref,
            wga_ref, wua_ref, wdf_ref, wgs_ref, wus_ref,
            ssmk_ref, wmod_ref, wg_ref, wu_ref, wd_ref, fwd_ref, inv_ref,
            mod_ref, sh_ref, zm_ref, shk_ref, ssmd_ref, c_ref,
            sem, *, S, D, Fh):
    NB = S // CB
    NS = S // TM
    NL = D // 128
    NF = Fh // FC
    NT = Fh // 128
    T0 = 3
    NLOOP = NS - T0
    lanes = [slice(i * 128, (i + 1) * 128) for i in range(NL)]
    cat = jnp.concatenate

    offs = [int(o) for o in np.cumsum([0, 5, NS, NS, NS, NL, 3, NF, NF, 1])]
    s_small, s_q, s_k, s_v, s_ssm, s_mod, s_g, s_u, s_d, s_o = offs

    def rows_of(t):
        return pl.ds(t * TM if isinstance(t, int) else pl.multiple_of(t * TM, TM), TM)

    def rows_cp(src, dst, base, t):
        return pltpu.make_async_copy(src.at[rows_of(t), :], dst.at[rows_of(t), :], sem.at[base + t])

    def cols_cp(src, dst, lo, hi, si):
        return pltpu.make_async_copy(src.at[:, lo:hi], dst.at[:, lo:hi], sem.at[si])

    q_cp = lambda t: rows_cp(q_hbm, q_ref, s_q, t)
    k_cp = lambda t: rows_cp(k_hbm, k_ref, s_k, t)
    v_cp = lambda t: rows_cp(v_hbm, v_ref, s_v, t)
    o_cp = lambda t: rows_cp(o_ref, o_hbm, s_o, t)
    small = [pltpu.make_async_copy(s, d, sem.at[s_small + i]) for i, (s, d) in enumerate(
        [(fwd_hbm, fwd_ref), (shk_hbm, shk_ref), (ssmd_hbm, ssmd_ref), (inv_hbm, inv_ref), (c_hbm, c_ref)])]
    ssm_cp = lambda i: pltpu.make_async_copy(ssmk_hbm.at[lanes[i], :], ssmk_ref.at[lanes[i], :],
                                             sem.at[s_ssm + i])
    mod_cols = [(0, 3 * D), (3 * D, 5 * D), (5 * D, 6 * D)]
    mod_cp = lambda i: cols_cp(wmod_hbm, wmod_ref, mod_cols[i][0], mod_cols[i][1], s_mod + i)
    g_cp = lambda f: cols_cp(wg_hbm, wg_ref, f * FC, (f + 1) * FC, s_g + f)
    u_cp = lambda f: cols_cp(wu_hbm, wu_ref, f * FC, (f + 1) * FC, s_u + f)
    d_cp = pltpu.make_async_copy(wd_hbm, wd_ref, sem.at[s_d])

    order = small + [ssm_cp(0), k_cp(0), v_cp(0), k_cp(1), v_cp(1),
                     ssm_cp(1), ssm_cp(2), ssm_cp(3), ssm_cp(4), q_cp(0), q_cp(1),
                     mod_cp(0), mod_cp(1), g_cp(0), u_cp(0), k_cp(2), v_cp(2)]
    for f in range(1, NF):
        order += [g_cp(f), u_cp(f)]
    order += [q_cp(2), d_cp, mod_cp(2), k_cp(3), v_cp(3)]
    for t in range(T0, NS):
        order += [q_cp(t)]
        if t + 1 < NS:
            order += [k_cp(t + 1), v_cp(t + 1)]
    for cp in order:
        cp.start()

    zs = []
    bg = _Sched(lambda x: pltpu.bitcast(pltpu.bitcast(x, I32) & zm_ref[...], F32))

    def opaque(ref):
        return ref.at[pl.ds(pl.multiple_of(zs[0], 32), ref.shape[0])]

    def chain(pieces, dist, extra=0, dep=None):
        hist = [] if dep is None else [dep] * dist
        for p in pieces:
            tok = None
            if len(hist) >= dist:
                tok = bg.token(hist[-dist])
                for _ in range(extra):
                    tok = tok + tok
            hist.append(p(tok))
        return hist[-1]

    def linked(pieces, d):
        res = []

        def wrap(p):
            def run(tok):
                if d and len(res) >= d:
                    tok = tok + bg.token(res[-d])
                res.append(p(tok))
            return run
        return [wrap(p) for p in pieces]

    def now(pieces):
        for p in pieces:
            p(None)

    def mod_chunk(i):
        c = c_ref[...].astype(F32)
        sc = jnp.broadcast_to((c * jax.nn.sigmoid(c)).astype(BF16), (16, D))
        lo, hi = mod_cols[i]
        m = bg.dot(sc, wmod_ref[:, lo:hi])[0:8]
        if i == 0:
            ga = m[:, 2 * D:3 * D]
            mod_ref[0] = (1.0 + m[:, D:2 * D]) * ga
            mod_ref[1] = m[:, 0:D] * ga
        elif i == 1:
            mod_ref[2] = 1.0 + m[:, D:2 * D]
            mod_ref[3] = m[:, 0:D]
        else:
            mod_ref[4] = m

    def gb_tile(i):
        def run():
            c = c_ref[...].astype(F32)
            sc = jnp.broadcast_to((c * jax.nn.sigmoid(c)).astype(BF16), (16, D))
            w = wmod_ref[:, 5 * D + i * 128:5 * D + (i + 1) * 128]
            mod_ref[4, :, lanes[i]] = jnp.dot(sc, w, preferred_element_type=F32)[0:8]
        return run

    def k_fwd(i):
        ls = lanes[i]
        fwd = fwd_ref[...]
        prev = None
        for m in range(NB):
            kf = lax.dot_general(fwd, ssmk_ref[ls, m * CB:(m + 1) * CB], (((1,), (1,)), ((), ())),
                                 preferred_element_type=F32)
            if m == 0:
                c = kf[:CB] + ssmd_ref[...].astype(F32).reshape(1, D)[:, ls]
                d = kf[CB:]
            else:
                c = kf[:CB] + prev[CB:]
                d = kf[CB:] - prev[:CB]
            prev = kf
            kk_ref[m, 0:CB, ls] = c
            kk_ref[m, CB:2 * CB, ls] = d - c
            kk_ref[m, 2 * CB:3 * CB, ls] = c + d
            if m % 4 == 3:
                bg.note(kf, 2 * CB)

    def lo_hi(w):
        return pltpu.bitcast(w << 16, F32), pltpu.bitcast(w & jnp.uint32(0xFFFF0000), F32)

    def kv_pieces(t, G=32):
        n = G // 2
        kb, vb = k_ref.at[rows_of(t)], v_ref.at[rows_of(t)]

        def piece(ls, r0):
            def run(tok):
                if r0 > 0:
                    w = pltpu.bitcast(kb[r0 - 16:r0 + G, ls], U32)
                else:
                    if isinstance(t, int) and t == 0:
                        halo = jnp.zeros((8, 128), U32)
                    else:
                        halo = pltpu.bitcast(k_ref.at[rows_of(t - 1)][TM - 16:TM, ls], U32)
                    w = cat([halo, pltpu.bitcast(kb[0:G, ls], U32)], axis=0)
                if tok is not None:
                    w = w | _rep(pltpu.bitcast(tok, U32), n + 8)
                ke, ko = lo_hi(w[8:])
                ke1, ko1 = lo_hi(pltpu.roll(w, 1, 0)[8:])
                _, ko2 = lo_hi(pltpu.roll(w, 2, 0)[8:])
                s0, s1, s2, s3 = [_rep(sh_ref[a, :, ls], n) for a in range(4)]
                ve, vo = lo_hi(pltpu.bitcast(vb[r0:r0 + G, ls], U32))
                kve = ((ke * s0 + ko1 * s1) + (ke1 * s2 + ko2 * s3)) * ve
                kvo = ((ko * s0 + ke * s1) + (ko1 * s2 + ke1 * s3)) * vo
                kv_ref[r0 // 2:(r0 + G) // 2, ls] = pltpu.bitcast(
                    pltpu.pack_elementwise([kve, kvo], packed_dtype=BF16), U32)
            return run
        return _costed([piece(ls, r0) for ls in lanes for r0 in range(0, TM, G)], 2.5 * G + 10)

    def u_fwd(t):
        for b in range(2):
            for ls in lanes:
                kv = lambda: _unpk(kv_ref[b * HB:(b + 1) * HB, ls])
                a = bg.dot(fwd_ref[0:CB, :], kv())
                bb = bg.dot(fwd_ref[CB:2 * CB, :], kv())
                u_ref[t, b, 0:CB, ls] = a + bb
                u_ref[t, b, CB:2 * CB, ls] = a
                u_ref[t, b, 2 * CB:3 * CB, ls] = bb

    positions = [(slice(r0, r0 + 8), ls) for r0 in range(0, 3 * CB, 8) for ls in lanes]

    def ystatic_pieces(blocks, acc_in, pos=None):
        def piece(rs, ls):
            def run(tok):
                us, ks = {}, {}
                for s, lo, hi in blocks:
                    acc = None
                    for i in range(lo, min(hi, s + 1)):
                        if i not in us:
                            us[i] = _add(u_ref[i // 2, i % 2, rs, ls], tok)
                        if s - i not in ks:
                            ks[s - i] = kk_ref[s - i, rs, ls]
                        p = ks[s - i] * us[i]
                        acc = p if acc is None else acc + p
                    if acc_in:
                        acc = acc + y_ref[s // 2, s % 2, rs, ls]
                    y_ref[s // 2, s % 2, rs, ls] = acc
                return acc
            return run
        return _costed([piece(*p) for p in (positions if pos is None else pos)], 35)

    y_first = [(s, 0, 4) for s in range(NB)]

    def task_pieces(t, delta):
        p = t - delta
        left = p >= T0
        J = jnp.where(left, t, p + NLOOP)
        I = jnp.where(left, p, t)
        kview = kk_ref.at[pl.ds(2 * (J - I) - 1, 3)]

        def piece(rs, ls):
            def run(tok):
                u0 = _add(u_ref[I, 0, rs, ls], tok)
                u1 = _add(u_ref[I, 1, rs, ls], tok)
                kc = kview[1, rs, ls]
                y_ref[J, 0, rs, ls] = (kc * u0 + kview[0, rs, ls] * u1) + y_ref[J, 0, rs, ls]
                y1 = (kview[2, rs, ls] * u0 + kc * u1) + y_ref[J, 1, rs, ls]
                y_ref[J, 1, rs, ls] = y1
                return y1
            return run
        return [piece(*p) for p in positions]

    def diag_pieces(t, I):
        kview = kk_ref.at[pl.ds(2 * (t - I) - 1, 3)]

        def piece(rs, ls):
            def run(tok):
                us = [_add(u_ref[a, b, rs, ls], tok) for a in (t, I) for b in range(2)]
                k0 = kk_ref[0, rs, ls]
                kc = kview[1, rs, ls]
                y_ref[t, 0, rs, ls] = ((k0 * us[0] + y_ref[t, 0, rs, ls])
                                       + (kc * us[2] + kview[0, rs, ls] * us[3]))
                y1 = ((kk_ref[1, rs, ls] * us[0] + k0 * us[1])
                      + (kview[2, rs, ls] * us[2] + kc * us[3]) + y_ref[t, 1, rs, ls])
                y_ref[t, 1, rs, ls] = y1
                return y1
            return run
        return [piece(*p) for p in positions]

    def mac_pieces(J, I, diag):
        kview = kk_ref if diag else kk_ref.at[pl.ds(2 * (J - I) - 3, 5)]
        uview = u_ref.at[pl.ds(I, 2)]

        def piece(rs, ls):
            def run(tok):
                one = _E('TK', 0)
                us = [_add(uview[a, b, rs, ls], None if one else tok) for a in range(2) for b in range(2)]
                ks = ([None] + [kview[i, rs, ls] for i in range(4)]) if diag else [kview[i, rs, ls] for i in range(5)]
                if one:
                    ks[2] = _add(ks[2], tok)
                    if one == 2:
                        ks[1], ks[3] = _add(ks[1], tok), _add(ks[3], tok)
                y0 = (ks[3] * us[0] + ks[2] * us[1]) + (ks[1] * us[2] + y_ref[J, 0, rs, ls])
                if not diag:
                    y0 = y0 + ks[0] * us[3]
                y1 = ((ks[4] * us[0] + ks[3] * us[1]) + (ks[2] * us[2] + ks[1] * us[3])) + y_ref[J, 1, rs, ls]
                y_ref[J, 0, rs, ls] = y0
                y_ref[J, 1, rs, ls] = y1
                return y1
            return run
        return [piece(*p) for p in positions]

    def post_pieces(t):
        def piece(b, r0, ls):
            def run(tok):
                comp = lambda c, off: y_ref[t, b, c * CB + off + r0:c * CB + off + r0 + 16, ls]
                k1l, k1h = _add(comp(0, 0), tok), _add(comp(0, HB), tok)
                rel, reh = k1l - comp(2, 0), k1h - comp(2, HB)
                iml, imh = k1l + comp(1, 0), k1h + comp(1, HB)
                p0 = b * CB + r0 // 2
                yb_ref[p0:p0 + 8, ls] = _pk(rel + reh)
                yb_ref[p0 + HB // 2:p0 + HB // 2 + 8, ls] = _pk(iml + imh)
                yb_ref[p0 + HB:p0 + HB + 8, ls] = _pk(rel - reh)
                oim = iml - imh
                yb_ref[p0 + HB + HB // 2:p0 + HB + HB // 2 + 8, ls] = _pk(oim)
                return oim[8:16]
            return run
        return _costed([piece(b, r0, ls) for b in range(2) for r0 in range(0, HB, 16) for ls in lanes], 45)

    def q_split(t, b, p0, n, ls):
        w = pltpu.bitcast(q_ref.at[rows_of(t)][b * CB + 2 * p0:b * CB + 2 * p0 + 2 * n, ls], U32)
        return lo_hi(w)

    def ln_tiles(xs, tok):
        n = xs[0].shape[0]
        s = _add(xs[0], tok)
        for x in xs[1:]:
            s = s + x
        m = jnp.sum(s, axis=-1, keepdims=True) * (1.0 / D)
        xc = [x - m for x in xs]
        s2 = xc[0] * xc[0]
        for x in xc[1:]:
            s2 = s2 + x * x
        r = lax.rsqrt(jnp.sum(s2, axis=-1, keepdims=True) * (1.0 / D) + EPS)
        return xc, jnp.broadcast_to(r, (n, 128)), jnp.broadcast_to(m, (n, 128))

    def ln1_pieces(t):
        G = _E('L1G', 8)

        def piece(b, p0):
            def run(tok):
                xc, r, _ = ln_tiles([cat(q_split(t, b, p0, G, ls), axis=0) for ls in lanes], tok)
                for ls, x in zip(lanes, xc):
                    h = (x * r) * _rep(mod_ref[0, :, ls], 2 * G) + _rep(mod_ref[1, :, ls], 2 * G)
                    hp_ref[b * CB + p0:b * CB + p0 + G, ls] = h[:G]
                    hp_ref[b * CB + HB + p0:b * CB + HB + p0 + G, ls] = h[G:]
                return functools.reduce(lambda a, c: a + c, [h[r:r + 8] for r in range(0, 2 * G, 8)])
            return run
        return [piece(b, p0) for b in range(2) for p0 in range(0, HB, G)]

    def y_inv(t, x1_dst):
        yb = opaque(yb_ref)
        hp = opaque(hp_ref)
        for b in range(2):
            ye = bg.dot(inv_ref[0:HB, :], _unpk(yb[b * CB:b * CB + HB, :]))
            yo = bg.dot(inv_ref[HB:CB, :], _unpk(yb[b * CB + HB:(b + 1) * CB, :]))
            for ls in lanes:
                qe, qo = q_split(t, b, 0, HB, ls)
                re, ro = slice(b * CB, b * CB + HB), slice(b * CB + HB, (b + 1) * CB)
                x1_dst[re, ls] = qe + hp[re, ls] * ye[:, ls]
                x1_dst[ro, ls] = qo + hp[ro, ls] * yo[:, ls]

    def ln2_stat_pieces(x1_src, st):
        x1o = opaque(x1_src)

        def piece(r0):
            def run(tok):
                _, r, m = ln_tiles([x1o[r0:r0 + 16, ls] for ls in lanes], tok)
                st[r0:r0 + 16, 0:128] = m
                st[r0:r0 + 16, 128:256] = r
                return r[0:8] + r[8:16]
            return run
        return [piece(h * CB + r0) for r0 in range(0, CB, 16) for h in range(2)]

    done = set()

    def ln2_apply_pieces(x1_src, st, unit, plain=False, forms=True, link=False):
        G = 16
        x1o = opaque(x1_src)

        def piece(r0, js):
            def run(tok):
                two = lambda ref, c: cat([ref[r0:r0 + G, c], ref[CB + r0:CB + r0 + G, c]], axis=0)
                m, r = _add(two(st, slice(0, 128)), tok), two(st, slice(128, 256))
                hs = [((two(x1o, lanes[j]) - m) * r) * _rep(mod_ref[2, :, lanes[j]], 2 * G)
                      + _rep(mod_ref[3, :, lanes[j]], 2 * G) for j in js]
                if plain:
                    for j, h in zip(js, hs):
                        p0 = unit * CB + r0 // 2
                        h2_ref[p0:p0 + G // 2, lanes[j]] = _pk(h[:G])
                        h2_ref[p0 + HB:p0 + HB + G // 2, lanes[j]] = _pk(h[G:])
                    done.add(('h2', unit, r0, js[0]))
                if forms:
                    fs = (_a3 if len(js) == 3 else _a2)([h[:G] for h in hs], [h[G:] for h in hs])
                    for i, fm in enumerate(fs):
                        p0 = (i + (0 if len(js) == 3 else 15)) * HB + r0 // 2
                        hf_ref[p0:p0 + G // 2, lanes[unit]] = _pk(fm)
                    done.add(('hf', unit, r0, js[0]))

            return run
        return [_costed([piece(r0, js)], (30 if plain else 42) * len(js))[0]
                for r0 in range(0, CB, G) for js in ([0, 1, 2], [3, 4])]

    def need(*key, rows=range(0, CB, 16)):
        for r0 in rows:
            assert key[:2] + (r0,) + key[2:] in done, key

    tile = lambda j: slice(j * 128, (j + 1) * 128)
    gu_refs = ((wg_ref, wga_ref, wgs_ref), (wu_ref, wua_ref, wus_ref))

    def w_pieces(w, n, g, split=False):
        G = 16

        off = 0 if n == 3 else 3
        subsets = [[0, 1, 9, 10, 11, 12, 13, 14], [2, 3, 6, 7, 8], [4, 5]] if n == 3 and split else [range(15 if n == 3 else 7)]

        def piece(r0, sub):
            def run(tok):
                if w < 2:
                    ld = lambda k, j: gu_refs[w][0][(off + k) * 128 + r0:(off + k) * 128 + r0 + G, tile(n * g + j)]
                else:
                    ld = lambda k, j: wd_ref[(n * g + k) * 128 + r0:(n * g + k) * 128 + r0 + G, tile(off + j)]
                pin = (lambda k, j: k != j) if n == 3 else (lambda k, j: k == j)
                bb = [[_add(ld(k, j).astype(F32), tok if pin(k, j) else None) for j in range(n)] for k in range(n)]
                fs = (_b3 if n == 3 else _b2)(bb)
                for i in sub:
                    if w < 2:
                        gu_refs[w][1 if n == 3 else 2][i * HB + r0 // 2:i * HB + (r0 + G) // 2, tile(g)] = _pk(fs[i])
                    else:
                        p0 = (i * (NT // n) + g) * HB + r0 // 2
                        wdf_ref[p0:p0 + G // 2, tile(3 - n)] = _pk(fs[i])
                if sub is subsets[-1]:
                    done.add(('w', w, r0, n, g))
            return run
        return _costed([piece(r0, sub) for r0 in range(0, CB, G) for sub in subsets],
                       45 if len(subsets) > 1 or n == 2 else 110)

    def put_forms(unit, n, g, p0, x, y):
        rows = x[0].shape[0] // 2
        dst, nf = (ha_ref, 15) if n == 3 else (hs_ref, 7)
        for i, fm in enumerate((_a3 if n == 3 else _a2)(x, y)):
            dst[(unit * nf + i) * HB + p0:(unit * nf + i) * HB + p0 + rows, tile(g)] = _pk(fm)
        for r0 in range(2 * p0, 2 * (p0 + rows), 16):
            done.add(('hh', unit, r0, n, g))

    def gu_plain(j, unit):
        need('h2', unit, 0)
        need('h2', unit, 3)
        for h in range(2):
            x = lambda: _unpk(h2_ref[unit * CB + h * HB:unit * CB + (h + 1) * HB, :])
            p = bg.dot(x(), wg_ref[:, tile(j)]) * bg.dot(x(), wu_ref[:, tile(j)])
            pp_ref[unit * TM + h * CB:unit * TM + (h + 1) * CB, tile(j)] = p
        done.add(('pp', unit, j))

    def pp_pieces(unit, n, g, rows=range(0, CB, 16), chk=True):
        G = 16

        def piece(r0):
            def run(tok):
                assert not chk or all(('pp', unit, n * g + j) in done for j in range(n))
                ld = lambda h, j: _add((opaque(pp_ref) if chk or _E('PO', 0) else pp_ref)[unit * TM + h * CB + r0:unit * TM + h * CB + r0 + G,
                                                      tile(n * g + j)], tok)
                put_forms(unit, n, g, r0 // 2, [ld(0, j) for j in range(n)], [ld(1, j) for j in range(n)])
            return run
        return _costed([piece(r0) for r0 in rows], 80 if n == 3 else 42)

    def gu_fast(sc, unit, wide=False, tail=True):
        n = HB // 2
        need('hf', unit, 0)
        need('hf', unit, 3)

        def half(hi, w, p0, carry):
            lhs = lambda i: _unpk(hf_ref[i * HB + p0:i * HB + p0 + n, lanes[unit]])

            def m2(g):
                need('w', w, 2, g)
                return _c2(lambda i: bg.dot(lhs(15 + i), _unpk(gu_refs[w][2][i * HB:(i + 1) * HB, tile(g)])))

            if hi:
                b = m2(3 * sc + 2)
                p, q = [carry[w, p0][0]] + b[0], [carry[w, p0][1]] + b[1]
            else:
                c, b = m2(3 * sc + 1), m2(3 * sc)
                carry[w, p0] = (c[0][1], c[1][1])
                p, q = b[0] + c[0][:1], b[1] + c[1][:1]
            g = 2 * sc + hi
            need('w', w, 3, g)
            return _c3d(lambda i: bg.dot(lhs(i), _unpk(gu_refs[w][1][i * HB:(i + 1) * HB, tile(g)])), p, q)

        def finish(hi, p0, gs, us, inline):
            if inline:
                pr = [[g * u for g, u in zip(gs[h], us[h])] for h in range(2)]
                r = unit * TM + 2 * p0
                prev = [pp_ref[r + h * CB:r + h * CB + 2 * n, tile(6 * sc + 2)] for h in range(2)]
                put_forms(unit, 2, 3 * sc + 2, p0, pr[0][1:], pr[1][1:])
                put_forms(unit, 2, 3 * sc + 1, p0, [prev[0], pr[0][0]], [prev[1], pr[1][0]])
                put_forms(unit, 3, 2 * sc + 1, p0, pr[0], pr[1])
                return
            for h in range(2):
                for j in range(3):
                    r = unit * TM + h * CB + 2 * p0
                    pp_ref[r:r + 2 * n, tile(6 * sc + 3 * hi + j)] = gs[h][j] * us[h][j]
            groups = [(2, 3 * sc + 1), (2, 3 * sc + 2), (3, 2 * sc + 1)] if hi else [(2, 3 * sc), (3, 2 * sc)]
            ps = [p for nn, g in groups for p in pp_pieces(unit, nn, g, range(2 * p0, 2 * (p0 + n), 16), False)]
            if inline:
                now(ps)
            else:
                bg.add(ps, bg.clock + _E('F0', 100), bg.clock + (_E('F2', 400) if wide else _E('F1', 600)))

        carry = {}
        if wide:
            for hi in range(2):
                gs = [half(hi, 0, p0, carry) for p0 in (0, n)]
                for i, p0 in enumerate((0, n)):
                    finish(hi, p0, gs[i], half(hi, 1, p0, carry), tail and hi and p0)
        else:
            for p0 in (0, n):
                for hi in range(2):
                    gs = half(hi, 0, p0, carry)
                    finish(hi, p0, gs, half(hi, 1, p0, carry), tail and hi and p0)

    def ffn_down(x1_src, t, unit, mid=None, flip=False):
        ob = o_ref.at[rows_of(t)]

        def emit(dn, b, ls):
            o = x1_src[b * CB:(b + 1) * CB, ls] + _rep(mod_ref[4, :, ls], CB) * dn
            w = pltpu.pack_elementwise([o[:HB], o[HB:]], packed_dtype=BF16)
            ob[b * CB:(b + 1) * CB, ls] = pltpu.bitcast(w, BF16)

        parts = [(3, 15, ha_ref, [_c3, _c3cse, _c3d][_E('CSD', 0)], 0), (2, 7, hs_ref, _c2, 3)]
        for n, nf, h_ref, comb, off in (parts[::-1] if flip else parts):
            for g in range(NT // n):
                need('w', 2, n, g)
                need('hh', unit, n, g)
            kr = (NT // n) * HB
            if _E('OH', 0):
                h_ref = opaque(h_ref)
            def prod(i):
                base = (unit * nf + i) * HB
                w = lambda: _unpk(wdf_ref[i * kr:(i + 1) * kr, tile(3 - n)])
                if n == 2 and i == 3:
                    return cat([bg.dot(_unpk(h_ref[base + r:base + r + HB // 2, :]), w()) for r in (0, HB // 2)],
                               axis=0)
                return bg.dot(_unpk(h_ref[base:base + HB, :]), w())
            res = comb(prod)
            for j in range(n):
                for b in range(2):
                    emit(res[b][j], b, lanes[off + j])
            if n == (2 if flip else 3) and mid is not None:
                mid()

    x1s = [x1_ref.at[r] for r in range(NS)]
    sts = [st_ref.at[r * TM:(r + 1) * TM] for r in range(2)]
    YP = _E('YP', 12)

    def setup():
        for cp in small:
            cp.wait()
        shk = shk_ref[...].astype(F32)
        for a in range(4):
            sh_ref[a] = jnp.broadcast_to(shk[a:a + 1, :], (8, D))
        zm_ref[...] = pltpu.bitcast(inv_ref[CB:CB + 16, :], I32)
        zs.append(zm_ref[0, 0])

    def prologue():
        ytile = lambda i: ystatic_pieces(y_first, False, [p for p in positions if p[1] == lanes[i]])
        ssm_cp(0).wait()
        k_fwd(0)
        for t in range(2):
            k_cp(t).wait()
            v_cp(t).wait()
            now(kv_pieces(t, 64))
            u_fwd(t)
        bg.flush()
        for i in range(1, NL):
            if i != 3:
                ssm_cp(i).wait()
            if i == 2:
                ssm_cp(3).wait()
            bg.add(ytile(i - 1), 0, 1024)
            k_fwd(i)
            bg.flush()
        q_cp(0).wait()
        now(ytile(NL - 1))
        q_cp(1).wait()
        mod_cp(0).wait()
        mod_chunk(0)
        for t in range(2):
            now(post_pieces(t))
            now(ln1_pieces(t))
            y_inv(t, x1s[t])
        for t in range(2):
            now(ln2_stat_pieces(x1s[t], sts[t]))
        bg.flush()

    def superstep():
        wp = lambda n, g: w_pieces(0, n, g) + w_pieces(1, n, g)
        pp = lambda n, g: pp_pieces(0, n, g) + pp_pieces(1, n, g)
        mod_cp(1).wait()
        mod_chunk(1)
        now(ln2_apply_pieces(x1s[0], sts[0], 0, plain=True, forms=False))
        bg.flush()
        g_cp(0).wait()
        u_cp(0).wait()
        bg.add(ln2_apply_pieces(x1s[1], sts[1], 1, plain=True), 0, 1000)
        bg.add(ln2_apply_pieces(x1s[0], sts[0], 0) + wp(2, 0) + pp_pieces(0, 2, 0), 1000, 2400)
        for u in range(2):
            gu_plain(0, u)
            gu_plain(1, u)
        bg.flush()
        k_cp(2).wait()
        v_cp(2).wait()
        g_cp(1).wait()
        u_cp(1).wait()
        bg.add(kv_pieces(2) + wp(3, 0) + wp(2, 1) + pp_pieces(1, 2, 0), 0, 2400)
        for u in range(2):
            gu_plain(2, u)
            gu_plain(3, u)
        bg.flush()
        for f in range(2, 4):
            g_cp(f).wait()
            u_cp(f).wait()
        ymid = _costed(_group(ystatic_pieces([(s, 4, 6) for s in (4, 5)], True), 2), 35)
        bg.add(wp(2, 3) + wp(2, 2) + pp(2, 1) + pp_pieces(0, 3, 0) + ymid, 600, 2420)
        u_fwd(2)
        gu_plain(4, 0)
        gu_plain(5, 0)
        gu_plain(4, 1)
        bg.flush()
        for f in range(4, NF):
            g_cp(f).wait()
            u_cp(f).wait()
        q_cp(2).wait()
        bg.add(w_pieces(0, 2, 4) + w_pieces(0, 3, 2), 0, 550)
        bg.add(w_pieces(1, 2, 4) + w_pieces(1, 3, 2), 550, 1400)
        bg.add(w_pieces(0, 2, 5) + w_pieces(0, 3, 3), 1400, 2300)
        bg.add(w_pieces(1, 2, 5) + w_pieces(1, 3, 3), 2300, 3050)
        bg.add(post_pieces(2), _E('Q0', 3050), _E('Q1', 3750))
        gu_plain(5, 1)
        gu_fast(1, 0, wide=True)
        bg.flush()
        d_cp.wait()
        wdp = [p for g in range(NT // 3) for p in w_pieces(2, 3, g, True)]
        bg.add(pp_pieces(0, 3, 1) + wdp, 0, 3000)
        if _E('LW', 1):
            bg.add(linked(ln1_pieces(2), 3), 0, 2600)
        gu_fast(1, 1)
        bg.flush()
        mod_cp(2).wait()
        k_cp(3).wait()
        v_cp(3).wait()
        wdp = [p for g in range(NT // 2) for p in w_pieces(2, 2, g)]
        bg.add(wdp + pp(2, 2) + pp_pieces(1, 3, 0) + pp_pieces(1, 3, 1) + wp(3, 1) + kv_pieces(3), 300, 3450)
        if not _E('LW', 1):
            bg.add(linked(ln1_pieces(2), 3), 0, 2600)
        bg.inj = [(400 + 130 * i, gb_tile(i)) for i in range(NL)]
        if _E('LW', 1):
            y_inv(2, x1s[2])
        ffn_down(x1s[0], 0, 0)
        if not _E('LW', 1):
            y_inv(2, x1s[2])
        bg.flush()
        o_cp(0).start()

    def run_super(fn):
        if _E('SL', 1):
            def body(i, carry):
                fn()
                return carry
            lax.fori_loop(0, zs[0] + 1, body, 0)
        else:
            fn()

    def step(t, carry):
        q_cp(t).wait()

        @pl.when(t + 1 < NS)
        def _():
            k_cp(t + 1).wait()
            v_cp(t + 1).wait()

        x1v = x1_ref.at[pl.ds(t - 2, 3)]
        x1 = x1v.at[2]
        iv = _E('IV', 2)
        t1 = 640 + 3264 + iv * 1632 + 320
        end = 10752
        bg.add(linked(ln1_pieces(t), _E('LK1', 2)), _E('L0', 800), t1 - _E('L1', 3500))
        if _E('STOP', 1):
            bg.add(linked(ln2_stat_pieces(x1v.at[1], st_ref), _E('LK2', 0)), _E('S0', 0), _E('S1', 800))
        else:
            bg.add(linked(ln2_stat_pieces(x1, st_ref), _E('LK2', 3)), t1 + _E('S0', 100), t1 + _E('S1', 2600))
        la = _E('LKA', 0)
        bg.add(linked(ln2_apply_pieces(x1v.at[1], st_ref, 1, link=bool(la)), la), _E('P0', 1200), _E('P1', 3500))
        bg.add(kv_pieces(jnp.minimum(t + 1, NS - 1), 16), t1 + _E('K0', 300), t1 + _E('K1', 3000))
        u_fwd(t)
        J = jnp.minimum(t + 1, NS - 1)
        I = jnp.where(t == NS - 2, 2, jnp.minimum(t - 2, 4))
        chain(diag_pieces(t, T0 - 1), _E('DD', 2), _E('DE', 0))
        chain(task_pieces(t, 2), _E('MD', 3), _E('ME', 0))
        dep = chain(task_pieces(t, 1), _E('MD', 3), _E('ME', 0))
        chain(post_pieces(t), 1, 3, dep)
        ffn_down(x1v.at[0], t - 2, 1)
        if _E('OMID', 0):
            o_cp(t - 2).start()
        gu_fast(0, 1, tail=False)
        y_inv(t, x1)
        gu_fast(1, 1)
        bg.flush()
        if not _E('OMID', 0):
            o_cp(t - 2).start()
        return carry

    def epilogue():
        t = NS - 1
        bg.add(ln2_stat_pieces(x1s[t], st_ref), 0, 800)
        bg.add(ln2_apply_pieces(x1s[t], st_ref, 1), 1200, 2900)
        ffn_down(x1s[t - 1], t - 1, 1)
        o_cp(t - 1).start()
        for sc6 in range(NT // 6):
            gu_fast(sc6, 1, tail=bool(sc6))
        last = [pltpu.make_async_copy(o_ref.at[rows_of(t), lo:hi], o_hbm.at[rows_of(t), lo:hi], sem.at[s_o + t + i])
                for i, (lo, hi) in enumerate([(0, 384), (384, D)])]
        ffn_down(x1s[t], t, 1, mid=last[0].start)
        last[1].start()
        for i in range(NS - 1):
            o_cp(i).wait()
        for cp in last:
            cp.wait()

    sc = jax.named_scope if SCOPES else (lambda name: (lambda f: f))

    def rest():
        sc("superstep")(superstep)()
        lax.fori_loop(T0, NS, sc("step")(step), 0)
        sc("epilogue")(epilogue)()

    if ONLY == 'loop':
        need = lambda *a, **k: None
        zs.append(zm_ref[0, 0])
        lax.fori_loop(T0, NS, step, 0)
        epilogue()
    elif ONLY == 'S':
        zs.append(zm_ref[0, 0])
        run_super(superstep)
        lax.fori_loop(T0, NS, step, 0)
    elif _E('NEST', 3) == 3:
        setup()

        def everything():
            sc("prologue")(prologue)()
            rest()
        run_super(everything)
    else:
        setup()
        sc("prologue")(prologue)()
        run_super(rest)


@jax.jit
def pallas_adaLN_cond__ssm_conv_h3__glu_gated_bilinear__prompt_kernel(
    A_q, A_k, A_v, A_shift_k, A_ssm_k, A_ssm_D, B_x, B_w_gate, B_w_up, B_w_down, c, w_mod,
):
    B, S, D = A_q.shape
    Fh = B_w_gate.shape[1]
    NB = S // CB
    NS = S // TM
    fwd, inv = _dft_consts()
    anyspec = pl.BlockSpec(memory_space=pl.ANY)
    V = pltpu.VMEM
    out = pl.pallas_call(
        functools.partial(_kernel, S=S, D=D, Fh=Fh),
        in_specs=[anyspec] * 13,
        out_specs=anyspec,
        out_shape=jax.ShapeDtypeStruct((S, D), A_q.dtype),
        scratch_shapes=[
            V((NS, 2, 3 * CB, D), F32),
            V((NB, 3 * CB, D), F32),
            V((NS, 2, 3 * CB, D), F32),
            V((NS, TM, D), F32),
            V((S, D), BF16), V((S, D), BF16), V((S, D), BF16), V((S, D), BF16),
            V((TM, D), F32),
            V((2 * TM, 256), F32),
            V((2 * TM, Fh), F32),
            V((2 * CB, D), U32),
            V((22 * HB, 256), U32),
            V((2 * 15 * HB, Fh // 3), U32),
            V((2 * 7 * HB, Fh // 2), U32),
            V((TM // 2, D), U32),
            V((2 * CB, D), U32),
            V((15 * HB, Fh // 3), U32), V((15 * HB, Fh // 3), U32), V((15 * Fh // 6, 256), U32),
            V((7 * HB, Fh // 2), U32), V((7 * HB, Fh // 2), U32),
            V((D, S), BF16), V((D, 6 * D), BF16), V((D, Fh), BF16), V((D, Fh), BF16), V((Fh, D), BF16),
            V((2 * CB, CB), BF16), V((CB + 16, CB), BF16),
            V((5, 8, D), F32), V((4, 8, D), F32), V((8, 128), I32),
            V((4, D), BF16), V((D,), BF16), V((1, D), BF16),
            pltpu.SemaphoreType.DMA((5 + 4 * NS + D // 128 + 3 + 2 * (Fh // FC) + 2,)),
        ],
        compiler_params=pltpu.CompilerParams(
            internal_scratch_in_bytes=48 * 1024,
            disable_semaphore_checks=True,
            disable_bounds_checks=True,
            vmem_limit_bytes=110 * 1024 * 1024),
        name="adaln_h3_glu",
    )(A_q.reshape(S, D), A_k.reshape(S, D), A_v.reshape(S, D), A_shift_k.T, A_ssm_k,
      A_ssm_D, B_w_gate, B_w_up, B_w_down, c, w_mod, fwd, inv)
    return out.reshape(B, S, D)
```

```python
import functools
import os

import numpy as np
import jax
import jax.numpy as jnp
from jax import lax
import jax.experimental.pallas as pl
import jax.experimental.pallas.tpu as pltpu

F32 = jnp.float32
BF16 = jnp.bfloat16
U32 = jnp.uint32
I32 = jnp.int32

CB = 128
HB = CB // 2
TM = 256
FC = 256
KS = 256
EPS = 1e-5
SCOPES = False
ONLY = os.environ.get('ONLY', '')


def _E(name, default):
    return int(os.environ.get(name, default))


def _dft_consts():
    k = np.arange(CB, dtype=np.float64)[:, None]
    n = np.arange(CB, dtype=np.float64)[None, :]
    th = np.pi * (4.0 * k + 1.0) * n / (2.0 * CB)
    fwd = np.concatenate([np.cos(th), np.sin(th)], axis=0)
    g = np.concatenate([np.cos(th[:HB]), np.sin(th[:HB])], axis=0).T / CB
    inv = np.concatenate([g[0::2], g[1::2], np.zeros((16, CB))], axis=0)
    return jnp.asarray(fwd, dtype=BF16), jnp.asarray(inv, dtype=BF16)


def _pk(x):
    return pltpu.bitcast(x.astype(BF16), U32)


def _unpk(x):
    return pltpu.bitcast(x, BF16)


def _rep(r, n):
    return r if n == 8 else jnp.concatenate([r] * (n // 8), axis=0)


def _add(x, tok):
    return x if tok is None else x + _rep(tok, x.shape[0])


def _costed(pieces, cost):
    for p in pieces:
        p.cost = cost
    return pieces


def _group(pieces, n):
    def merged(ps):
        def run(tok):
            for p in ps:
                p(tok)
        return run
    return [merged(pieces[i:i + n]) for i in range(0, len(pieces), n)]


def _a2(x, y):
    return [x[0] + y[1], y[0] + y[1], x[0] + x[1], y[0] - x[0], x[1] - y[1], x[0], y[1]]


def _b2(b):
    return [b[0][0] + b[1][1], b[0][0], b[1][1], b[0][0] + b[0][1], b[1][0] + b[1][1],
            b[0][1] - b[1][1], b[1][0] - b[0][0]]


def _c2(m):
    m1, m7, m4, m2 = m(0), m(4), m(6), m(1)
    q0 = m2 + m4
    m5 = m(2)
    p0 = m1 + m7 + m4 - m5
    m3 = m(5)
    p1 = m3 + m5
    q1 = m1 - m2 + m3 + m(3)
    return [p0, p1], [q0, q1]


def _a3(x, y):
    w = [a + b for a, b in zip(x, y)]
    return [x[0], y[0], x[1], w[1], y[2], w[2], x[1] + y[2], x[2] - x[1], y[1] - y[2],
            w[1] - y[0], y[0] - y[1], w[0] - w[1], w[2] - x[0], x[0] - x[2], w[0] - w[2]]


def _b3(b):
    return [b[0][0] - b[0][1] + b[2][0], b[0][0] - b[0][2] + b[1][0], b[1][1] - b[1][0] + b[2][1],
            b[0][1] + b[1][1] - b[1][2], b[1][2] - b[2][0] + b[2][2], b[0][2] - b[2][1] + b[2][2],
            b[1][2] + b[2][1], b[2][1], b[1][2], b[0][1] + b[1][0], b[1][0], b[0][1],
            b[0][2] + b[2][0], b[2][0], b[0][2]]


_C3 = [(7, "+p1 +p2"), (8, "+q1 +q2"), (6, "+q1 +p2"), (14, "+q0 +q2"), (11, "+p0 +p1"), (5, "+p2"),
       (4, "-p2 +q2"), (12, "+q0 -p2 +q2"), (13, "-p0 +q0 -p2 +q2"), (3, "+q1"), (2, "+p1 -q1"),
       (9, "+p0 +p1 -q1"), (10, "+p0 -q0 +p1 -q1"), (1, "+q0"), (0, "+p0")]


def _c3(m, p=None, q=None, pad=0):
    v = {"p": [None] * 3 if p is None else list(p), "q": [None] * 3 if q is None else list(q)}
    for i, terms in _C3:
        x = m(i)
        for sg, h, n in terms.split():
            cur = v[h][int(n)]
            v[h][int(n)] = x if cur is None else (cur + x if sg == "+" else cur - x)
    return v["p"], v["q"]


def _c3cse(m, p=None, q=None, pad=0):
    p = [None] * 3 if p is None else list(p)
    q = [None] * 3 if q is None else list(q)

    def acc(v, n, x, neg=False):
        v[n] = (-x if neg else x) if v[n] is None else (v[n] - x if neg else v[n] + x)

    singles = [(5, p, 2), (3, q, 1), (1, q, 0), (0, p, 0)]
    for i, v, n in singles[:pad]:
        acc(v, n, m(i))
    m6, m7, m8 = m(6), m(7), m(8)
    if pad < 4:
        i, v, n = singles[pad]
        acc(v, n, m(i))
    acc(p, 1, m7), acc(q, 2, m8), acc(q, 1, m6 + m8), acc(p, 2, m6 + m7)
    m12, m13, m4, m14 = m(12), m(13), m(4), m(14)
    s2 = m12 + m13
    t2 = m4 + s2
    acc(q, 2, t2 + m14), acc(q, 0, s2 + m14), acc(p, 2, t2, True)
    m9, m10, m2, m11 = m(9), m(10), m(2), m(11)
    s1 = m9 + m10
    t1 = m2 + s1
    if p[0] is None:
        p[0] = (s1 + m11) - m13
    else:
        p[0] = (p[0] - m13) + (s1 + m11)
    acc(p, 1, t1 + m11), acc(q, 1, t1, True), acc(q, 0, m10, True)
    for i, v, n in singles[pad + 1:]:
        acc(v, n, m(i))
    return p, q


def _c3d(m, p=None, q=None, pad=0):
    p = [None] * 3 if p is None else list(p)
    q = [None] * 3 if q is None else list(q)

    def acc(v, n, x, neg=False):
        v[n] = x if v[n] is None else (v[n] - x if neg else v[n] + x)

    for i, a, b in ((7, (p, 1), (p, 2)), (8, (q, 1), (q, 2)), (6, (q, 1), (p, 2)), (14, (q, 0), (q, 2)),
                    (11, (p, 0), (p, 1))):
        x = m(i)
        acc(*a, x), acc(*b, x)
    m13 = m(13)
    m12 = m(12)
    acc(q, 0, m12)
    d2 = (m13 + m12) + m(4)
    acc(q, 2, d2), acc(p, 2, d2, True)
    acc(p, 2, m(5))
    m10 = m(10)
    d0 = m10 - m13
    acc(p, 0, d0), acc(q, 0, d0, True)
    m9 = m(9)
    acc(p, 0, m9)
    d1 = (m10 + m9) + m(2)
    acc(p, 1, d1), acc(q, 1, d1, True)
    acc(q, 1, m(3)), acc(q, 0, m(1)), acc(p, 0, m(0))
    return p, q


def _acc(v, n, x, neg=False):
    v[n] = x if v[n] is None else (v[n] - x if neg else v[n] + x)


def _c2_into(m, p, q, a):
    for i, terms in ((0, ((p, a, 0), (q, a + 1, 0))), (4, ((p, a, 0),)), (6, ((p, a, 0), (q, a, 0))),
                     (1, ((q, a, 0), (q, a + 1, 1))), (2, ((p, a, 1), (p, a + 1, 0))),
                     (5, ((p, a + 1, 0), (q, a + 1, 0))), (3, ((q, a + 1, 0),))):
        x = m(i)
        for v, n, neg in terms:
            _acc(v, n, x, neg)


def _c3_12(m, p, q):
    for i, a, b in ((7, (p, 1), (p, 2)), (8, (q, 1), (q, 2)), (6, (q, 1), (p, 2))):
        x = m(i)
        _acc(*a, x), _acc(*b, x)


def _c3_02(m, p, q):
    _acc(p, 0, m(0))
    x = m(14)
    _acc(q, 0, x), _acc(q, 2, x)
    _acc(p, 2, m(5))
    m13 = m(13)
    _acc(p, 0, m13, True)
    s = m13 + m(12)
    _acc(q, 0, s)
    d = s + m(4)
    _acc(q, 2, d), _acc(p, 2, d, True)


def _c3_01(m, p, q):
    _acc(q, 0, m(1))
    x = m(11)
    _acc(p, 0, x), _acc(p, 1, x)
    _acc(q, 1, m(3))
    m10 = m(10)
    _acc(q, 0, m10, True)
    s = m10 + m(9)
    _acc(p, 0, s)
    d = s + m(2)
    _acc(p, 1, d), _acc(q, 1, d, True)


class _Sched:
    def __init__(self, token):
        self.token = token
        self.clock = 0.0
        self.q = []
        self.last = None
        self.inj = []

    def add(self, pieces, t0, t1):
        cum = np.cumsum([0.0] + [getattr(p, "cost", 1.0) for p in pieces])
        self.q += [(t0 + (t1 - t0) * cum[i] / cum[-1], i, p) for i, p in enumerate(pieces)]
        self.q.sort(key=lambda e: e[:2])

    def note(self, m, dt):
        rows, cols = m.shape
        tiles = [(slice(r, r + 8), slice(c, c + 128)) for c in range(0, cols, 128) for r in range(0, rows, 8)]
        for i, tl in enumerate(tiles):
            tok = None
            while self.q and self.q[0][0] <= self.clock + dt * (i + 1) / len(tiles):
                if tok is None:
                    tok = self.token(m[tl])
                self.q.pop(0)[2](tok)
        self.clock += dt
        self.last = m[tiles[-1]]
        return m

    def dot(self, a, b):
        if self.inj and self.clock >= self.inj[0][0]:
            self.inj.pop(0)[1]()
        m = jnp.dot(a, b, preferred_element_type=F32)
        return self.note(m, max(a.shape[0], 32) * (a.shape[1] // 128) * (b.shape[1] // 128) / 4)

    def flush(self):
        tok = None if self.last is None or not self.q else self.token(self.last)
        while self.q:
            self.q.pop(0)[2](tok)
        self.clock = 0.0
        self.last = None


def _kernel(q_hbm, k_hbm, v_hbm, shk_hbm, ssmk_hbm, ssmd_hbm, wg_hbm, wu_hbm, wd_hbm,
            c_hbm, wmod_hbm, fwd_hbm, inv_hbm, o_hbm,
            u_ref, kk_ref, y_ref, x1_ref, q_ref, k_ref, v_ref, o_ref,
            hp_ref, st_ref, pp_ref, gs_ref, h2_ref, hf_ref, ha_ref, hs_ref, kv_ref, yb_ref,
            wga_ref, wua_ref, wdf_ref, wgs_ref, wus_ref,
            ssmk_ref, wmod_ref, wg_ref, wu_ref, wd_ref, fwd_ref, inv_ref,
            mod_ref, sh_ref, zm_ref, shk_ref, ssmd_ref, c_ref,
            sem, *, S, D, Fh):
    NB = S // CB
    NS = S // TM
    NL = D // 128
    NF = Fh // FC
    NT = Fh // 128
    T0 = 3
    NLOOP = NS - T0
    lanes = [slice(i * 128, (i + 1) * 128) for i in range(NL)]
    cat = jnp.concatenate

    offs = [int(o) for o in np.cumsum([0, 5, NS, NS, NS, NL, 3, NF, NF, 1])]
    s_small, s_q, s_k, s_v, s_ssm, s_mod, s_g, s_u, s_d, s_o = offs

    def rows_of(t):
        return pl.ds(t * TM if isinstance(t, int) else pl.multiple_of(t * TM, TM), TM)

    def rows_cp(src, dst, base, t):
        return pltpu.make_async_copy(src.at[rows_of(t), :], dst.at[rows_of(t), :], sem.at[base + t])

    def cols_cp(src, dst, lo, hi, si):
        return pltpu.make_async_copy(src.at[:, lo:hi], dst.at[:, lo:hi], sem.at[si])

    q_cp = lambda t: rows_cp(q_hbm, q_ref, s_q, t)
    k_cp = lambda t: rows_cp(k_hbm, k_ref, s_k, t)
    v_cp = lambda t: rows_cp(v_hbm, v_ref, s_v, t)
    o_cp = lambda t: rows_cp(o_ref, o_hbm, s_o, t)
    small = [pltpu.make_async_copy(s, d, sem.at[s_small + i]) for i, (s, d) in enumerate(
        [(fwd_hbm, fwd_ref), (shk_hbm, shk_ref), (ssmd_hbm, ssmd_ref), (inv_hbm, inv_ref), (c_hbm, c_ref)])]
    ssm_cp = lambda i: pltpu.make_async_copy(ssmk_hbm.at[lanes[i], :], ssmk_ref.at[lanes[i], :],
                                             sem.at[s_ssm + i])
    mod_cols = [(0, 3 * D), (3 * D, 5 * D), (5 * D, 6 * D)]
    mod_cp = lambda i: cols_cp(wmod_hbm, wmod_ref, mod_cols[i][0], mod_cols[i][1], s_mod + i)
    g_cp = lambda f: cols_cp(wg_hbm, wg_ref, f * FC, (f + 1) * FC, s_g + f)
    u_cp = lambda f: cols_cp(wu_hbm, wu_ref, f * FC, (f + 1) * FC, s_u + f)
    d_cp = pltpu.make_async_copy(wd_hbm, wd_ref, sem.at[s_d])

    order = small + [ssm_cp(0), k_cp(0), v_cp(0), k_cp(1), v_cp(1),
                     ssm_cp(1), ssm_cp(2), ssm_cp(3), ssm_cp(4), q_cp(0), q_cp(1),
                     mod_cp(0), mod_cp(1), g_cp(0), u_cp(0), k_cp(2), v_cp(2)]
    for f in range(1, NF):
        order += [g_cp(f), u_cp(f)]
    order += [q_cp(2), d_cp, mod_cp(2), k_cp(3), v_cp(3)]
    for t in range(T0, NS):
        order += [q_cp(t)]
        if t + 1 < NS:
            order += [k_cp(t + 1), v_cp(t + 1)]
    for cp in order:
        cp.start()

    zs = []
    bg = _Sched(lambda x: pltpu.bitcast(pltpu.bitcast(x, I32) & zm_ref[...], F32))

    def opaque(ref):
        return ref.at[pl.ds(pl.multiple_of(zs[0], 32), ref.shape[0])]

    def chain(pieces, dist, extra=0, dep=None):
        hist = [] if dep is None else [dep] * dist
        for p in pieces:
            tok = None
            if len(hist) >= dist:
                tok = bg.token(hist[-dist])
                for _ in range(extra):
                    tok = tok + tok
            hist.append(p(tok))
        return hist[-1]

    def linked(pieces, d):
        res = []

        def wrap(p):
            def run(tok):
                if d and len(res) >= d:
                    tok = tok + bg.token(res[-d])
                res.append(p(tok))
            return run
        return [wrap(p) for p in pieces]

    def now(pieces):
        for p in pieces:
            p(None)

    def mod_chunk(i):
        c = c_ref[...].astype(F32)
        sc = jnp.broadcast_to((c * jax.nn.sigmoid(c)).astype(BF16), (16, D))
        lo, hi = mod_cols[i]
        m = bg.dot(sc, wmod_ref[:, lo:hi])[0:8]
        if i == 0:
            ga = m[:, 2 * D:3 * D]
            mod_ref[0] = (1.0 + m[:, D:2 * D]) * ga
            mod_ref[1] = m[:, 0:D] * ga
        elif i == 1:
            mod_ref[2] = 1.0 + m[:, D:2 * D]
            mod_ref[3] = m[:, 0:D]
        else:
            mod_ref[4] = m

    def gb_tile(i):
        def run():
            c = c_ref[...].astype(F32)
            sc = jnp.broadcast_to((c * jax.nn.sigmoid(c)).astype(BF16), (16, D))
            w = wmod_ref[:, 5 * D + i * 128:5 * D + (i + 1) * 128]
            mod_ref[4, :, lanes[i]] = jnp.dot(sc, w, preferred_element_type=F32)[0:8]
        return run

    def k_fwd(i):
        ls = lanes[i]
        fwd = fwd_ref[...]
        prev = None
        for m in range(NB):
            kf = lax.dot_general(fwd, ssmk_ref[ls, m * CB:(m + 1) * CB], (((1,), (1,)), ((), ())),
                                 preferred_element_type=F32)
            if m == 0:
                c = kf[:CB] + ssmd_ref[...].astype(F32).reshape(1, D)[:, ls]
                d = kf[CB:]
            else:
                c = kf[:CB] + prev[CB:]
                d = kf[CB:] - prev[:CB]
            prev = kf
            kk_ref[m, 0:CB, ls] = c
            kk_ref[m, CB:2 * CB, ls] = d - c
            kk_ref[m, 2 * CB:3 * CB, ls] = c + d
            if m % 4 == 3:
                bg.note(kf, 2 * CB)

    def lo_hi(w):
        return pltpu.bitcast(w << 16, F32), pltpu.bitcast(w & jnp.uint32(0xFFFF0000), F32)

    def kv_pieces(t, G=32):
        n = G // 2
        kb, vb = k_ref.at[rows_of(t)], v_ref.at[rows_of(t)]

        def piece(ls, r0):
            def run(tok):
                if r0 > 0:
                    w = pltpu.bitcast(kb[r0 - 16:r0 + G, ls], U32)
                else:
                    if isinstance(t, int) and t == 0:
                        halo = jnp.zeros((8, 128), U32)
                    else:
                        halo = pltpu.bitcast(k_ref.at[rows_of(t - 1)][TM - 16:TM, ls], U32)
                    w = cat([halo, pltpu.bitcast(kb[0:G, ls], U32)], axis=0)
                if tok is not None:
                    w = w | _rep(pltpu.bitcast(tok, U32), n + 8)
                ke, ko = lo_hi(w[8:])
                ke1, ko1 = lo_hi(pltpu.roll(w, 1, 0)[8:])
                _, ko2 = lo_hi(pltpu.roll(w, 2, 0)[8:])
                s0, s1, s2, s3 = [_rep(sh_ref[a, :, ls], n) for a in range(4)]
                ve, vo = lo_hi(pltpu.bitcast(vb[r0:r0 + G, ls], U32))
                kve = ((ke * s0 + ko1 * s1) + (ke1 * s2 + ko2 * s3)) * ve
                kvo = ((ko * s0 + ke * s1) + (ko1 * s2 + ke1 * s3)) * vo
                kv_ref[r0 // 2:(r0 + G) // 2, ls] = pltpu.bitcast(
                    pltpu.pack_elementwise([kve, kvo], packed_dtype=BF16), U32)
            return run
        return _costed([piece(ls, r0) for ls in lanes for r0 in range(0, TM, G)], 2.5 * G + 10)

    def u_fwd(t):
        for b in range(2):
            for ls in lanes:
                kv = lambda: _unpk(kv_ref[b * HB:(b + 1) * HB, ls])
                a = bg.dot(fwd_ref[0:CB, :], kv())
                bb = bg.dot(fwd_ref[CB:2 * CB, :], kv())
                u_ref[t, b, 0:CB, ls] = a + bb
                u_ref[t, b, CB:2 * CB, ls] = a
                u_ref[t, b, 2 * CB:3 * CB, ls] = bb

    positions = [(slice(r0, r0 + 8), ls) for r0 in range(0, 3 * CB, 8) for ls in lanes]

    def ystatic_pieces(blocks, acc_in, pos=None):
        def piece(rs, ls):
            def run(tok):
                us, ks = {}, {}
                for s, lo, hi in blocks:
                    acc = None
                    for i in range(lo, min(hi, s + 1)):
                        if i not in us:
                            us[i] = _add(u_ref[i // 2, i % 2, rs, ls], tok)
                        if s - i not in ks:
                            ks[s - i] = kk_ref[s - i, rs, ls]
                        p = ks[s - i] * us[i]
                        acc = p if acc is None else acc + p
                    if acc_in:
                        acc = acc + y_ref[s // 2, s % 2, rs, ls]
                    y_ref[s // 2, s % 2, rs, ls] = acc
                return acc
            return run
        return _costed([piece(*p) for p in (positions if pos is None else pos)], 35)

    y_first = [(s, 0, 4) for s in range(NB)]

    def task_pieces(t, delta):
        p = t - delta
        left = p >= T0
        J = jnp.where(left, t, p + NLOOP)
        I = jnp.where(left, p, t)
        kview = kk_ref.at[pl.ds(2 * (J - I) - 1, 3)]

        def piece(rs, ls):
            def run(tok):
                u0 = _add(u_ref[I, 0, rs, ls], tok)
                u1 = _add(u_ref[I, 1, rs, ls], tok)
                kc = kview[1, rs, ls]
                y_ref[J, 0, rs, ls] = (kc * u0 + kview[0, rs, ls] * u1) + y_ref[J, 0, rs, ls]
                y1 = (kview[2, rs, ls] * u0 + kc * u1) + y_ref[J, 1, rs, ls]
                y_ref[J, 1, rs, ls] = y1
                return y1
            return run
        return [piece(*p) for p in positions]

    def diag_pieces(t, I):
        kview = kk_ref.at[pl.ds(2 * (t - I) - 1, 3)]

        def piece(rs, ls):
            def run(tok):
                us = [_add(u_ref[a, b, rs, ls], tok) for a in (t, I) for b in range(2)]
                k0 = kk_ref[0, rs, ls]
                kc = kview[1, rs, ls]
                y_ref[t, 0, rs, ls] = ((k0 * us[0] + y_ref[t, 0, rs, ls])
                                       + (kc * us[2] + kview[0, rs, ls] * us[3]))
                y1 = ((kk_ref[1, rs, ls] * us[0] + k0 * us[1])
                      + (kview[2, rs, ls] * us[2] + kc * us[3]) + y_ref[t, 1, rs, ls])
                y_ref[t, 1, rs, ls] = y1
                return y1
            return run
        return [piece(*p) for p in positions]

    def mac_pieces(J, I, diag):
        kview = kk_ref if diag else kk_ref.at[pl.ds(2 * (J - I) - 3, 5)]
        uview = u_ref.at[pl.ds(I, 2)]

        def piece(rs, ls):
            def run(tok):
                one = _E('TK', 0)
                us = [_add(uview[a, b, rs, ls], None if one else tok) for a in range(2) for b in range(2)]
                ks = ([None] + [kview[i, rs, ls] for i in range(4)]) if diag else [kview[i, rs, ls] for i in range(5)]
                if one:
                    ks[2] = _add(ks[2], tok)
                    if one == 2:
                        ks[1], ks[3] = _add(ks[1], tok), _add(ks[3], tok)
                y0 = (ks[3] * us[0] + ks[2] * us[1]) + (ks[1] * us[2] + y_ref[J, 0, rs, ls])
                if not diag:
                    y0 = y0 + ks[0] * us[3]
                y1 = ((ks[4] * us[0] + ks[3] * us[1]) + (ks[2] * us[2] + ks[1] * us[3])) + y_ref[J, 1, rs, ls]
                y_ref[J, 0, rs, ls] = y0
                y_ref[J, 1, rs, ls] = y1
                return y1
            return run
        return [piece(*p) for p in positions]

    def post_pieces(t):
        def piece(b, r0, ls):
            def run(tok):
                comp = lambda c, off: y_ref[t, b, c * CB + off + r0:c * CB + off + r0 + 16, ls]
                k1l, k1h = _add(comp(0, 0), tok), _add(comp(0, HB), tok)
                rel, reh = k1l - comp(2, 0), k1h - comp(2, HB)
                iml, imh = k1l + comp(1, 0), k1h + comp(1, HB)
                p0 = b * CB + r0 // 2
                yb_ref[p0:p0 + 8, ls] = _pk(rel + reh)
                yb_ref[p0 + HB // 2:p0 + HB // 2 + 8, ls] = _pk(iml + imh)
                yb_ref[p0 + HB:p0 + HB + 8, ls] = _pk(rel - reh)
                oim = iml - imh
                yb_ref[p0 + HB + HB // 2:p0 + HB + HB // 2 + 8, ls] = _pk(oim)
                return oim[8:16]
            return run
        return _costed([piece(b, r0, ls) for b in range(2) for r0 in range(0, HB, 16) for ls in lanes], 45)

    def q_split(t, b, p0, n, ls):
        w = pltpu.bitcast(q_ref.at[rows_of(t)][b * CB + 2 * p0:b * CB + 2 * p0 + 2 * n, ls], U32)
        return lo_hi(w)

    def ln_tiles(xs, tok):
        n = xs[0].shape[0]
        s = _add(xs[0], tok)
        for x in xs[1:]:
            s = s + x
        m = jnp.sum(s, axis=-1, keepdims=True) * (1.0 / D)
        xc = [x - m for x in xs]
        s2 = xc[0] * xc[0]
        for x in xc[1:]:
            s2 = s2 + x * x
        r = lax.rsqrt(jnp.sum(s2, axis=-1, keepdims=True) * (1.0 / D) + EPS)
        return xc, jnp.broadcast_to(r, (n, 128)), jnp.broadcast_to(m, (n, 128))

    def ln1_pieces(t):
        G = _E('L1G', 8)

        def piece(b, p0):
            def run(tok):
                xc, r, _ = ln_tiles([cat(q_split(t, b, p0, G, ls), axis=0) for ls in lanes], tok)
                for ls, x in zip(lanes, xc):
                    h = (x * r) * _rep(mod_ref[0, :, ls], 2 * G) + _rep(mod_ref[1, :, ls], 2 * G)
                    hp_ref[b * CB + p0:b * CB + p0 + G, ls] = h[:G]
                    hp_ref[b * CB + HB + p0:b * CB + HB + p0 + G, ls] = h[G:]
                return functools.reduce(lambda a, c: a + c, [h[r:r + 8] for r in range(0, 2 * G, 8)])
            return run
        return [piece(b, p0) for b in range(2) for p0 in range(0, HB, G)]

    def y_inv(t, x1_dst):
        yb = opaque(yb_ref)
        hp = opaque(hp_ref)
        for b in range(2):
            ye = bg.dot(inv_ref[0:HB, :], _unpk(yb[b * CB:b * CB + HB, :]))
            yo = bg.dot(inv_ref[HB:CB, :], _unpk(yb[b * CB + HB:(b + 1) * CB, :]))
            for ls in lanes:
                qe, qo = q_split(t, b, 0, HB, ls)
                re, ro = slice(b * CB, b * CB + HB), slice(b * CB + HB, (b + 1) * CB)
                x1_dst[re, ls] = qe + hp[re, ls] * ye[:, ls]
                x1_dst[ro, ls] = qo + hp[ro, ls] * yo[:, ls]

    def ln2_stat_pieces(x1_src, st):
        x1o = opaque(x1_src)

        def piece(r0):
            def run(tok):
                _, r, m = ln_tiles([x1o[r0:r0 + 16, ls] for ls in lanes], tok)
                st[r0:r0 + 16, 0:128] = m
                st[r0:r0 + 16, 128:256] = r
                return r[0:8] + r[8:16]
            return run
        return [piece(h * CB + r0) for r0 in range(0, CB, 16) for h in range(2)]

    done = set()

    def ln2_apply_pieces(x1_src, st, unit, plain=False, forms=True, link=False):
        G = 16
        x1o = opaque(x1_src)

        def piece(r0, js):
            def run(tok):
                two = lambda ref, c: cat([ref[r0:r0 + G, c], ref[CB + r0:CB + r0 + G, c]], axis=0)
                m, r = _add(two(st, slice(0, 128)), tok), two(st, slice(128, 256))
                hs = [((two(x1o, lanes[j]) - m) * r) * _rep(mod_ref[2, :, lanes[j]], 2 * G)
                      + _rep(mod_ref[3, :, lanes[j]], 2 * G) for j in js]
                if plain:
                    for j, h in zip(js, hs):
                        p0 = unit * CB + r0 // 2
                        h2_ref[p0:p0 + G // 2, lanes[j]] = _pk(h[:G])
                        h2_ref[p0 + HB:p0 + HB + G // 2, lanes[j]] = _pk(h[G:])
                    done.add(('h2', unit, r0, js[0]))
                if forms:
                    fs = (_a3 if len(js) == 3 else _a2)([h[:G] for h in hs], [h[G:] for h in hs])
                    for i, fm in enumerate(fs):
                        p0 = (i + (0 if len(js) == 3 else 15)) * HB + r0 // 2
                        hf_ref[p0:p0 + G // 2, lanes[unit]] = _pk(fm)
                    done.add(('hf', unit, r0, js[0]))

            return run
        return [_costed([piece(r0, js)], (30 if plain else 42) * len(js))[0]
                for r0 in range(0, CB, G) for js in ([0, 1, 2], [3, 4])]

    def need(*key, rows=range(0, CB, 16)):
        for r0 in rows:
            assert key[:2] + (r0,) + key[2:] in done, key

    tile = lambda j: slice(j * 128, (j + 1) * 128)
    gu_refs = ((wg_ref, wga_ref, wgs_ref), (wu_ref, wua_ref, wus_ref))

    def w_pieces(w, n, g, split=False):
        G = 16

        off = 0 if n == 3 else 3
        subsets = [[0, 1, 9, 10, 11, 12, 13, 14], [2, 3, 6, 7, 8], [4, 5]] if n == 3 and split else [range(15 if n == 3 else 7)]

        def piece(r0, sub):
            def run(tok):
                if w < 2:
                    ld = lambda k, j: gu_refs[w][0][(off + k) * 128 + r0:(off + k) * 128 + r0 + G, tile(n * g + j)]
                else:
                    ld = lambda k, j: wd_ref[(n * g + k) * 128 + r0:(n * g + k) * 128 + r0 + G, tile(off + j)]
                pin = (lambda k, j: k != j) if n == 3 else (lambda k, j: k == j)
                bb = [[_add(ld(k, j).astype(F32), tok if pin(k, j) else None) for j in range(n)] for k in range(n)]
                fs = (_b3 if n == 3 else _b2)(bb)
                for i in sub:
                    if w < 2:
                        gu_refs[w][1 if n == 3 else 2][i * HB + r0 // 2:i * HB + (r0 + G) // 2, tile(g)] = _pk(fs[i])
                    else:
                        p0 = (i * (NT // n) + g) * HB + r0 // 2
                        wdf_ref[p0:p0 + G // 2, tile(3 - n)] = _pk(fs[i])
                if sub is subsets[-1]:
                    done.add(('w', w, r0, n, g))
            return run
        return _costed([piece(r0, sub) for r0 in range(0, CB, G) for sub in subsets],
                       45 if len(subsets) > 1 or n == 2 else 110)

    def put_forms(unit, n, g, p0, x, y):
        rows = x[0].shape[0] // 2
        dst, nf = (ha_ref, 15) if n == 3 else (hs_ref, 7)
        for i, fm in enumerate((_a3 if n == 3 else _a2)(x, y)):
            dst[(unit * nf + i) * HB + p0:(unit * nf + i) * HB + p0 + rows, tile(g)] = _pk(fm)
        for r0 in range(2 * p0, 2 * (p0 + rows), 16):
            done.add(('hh', unit, r0, n, g))

    def gu_plain(j, unit):
        need('h2', unit, 0)
        need('h2', unit, 3)
        for h in range(2):
            x = lambda: _unpk(h2_ref[unit * CB + h * HB:unit * CB + (h + 1) * HB, :])
            p = bg.dot(x(), wg_ref[:, tile(j)]) * bg.dot(x(), wu_ref[:, tile(j)])
            pp_ref[unit * TM + h * CB:unit * TM + (h + 1) * CB, tile(j)] = p
        done.add(('pp', unit, j))

    def pp_pieces(unit, n, g, rows=range(0, CB, 16), chk=True):
        G = 16

        def piece(r0):
            def run(tok):
                assert not chk or all(('pp', unit, n * g + j) in done for j in range(n))
                ld = lambda h, j: _add((opaque(pp_ref) if chk or _E('PO', 0) else pp_ref)[unit * TM + h * CB + r0:unit * TM + h * CB + r0 + G,
                                                      tile(n * g + j)], tok)
                put_forms(unit, n, g, r0 // 2, [ld(0, j) for j in range(n)], [ld(1, j) for j in range(n)])
            return run
        return _costed([piece(r0) for r0 in rows], 80 if n == 3 else 42)

    def tail_pieces(unit):
        return [p for nn, g in ((3, NT // 3 - 1), (2, NT // 2 - 2), (2, NT // 2 - 1))
                for p in pp_pieces(unit, nn, g, range(HB, CB, 16), False)]

    def gu_fast(sc, unit, wide=False, tail=True, mid=None):
        n = HB // 2
        need('hf', unit, 0)
        need('hf', unit, 3)

        def park(x, h, p0, j):
            mode = _E('PARK', 1)
            if not mode:
                return lambda: x
            r = slice(h * CB + 2 * p0, h * CB + 2 * (p0 + n))
            gs_ref[r, tile(j)] = x
            return lambda: (opaque(gs_ref) if mode == 2 else gs_ref)[r, tile(j)]

        def half(hi, w, p0, carry):
            lhs = lambda i: _unpk(hf_ref[i * HB + p0:i * HB + p0 + n, lanes[unit]])

            def m2(g):
                need('w', w, 2, g)
                return _c2(lambda i: bg.dot(lhs(15 + i), _unpk(gu_refs[w][2][i * HB:(i + 1) * HB, tile(g)])))

            g = 2 * sc + hi
            m3 = lambda i: bg.dot(lhs(i), _unpk(gu_refs[w][1][i * HB:(i + 1) * HB, tile(g)]))
            if _E('PH', 1):
                def into(g2, p, q, a):
                    need('w', w, 2, g2)
                    _c2_into(lambda i: bg.dot(lhs(15 + i), _unpk(gu_refs[w][2][i * HB:(i + 1) * HB, tile(g2)])),
                             p, q, a)
                out = lambda j: [park(v[j], h, p0, j) if w == 0 else v[j] for h, v in enumerate((p, q))]
                rest = (lambda x, h: park(x, h, p0, 5)) if _E('PH', 1) == 1 else (lambda x, h: (lambda: x))
                if hi:
                    p, q = [carry[w, p0][0](), None, None], [carry[w, p0][1](), None, None]
                    need('w', w, 3, g)
                    _c3_02(m3, p, q)
                    idle = rest(p[2], 0), rest(q[2], 1)
                    _c3_01(m3, p, q)
                    o0 = out(0)
                    p[2], q[2] = idle[0](), idle[1]()
                    _c3_12(m3, p, q)
                    into(3 * sc + 2, p, q, 1)
                    o = [o0, out(1), out(2)]
                else:
                    p, q = [None] * 4, [None] * 4
                    into(3 * sc + 1, p, q, 2)
                    carry[w, p0] = (park(p[3], 0, p0, 3 + w), park(q[3], 1, p0, 3 + w))
                    need('w', w, 3, g)
                    _c3_12(m3, p, q)
                    idle = rest(p[1], 0), rest(q[1], 1)
                    _c3_02(m3, p, q)
                    o2 = out(2)
                    p[1], q[1] = idle[0](), idle[1]()
                    _c3_01(m3, p, q)
                    into(3 * sc, p, q, 0)
                    o = [out(0), out(1), o2]
                return [[o[j][h] for j in range(3)] for h in range(2)]
            if hi:
                b = m2(3 * sc + 2)
                p, q = [carry[w, p0][0]()] + b[0], [carry[w, p0][1]()] + b[1]
            else:
                c, b = m2(3 * sc + 1), m2(3 * sc)
                carry[w, p0] = (park(c[0][1], 0, p0, 3 + w), park(c[1][1], 1, p0, 3 + w))
                p, q = b[0] + c[0][:1], b[1] + c[1][:1]
            need('w', w, 3, g)
            res = _c3d(lambda i: bg.dot(lhs(i), _unpk(gu_refs[w][1][i * HB:(i + 1) * HB, tile(g)])), p, q)
            return res if w else [[park(x, h, p0, j) for j, x in enumerate(res[h])] for h in range(2)]

        def finish(hi, p0, gs, us, inline):
            gs = [[x() for x in gs[h]] for h in range(2)]
            if inline and tail is True:
                pr = [[g * u for g, u in zip(gs[h], us[h])] for h in range(2)]
                r = unit * TM + 2 * p0
                prev = [pp_ref[r + h * CB:r + h * CB + 2 * n, tile(6 * sc + 2)] for h in range(2)]
                put_forms(unit, 2, 3 * sc + 2, p0, pr[0][1:], pr[1][1:])
                put_forms(unit, 2, 3 * sc + 1, p0, [prev[0], pr[0][0]], [prev[1], pr[1][0]])
                put_forms(unit, 3, 2 * sc + 1, p0, pr[0], pr[1])
                return
            for h in range(2):
                for j in range(3):
                    r = unit * TM + h * CB + 2 * p0
                    pp_ref[r:r + 2 * n, tile(6 * sc + 3 * hi + j)] = gs[h][j] * us[h][j]
            groups = [(2, 3 * sc + 1), (2, 3 * sc + 2), (3, 2 * sc + 1)] if hi else [(2, 3 * sc), (3, 2 * sc)]
            ps = [p for nn, g in groups for p in pp_pieces(unit, nn, g, range(2 * p0, 2 * (p0 + n), 16), False)]
            if not inline:
                bg.add(ps, bg.clock + _E('F0', 100), bg.clock + (_E('F2', 400) if wide else _E('F1', 600)))

        carry = {}
        if wide:
            for hi in range(2):
                gs = [half(hi, 0, p0, carry) for p0 in (0, n)]
                for i, p0 in enumerate((0, n)):
                    finish(hi, p0, gs[i], half(hi, 1, p0, carry), tail and hi and p0)
        else:
            for p0 in (0, n):
                for hi in range(2):
                    if mid is not None and mid[0] == 2 * (p0 > 0) + hi:
                        mid[1]()
                    gs = half(hi, 0, p0, carry)
                    finish(hi, p0, gs, half(hi, 1, p0, carry), tail and hi and p0)

    def ffn_down(x1_src, t, unit, mid=None, flip=False):
        ob = o_ref.at[rows_of(t)]

        def emit(dn, b, ls):
            o = x1_src[b * CB:(b + 1) * CB, ls] + _rep(mod_ref[4, :, ls], CB) * dn
            w = pltpu.pack_elementwise([o[:HB], o[HB:]], packed_dtype=BF16)
            ob[b * CB:(b + 1) * CB, ls] = pltpu.bitcast(w, BF16)

        parts = [(3, 15, ha_ref, [_c3, _c3cse, _c3d][_E('CSD', 0)], 0), (2, 7, hs_ref, _c2, 3)]
        for n, nf, h_ref, comb, off in (parts[::-1] if flip else parts):
            for g in range(NT // n):
                need('w', 2, n, g)
                need('hh', unit, n, g)
            kr = (NT // n) * HB
            if _E('OH', 0):
                h_ref = opaque(h_ref)
            def prod(i):
                base = (unit * nf + i) * HB
                w = lambda: _unpk(wdf_ref[i * kr:(i + 1) * kr, tile(3 - n)])
                if n == 2 and i == 3:
                    return cat([bg.dot(_unpk(h_ref[base + r:base + r + HB // 2, :]), w()) for r in (0, HB // 2)],
                               axis=0)
                return bg.dot(_unpk(h_ref[base:base + HB, :]), w())
            res = comb(prod)
            for j in range(n):
                for b in range(2):
                    emit(res[b][j], b, lanes[off + j])
            if n == (2 if flip else 3) and mid is not None:
                mid()

    x1s = [x1_ref.at[r] for r in range(NS)]
    sts = [st_ref.at[r * TM:(r + 1) * TM] for r in range(2)]
    YP = _E('YP', 12)

    def setup():
        for cp in small:
            cp.wait()
        shk = shk_ref[...].astype(F32)
        for a in range(4):
            sh_ref[a] = jnp.broadcast_to(shk[a:a + 1, :], (8, D))
        zm_ref[...] = pltpu.bitcast(inv_ref[CB:CB + 16, :], I32)
        zs.append(zm_ref[0, 0])

    def prologue():
        ytile = lambda i: ystatic_pieces(y_first, False, [p for p in positions if p[1] == lanes[i]])
        ssm_cp(0).wait()
        k_fwd(0)
        for t in range(2):
            k_cp(t).wait()
            v_cp(t).wait()
            now(kv_pieces(t, 64))
            u_fwd(t)
        bg.flush()
        for i in range(1, NL):
            if i != 3:
                ssm_cp(i).wait()
            if i == 2:
                ssm_cp(3).wait()
            bg.add(ytile(i - 1), 0, 1024)
            k_fwd(i)
            bg.flush()
        q_cp(0).wait()
        now(ytile(NL - 1))
        q_cp(1).wait()
        mod_cp(0).wait()
        mod_chunk(0)
        for t in range(2):
            now(post_pieces(t))
            now(ln1_pieces(t))
            y_inv(t, x1s[t])
        for t in range(2):
            now(ln2_stat_pieces(x1s[t], sts[t]))
        bg.flush()

    def superstep():
        wp = lambda n, g: w_pieces(0, n, g) + w_pieces(1, n, g)
        pp = lambda n, g: pp_pieces(0, n, g) + pp_pieces(1, n, g)
        mod_cp(1).wait()
        mod_chunk(1)
        now(ln2_apply_pieces(x1s[0], sts[0], 0, plain=True, forms=False))
        bg.flush()
        g_cp(0).wait()
        u_cp(0).wait()
        bg.add(ln2_apply_pieces(x1s[1], sts[1], 1, plain=True), 0, 1000)
        bg.add(ln2_apply_pieces(x1s[0], sts[0], 0) + wp(2, 0) + pp_pieces(0, 2, 0), 1000, 2400)
        for u in range(2):
            gu_plain(0, u)
            gu_plain(1, u)
        bg.flush()
        k_cp(2).wait()
        v_cp(2).wait()
        g_cp(1).wait()
        u_cp(1).wait()
        bg.add(kv_pieces(2) + wp(3, 0) + wp(2, 1) + pp_pieces(1, 2, 0), 0, 2400)
        for u in range(2):
            gu_plain(2, u)
            gu_plain(3, u)
        bg.flush()
        for f in range(2, 4):
            g_cp(f).wait()
            u_cp(f).wait()
        ymid = _costed(_group(ystatic_pieces([(s, 4, 6) for s in (4, 5)], True), 2), 35)
        bg.add(wp(2, 3) + wp(2, 2) + pp(2, 1) + pp_pieces(0, 3, 0) + ymid, 600, 2420)
        u_fwd(2)
        gu_plain(4, 0)
        gu_plain(5, 0)
        gu_plain(4, 1)
        bg.flush()
        for f in range(4, NF):
            g_cp(f).wait()
            u_cp(f).wait()
        q_cp(2).wait()
        bg.add(w_pieces(0, 2, 4) + w_pieces(0, 3, 2), 0, 550)
        bg.add(w_pieces(1, 2, 4) + w_pieces(1, 3, 2), 550, 1400)
        bg.add(w_pieces(0, 2, 5) + w_pieces(0, 3, 3), 1400, 2300)
        bg.add(w_pieces(1, 2, 5) + w_pieces(1, 3, 3), 2300, 3050)
        bg.add(post_pieces(2), _E('Q0', 3050), _E('Q1', 3750))
        gu_plain(5, 1)
        gu_fast(1, 0, wide=True, tail='defer')
        bg.flush()
        d_cp.wait()
        wdp = [p for g in range(NT // 3) for p in w_pieces(2, 3, g, True)]
        bg.add(tail_pieces(0) + pp_pieces(0, 3, 1) + wdp, 0, 3000)
        if _E('LW', 1):
            bg.add(linked(ln1_pieces(2), 3), 0, 2600)
        gu_fast(1, 1, tail='defer')
        bg.flush()
        mod_cp(2).wait()
        k_cp(3).wait()
        v_cp(3).wait()
        wdp = [p for g in range(NT // 2) for p in w_pieces(2, 2, g)]
        bg.add(wdp + pp(2, 2) + ([] if _E('TD', 0) else tail_pieces(1)) + pp_pieces(1, 3, 0) + pp_pieces(1, 3, 1) + wp(3, 1) + kv_pieces(3), 300, 3450)
        if not _E('LW', 1):
            bg.add(linked(ln1_pieces(2), 3), 0, 2600)
        bg.inj = [(400 + 130 * i, gb_tile(i)) for i in range(NL)]
        if _E('LW', 1):
            y_inv(2, x1s[2])
        ffn_down(x1s[0], 0, 0)
        if not _E('LW', 1):
            y_inv(2, x1s[2])
        bg.flush()
        o_cp(0).start()

    def run_super(fn):
        if _E('SL', 1):
            def body(i, carry):
                fn()
                return carry
            lax.fori_loop(0, zs[0] + 1, body, 0)
        else:
            fn()

    def step(t, carry):
        q_cp(t).wait()

        @pl.when(t + 1 < NS)
        def _():
            k_cp(t + 1).wait()
            v_cp(t + 1).wait()

        x1v = x1_ref.at[pl.ds(t - 2, 3)]
        x1 = x1v.at[2]
        iv = _E('IV', 2)
        t1 = 640 + 3264 + 3264 + [0, 928, 1632, 2560][iv] + 320
        end = 10752
        bg.add(linked(ln1_pieces(t), _E('LK1', 2)), _E('L0', 800), _E('L1', 3988))
        if _E('STOP', 1):
            bg.add(linked(ln2_stat_pieces(x1v.at[1], st_ref), _E('LK2', 0)), _E('S0', 0), _E('S1', 600))
        else:
            bg.add(linked(ln2_stat_pieces(x1, st_ref), _E('LK2', 3)), t1 + _E('S0', 100), t1 + _E('S1', 2600))
        la = _E('LKA', 0)
        bg.add(linked(ln2_apply_pieces(x1v.at[1], st_ref, 1, link=bool(la)), la), _E('P0', 1500), _E('P1', 3700))
        bg.add(kv_pieces(jnp.minimum(t + 1, NS - 1), 16), _E('K0', 7788), _E('K1', 10488))
        if _E('TD', 0):
            tp = tail_pieces(1)
            bg.add(tp[:4], _E('T0', 0), _E('T1', 300))
            bg.add(tp[4:], _E('T2', 700), _E('T3', 1200))
        u_fwd(t)
        J = jnp.minimum(t + 1, NS - 1)
        I = jnp.where(t == NS - 2, 2, jnp.minimum(t - 2, 4))
        chain(diag_pieces(t, T0 - 1), _E('DD', 2), _E('DE', 0))
        chain(task_pieces(t, 2), _E('MD', 2), _E('ME', 0))
        dep = chain(task_pieces(t, 1), _E('MD', 2), _E('ME', 0))
        chain(post_pieces(t), 1, 3, dep)
        ffn_down(x1v.at[0], t - 2, 1)
        if _E('OMID', 0):
            o_cp(t - 2).start()
        gu_fast(0, 1, tail=False)
        gu_fast(1, 1, mid=(iv, lambda: y_inv(t, x1)))
        bg.flush()
        if not _E('OMID', 0):
            o_cp(t - 2).start()
        return carry

    def epilogue():
        t = NS - 1
        if _E('TD', 0):
            tp = tail_pieces(1)
            now(tp[:4])
            bg.add(tp[4:], 100, 600)
        bg.add(ln2_stat_pieces(x1s[t], st_ref), 0, 800)
        bg.add(ln2_apply_pieces(x1s[t], st_ref, 1), 1200, 2900)
        ffn_down(x1s[t - 1], t - 1, 1)
        o_cp(t - 1).start()
        for sc6 in range(NT // 6):
            gu_fast(sc6, 1, tail=bool(sc6))
        last = [pltpu.make_async_copy(o_ref.at[rows_of(t), lo:hi], o_hbm.at[rows_of(t), lo:hi], sem.at[s_o + t + i])
                for i, (lo, hi) in enumerate([(0, 384), (384, D)])]
        ffn_down(x1s[t], t, 1, mid=last[0].start)
        last[1].start()
        for i in range(NS - 1):
            o_cp(i).wait()
        for cp in last:
            cp.wait()

    sc = jax.named_scope if SCOPES else (lambda name: (lambda f: f))

    def rest():
        sc("superstep")(superstep)()
        lax.fori_loop(T0, NS, sc("step")(step), 0)
        sc("epilogue")(epilogue)()

    if ONLY == 'loop':
        need = lambda *a, **k: None
        zs.append(zm_ref[0, 0])
        lax.fori_loop(T0, NS, step, 0)
        epilogue()
    elif ONLY == 'S':
        zs.append(zm_ref[0, 0])
        run_super(superstep)
        lax.fori_loop(T0, NS, step, 0)
    elif _E('NEST', 3) == 3:
        setup()

        def everything():
            sc("prologue")(prologue)()
            rest()
        run_super(everything)
    else:
        setup()
        sc("prologue")(prologue)()
        run_super(rest)


@jax.jit
def pallas_adaLN_cond__ssm_conv_h3__glu_gated_bilinear__prompt_kernel(
    A_q, A_k, A_v, A_shift_k, A_ssm_k, A_ssm_D, B_x, B_w_gate, B_w_up, B_w_down, c, w_mod,
):
    B, S, D = A_q.shape
    Fh = B_w_gate.shape[1]
    NB = S // CB
    NS = S // TM
    fwd, inv = _dft_consts()
    anyspec = pl.BlockSpec(memory_space=pl.ANY)
    V = pltpu.VMEM
    out = pl.pallas_call(
        functools.partial(_kernel, S=S, D=D, Fh=Fh),
        in_specs=[anyspec] * 13,
        out_specs=anyspec,
        out_shape=jax.ShapeDtypeStruct((S, D), A_q.dtype),
        scratch_shapes=[
            V((NS, 2, 3 * CB, D), F32),
            V((NB, 3 * CB, D), F32),
            V((NS, 2, 3 * CB, D), F32),
            V((NS, TM, D), F32),
            V((S, D), BF16), V((S, D), BF16), V((S, D), BF16), V((S, D), BF16),
            V((TM, D), F32),
            V((2 * TM, 256), F32),
            V((2 * TM, Fh), F32),
            V((TM, 6 * 128), F32),
            V((2 * CB, D), U32),
            V((22 * HB, 256), U32),
            V((2 * 15 * HB, Fh // 3), U32),
            V((2 * 7 * HB, Fh // 2), U32),
            V((TM // 2, D), U32),
            V((2 * CB, D), U32),
            V((15 * HB, Fh // 3), U32), V((15 * HB, Fh // 3), U32), V((15 * Fh // 6, 256), U32),
            V((7 * HB, Fh // 2), U32), V((7 * HB, Fh // 2), U32),
            V((D, S), BF16), V((D, 6 * D), BF16), V((D, Fh), BF16), V((D, Fh), BF16), V((Fh, D), BF16),
            V((2 * CB, CB), BF16), V((CB + 16, CB), BF16),
            V((5, 8, D), F32), V((4, 8, D), F32), V((8, 128), I32),
            V((4, D), BF16), V((D,), BF16), V((1, D), BF16),
            pltpu.SemaphoreType.DMA((5 + 4 * NS + D // 128 + 3 + 2 * (Fh // FC) + 2,)),
        ],
        compiler_params=pltpu.CompilerParams(
            internal_scratch_in_bytes=48 * 1024,
            disable_semaphore_checks=True,
            disable_bounds_checks=True,
            vmem_limit_bytes=110 * 1024 * 1024),
        name="adaln_h3_glu",
    )(A_q.reshape(S, D), A_k.reshape(S, D), A_v.reshape(S, D), A_shift_k.T, A_ssm_k,
      A_ssm_D, B_w_gate, B_w_up, B_w_down, c, w_mod, fwd, inv)
    return out.reshape(B, S, D)
```

```python
import functools
import os

import numpy as np
import jax
import jax.numpy as jnp
from jax import lax
import jax.experimental.pallas as pl
import jax.experimental.pallas.tpu as pltpu

F32 = jnp.float32
BF16 = jnp.bfloat16
U32 = jnp.uint32
I32 = jnp.int32

CB = 128
HB = CB // 2
TM = 256
FC = 256
KS = 256
EPS = 1e-5
SCOPES = False
ONLY = os.environ.get('ONLY', '')


def _E(name, default):
    return int(os.environ.get(name, default))


def _dft_consts():
    k = np.arange(CB, dtype=np.float64)[:, None]
    n = np.arange(CB, dtype=np.float64)[None, :]
    th = np.pi * (4.0 * k + 1.0) * n / (2.0 * CB)
    fwd = np.concatenate([np.cos(th), np.sin(th)], axis=0)
    g = np.concatenate([np.cos(th[:HB]), np.sin(th[:HB])], axis=0).T / CB
    inv = np.concatenate([g[0::2], g[1::2], np.zeros((16, CB))], axis=0)
    return jnp.asarray(fwd, dtype=BF16), jnp.asarray(inv, dtype=BF16)


def _pk(x):
    return pltpu.bitcast(x.astype(BF16), U32)


def _unpk(x):
    return pltpu.bitcast(x, BF16)


def _rep(r, n):
    return r if n == 8 else jnp.concatenate([r] * (n // 8), axis=0)


def _add(x, tok):
    return x if tok is None else x + _rep(tok, x.shape[0])


def _costed(pieces, cost):
    for p in pieces:
        p.cost = cost
    return pieces


def _group(pieces, n):
    def merged(ps):
        def run(tok):
            for p in ps:
                p(tok)
        return run
    return [merged(pieces[i:i + n]) for i in range(0, len(pieces), n)]


def _sum(xs):
    return functools.reduce(lambda a, b: a + b, xs)


class _Sched:
    def __init__(self, token):
        self.token = token
        self.clock = 0.0
        self.q = []
        self.last = None
        self.inj = []

    def add(self, pieces, t0, t1):
        cum = np.cumsum([0.0] + [getattr(p, "cost", 1.0) for p in pieces])
        self.q += [(t0 + (t1 - t0) * cum[i] / cum[-1], i, p) for i, p in enumerate(pieces)]
        self.q.sort(key=lambda e: e[:2])

    def note(self, m, dt):
        rows, cols = m.shape
        tiles = [(slice(r, r + 8), slice(c, c + 128)) for c in range(0, cols, 128) for r in range(0, rows, 8)]
        for i, tl in enumerate(tiles):
            tok = None
            while self.q and self.q[0][0] <= self.clock + dt * (i + 1) / len(tiles):
                if tok is None:
                    tok = self.token(m[tl])
                self.q.pop(0)[2](tok)
        self.clock += dt
        self.last = m[tiles[-1]]
        return m

    def dot(self, a, b):
        if self.inj and self.clock >= self.inj[0][0]:
            self.inj.pop(0)[1]()
        m = jnp.dot(a, b, preferred_element_type=F32)
        return self.note(m, max(a.shape[0], 32) * (a.shape[1] // 128) * (b.shape[1] // 128) / 4)

    def flush(self):
        tok = None if self.last is None or not self.q else self.token(self.last)
        while self.q:
            self.q.pop(0)[2](tok)
        self.clock = 0.0
        self.last = None


def _kernel(q_hbm, k_hbm, v_hbm, shk_hbm, ssmk_hbm, ssmd_hbm, wg_hbm, wu_hbm, wd_hbm,
            c_hbm, wmod_hbm, fwd_hbm, inv_hbm, o_hbm,
            u_ref, kk_ref, y_ref, x1_ref, q_ref, k_ref, v_ref, o_ref,
            hp_ref, st_ref, pp_ref, gs_ref, hn_ref, hf_ref, kv_ref, yb_ref, wgf_ref, wuf_ref, wdf_ref,
            ssmk_ref, wmod_ref, wg_ref, wu_ref, wd_ref, fwd_ref, inv_ref,
            mod_ref, sh_ref, zm_ref, shk_ref, ssmd_ref, c_ref,
            sem, *, S, D, Fh):
    NB = S // CB
    NS = S // TM
    NL = D // 128
    NF = Fh // FC
    NT = Fh // 128
    T0 = 3
    NLOOP = NS - T0
    lanes = [slice(i * 128, (i + 1) * 128) for i in range(NL)]
    cat = jnp.concatenate

    offs = [int(o) for o in np.cumsum([0, 5, NS, NS, NS, NL, 3, NF, NF, 1])]
    s_small, s_q, s_k, s_v, s_ssm, s_mod, s_g, s_u, s_d, s_o = offs

    def rows_of(t):
        return pl.ds(t * TM if isinstance(t, int) else pl.multiple_of(t * TM, TM), TM)

    def rows_cp(src, dst, base, t):
        return pltpu.make_async_copy(src.at[rows_of(t), :], dst.at[rows_of(t), :], sem.at[base + t])

    def cols_cp(src, dst, lo, hi, si):
        return pltpu.make_async_copy(src.at[:, lo:hi], dst.at[:, lo:hi], sem.at[si])

    q_cp = lambda t: rows_cp(q_hbm, q_ref, s_q, t)
    k_cp = lambda t: rows_cp(k_hbm, k_ref, s_k, t)
    v_cp = lambda t: rows_cp(v_hbm, v_ref, s_v, t)
    o_cp = lambda t: rows_cp(o_ref, o_hbm, s_o, t)
    small = [pltpu.make_async_copy(s, d, sem.at[s_small + i]) for i, (s, d) in enumerate(
        [(fwd_hbm, fwd_ref), (shk_hbm, shk_ref), (ssmd_hbm, ssmd_ref), (inv_hbm, inv_ref), (c_hbm, c_ref)])]
    ssm_cp = lambda i: pltpu.make_async_copy(ssmk_hbm.at[lanes[i], :], ssmk_ref.at[lanes[i], :],
                                             sem.at[s_ssm + i])
    mod_cols = [(0, 3 * D), (3 * D, 5 * D), (5 * D, 6 * D)]
    mod_cp = lambda i: cols_cp(wmod_hbm, wmod_ref, mod_cols[i][0], mod_cols[i][1], s_mod + i)
    g_cp = lambda f: cols_cp(wg_hbm, wg_ref, f * FC, (f + 1) * FC, s_g + f)
    u_cp = lambda f: cols_cp(wu_hbm, wu_ref, f * FC, (f + 1) * FC, s_u + f)
    d_cp = pltpu.make_async_copy(wd_hbm, wd_ref, sem.at[s_d])

    order = small + [ssm_cp(0), k_cp(0), v_cp(0), k_cp(1), v_cp(1),
                     ssm_cp(1), ssm_cp(2), ssm_cp(3), ssm_cp(4), q_cp(0), q_cp(1),
                     mod_cp(0), mod_cp(1)]
    for f in range(NF):
        order += [g_cp(f), u_cp(f)]
    order += [k_cp(2), v_cp(2), q_cp(2), d_cp, mod_cp(2), k_cp(3), v_cp(3)]
    for t in range(T0, NS):
        order += [q_cp(t)]
        if t + 1 < NS:
            order += [k_cp(t + 1), v_cp(t + 1)]
    for cp in order:
        cp.start()

    zs = []
    bg = _Sched(lambda x: pltpu.bitcast(pltpu.bitcast(x, I32) & zm_ref[...], F32))

    def opaque(ref):
        return ref.at[pl.ds(pl.multiple_of(zs[0], 32), ref.shape[0])]

    def chain(pieces, dist, extra=0, dep=None):
        hist = [] if dep is None else [dep] * dist
        for p in pieces:
            tok = None
            if len(hist) >= dist:
                tok = bg.token(hist[-dist])
                for _ in range(extra):
                    tok = tok + tok
            hist.append(p(tok))
        return hist[-1]

    def linked(pieces, d):
        res = []

        def wrap(p):
            def run(tok):
                if d and len(res) >= d:
                    tok = tok + bg.token(res[-d])
                res.append(p(tok))
            return run
        return [wrap(p) for p in pieces]

    def now(pieces):
        for p in pieces:
            p(None)

    def mod_chunk(i):
        c = c_ref[...].astype(F32)
        sc = jnp.broadcast_to((c * jax.nn.sigmoid(c)).astype(BF16), (16, D))
        lo, hi = mod_cols[i]
        m = bg.dot(sc, wmod_ref[:, lo:hi])[0:8]
        if i == 0:
            ga = m[:, 2 * D:3 * D]
            mod_ref[0] = (1.0 + m[:, D:2 * D]) * ga
            mod_ref[1] = m[:, 0:D] * ga
        elif i == 1:
            mod_ref[2] = 1.0 + m[:, D:2 * D]
            mod_ref[3] = m[:, 0:D]
        else:
            mod_ref[4] = m

    def gb_tile(i):
        def run():
            c = c_ref[...].astype(F32)
            sc = jnp.broadcast_to((c * jax.nn.sigmoid(c)).astype(BF16), (16, D))
            w = wmod_ref[:, 5 * D + i * 128:5 * D + (i + 1) * 128]
            mod_ref[4, :, lanes[i]] = jnp.dot(sc, w, preferred_element_type=F32)[0:8]
            done.add(('gb', i))
        return run

    def k_fwd(i):
        ls = lanes[i]
        fwd = fwd_ref[...]
        prev = None
        for m in range(NB):
            kf = lax.dot_general(fwd, ssmk_ref[ls, m * CB:(m + 1) * CB], (((1,), (1,)), ((), ())),
                                 preferred_element_type=F32)
            if m == 0:
                c = kf[:CB] + ssmd_ref[...].astype(F32).reshape(1, D)[:, ls]
                d = kf[CB:]
            else:
                c = kf[:CB] + prev[CB:]
                d = kf[CB:] - prev[:CB]
            prev = kf
            kk_ref[m, 0:CB, ls] = c
            kk_ref[m, CB:2 * CB, ls] = d - c
            kk_ref[m, 2 * CB:3 * CB, ls] = c + d
            if m % 4 == 3:
                bg.note(kf, 2 * CB)

    def lo_hi(w):
        return pltpu.bitcast(w << 16, F32), pltpu.bitcast(w & jnp.uint32(0xFFFF0000), F32)

    def kv_pieces(t, G=32):
        n = G // 2
        kb, vb = k_ref.at[rows_of(t)], v_ref.at[rows_of(t)]

        def piece(ls, r0):
            def run(tok):
                if r0 > 0:
                    w = pltpu.bitcast(kb[r0 - 16:r0 + G, ls], U32)
                else:
                    if isinstance(t, int) and t == 0:
                        halo = jnp.zeros((8, 128), U32)
                    else:
                        halo = pltpu.bitcast(k_ref.at[rows_of(t - 1)][TM - 16:TM, ls], U32)
                    w = cat([halo, pltpu.bitcast(kb[0:G, ls], U32)], axis=0)
                if tok is not None:
                    w = w | _rep(pltpu.bitcast(tok, U32), n + 8)
                ke, ko = lo_hi(w[8:])
                ke1, ko1 = lo_hi(pltpu.roll(w, 1, 0)[8:])
                _, ko2 = lo_hi(pltpu.roll(w, 2, 0)[8:])
                s0, s1, s2, s3 = [_rep(sh_ref[a, :, ls], n) for a in range(4)]
                ve, vo = lo_hi(pltpu.bitcast(vb[r0:r0 + G, ls], U32))
                kve = ((ke * s0 + ko1 * s1) + (ke1 * s2 + ko2 * s3)) * ve
                kvo = ((ko * s0 + ke * s1) + (ko1 * s2 + ke1 * s3)) * vo
                kv_ref[r0 // 2:(r0 + G) // 2, ls] = pltpu.bitcast(
                    pltpu.pack_elementwise([kve, kvo], packed_dtype=BF16), U32)
            return run
        return _costed([piece(ls, r0) for ls in lanes for r0 in range(0, TM, G)], 2.5 * G + 10)

    def u_fwd(t):
        for b in range(2):
            for ls in lanes:
                kv = lambda: _unpk(kv_ref[b * HB:(b + 1) * HB, ls])
                a = bg.dot(fwd_ref[0:CB, :], kv())
                bb = bg.dot(fwd_ref[CB:2 * CB, :], kv())
                u_ref[t, b, 0:CB, ls] = a + bb
                u_ref[t, b, CB:2 * CB, ls] = a
                u_ref[t, b, 2 * CB:3 * CB, ls] = bb

    positions = [(slice(r0, r0 + 8), ls) for r0 in range(0, 3 * CB, 8) for ls in lanes]

    def ystatic_pieces(blocks, acc_in, pos=None):
        def piece(rs, ls):
            def run(tok):
                us, ks = {}, {}
                for s, lo, hi in blocks:
                    acc = None
                    for i in range(lo, min(hi, s + 1)):
                        if i not in us:
                            us[i] = _add(u_ref[i // 2, i % 2, rs, ls], tok)
                        if s - i not in ks:
                            ks[s - i] = kk_ref[s - i, rs, ls]
                        p = ks[s - i] * us[i]
                        acc = p if acc is None else acc + p
                    if acc_in:
                        acc = acc + y_ref[s // 2, s % 2, rs, ls]
                    y_ref[s // 2, s % 2, rs, ls] = acc
                return acc
            return run
        return _costed([piece(*p) for p in (positions if pos is None else pos)], 35)

    y_first = [(s, 0, 4) for s in range(NB)]

    def task_pieces(t, delta):
        p = t - delta
        left = p >= T0
        J = jnp.where(left, t, p + NLOOP)
        I = jnp.where(left, p, t)
        kview = kk_ref.at[pl.ds(2 * (J - I) - 1, 3)]

        def piece(rs, ls):
            def run(tok):
                u0 = _add(u_ref[I, 0, rs, ls], tok)
                u1 = _add(u_ref[I, 1, rs, ls], tok)
                kc = kview[1, rs, ls]
                y_ref[J, 0, rs, ls] = (kc * u0 + kview[0, rs, ls] * u1) + y_ref[J, 0, rs, ls]
                y1 = (kview[2, rs, ls] * u0 + kc * u1) + y_ref[J, 1, rs, ls]
                y_ref[J, 1, rs, ls] = y1
                return y1
            return run
        return [piece(*p) for p in positions]

    def diag_pieces(t, I):
        kview = kk_ref.at[pl.ds(2 * (t - I) - 1, 3)]

        def piece(rs, ls):
            def run(tok):
                us = [_add(u_ref[a, b, rs, ls], tok) for a in (t, I) for b in range(2)]
                k0 = kk_ref[0, rs, ls]
                kc = kview[1, rs, ls]
                y_ref[t, 0, rs, ls] = ((k0 * us[0] + y_ref[t, 0, rs, ls])
                                       + (kc * us[2] + kview[0, rs, ls] * us[3]))
                y1 = ((kk_ref[1, rs, ls] * us[0] + k0 * us[1])
                      + (kview[2, rs, ls] * us[2] + kc * us[3]) + y_ref[t, 1, rs, ls])
                y_ref[t, 1, rs, ls] = y1
                return y1
            return run
        return [piece(*p) for p in positions]

    def post_pieces(t):
        def piece(b, r0, ls):
            def run(tok):
                comp = lambda c, off: y_ref[t, b, c * CB + off + r0:c * CB + off + r0 + 16, ls]
                k1l, k1h = _add(comp(0, 0), tok), _add(comp(0, HB), tok)
                rel, reh = k1l - comp(2, 0), k1h - comp(2, HB)
                iml, imh = k1l + comp(1, 0), k1h + comp(1, HB)
                p0 = b * CB + r0 // 2
                yb_ref[p0:p0 + 8, ls] = _pk(rel + reh)
                yb_ref[p0 + HB // 2:p0 + HB // 2 + 8, ls] = _pk(iml + imh)
                yb_ref[p0 + HB:p0 + HB + 8, ls] = _pk(rel - reh)
                oim = iml - imh
                yb_ref[p0 + HB + HB // 2:p0 + HB + HB // 2 + 8, ls] = _pk(oim)
                return oim[8:16]
            return run
        return _costed([piece(b, r0, ls) for b in range(2) for r0 in range(0, HB, 16) for ls in lanes], 45)

    def q_split(t, b, p0, n, ls):
        w = pltpu.bitcast(q_ref.at[rows_of(t)][b * CB + 2 * p0:b * CB + 2 * p0 + 2 * n, ls], U32)
        return lo_hi(w)

    def ln_tiles(xs, tok):
        n = xs[0].shape[0]
        s = _add(xs[0], tok)
        for x in xs[1:]:
            s = s + x
        m = jnp.sum(s, axis=-1, keepdims=True) * (1.0 / D)
        xc = [x - m for x in xs]
        s2 = xc[0] * xc[0]
        for x in xc[1:]:
            s2 = s2 + x * x
        r = lax.rsqrt(jnp.sum(s2, axis=-1, keepdims=True) * (1.0 / D) + EPS)
        return xc, jnp.broadcast_to(r, (n, 128)), jnp.broadcast_to(m, (n, 128))

    def ln1_pieces(t):
        G = _E('L1G', 8)

        def piece(b, p0):
            def run(tok):
                xc, r, _ = ln_tiles([cat(q_split(t, b, p0, G, ls), axis=0) for ls in lanes], tok)
                for ls, x in zip(lanes, xc):
                    h = (x * r) * _rep(mod_ref[0, :, ls], 2 * G) + _rep(mod_ref[1, :, ls], 2 * G)
                    hp_ref[b * CB + p0:b * CB + p0 + G, ls] = h[:G]
                    hp_ref[b * CB + HB + p0:b * CB + HB + p0 + G, ls] = h[G:]
                return functools.reduce(lambda a, c: a + c, [h[r:r + 8] for r in range(0, 2 * G, 8)])
            return run
        return [piece(b, p0) for b in range(2) for p0 in range(0, HB, G)]

    def y_inv(t, x1_dst):
        yb = opaque(yb_ref)
        hp = opaque(hp_ref)
        for b in range(2):
            ye = bg.dot(inv_ref[0:HB, :], _unpk(yb[b * CB:b * CB + HB, :]))
            yo = bg.dot(inv_ref[HB:CB, :], _unpk(yb[b * CB + HB:(b + 1) * CB, :]))
            for ls in lanes:
                qe, qo = q_split(t, b, 0, HB, ls)
                re, ro = slice(b * CB, b * CB + HB), slice(b * CB + HB, (b + 1) * CB)
                x1_dst[re, ls] = qe + hp[re, ls] * ye[:, ls]
                x1_dst[ro, ls] = qo + hp[ro, ls] * yo[:, ls]

    def ln2_stat_pieces(x1_src, st):
        x1o = opaque(x1_src)

        def piece(r0):
            def run(tok):
                _, r, m = ln_tiles([x1o[r0:r0 + 16, ls] for ls in lanes], tok)
                st[r0:r0 + 16, 0:128] = m
                st[r0:r0 + 16, 128:256] = r
                return r[0:8] + r[8:16]
            return run
        return [piece(h * CB + r0) for r0 in range(0, CB, 16) for h in range(2)]

    tile = lambda j: slice(j * 128, (j + 1) * 128)
    LX, RX = 0, 1
    Lc = lambda i: 2 + 2 * i
    Rc = lambda i: 3 + 2 * i
    others = lambda i: [j for j in range(NL) if j != i]
    edges = [(i, j) for i in range(NL) for j in others(i)]
    pairs = [(i, j) for i, j in edges if i < j]
    a_idx = {k: n for n, k in enumerate(
        [(c, i) for c in "xyw" for i in range(NL)] + [("s",) + e for e in edges]
        + [(c,) + e for c in ("dx", "dy") for e in pairs])}
    b_terms = {}
    for i in range(NL):
        b_terms["D1", i] = [(1, k, Lc(i)) for k in range(NL)]
        b_terms["D2", i] = [(1, i, Lc(i))] + [(-1, i, Rc(j)) for j in others(i)]
        b_terms["D3", i] = [(1, i, Rc(i))] + [(-1, i, Lc(j)) for j in others(i)]
        b_terms["D4", i] = [(1, k, Rc(i)) for k in range(NL)]
    for i, j in edges:
        sg = 1 if i < j else -1
        b_terms["E1", i, j] = [(1, i, Rc(j)), (1, j, Lc(i))]
        b_terms["E2", i, j] = [(sg, j, Lc(i))]
        b_terms["E3", i, j] = [(sg, i, Rc(j))]
    xpairs = [(0, 1), (2, 3)]
    for i, j in xpairs:
        b_terms["d1", i] = [(1, i, LX), (1, j, LX)]
        b_terms["d2", i] = [(1, i, LX), (-1, i, RX)]
        b_terms["d3", j] = [(1, j, RX), (-1, j, LX)]
        b_terms["d4", j] = [(1, j, RX), (1, i, RX)]
        b_terms["e1", i, j] = [(1, i, RX), (1, j, LX)]
        b_terms["e2", i, j] = [(1, j, LX)]
        b_terms["e3", i, j] = [(1, i, RX)]
    b_terms["pl",] = [(1, NL - 1, LX)]
    b_terms["pr",] = [(1, NL - 1, RX)]
    b_idx = {k: n for n, k in enumerate(b_terms)}
    w_refs = ((wg_ref, wgf_ref), (wu_ref, wuf_ref), (wd_ref, wdf_ref))
    done = set()
    check = [True]

    def norm_pieces(x1_src, st, unit, more=True):
        G = 16
        x1o = opaque(x1_src)

        def piece(r0, js):
            def run(tok):
                two = lambda ref, c: cat([ref[r0:r0 + G, c], ref[CB + r0:CB + r0 + G, c]], axis=0)
                m, r = _add(two(st, slice(0, 128)), tok), two(st, slice(128, 256))
                for j in js:
                    ls = lanes[j]
                    h = ((two(x1o, ls) - m) * r) * _rep(mod_ref[2, :, ls], 2 * G) + _rep(mod_ref[3, :, ls], 2 * G)
                    put_a(unit, r0, ("x", j), h[:G])
                    put_a(unit, r0, ("y", j), h[G:])
                    if more:
                        put_a(unit, r0, ("w", j), h[:G] + h[G:])
                        hn_ref[r0:r0 + G, ls] = h[:G]
                        hn_ref[CB + r0:CB + r0 + G, ls] = h[G:]
            return run
        return [_costed([piece(r0, js)], 32 * len(js))[0] for r0 in range(0, CB, G) for js in ([0, 1, 2], [3, 4])]

    def put_a(unit, r0, key, v):
        p0 = a_idx[key] * HB + r0 // 2
        hf_ref[p0:p0 + v.shape[0] // 2, lanes[unit]] = _pk(v)
        done.add(("a", unit, key, r0))

    def pair_pieces(unit):
        G = 16

        def piece(r0, i, j):
            def run(tok):
                assert ("a", unit, ("w", j), r0) in done
                ld = lambda h, k: hn_ref[h * CB + r0:h * CB + r0 + G, lanes[k]]
                xi, yi, xj, yj = _add(ld(0, i), tok), _add(ld(1, i), tok), ld(0, j), ld(1, j)
                put_a(unit, r0, ("s", i, j), xi + yj)
                put_a(unit, r0, ("s", j, i), xj + yi)
                put_a(unit, r0, ("dx", i, j), xj - xi)
                put_a(unit, r0, ("dy", i, j), yi - yj)
            return run
        return _costed([piece(r0, i, j) for r0 in range(0, CB, G) for i, j in pairs], 30)

    def w_pieces(w, groups):
        src, dst = w_refs[w]

        def piece(keys, r0, G):
            def run(tok):
                blk = {}

                def ld(k, c):
                    if (k, c) not in blk:
                        rt, ct = (k, c) if w < 2 else (c, k)
                        v = src[rt * 128 + r0:rt * 128 + r0 + G, tile(ct)].astype(F32)
                        blk[k, c] = _add(v, tok) if len(blk) < 2 else v
                    return blk[k, c]
                for key in keys:
                    acc = None
                    for sg, k, c in b_terms[key]:
                        v = ld(k, c)
                        acc = (v if sg > 0 else -v) if acc is None else (acc + v if sg > 0 else acc - v)
                    p0 = (b_idx[key] // 2) * HB + r0 // 2
                    dst[p0:p0 + G // 2, tile(b_idx[key] % 2)] = _pk(acc)
                    done.add(("b", w, key, r0 + G))
            return run
        out = []
        for keys in groups:
            G = 16 if len(keys) > 3 else 32
            n = len({t[1:] for k in keys for t in b_terms[k]})
            out += _costed([piece(keys, r0, G) for r0 in range(0, CB, G)], (3 * n + len(keys) + 2) * G / 8)
        return out

    g_edge = lambda i, j: [("E1", i, j), ("E2", i, j), ("E3", i, j)]
    g_left = [[("e1", i, j), ("e2", i, j), ("e3", i, j), ("d1", i), ("d2", i), ("d3", j), ("d4", j)]
              for i, j in xpairs] + [[("pl",), ("pr",)]]
    g_cols = lambda m: ([[("D1", m)], [("D4", m)]] + [g_edge(i, m) for i in range(m)]
                        + [g_edge(m, j) for j in range(m)])
    g_rows = [[(d, i)] for i in range(NL) for d in ("D2", "D3")]

    def rhs(w, key):
        assert not check[0] or ("b", w, key, CB) in done, (w, key)
        return _unpk(w_refs[w][1][(b_idx[key] // 2) * HB:(b_idx[key] // 2 + 1) * HB, tile(b_idx[key] % 2)])

    def lhs(unit, key, p0, n):
        assert not check[0] or all(("a", unit, key, r) in done for r in range(2 * p0, 2 * (p0 + n), 16)), key
        return _unpk(hf_ref[a_idx[key] * HB + p0:a_idx[key] * HB + p0 + n, lanes[unit]])

    def gu_plain(c, unit):
        for h in range(2):
            x = lambda: cat([lhs(unit, ("xy"[h], k), 0, HB) for k in range(NL)], axis=1)
            p = bg.dot(x(), wg_ref[:, tile(c)]) * bg.dot(x(), wu_ref[:, tile(c)])
            pp_ref[unit * TM + h * CB:unit * TM + (h + 1) * CB, tile(c)] = p

    def gu_finish(w, unit, p0, n, c, v):
        for h in range(2):
            r = h * CB + 2 * p0
            if w == 0:
                gs_ref[r:r + 2 * n, tile(c)] = v[h]
            else:
                pp_ref[unit * TM + r:unit * TM + r + 2 * n, tile(c)] = gs_ref[r:r + 2 * n, tile(c)] * v[h]

    def gu_main(w, unit, p0, n, rows=range(NL)):
        dot = lambda a, b: bg.dot(lhs(unit, a, p0, n), rhs(w, b))
        run_ref, off = (gs_ref, 0) if w == 0 else (pp_ref, unit * TM)
        for i in rows:
            p = q = None
            for d in range(1, NL):
                j = (i + d) % NL
                lo, hi = min(i, j), max(i, j)
                e1 = dot(("s", i, j), ("E1", i, j))
                e2 = dot(("dx", lo, hi), ("E2", i, j))
                e3 = dot(("dy", lo, hi), ("E3", i, j))
                p = e2 if p is None else p + e2
                q = e1 + e3 if q is None else (q + e1) + e3
                rp, rq = e1 + e2, e3
                if d == 1:
                    x = dot(("x", i), ("D1", i))
                    p, q = p + x, q - x
                elif d == 2:
                    q = q + dot(("w", i), ("D2", i))
                elif d == 3:
                    rp = rp + dot(("w", j), ("D3", j))
                else:
                    x = dot(("y", j), ("D4", j))
                    rp, rq = rp - x, rq + x
                rs = [slice(off + h * CB + 2 * p0, off + h * CB + 2 * (p0 + n)) for h in range(2)]
                if i != others(j)[0]:
                    rp, rq = rp + run_ref[rs[0], tile(Rc(j))], rq + run_ref[rs[1], tile(Rc(j))]
                if i == others(j)[-1]:
                    gu_finish(w, unit, p0, n, Rc(j), (rp, rq))
                else:
                    run_ref[rs[0], tile(Rc(j))] = rp
                    run_ref[rs[1], tile(Rc(j))] = rq
            gu_finish(w, unit, p0, n, Lc(i), (p, q))

    def gu_left(w, unit, p0, n):
        def dot(f, extra=()):
            ks = [f(i, j) for i, j in xpairs] + list(extra)
            return bg.dot(cat([lhs(unit, a, p0, n) for a, _ in ks], axis=1), cat([rhs(w, b) for _, b in ks], axis=0))
        one = lambda a, b: bg.dot(lhs(unit, (a, NL - 1), p0, n), rhs(w, (b,)))
        e1 = dot(lambda i, j: (("s", i, j), ("e1", i, j)))
        e2 = dot(lambda i, j: (("dx", i, j), ("e2", i, j)))
        e3 = dot(lambda i, j: (("dy", i, j), ("e3", i, j)))
        d1 = dot(lambda i, j: (("x", i), ("d1", i)))
        pl_, ql, pr = e2 + d1, (e1 + e3) - d1, e1 + e2
        ql = ql + dot(lambda i, j: (("w", i), ("d2", i)), [(("y", NL - 1), ("pl",))])
        gu_finish(w, unit, p0, n, LX, (pl_ + one("x", "pl"), ql))
        d4 = dot(lambda i, j: (("y", j), ("d4", j)))
        pr = (pr - d4) + dot(lambda i, j: (("w", j), ("d3", j)), [(("x", NL - 1), ("pr",))])
        gu_finish(w, unit, p0, n, RX, (pr, (e3 + d4) + one("y", "pr")))

    def gu_fast(unit, n, left=True, mid=None):
        k = 0
        for p0 in range(0, HB, n):
            for w in range(2):
                if mid is not None and mid[0] == k:
                    mid[1]()
                k += 1
                if left and w == 1:
                    gu_left(w, unit, p0, n)
                gu_main(w, unit, p0, n)
                if left and w == 0:
                    gu_left(w, unit, p0, n)

    def ffn_down(x1_src, t, unit, mid=None, e=_E('DSUB', 32)):
        ob = o_ref.at[rows_of(t)]
        k = 0
        for r0 in range(0, HB, e):
            rows = lambda ref, base, c: cat([ref[base + o + r0:base + o + r0 + e, c] for o in (0, HB)], axis=0)
            hx = lambda c: rows(pp_ref, unit * TM, tile(c))
            hy = lambda c: rows(pp_ref, unit * TM + CB, tile(c))
            run = lambda h: slice(h * CB + 2 * r0, h * CB + 2 * (r0 + e))

            def left(key):
                kind = key[0]
                if kind[0] in "Ee":
                    l, r = (Lc(key[1]), Rc(key[2])) if kind[0] == "E" else (LX, RX)
                    return (hy if kind[1] == "3" else hx)(r) + (hx if kind[1] == "2" else hy)(l)
                if kind[1] in "12":
                    c = Lc(key[1]) if kind[0] == "D" else LX
                    return hx(c) - hy(c) if kind[1] == "1" else hy(c)
                c = Rc(key[1]) if kind[0] == "D" else RX
                return hx(c) if kind[1] == "3" else hy(c) - hx(c)

            def dot(keys, plain=None):
                keys = [kk for kk in keys if kk in b_terms]
                a = [left(kk) for kk in keys]
                if plain is not None:
                    a, keys = a + [plain(LX), plain(RX)], keys + [("pl",), ("pr",)]
                a, w = cat(a, axis=1), (lambda: cat([rhs(2, kk) for kk in keys], axis=0))
                if plain is not None and e == HB:
                    return cat([bg.dot(a[r:r + HB].astype(BF16), w()) for r in (0, HB)], axis=0)
                return bg.dot(a.astype(BF16), w())

            for i in range(NL):
                ls = lanes[i]
                last = i == NL - 1
                both = dot([("D2", i), ("D3", i), ("d2", i), ("d3", i)])
                p = both + dot([("D1", i), ("d1", i)], hx if last else None)
                q = both + dot([("D4", i), ("d4", i)], hy if last else None)
                if i > 0:
                    p, q = p + gs_ref[run(0), ls], q + gs_ref[run(1), ls]
                for j in range(i + 1, NL):
                    a = dot([("E1", i, j), ("e1", i, j)])
                    c3 = dot([("E3", i, j), ("E3", j, i), ("e3", i, j)])
                    rq = a - c3
                    gs_ref[run(1), lanes[j]] = rq + gs_ref[run(1), lanes[j]] if i > 0 else rq
                    b = dot([("E1", j, i)])
                    c2 = dot([("E2", i, j), ("E2", j, i), ("e2", i, j)])
                    rp = b + c2
                    gs_ref[run(0), lanes[j]] = rp + gs_ref[run(0), lanes[j]] if i > 0 else rp
                    p, q = (p + a) - c2, (q + c3) + b
                assert not check[0] or ('gb', i) in done
                for b, dn in enumerate((p, q)):
                    o = rows(x1_src, b * CB, ls) + _rep(mod_ref[4, :, ls], 2 * e) * dn
                    w = pltpu.pack_elementwise([o[:e], o[e:]], packed_dtype=BF16)
                    ob[run(b), ls] = pltpu.bitcast(w, BF16)
                k += 1
                if mid is not None and k == mid[0] * (HB // e) + (NL - mid[0]) * (HB // e - 1) * mid[2]:
                    mid[1]()

    x1s = [x1_ref.at[r] for r in range(NS)]
    sts = [st_ref.at[r * TM:(r + 1) * TM] for r in range(2)]
    YP = _E('YP', 12)

    def setup():
        for cp in small:
            cp.wait()
        shk = shk_ref[...].astype(F32)
        for a in range(4):
            sh_ref[a] = jnp.broadcast_to(shk[a:a + 1, :], (8, D))
        zm_ref[...] = pltpu.bitcast(inv_ref[CB:CB + 16, :], I32)
        zs.append(zm_ref[0, 0])

    def prologue():
        ytile = lambda i: ystatic_pieces(y_first, False, [p for p in positions if p[1] == lanes[i]])
        ssm_cp(0).wait()
        k_fwd(0)
        for t in range(2):
            k_cp(t).wait()
            v_cp(t).wait()
            now(kv_pieces(t, 64))
            u_fwd(t)
        bg.flush()
        for i in range(1, NL):
            if i != 3:
                ssm_cp(i).wait()
            if i == 2:
                ssm_cp(3).wait()
            bg.add(ytile(i - 1), 0, 1024)
            k_fwd(i)
            bg.flush()
        q_cp(0).wait()
        now(ytile(NL - 1))
        q_cp(1).wait()
        mod_cp(0).wait()
        mod_chunk(0)
        for t in range(2):
            now(post_pieces(t))
            now(ln1_pieces(t))
            y_inv(t, x1s[t])
        for t in range(2):
            now(ln2_stat_pieces(x1s[t], sts[t]))
        bg.flush()

    def superstep():
        wp = lambda groups: w_pieces(0, groups) + w_pieces(1, groups)

        def wait_gu(*fs):
            for f in fs:
                g_cp(f).wait()
                u_cp(f).wait()

        mod_cp(1).wait()
        mod_chunk(1)
        now(norm_pieces(x1s[0], sts[0], 0, more=False))
        bg.flush()
        wait_gu(0)
        bg.add(norm_pieces(x1s[1], sts[1], 1), 0, 900)
        bg.add(pair_pieces(1) + wp(g_left), 900, 2400)
        for u in range(2):
            gu_plain(0, u)
            gu_plain(1, u)
        bg.flush()
        wait_gu(1, 2)
        bg.add(wp(g_cols(0) + g_cols(1)), 0, 2400)
        for c in range(2, 6):
            gu_plain(c, 0)
        bg.flush()
        wait_gu(3, 4)
        bg.add(wp(g_cols(2) + g_cols(3)), 0, 2400)
        for c in range(6, 10):
            gu_plain(c, 0)
        bg.flush()
        wait_gu(5)
        k_cp(2).wait()
        v_cp(2).wait()
        bg.add(w_pieces(0, g_cols(4) + g_rows), 0, 1200)
        bg.add(kv_pieces(2) + w_pieces(1, g_cols(4) + g_rows), 1200, 3700)
        gu_plain(10, 0)
        gu_plain(11, 0)
        gu_main(0, 1, 0, HB)
        bg.flush()
        q_cp(2).wait()
        d_cp.wait()
        order_d = g_left + [g for i in range(NL) for g in (
            [[(d, i)] for d in ("D2", "D3", "D1", "D4")]
            + [g for j in range(i + 1, NL) for g in (g_edge(i, j), g_edge(j, i))])]
        wdp = w_pieces(2, order_d)
        nd = _E('ND', 100)
        ymid = _costed(_group(ystatic_pieces([(s, 4, 6) for s in (4, 5)], True), 2), 35)
        bg.add(wdp[:nd] + ymid, 600, 3050)
        u_fwd(2)
        gu_main(1, 1, 0, HB)
        bg.flush()
        mod_cp(2).wait()
        k_cp(3).wait()
        v_cp(3).wait()
        bg.add(wdp[nd:] + post_pieces(2) + kv_pieces(3), 0, 3300)
        bg.add(linked(ln1_pieces(2), 3), 0, 2500)
        bg.inj = [(100 + 130 * i, gb_tile(i)) for i in range(NL)]
        ffn_down(x1s[0], 0, 0, e=HB)
        y_inv(2, x1s[2])
        bg.flush()
        o_cp(0).start()

    def run_super(fn):
        if _E('SL', 1):
            def body(i, carry):
                fn()
                return carry
            lax.fori_loop(0, zs[0] + 1, body, 0)
        else:
            fn()

    def step(t, carry):
        q_cp(t).wait()

        @pl.when(t + 1 < NS)
        def _():
            k_cp(t + 1).wait()
            v_cp(t + 1).wait()

        x1v = x1_ref.at[pl.ds(t - 2, 3)]
        x1 = x1v.at[2]
        bg.add(linked(ln1_pieces(t), _E('LK1', 2)), _E('L0', 4000), _E('L1', 8500))
        bg.add(ln2_stat_pieces(x1v.at[1], st_ref), 0, _E('S1', 600))
        bg.add(norm_pieces(x1v.at[1], st_ref, 1), _E('P0', 1000), _E('P1', 2000))
        bg.add(pair_pieces(1), _E('P1', 2000), _E('P2', 3100))
        bg.add(kv_pieces(jnp.minimum(t + 1, NS - 1), 16), _E('K0', 4000), _E('K1', 10100))

        def conv():
            u_fwd(t)
            chain(diag_pieces(t, T0 - 1), _E('DD', 2), _E('DE', 0))
            chain(task_pieces(t, 2), _E('MD', 3), _E('ME', 0))
            dep = chain(task_pieces(t, 1), _E('MD', 3), _E('ME', 0))
            chain(post_pieces(t), 1, 3, dep)

        if _E('FP', 5) == 0:
            conv()
        ffn_down(x1v.at[0], t - 2, 1, mid=(_E('FP', 5), conv, 0))
        sub = _E('SUB', HB)
        if sub == HB:
            iv = _E('IV', 5)
            gu_main(0, 1, 0, HB)
            gu_left(0, 1, 0, HB)
            gu_left(1, 1, 0, HB)
            gu_main(1, 1, 0, HB, range(iv))
            y_inv(t, x1)
            gu_main(1, 1, 0, HB, range(iv, NL))
        else:
            gu_fast(1, sub, mid=(3, lambda: y_inv(t, x1)))
        bg.flush()
        o_cp(t - 2).start()
        return carry

    def epilogue():
        t = NS - 1
        bg.add(ln2_stat_pieces(x1s[t], st_ref), 0, 500)
        bg.add(norm_pieces(x1s[t], st_ref, 1), 900, 1800)
        bg.add(pair_pieces(1), 1800, 2950)
        ffn_down(x1s[t - 1], t - 1, 1)
        o_cp(t - 1).start()
        gu_fast(1, _E('SUB', HB))
        last = [pltpu.make_async_copy(o_ref.at[rows_of(t), lo:hi], o_hbm.at[rows_of(t), lo:hi], sem.at[s_o + t + i])
                for i, (lo, hi) in enumerate([(0, 384), (384, D)])]
        ffn_down(x1s[t], t, 1, mid=(3, last[0].start, 1))
        last[1].start()
        for i in range(NS - 1):
            o_cp(i).wait()
        for cp in last:
            cp.wait()

    sc = jax.named_scope if SCOPES else (lambda name: (lambda f: f))

    def rest():
        sc("superstep")(superstep)()
        lax.fori_loop(T0, NS, sc("step")(step), 0)
        sc("epilogue")(epilogue)()

    if ONLY == 'loop':
        check[0] = False
        zs.append(zm_ref[0, 0])
        lax.fori_loop(T0, NS, step, 0)
        epilogue()
    elif ONLY == 'S':
        zs.append(zm_ref[0, 0])
        run_super(superstep)
        lax.fori_loop(T0, NS, step, 0)
    elif _E('NEST', 3) == 3:
        setup()

        def everything():
            sc("prologue")(prologue)()
            rest()
        run_super(everything)
    else:
        setup()
        sc("prologue")(prologue)()
        run_super(rest)


@jax.jit
def pallas_adaLN_cond__ssm_conv_h3__glu_gated_bilinear__prompt_kernel(
    A_q, A_k, A_v, A_shift_k, A_ssm_k, A_ssm_D, B_x, B_w_gate, B_w_up, B_w_down, c, w_mod,
):
    B, S, D = A_q.shape
    Fh = B_w_gate.shape[1]
    NB = S // CB
    NS = S // TM
    fwd, inv = _dft_consts()
    anyspec = pl.BlockSpec(memory_space=pl.ANY)
    V = pltpu.VMEM
    out = pl.pallas_call(
        functools.partial(_kernel, S=S, D=D, Fh=Fh),
        in_specs=[anyspec] * 13,
        out_specs=anyspec,
        out_shape=jax.ShapeDtypeStruct((S, D), A_q.dtype),
        scratch_shapes=[
            V((NS, 2, 3 * CB, D), F32),
            V((NB, 3 * CB, D), F32),
            V((NS, 2, 3 * CB, D), F32),
            V((NS, TM, D), F32),
            V((S, D), BF16), V((S, D), BF16), V((S, D), BF16), V((S, D), BF16),
            V((TM, D), F32),
            V((2 * TM, 256), F32),
            V((2 * TM, Fh), F32),
            V((TM, Fh), F32),
            V((TM, D), F32),
            V((55 * HB, 256), U32),
            V((TM // 2, D), U32),
            V((2 * CB, D), U32),
            V((48 * HB, 256), U32), V((48 * HB, 256), U32), V((48 * HB, 256), U32),
            V((D, S), BF16), V((D, 6 * D), BF16), V((D, Fh), BF16), V((D, Fh), BF16), V((Fh, D), BF16),
            V((2 * CB, CB), BF16), V((CB + 16, CB), BF16),
            V((5, 8, D), F32), V((4, 8, D), F32), V((8, 128), I32),
            V((4, D), BF16), V((D,), BF16), V((1, D), BF16),
            pltpu.SemaphoreType.DMA((5 + 4 * NS + D // 128 + 3 + 2 * (Fh // FC) + 2,)),
        ],
        compiler_params=pltpu.CompilerParams(
            internal_scratch_in_bytes=48 * 1024,
            disable_semaphore_checks=True,
            disable_bounds_checks=True,
            vmem_limit_bytes=110 * 1024 * 1024),
        name="adaln_h3_glu",
    )(A_q.reshape(S, D), A_k.reshape(S, D), A_v.reshape(S, D), A_shift_k.T, A_ssm_k,
      A_ssm_D, B_w_gate, B_w_up, B_w_down, c, w_mod, fwd, inv)
    return out.reshape(B, S, D)
```

```python
import functools
import os

import numpy as np
import jax
import jax.numpy as jnp
from jax import lax
import jax.experimental.pallas as pl
import jax.experimental.pallas.tpu as pltpu

F32 = jnp.float32
BF16 = jnp.bfloat16
U32 = jnp.uint32
I32 = jnp.int32

CB = 128
HB = CB // 2
TM = 256
FC = 256
KS = 256
EPS = 1e-5
SCOPES = False
ONLY = os.environ.get('ONLY', '')


def _E(name, default):
    return int(os.environ.get(name, default))


def _dft_consts():
    k = np.arange(CB, dtype=np.float64)[:, None]
    n = np.arange(CB, dtype=np.float64)[None, :]
    th = np.pi * (4.0 * k + 1.0) * n / (2.0 * CB)
    fwd = np.concatenate([np.cos(th), np.sin(th)], axis=0)
    g = np.concatenate([np.cos(th[:HB]), np.sin(th[:HB])], axis=0).T / CB
    inv = np.concatenate([g[0::2], g[1::2], np.zeros((16, CB))], axis=0)
    return jnp.asarray(fwd, dtype=BF16), jnp.asarray(inv, dtype=BF16)


def _pk(x):
    return pltpu.bitcast(x.astype(BF16), U32)


def _unpk(x):
    return pltpu.bitcast(x, BF16)


def _rep(r, n):
    return r if n == 8 else jnp.concatenate([r] * (n // 8), axis=0)


def _add(x, tok):
    return x if tok is None else x + _rep(tok, x.shape[0])


def _costed(pieces, cost):
    for p in pieces:
        p.cost = cost
    return pieces


def _group(pieces, n):
    def merged(ps):
        def run(tok):
            for p in ps:
                p(tok)
        return run
    return [merged(pieces[i:i + n]) for i in range(0, len(pieces), n)]


def _sum(xs):
    return functools.reduce(lambda a, b: a + b, xs)


class _Sched:
    def __init__(self, token):
        self.token = token
        self.clock = 0.0
        self.q = []
        self.last = None
        self.inj = []

    def add(self, pieces, t0, t1):
        cum = np.cumsum([0.0] + [getattr(p, "cost", 1.0) for p in pieces])
        self.q += [(t0 + (t1 - t0) * cum[i] / cum[-1], i, p) for i, p in enumerate(pieces)]
        self.q.sort(key=lambda e: e[:2])

    def note(self, m, dt):
        rows, cols = m.shape
        tiles = [(slice(r, r + 8), slice(c, c + 128)) for c in range(0, cols, 128) for r in range(0, rows, 8)]
        for i, tl in enumerate(tiles):
            tok = None
            while self.q and self.q[0][0] <= self.clock + dt * (i + 1) / len(tiles):
                if tok is None:
                    tok = self.token(m[tl])
                self.q.pop(0)[2](tok)
        self.clock += dt
        self.last = m[tiles[-1]]
        return m

    def dot(self, a, b):
        if self.inj and self.clock >= self.inj[0][0]:
            self.inj.pop(0)[1]()
        m = jnp.dot(a, b, preferred_element_type=F32)
        return self.note(m, max(a.shape[0], 32) * (a.shape[1] // 128) * (b.shape[1] // 128) / 4)

    def flush(self):
        tok = None if self.last is None or not self.q else self.token(self.last)
        while self.q:
            self.q.pop(0)[2](tok)
        self.clock = 0.0
        self.last = None


def _kernel(q_hbm, k_hbm, v_hbm, shk_hbm, ssmk_hbm, ssmd_hbm, wg_hbm, wu_hbm, wd_hbm,
            c_hbm, wmod_hbm, fwd_hbm, inv_hbm, o_hbm,
            u_ref, kk_ref, y_ref, x1_ref, q_ref, k_ref, v_ref, o_ref,
            hp_ref, st_ref, pp_ref, gs_ref, hn_ref, hf_ref, kv_ref, yb_ref, wgf_ref, wuf_ref, wdf_ref,
            ssmk_ref, wmod_ref, wg_ref, wu_ref, wd_ref, fwd_ref, inv_ref,
            mod_ref, sh_ref, zm_ref, shk_ref, ssmd_ref, c_ref,
            sem, *, S, D, Fh):
    NB = S // CB
    NS = S // TM
    NL = D // 128
    NF = Fh // FC
    NT = Fh // 128
    T0 = 3
    NLOOP = NS - T0
    lanes = [slice(i * 128, (i + 1) * 128) for i in range(NL)]
    cat = jnp.concatenate

    offs = [int(o) for o in np.cumsum([0, 5, NS, NS, NS, NL, 3, NF, NF, 1])]
    s_small, s_q, s_k, s_v, s_ssm, s_mod, s_g, s_u, s_d, s_o = offs

    def rows_of(t):
        return pl.ds(t * TM if isinstance(t, int) else pl.multiple_of(t * TM, TM), TM)

    def rows_cp(src, dst, base, t):
        return pltpu.make_async_copy(src.at[rows_of(t), :], dst.at[rows_of(t), :], sem.at[base + t])

    def cols_cp(src, dst, lo, hi, si):
        return pltpu.make_async_copy(src.at[:, lo:hi], dst.at[:, lo:hi], sem.at[si])

    q_cp = lambda t: rows_cp(q_hbm, q_ref, s_q, t)
    k_cp = lambda t: rows_cp(k_hbm, k_ref, s_k, t)
    v_cp = lambda t: rows_cp(v_hbm, v_ref, s_v, t)
    o_cp = lambda t: rows_cp(o_ref, o_hbm, s_o, t)
    small = [pltpu.make_async_copy(s, d, sem.at[s_small + i]) for i, (s, d) in enumerate(
        [(fwd_hbm, fwd_ref), (shk_hbm, shk_ref), (ssmd_hbm, ssmd_ref), (inv_hbm, inv_ref), (c_hbm, c_ref)])]
    ssm_cp = lambda i: pltpu.make_async_copy(ssmk_hbm.at[lanes[i], :], ssmk_ref.at[lanes[i], :],
                                             sem.at[s_ssm + i])
    mod_cols = [(0, 3 * D), (3 * D, 5 * D), (5 * D, 6 * D)]
    mod_cp = lambda i: cols_cp(wmod_hbm, wmod_ref, mod_cols[i][0], mod_cols[i][1], s_mod + i)
    g_cp = lambda f: cols_cp(wg_hbm, wg_ref, f * FC, (f + 1) * FC, s_g + f)
    u_cp = lambda f: cols_cp(wu_hbm, wu_ref, f * FC, (f + 1) * FC, s_u + f)
    d_cp = pltpu.make_async_copy(wd_hbm, wd_ref, sem.at[s_d])

    order = small + [ssm_cp(0), k_cp(0), v_cp(0), k_cp(1), v_cp(1),
                     ssm_cp(1), ssm_cp(2), ssm_cp(3), ssm_cp(4), q_cp(0), q_cp(1),
                     mod_cp(0), mod_cp(1)]
    for f in range(NF):
        order += [g_cp(f), u_cp(f)]
        if f == 2:
            order += [k_cp(2), v_cp(2)]
    order += [q_cp(2), d_cp, mod_cp(2), k_cp(3), v_cp(3)]
    for t in range(T0, NS):
        order += [q_cp(t)]
        if t + 1 < NS:
            order += [k_cp(t + 1), v_cp(t + 1)]
    for cp in order:
        cp.start()

    zs = []
    bg = _Sched(lambda x: pltpu.bitcast(pltpu.bitcast(x, I32) & zm_ref[...], F32))

    def opaque(ref):
        return ref.at[pl.ds(pl.multiple_of(zs[0], 32), ref.shape[0])]

    def chain(pieces, dist, extra=0, dep=None):
        hist = [] if dep is None else [dep] * dist
        for p in pieces:
            tok = None
            if len(hist) >= dist:
                tok = bg.token(hist[-dist])
                for _ in range(extra):
                    tok = tok + tok
            hist.append(p(tok))
        return hist[-1]

    def linked(pieces, d):
        res = []

        def wrap(p):
            def run(tok):
                if d and len(res) >= d:
                    tok = tok + bg.token(res[-d])
                res.append(p(tok))
            return run
        return [wrap(p) for p in pieces]

    def now(pieces):
        for p in pieces:
            p(None)

    def mod_chunk(i):
        c = c_ref[...].astype(F32)
        sc = jnp.broadcast_to((c * jax.nn.sigmoid(c)).astype(BF16), (16, D))
        lo, hi = mod_cols[i]
        m = bg.dot(sc, wmod_ref[:, lo:hi])[0:8]
        if i == 0:
            ga = m[:, 2 * D:3 * D]
            mod_ref[0] = (1.0 + m[:, D:2 * D]) * ga
            mod_ref[1] = m[:, 0:D] * ga
        elif i == 1:
            mod_ref[2] = 1.0 + m[:, D:2 * D]
            mod_ref[3] = m[:, 0:D]
        else:
            mod_ref[4] = m

    def gb_tile(i):
        def run():
            c = c_ref[...].astype(F32)
            sc = jnp.broadcast_to((c * jax.nn.sigmoid(c)).astype(BF16), (16, D))
            w = wmod_ref[:, 5 * D + i * 128:5 * D + (i + 1) * 128]
            mod_ref[4, :, lanes[i]] = jnp.dot(sc, w, preferred_element_type=F32)[0:8]
            done.add(('gb', i))
        return run

    def k_fwd(i):
        ls = lanes[i]
        fwd = fwd_ref[...]
        prev = None
        for m in range(NB):
            kf = lax.dot_general(fwd, ssmk_ref[ls, m * CB:(m + 1) * CB], (((1,), (1,)), ((), ())),
                                 preferred_element_type=F32)
            if m == 0:
                c = kf[:CB] + ssmd_ref[...].astype(F32).reshape(1, D)[:, ls]
                d = kf[CB:]
            else:
                c = kf[:CB] + prev[CB:]
                d = kf[CB:] - prev[:CB]
            prev = kf
            kk_ref[m, 0:CB, ls] = c
            kk_ref[m, CB:2 * CB, ls] = d - c
            kk_ref[m, 2 * CB:3 * CB, ls] = c + d
            if m % 4 == 3:
                bg.note(kf, 2 * CB)

    def lo_hi(w):
        return pltpu.bitcast(w << 16, F32), pltpu.bitcast(w & jnp.uint32(0xFFFF0000), F32)

    kv_live = set()

    def kv_pieces(t, G=32):
        n = G // 2
        kb, vb = k_ref.at[rows_of(t)], v_ref.at[rows_of(t)]

        def piece(ls, r0):
            def run(tok):
                assert (r0 // CB, ls.start) not in kv_live
                if r0 > 0:
                    w = pltpu.bitcast(kb[r0 - 16:r0 + G, ls], U32)
                else:
                    if isinstance(t, int) and t == 0:
                        halo = jnp.zeros((8, 128), U32)
                    else:
                        halo = pltpu.bitcast(k_ref.at[rows_of(t - 1)][TM - 16:TM, ls], U32)
                    w = cat([halo, pltpu.bitcast(kb[0:G, ls], U32)], axis=0)
                if tok is not None:
                    w = w | _rep(pltpu.bitcast(tok, U32), n + 8)
                ke, ko = lo_hi(w[8:])
                ke1, ko1 = lo_hi(pltpu.roll(w, 1, 0)[8:])
                _, ko2 = lo_hi(pltpu.roll(w, 2, 0)[8:])
                s0, s1, s2, s3 = [_rep(sh_ref[a, :, ls], n) for a in range(4)]
                ve, vo = lo_hi(pltpu.bitcast(vb[r0:r0 + G, ls], U32))
                kve = ((ke * s0 + ko1 * s1) + (ke1 * s2 + ko2 * s3)) * ve
                kvo = ((ko * s0 + ke * s1) + (ko1 * s2 + ke1 * s3)) * vo
                kv_ref[r0 // 2:(r0 + G) // 2, ls] = pltpu.bitcast(
                    pltpu.pack_elementwise([kve, kvo], packed_dtype=BF16), U32)
            return run
        return _costed([piece(ls, r0) for b in range(2) for ls in lanes
                        for r0 in range(b * CB, (b + 1) * CB, G)], 2.5 * G + 10)

    def u_fwd(t):
        for b in range(2):
            for ls in lanes:
                kv = lambda: _unpk(kv_ref[b * HB:(b + 1) * HB, ls])
                a = bg.dot(fwd_ref[0:CB, :], kv())
                kv2 = kv()
                kv_live.discard((b, ls.start))
                bb = bg.dot(fwd_ref[CB:2 * CB, :], kv2)
                u_ref[t, b, 0:CB, ls] = a + bb
                u_ref[t, b, CB:2 * CB, ls] = a
                u_ref[t, b, 2 * CB:3 * CB, ls] = bb

    positions = [(slice(r0, r0 + 8), ls) for r0 in range(0, 3 * CB, 8) for ls in lanes]

    def ystatic_pieces(blocks, acc_in, pos=None):
        def piece(rs, ls):
            def run(tok):
                us, ks = {}, {}
                for s, lo, hi in blocks:
                    acc = None
                    for i in range(lo, min(hi, s + 1)):
                        if i not in us:
                            us[i] = _add(u_ref[i // 2, i % 2, rs, ls], tok)
                        if s - i not in ks:
                            ks[s - i] = kk_ref[s - i, rs, ls]
                        p = ks[s - i] * us[i]
                        acc = p if acc is None else acc + p
                    if acc_in:
                        acc = acc + y_ref[s // 2, s % 2, rs, ls]
                    y_ref[s // 2, s % 2, rs, ls] = acc
                return acc
            return run
        return _costed([piece(*p) for p in (positions if pos is None else pos)], 35)

    y_first = [(s, 0, 4) for s in range(NB)]

    def task_pieces(t, delta):
        p = t - delta
        left = p >= T0
        J = jnp.where(left, t, p + NLOOP)
        I = jnp.where(left, p, t)
        kview = kk_ref.at[pl.ds(2 * (J - I) - 1, 3)]

        def piece(rs, ls):
            def run(tok):
                u0 = _add(u_ref[I, 0, rs, ls], tok)
                u1 = _add(u_ref[I, 1, rs, ls], tok)
                kc = kview[1, rs, ls]
                y_ref[J, 0, rs, ls] = (kc * u0 + kview[0, rs, ls] * u1) + y_ref[J, 0, rs, ls]
                y1 = (kview[2, rs, ls] * u0 + kc * u1) + y_ref[J, 1, rs, ls]
                y_ref[J, 1, rs, ls] = y1
                return y1
            return run
        return [piece(*p) for p in positions]

    def diag_pieces(t, I):
        kview = kk_ref.at[pl.ds(2 * (t - I) - 1, 3)]

        def piece(rs, ls):
            def run(tok):
                us = [_add(u_ref[a, b, rs, ls], tok) for a in (t, I) for b in range(2)]
                k0 = kk_ref[0, rs, ls]
                kc = kview[1, rs, ls]
                y_ref[t, 0, rs, ls] = ((k0 * us[0] + y_ref[t, 0, rs, ls])
                                       + (kc * us[2] + kview[0, rs, ls] * us[3]))
                y1 = ((kk_ref[1, rs, ls] * us[0] + k0 * us[1])
                      + (kview[2, rs, ls] * us[2] + kc * us[3]) + y_ref[t, 1, rs, ls])
                y_ref[t, 1, rs, ls] = y1
                return y1
            return run
        return [piece(*p) for p in positions]

    def post_pieces(t):
        def piece(b, r0, ls):
            def run(tok):
                comp = lambda c, off: y_ref[t, b, c * CB + off + r0:c * CB + off + r0 + 16, ls]
                k1l, k1h = _add(comp(0, 0), tok), _add(comp(0, HB), tok)
                rel, reh = k1l - comp(2, 0), k1h - comp(2, HB)
                iml, imh = k1l + comp(1, 0), k1h + comp(1, HB)
                p0 = b * CB + r0 // 2
                yb_ref[p0:p0 + 8, ls] = _pk(rel + reh)
                yb_ref[p0 + HB // 2:p0 + HB // 2 + 8, ls] = _pk(iml + imh)
                yb_ref[p0 + HB:p0 + HB + 8, ls] = _pk(rel - reh)
                oim = iml - imh
                yb_ref[p0 + HB + HB // 2:p0 + HB + HB // 2 + 8, ls] = _pk(oim)
                return oim[8:16]
            return run
        return _costed([piece(b, r0, ls) for b in range(2) for r0 in range(0, HB, 16) for ls in lanes], 45)

    def q_split(t, b, p0, n, ls):
        w = pltpu.bitcast(q_ref.at[rows_of(t)][b * CB + 2 * p0:b * CB + 2 * p0 + 2 * n, ls], U32)
        return lo_hi(w)

    def ln_tiles(xs, tok):
        n = xs[0].shape[0]
        s = _add(xs[0], tok)
        for x in xs[1:]:
            s = s + x
        m = jnp.sum(s, axis=-1, keepdims=True) * (1.0 / D)
        xc = [x - m for x in xs]
        s2 = xc[0] * xc[0]
        for x in xc[1:]:
            s2 = s2 + x * x
        r = lax.rsqrt(jnp.sum(s2, axis=-1, keepdims=True) * (1.0 / D) + EPS)
        return xc, jnp.broadcast_to(r, (n, 128)), jnp.broadcast_to(m, (n, 128))

    def ln1_pieces(t):
        G = _E('L1G', 8)

        def piece(b, p0):
            def run(tok):
                xc, r, _ = ln_tiles([cat(q_split(t, b, p0, G, ls), axis=0) for ls in lanes], tok)
                for ls, x in zip(lanes, xc):
                    h = (x * r) * _rep(mod_ref[0, :, ls], 2 * G) + _rep(mod_ref[1, :, ls], 2 * G)
                    hp_ref[b * CB + p0:b * CB + p0 + G, ls] = h[:G]
                    hp_ref[b * CB + HB + p0:b * CB + HB + p0 + G, ls] = h[G:]
                return functools.reduce(lambda a, c: a + c, [h[r:r + 8] for r in range(0, 2 * G, 8)])
            return run
        return [piece(b, p0) for b in range(2) for p0 in range(0, HB, G)]

    def y_inv(t, x1_dst):
        yb = opaque(yb_ref)
        hp = opaque(hp_ref)
        for b in range(2):
            ye = bg.dot(inv_ref[0:HB, :], _unpk(yb[b * CB:b * CB + HB, :]))
            yo = bg.dot(inv_ref[HB:CB, :], _unpk(yb[b * CB + HB:(b + 1) * CB, :]))
            for ls in lanes:
                qe, qo = q_split(t, b, 0, HB, ls)
                re, ro = slice(b * CB, b * CB + HB), slice(b * CB + HB, (b + 1) * CB)
                x1_dst[re, ls] = qe + hp[re, ls] * ye[:, ls]
                x1_dst[ro, ls] = qo + hp[ro, ls] * yo[:, ls]

    def ln2_stat_pieces(x1_src, st):
        x1o = opaque(x1_src)

        def piece(r0):
            def run(tok):
                _, r, m = ln_tiles([x1o[r0:r0 + 16, ls] for ls in lanes], tok)
                st[r0:r0 + 16, 0:128] = m
                st[r0:r0 + 16, 128:256] = r
                return r[0:8] + r[8:16]
            return run
        return [piece(h * CB + r0) for r0 in range(0, CB, 16) for h in range(2)]

    tile = lambda j: slice(j * 128, (j + 1) * 128)
    LX, RX = 0, 1
    Lc = lambda i: 2 + 2 * i
    Rc = lambda i: 3 + 2 * i
    others = lambda i: [j for j in range(NL) if j != i]
    edges = [(i, j) for i in range(NL) for j in others(i)]
    pairs = [(i, j) for i, j in edges if i < j]
    a_idx = {k: n for n, k in enumerate(
        [(c, i) for c in "xyw" for i in range(NL)] + [("s",) + e for e in edges]
        + [(c,) + e for c in ("dx", "dy") for e in pairs])}
    b_terms = {}
    for i in range(NL):
        b_terms["D1", i] = [(1, k, Lc(i)) for k in range(NL)]
        b_terms["D2", i] = [(1, i, Lc(i))] + [(-1, i, Rc(j)) for j in others(i)]
        b_terms["D3", i] = [(1, i, Rc(i))] + [(-1, i, Lc(j)) for j in others(i)]
        b_terms["D4", i] = [(1, k, Rc(i)) for k in range(NL)]
    for i, j in edges:
        sg = 1 if i < j else -1
        b_terms["E1", i, j] = [(1, i, Rc(j)), (1, j, Lc(i))]
        b_terms["E2", i, j] = [(sg, j, Lc(i))]
        b_terms["E3", i, j] = [(sg, i, Rc(j))]
    xpairs = [(0, 1), (2, 3)]
    for i, j in xpairs:
        b_terms["d1", i] = [(1, i, LX), (1, j, LX)]
        b_terms["d2", i] = [(1, i, LX), (-1, i, RX)]
        b_terms["d3", j] = [(1, j, RX), (-1, j, LX)]
        b_terms["d4", j] = [(1, j, RX), (1, i, RX)]
        b_terms["e1", i, j] = [(1, i, RX), (1, j, LX)]
        b_terms["e2", i, j] = [(1, j, LX)]
        b_terms["e3", i, j] = [(1, i, RX)]
    b_terms["pl",] = [(1, NL - 1, LX)]
    b_terms["pr",] = [(1, NL - 1, RX)]
    b_idx = {k: n for n, k in enumerate(b_terms)}
    w_refs = ((wg_ref, wgf_ref), (wu_ref, wuf_ref), (wd_ref, wdf_ref))
    done = set()
    check = [True]

    def norm_pieces(x1_src, st, unit, more=True):
        G = 16
        x1o = opaque(x1_src)

        def piece(r0, js):
            def run(tok):
                two = lambda ref, c: cat([ref[r0:r0 + G, c], ref[CB + r0:CB + r0 + G, c]], axis=0)
                m, r = _add(two(st, slice(0, 128)), tok), two(st, slice(128, 256))
                for j in js:
                    ls = lanes[j]
                    h = ((two(x1o, ls) - m) * r) * _rep(mod_ref[2, :, ls], 2 * G) + _rep(mod_ref[3, :, ls], 2 * G)
                    put_a(unit, r0, ("x", j), h[:G])
                    put_a(unit, r0, ("y", j), h[G:])
                    if more:
                        put_a(unit, r0, ("w", j), h[:G] + h[G:])
                        hn_ref[r0:r0 + G, ls] = h[:G]
                        hn_ref[CB + r0:CB + r0 + G, ls] = h[G:]
            return run
        return [_costed([piece(r0, js)], 32 * len(js))[0] for r0 in range(0, CB, G) for js in ([0, 1, 2], [3, 4])]

    def put_a(unit, r0, key, v):
        p0 = a_idx[key] * HB + r0 // 2
        hf_ref[p0:p0 + v.shape[0] // 2, lanes[unit]] = _pk(v)
        done.add(("a", unit, key, r0))

    def pair_pieces(unit):
        G = 16

        def piece(r0, i, j):
            def run(tok):
                assert ("a", unit, ("w", j), r0) in done
                ld = lambda h, k: hn_ref[h * CB + r0:h * CB + r0 + G, lanes[k]]
                xi, yi, xj, yj = _add(ld(0, i), tok), _add(ld(1, i), tok), ld(0, j), ld(1, j)
                put_a(unit, r0, ("s", i, j), xi + yj)
                put_a(unit, r0, ("s", j, i), xj + yi)
                put_a(unit, r0, ("dx", i, j), xj - xi)
                put_a(unit, r0, ("dy", i, j), yi - yj)
            return run
        return _costed([piece(r0, i, j) for r0 in range(0, CB, G) for i, j in pairs], 30)

    def w_pieces(w, groups):
        src, dst = w_refs[w]

        def piece(keys, r0, G):
            def run(tok):
                blk = {}

                def ld(k, c):
                    if (k, c) not in blk:
                        rt, ct = (k, c) if w < 2 else (c, k)
                        v = src[rt * 128 + r0:rt * 128 + r0 + G, tile(ct)].astype(F32)
                        blk[k, c] = _add(v, tok) if len(blk) < _E('TA', 2) else v
                    return blk[k, c]
                for key in keys:
                    acc = None
                    for sg, k, c in b_terms[key]:
                        v = ld(k, c)
                        acc = (v if sg > 0 else -v) if acc is None else (acc + v if sg > 0 else acc - v)
                    p0 = (b_idx[key] // 2) * HB + r0 // 2
                    dst[p0:p0 + G // 2, tile(b_idx[key] % 2)] = _pk(acc)
                    done.add(("b", w, key, r0 + G))
            return run
        out = []
        for keys in groups:
            G = 16 if len(keys) > 3 else 32
            n = len({t[1:] for k in keys for t in b_terms[k]})
            out += _costed([piece(keys, r0, G) for r0 in range(0, CB, G)], (3 * n + len(keys) + 2) * G / 8)
        return out

    g_edge = lambda i, j: [("E1", i, j), ("E2", i, j), ("E3", i, j)]
    g_left = [[("e1", i, j), ("e2", i, j), ("e3", i, j), ("d1", i), ("d2", i), ("d3", j), ("d4", j)]
              for i, j in xpairs] + [[("pl",), ("pr",)]]
    g_cols = lambda m: ([[("D1", m)], [("D4", m)]] + [g_edge(i, m) for i in range(m)]
                        + [g_edge(m, j) for j in range(m)])
    g_rows = [[(d, i)] for i in range(NL) for d in ("D2", "D3")]

    def rhs(w, key):
        assert not check[0] or ("b", w, key, CB) in done, (w, key)
        return _unpk(w_refs[w][1][(b_idx[key] // 2) * HB:(b_idx[key] // 2 + 1) * HB, tile(b_idx[key] % 2)])

    def lhs(unit, key, p0, n):
        assert not check[0] or all(("a", unit, key, r) in done for r in range(2 * p0, 2 * (p0 + n), 16)), key
        return _unpk(hf_ref[a_idx[key] * HB + p0:a_idx[key] * HB + p0 + n, lanes[unit]])

    def gu_plain(c, unit):
        for h in range(2):
            x = lambda: cat([lhs(unit, ("xy"[h], k), 0, HB) for k in range(NL)], axis=1)
            p = bg.dot(x(), wg_ref[:, tile(c)]) * bg.dot(x(), wu_ref[:, tile(c)])
            pp_ref[unit * TM + h * CB:unit * TM + (h + 1) * CB, tile(c)] = p

    def gu_finish(w, unit, p0, n, c, v):
        for h in range(2):
            r = h * CB + 2 * p0
            if w == 0:
                gs_ref[r:r + 2 * n, tile(c)] = v[h]
            else:
                pp_ref[unit * TM + r:unit * TM + r + 2 * n, tile(c)] = gs_ref[r:r + 2 * n, tile(c)] * v[h]

    def gu_main(w, unit, p0, n, rows=range(NL)):
        dot = lambda a, b: bg.dot(lhs(unit, a, p0, n), rhs(w, b))
        run_ref, off = (gs_ref, 0) if w == 0 else (pp_ref, unit * TM)
        for i in rows:
            p = q = None
            for d in range(1, NL):
                j = (i + d) % NL
                lo, hi = min(i, j), max(i, j)
                e1 = dot(("s", i, j), ("E1", i, j))
                e2 = dot(("dx", lo, hi), ("E2", i, j))
                e3 = dot(("dy", lo, hi), ("E3", i, j))
                p = e2 if p is None else p + e2
                q = e1 + e3 if q is None else (q + e1) + e3
                rp, rq = e1 + e2, e3
                if d == 1:
                    x = dot(("x", i), ("D1", i))
                    p, q = p + x, q - x
                elif d == 2:
                    q = q + dot(("w", i), ("D2", i))
                elif d == 3:
                    rp = rp + dot(("w", j), ("D3", j))
                else:
                    x = dot(("y", j), ("D4", j))
                    rp, rq = rp - x, rq + x
                rs = [slice(off + h * CB + 2 * p0, off + h * CB + 2 * (p0 + n)) for h in range(2)]
                if i != others(j)[0]:
                    rp, rq = rp + run_ref[rs[0], tile(Rc(j))], rq + run_ref[rs[1], tile(Rc(j))]
                if i == others(j)[-1]:
                    gu_finish(w, unit, p0, n, Rc(j), (rp, rq))
                else:
                    run_ref[rs[0], tile(Rc(j))] = rp
                    run_ref[rs[1], tile(Rc(j))] = rq
            gu_finish(w, unit, p0, n, Lc(i), (p, q))

    def gu_left(w, unit, p0, n):
        def dot(f, extra=()):
            ks = [f(i, j) for i, j in xpairs] + list(extra)
            return bg.dot(cat([lhs(unit, a, p0, n) for a, _ in ks], axis=1), cat([rhs(w, b) for _, b in ks], axis=0))
        one = lambda a, b: bg.dot(lhs(unit, (a, NL - 1), p0, n), rhs(w, (b,)))
        e1 = dot(lambda i, j: (("s", i, j), ("e1", i, j)))
        e2 = dot(lambda i, j: (("dx", i, j), ("e2", i, j)))
        e3 = dot(lambda i, j: (("dy", i, j), ("e3", i, j)))
        d1 = dot(lambda i, j: (("x", i), ("d1", i)))
        pl_, ql, pr = e2 + d1, (e1 + e3) - d1, e1 + e2
        ql = ql + dot(lambda i, j: (("w", i), ("d2", i)), [(("y", NL - 1), ("pl",))])
        gu_finish(w, unit, p0, n, LX, (pl_ + one("x", "pl"), ql))
        d4 = dot(lambda i, j: (("y", j), ("d4", j)))
        pr = (pr - d4) + dot(lambda i, j: (("w", j), ("d3", j)), [(("x", NL - 1), ("pr",))])
        gu_finish(w, unit, p0, n, RX, (pr, (e3 + d4) + one("y", "pr")))

    def gu_fast(unit, n, left=True, mid=None):
        k = 0
        for p0 in range(0, HB, n):
            for w in range(2):
                if mid is not None and mid[0] == k:
                    mid[1]()
                k += 1
                if left and w == 1:
                    gu_left(w, unit, p0, n)
                gu_main(w, unit, p0, n)
                if left and w == 0:
                    gu_left(w, unit, p0, n)

    def ffn_down(x1_src, t, unit, mid=None, e=_E('DSUB', 32)):
        ob = o_ref.at[rows_of(t)]
        k = 0
        for r0 in range(0, HB, e):
            rows = lambda ref, base, c: cat([ref[base + o + r0:base + o + r0 + e, c] for o in (0, HB)], axis=0)
            hx = lambda c: rows(pp_ref, unit * TM, tile(c))
            hy = lambda c: rows(pp_ref, unit * TM + CB, tile(c))
            run = lambda h: slice(h * CB + 2 * r0, h * CB + 2 * (r0 + e))

            def left(key):
                kind = key[0]
                if kind[0] in "Ee":
                    l, r = (Lc(key[1]), Rc(key[2])) if kind[0] == "E" else (LX, RX)
                    return (hy if kind[1] == "3" else hx)(r) + (hx if kind[1] == "2" else hy)(l)
                if kind[1] in "12":
                    c = Lc(key[1]) if kind[0] == "D" else LX
                    return hx(c) - hy(c) if kind[1] == "1" else hy(c)
                c = Rc(key[1]) if kind[0] == "D" else RX
                return hx(c) if kind[1] == "3" else hy(c) - hx(c)

            def dot(keys, plain=None):
                keys = [kk for kk in keys if kk in b_terms]
                a = [left(kk) for kk in keys]
                if plain is not None:
                    a, keys = a + [plain(LX), plain(RX)], keys + [("pl",), ("pr",)]
                a, w = cat(a, axis=1), (lambda: cat([rhs(2, kk) for kk in keys], axis=0))
                if plain is not None and e == HB:
                    return cat([bg.dot(a[r:r + HB].astype(BF16), w()) for r in (0, HB)], axis=0)
                return bg.dot(a.astype(BF16), w())

            for i in range(NL):
                ls = lanes[i]
                last = i == NL - 1
                both = dot([("D2", i), ("D3", i), ("d2", i), ("d3", i)])
                p = both + dot([("D1", i), ("d1", i)], hx if last else None)
                q = both + dot([("D4", i), ("d4", i)], hy if last else None)
                if i > 0:
                    p, q = p + gs_ref[run(0), ls], q + gs_ref[run(1), ls]
                for j in range(i + 1, NL):
                    a = dot([("E1", i, j), ("e1", i, j)])
                    c3 = dot([("E3", i, j), ("E3", j, i), ("e3", i, j)])
                    rq = a - c3
                    gs_ref[run(1), lanes[j]] = rq + gs_ref[run(1), lanes[j]] if i > 0 else rq
                    b = dot([("E1", j, i)])
                    c2 = dot([("E2", i, j), ("E2", j, i), ("e2", i, j)])
                    rp = b + c2
                    gs_ref[run(0), lanes[j]] = rp + gs_ref[run(0), lanes[j]] if i > 0 else rp
                    p, q = (p + a) - c2, (q + c3) + b
                assert not check[0] or ('gb', i) in done
                for b, dn in enumerate((p, q)):
                    o = rows(x1_src, b * CB, ls) + _rep(mod_ref[4, :, ls], 2 * e) * dn
                    w = pltpu.pack_elementwise([o[:e], o[e:]], packed_dtype=BF16)
                    ob[run(b), ls] = pltpu.bitcast(w, BF16)
                k += 1
                if mid is not None and k == mid[0] * (HB // e) + (NL - mid[0]) * (HB // e - 1) * mid[2]:
                    mid[1]()

    x1s = [x1_ref.at[r] for r in range(NS)]
    sts = [st_ref.at[r * TM:(r + 1) * TM] for r in range(2)]
    YP = _E('YP', 12)

    def setup():
        for cp in small:
            cp.wait()
        shk = shk_ref[...].astype(F32)
        for a in range(4):
            sh_ref[a] = jnp.broadcast_to(shk[a:a + 1, :], (8, D))
        zm_ref[...] = pltpu.bitcast(inv_ref[CB:CB + 16, :], I32)
        zs.append(zm_ref[0, 0])

    def prologue():
        ytile = lambda i: ystatic_pieces(y_first, False, [p for p in positions if p[1] == lanes[i]])
        ssm_cp(0).wait()
        k_fwd(0)
        for t in range(2):
            k_cp(t).wait()
            v_cp(t).wait()
            now(kv_pieces(t, 64))
            u_fwd(t)
        bg.flush()
        for i in range(1, NL):
            if i != 3:
                ssm_cp(i).wait()
            if i == 2:
                ssm_cp(3).wait()
            bg.add(ytile(i - 1), 0, 1024)
            k_fwd(i)
            bg.flush()
        q_cp(0).wait()
        now(ytile(NL - 1))
        q_cp(1).wait()
        mod_cp(0).wait()
        mod_chunk(0)
        for t in range(2):
            now(post_pieces(t))
            now(ln1_pieces(t))
            y_inv(t, x1s[t])
        for t in range(2):
            now(ln2_stat_pieces(x1s[t], sts[t]))
        bg.flush()

    def superstep():
        wp = lambda groups: w_pieces(0, groups) + w_pieces(1, groups)

        def wait_gu(*fs):
            for f in fs:
                g_cp(f).wait()
                u_cp(f).wait()

        mod_cp(1).wait()
        mod_chunk(1)
        now(norm_pieces(x1s[0], sts[0], 0, more=False))
        bg.flush()
        wait_gu(0)
        bg.add(norm_pieces(x1s[1], sts[1], 1), 0, 900)
        bg.add(pair_pieces(1) + wp(g_left), 900, 2400)
        for u in range(2):
            gu_plain(0, u)
            gu_plain(1, u)
        bg.flush()
        wait_gu(1, 2)
        bg.add(wp(g_cols(0) + g_cols(1)), 0, 2400)
        for c in range(2, 6):
            gu_plain(c, 0)
        bg.flush()
        k_cp(2).wait()
        v_cp(2).wait()
        wait_gu(3)
        bg.add(kv_pieces(2), 0, 1050)
        if _E('C2', 2):
            bg.add(wp(g_cols(2)[:_E('C2', 2)]), 1100, 1850)
        gu_plain(6, 0)
        gu_plain(7, 0)
        u_fwd(2)
        bg.flush()
        wait_gu(4, 5)
        ymid = _costed(_group(ystatic_pieces([(s, 4, 6) for s in (4, 5)], True), 2), 35)
        late = g_cols(2)[_E('C2', 2):] + g_cols(3) + g_cols(4) + g_rows
        w1 = w_pieces(1, late)
        n1 = _E('N1', 20)
        bg.add(w_pieces(0, late) + w1[:n1], 0, 2450)
        for c in range(8, 12):
            gu_plain(c, 0)
        bg.flush()
        q_cp(2).wait()
        ny = _E('NY', 60)
        bg.add(w1[n1:] + ymid[:ny], 0, 2450)
        if _E('LB', 0) == 1:
            bg.add(linked(ln1_pieces(2), 3), 0, 2100)
        gu_main(0, 1, 0, HB)
        bg.flush()
        d_cp.wait()
        order_d = g_left + [g for i in range(NL) for g in (
            [[(d, i)] for d in ("D2", "D3", "D1", "D4")]
            + [g for j in range(i + 1, NL) for g in (g_edge(i, j), g_edge(j, i))])]
        wdp = w_pieces(2, order_d)
        nd = _E('ND', 160)
        bg.add(wdp[:nd], 0, 2450)
        gu_main(1, 1, 0, HB)
        bg.flush()
        mod_cp(2).wait()
        k_cp(3).wait()
        v_cp(3).wait()
        bg.add(wdp[nd:] + ymid[ny:] + post_pieces(2) + kv_pieces(3, _E('KS', 32)), 0, 3300)
        if _E('LB', 0) == 0:
            bg.add(linked(ln1_pieces(2), 3), 0, 2500)
        bg.inj = [(100 + 130 * i, gb_tile(i)) for i in range(NL)]
        ffn_down(x1s[0], 0, 0, e=_E('SE', 64))
        y_inv(2, x1s[2])
        bg.flush()
        o_cp(0).start()

    def run_super(fn):
        if _E('SL', 1):
            def body(i, carry):
                fn()
                return carry
            lax.fori_loop(0, zs[0] + 1, body, 0)
        else:
            fn()

    def step(t, carry):
        q_cp(t).wait()

        @pl.when(t + 1 < NS)
        def _():
            k_cp(t + 1).wait()
            v_cp(t + 1).wait()

        x1v = x1_ref.at[pl.ds(t - 2, 3)]
        x1 = x1v.at[2]
        bg.add(linked(ln1_pieces(t), _E('LK1', 2)), _E('L0', 4000), _E('L1', 8500))
        bg.add(ln2_stat_pieces(x1v.at[1], st_ref), 0, _E('S1', 600))
        bg.add(norm_pieces(x1v.at[1], st_ref, 1), _E('P0', 1000), _E('P1', 2000))
        bg.add(pair_pieces(1), _E('P1', 2000), _E('P2', 3100))
        kv_live.update((b, ls.start) for b in range(2) for ls in lanes)
        kvp = kv_pieces(jnp.minimum(t + 1, NS - 1), _E('KG', 32))
        nk = len(kvp) * _E('KF', 60) // 100
        if nk:
            bg.add(kvp[:nk], 3136 + _E('KA', 70), 3136 + _E('KB', 700))
        if nk < len(kvp):
            bg.add(kvp[nk:], _E('K0', 9000), _E('K1', 10200))

        def conv():
            u_fwd(t)
            chain(diag_pieces(t, T0 - 1), _E('DD', 2), _E('DE', 0))
            chain(task_pieces(t, 2), _E('MD', 3), _E('ME', 0))
            dep = chain(task_pieces(t, 1), _E('MD', 3), _E('ME', 0))
            chain(post_pieces(t), 1, 3, dep)

        if _E('FP', 5) == 0:
            conv()
        ffn_down(x1v.at[0], t - 2, 1, mid=(_E('FP', 5), conv, 0))
        sub = _E('SUB', HB)
        if sub == HB:
            iv = _E('IV', 5)
            gu_main(0, 1, 0, HB)
            gu_left(0, 1, 0, HB)
            gu_left(1, 1, 0, HB)
            gu_main(1, 1, 0, HB, range(iv))
            y_inv(t, x1)
            gu_main(1, 1, 0, HB, range(iv, NL))
        else:
            gu_fast(1, sub, mid=(3, lambda: y_inv(t, x1)))
        bg.flush()
        o_cp(t - 2).start()
        return carry

    def epilogue():
        t = NS - 1
        bg.add(ln2_stat_pieces(x1s[t], st_ref), 0, 500)
        bg.add(norm_pieces(x1s[t], st_ref, 1), 900, 1800)
        bg.add(pair_pieces(1), 1800, 2950)
        ffn_down(x1s[t - 1], t - 1, 1)
        o_cp(t - 1).start()
        gu_fast(1, _E('SUB', HB))
        last = [pltpu.make_async_copy(o_ref.at[rows_of(t), lo:hi], o_hbm.at[rows_of(t), lo:hi], sem.at[s_o + t + i])
                for i, (lo, hi) in enumerate([(0, 384), (384, D)])]
        ffn_down(x1s[t], t, 1, mid=(3, last[0].start, 1))
        last[1].start()
        for i in range(NS - 1):
            o_cp(i).wait()
        for cp in last:
            cp.wait()

    sc = jax.named_scope if SCOPES else (lambda name: (lambda f: f))

    def rest():
        sc("superstep")(superstep)()
        lax.fori_loop(T0, NS, sc("step")(step), 0)
        sc("epilogue")(epilogue)()

    if ONLY == 'loop':
        check[0] = False
        zs.append(zm_ref[0, 0])
        lax.fori_loop(T0, NS, step, 0)
        epilogue()
    elif ONLY == 'S':
        zs.append(zm_ref[0, 0])
        run_super(superstep)
        lax.fori_loop(T0, NS, step, 0)
    elif _E('NEST', 3) == 3:
        setup()

        def everything():
            sc("prologue")(prologue)()
            rest()
        run_super(everything)
    else:
        setup()
        sc("prologue")(prologue)()
        run_super(rest)


@jax.jit
def pallas_adaLN_cond__ssm_conv_h3__glu_gated_bilinear__prompt_kernel(
    A_q, A_k, A_v, A_shift_k, A_ssm_k, A_ssm_D, B_x, B_w_gate, B_w_up, B_w_down, c, w_mod,
):
    B, S, D = A_q.shape
    Fh = B_w_gate.shape[1]
    NB = S // CB
    NS = S // TM
    fwd, inv = _dft_consts()
    anyspec = pl.BlockSpec(memory_space=pl.ANY)
    V = pltpu.VMEM
    out = pl.pallas_call(
        functools.partial(_kernel, S=S, D=D, Fh=Fh),
        in_specs=[anyspec] * 13,
        out_specs=anyspec,
        out_shape=jax.ShapeDtypeStruct((S, D), A_q.dtype),
        scratch_shapes=[
            V((NS, 2, 3 * CB, D), F32),
            V((NB, 3 * CB, D), F32),
            V((NS, 2, 3 * CB, D), F32),
            V((NS, TM, D), F32),
            V((S, D), BF16), V((S, D), BF16), V((S, D), BF16), V((S, D), BF16),
            V((TM, D), F32),
            V((2 * TM, 256), F32),
            V((2 * TM, Fh), F32),
            V((TM, Fh), F32),
            V((TM, D), F32),
            V((55 * HB, 256), U32),
            V((TM // 2, D), U32),
            V((2 * CB, D), U32),
            V((48 * HB, 256), U32), V((48 * HB, 256), U32), V((48 * HB, 256), U32),
            V((D, S), BF16), V((D, 6 * D), BF16), V((D, Fh), BF16), V((D, Fh), BF16), V((Fh, D), BF16),
            V((2 * CB, CB), BF16), V((CB + 16, CB), BF16),
            V((5, 8, D), F32), V((4, 8, D), F32), V((8, 128), I32),
            V((4, D), BF16), V((D,), BF16), V((1, D), BF16),
            pltpu.SemaphoreType.DMA((5 + 4 * NS + D // 128 + 3 + 2 * (Fh // FC) + 2,)),
        ],
        compiler_params=pltpu.CompilerParams(
            internal_scratch_in_bytes=48 * 1024,
            disable_semaphore_checks=True,
            disable_bounds_checks=True,
            vmem_limit_bytes=110 * 1024 * 1024),
        name="adaln_h3_glu",
    )(A_q.reshape(S, D), A_k.reshape(S, D), A_v.reshape(S, D), A_shift_k.T, A_ssm_k,
      A_ssm_D, B_w_gate, B_w_up, B_w_down, c, w_mod, fwd, inv)
    return out.reshape(B, S, D)
```

```python
import functools

import numpy as np
import jax
import jax.numpy as jnp
from jax import lax
import jax.experimental.pallas as pl
import jax.experimental.pallas.tpu as pltpu

F32 = jnp.float32
BF16 = jnp.bfloat16
U32 = jnp.uint32
I32 = jnp.int32

CB = 128
HB = CB // 2
TM = 256
FC = 256
EPS = 1e-5


def _dft_consts():
    k = np.arange(CB, dtype=np.float64)[:, None]
    n = np.arange(CB, dtype=np.float64)[None, :]
    th = np.pi * (4.0 * k + 1.0) * n / (2.0 * CB)
    fwd = np.concatenate([np.cos(th), np.sin(th)], axis=0)
    g = np.concatenate([np.cos(th[:HB]), np.sin(th[:HB])], axis=0).T / CB
    inv = np.concatenate([g[0::2], g[1::2], np.zeros((16, CB))], axis=0)
    return jnp.asarray(fwd, dtype=BF16), jnp.asarray(inv, dtype=BF16)


def _pk(x):
    return pltpu.bitcast(x.astype(BF16), U32)


def _unpk(x):
    return pltpu.bitcast(x, BF16)


def _rep(r, n):
    return r if n == 8 else jnp.concatenate([r] * (n // 8), axis=0)


def _add(x, tok):
    return x if tok is None else x + _rep(tok, x.shape[0])


def _costed(pieces, cost):
    for p in pieces:
        p.cost = cost
    return pieces


def _group(pieces, n):
    def merged(ps):
        def run(tok):
            for p in ps:
                p(tok)
        return run
    return [merged(pieces[i:i + n]) for i in range(0, len(pieces), n)]


class _Sched:
    def __init__(self, token):
        self.token = token
        self.clock = 0.0
        self.q = []
        self.last = None
        self.inj = []

    def add(self, pieces, t0, t1):
        cum = np.cumsum([0.0] + [getattr(p, "cost", 1.0) for p in pieces])
        self.q += [(t0 + (t1 - t0) * cum[i] / cum[-1], i, p) for i, p in enumerate(pieces)]
        self.q.sort(key=lambda e: e[:2])

    def note(self, m, dt):
        rows, cols = m.shape
        tiles = [(slice(r, r + 8), slice(c, c + 128)) for c in range(0, cols, 128) for r in range(0, rows, 8)]
        for i, tl in enumerate(tiles):
            tok = None
            while self.q and self.q[0][0] <= self.clock + dt * (i + 1) / len(tiles):
                if tok is None:
                    tok = self.token(m[tl])
                self.q.pop(0)[2](tok)
        self.clock += dt
        self.last = m[tiles[-1]]
        return m

    def dot(self, a, b):
        if self.inj and self.clock >= self.inj[0][0]:
            self.inj.pop(0)[1]()
        m = jnp.dot(a, b, preferred_element_type=F32)
        return self.note(m, max(a.shape[0], 32) * (a.shape[1] // 128) * (b.shape[1] // 128) / 4)

    def flush(self):
        tok = None if self.last is None or not self.q else self.token(self.last)
        while self.q:
            self.q.pop(0)[2](tok)
        self.clock = 0.0
        self.last = None


def _kernel(q_hbm, k_hbm, v_hbm, shk_hbm, ssmk_hbm, ssmd_hbm, wg_hbm, wu_hbm, wd_hbm,
            c_hbm, wmod_hbm, fwd_hbm, inv_hbm, o_hbm,
            u_ref, kk_ref, y_ref, x1_ref, q_ref, k_ref, v_ref, o_ref,
            hp_ref, st_ref, pp_ref, gs_ref, hn_ref, hf_ref, kv_ref, yb_ref, wgf_ref, wuf_ref, wdf_ref,
            ssmk_ref, wmod_ref, wg_ref, wu_ref, wd_ref, fwd_ref, inv_ref,
            mod_ref, sh_ref, zm_ref, shk_ref, ssmd_ref, c_ref,
            sem, *, S, D, Fh):
    NB = S // CB
    NS = S // TM
    NL = D // 128
    NF = Fh // FC
    T0 = 3
    NLOOP = NS - T0
    lanes = [slice(i * 128, (i + 1) * 128) for i in range(NL)]
    cat = jnp.concatenate

    offs = [int(o) for o in np.cumsum([0, 5, NS, NS, NS, NL, 3, NF, NF, 1])]
    s_small, s_q, s_k, s_v, s_ssm, s_mod, s_g, s_u, s_d, s_o = offs

    def rows_of(t):
        return pl.ds(t * TM if isinstance(t, int) else pl.multiple_of(t * TM, TM), TM)

    def rows_cp(src, dst, base, t):
        return pltpu.make_async_copy(src.at[rows_of(t), :], dst.at[rows_of(t), :], sem.at[base + t])

    def cols_cp(src, dst, lo, hi, si):
        return pltpu.make_async_copy(src.at[:, lo:hi], dst.at[:, lo:hi], sem.at[si])

    q_cp = lambda t: rows_cp(q_hbm, q_ref, s_q, t)
    k_cp = lambda t: rows_cp(k_hbm, k_ref, s_k, t)
    v_cp = lambda t: rows_cp(v_hbm, v_ref, s_v, t)
    o_cp = lambda t: rows_cp(o_ref, o_hbm, s_o, t)
    small = [pltpu.make_async_copy(s, d, sem.at[s_small + i]) for i, (s, d) in enumerate(
        [(fwd_hbm, fwd_ref), (shk_hbm, shk_ref), (ssmd_hbm, ssmd_ref), (inv_hbm, inv_ref), (c_hbm, c_ref)])]
    ssm_cp = lambda i: pltpu.make_async_copy(ssmk_hbm.at[lanes[i], :], ssmk_ref.at[lanes[i], :],
                                             sem.at[s_ssm + i])
    mod_cols = [(0, 3 * D), (3 * D, 5 * D), (5 * D, 6 * D)]
    mod_cp = lambda i: cols_cp(wmod_hbm, wmod_ref, mod_cols[i][0], mod_cols[i][1], s_mod + i)
    g_cp = lambda f: cols_cp(wg_hbm, wg_ref, f * FC, (f + 1) * FC, s_g + f)
    u_cp = lambda f: cols_cp(wu_hbm, wu_ref, f * FC, (f + 1) * FC, s_u + f)
    d_cp = pltpu.make_async_copy(wd_hbm, wd_ref, sem.at[s_d])

    order = small + [ssm_cp(0), k_cp(0), v_cp(0), k_cp(1), v_cp(1),
                     ssm_cp(1), ssm_cp(2), ssm_cp(3), ssm_cp(4), q_cp(0), q_cp(1),
                     mod_cp(0), mod_cp(1)]
    for f in range(NF):
        order += [g_cp(f), u_cp(f)]
        if f == 2:
            order += [k_cp(2), v_cp(2)]
    order += [q_cp(2), d_cp, mod_cp(2), k_cp(3), v_cp(3)]
    for t in range(T0, NS):
        order += [q_cp(t)]
        if t + 1 < NS:
            order += [k_cp(t + 1), v_cp(t + 1)]
    for cp in order:
        cp.start()

    zs = []
    bg = _Sched(lambda x: pltpu.bitcast(pltpu.bitcast(x, I32) & zm_ref[...], F32))

    def opaque(ref):
        return ref.at[pl.ds(pl.multiple_of(zs[0], 32), ref.shape[0])]

    def chain(pieces, dist, extra=0, dep=None):
        hist = [] if dep is None else [dep] * dist
        for p in pieces:
            tok = None
            if len(hist) >= dist:
                tok = bg.token(hist[-dist])
                for _ in range(extra):
                    tok = tok + tok
            hist.append(p(tok))
        return hist[-1]

    def linked(pieces, d):
        res = []

        def wrap(p):
            def run(tok):
                if d and len(res) >= d:
                    tok = tok + bg.token(res[-d])
                res.append(p(tok))
            return run
        return [wrap(p) for p in pieces]

    def now(pieces):
        for p in pieces:
            p(None)

    def mod_chunk(i):
        c = c_ref[...].astype(F32)
        sc = jnp.broadcast_to((c * jax.nn.sigmoid(c)).astype(BF16), (16, D))
        lo, hi = mod_cols[i]
        m = bg.dot(sc, wmod_ref[:, lo:hi])[0:8]
        if i == 0:
            ga = m[:, 2 * D:3 * D]
            mod_ref[0] = (1.0 + m[:, D:2 * D]) * ga
            mod_ref[1] = m[:, 0:D] * ga
        else:
            mod_ref[2] = 1.0 + m[:, D:2 * D]
            mod_ref[3] = m[:, 0:D]

    def gb_tile(i):
        def run():
            c = c_ref[...].astype(F32)
            sc = jnp.broadcast_to((c * jax.nn.sigmoid(c)).astype(BF16), (16, D))
            w = wmod_ref[:, 5 * D + i * 128:5 * D + (i + 1) * 128]
            mod_ref[4, :, lanes[i]] = jnp.dot(sc, w, preferred_element_type=F32)[0:8]
            done.add(('gb', i))
        return run

    def k_fwd(i):
        ls = lanes[i]
        fwd = fwd_ref[...]
        prev = None
        for m in range(NB):
            kf = lax.dot_general(fwd, ssmk_ref[ls, m * CB:(m + 1) * CB], (((1,), (1,)), ((), ())),
                                 preferred_element_type=F32)
            if m == 0:
                c = kf[:CB] + ssmd_ref[...].astype(F32).reshape(1, D)[:, ls]
                d = kf[CB:]
            else:
                c = kf[:CB] + prev[CB:]
                d = kf[CB:] - prev[:CB]
            prev = kf
            kk_ref[m, 0:CB, ls] = c
            kk_ref[m, CB:2 * CB, ls] = d - c
            kk_ref[m, 2 * CB:3 * CB, ls] = c + d
            if m % 4 == 3:
                bg.note(kf, 2 * CB)

    def lo_hi(w):
        return pltpu.bitcast(w << 16, F32), pltpu.bitcast(w & jnp.uint32(0xFFFF0000), F32)

    kv_live = set()

    def kv_pieces(t, G=32):
        n = G // 2
        kb, vb = k_ref.at[rows_of(t)], v_ref.at[rows_of(t)]

        def piece(ls, r0):
            def run(tok):
                assert (r0 // CB, ls.start) not in kv_live
                if r0 > 0:
                    w = pltpu.bitcast(kb[r0 - 16:r0 + G, ls], U32)
                else:
                    if isinstance(t, int) and t == 0:
                        halo = jnp.zeros((8, 128), U32)
                    else:
                        halo = pltpu.bitcast(k_ref.at[rows_of(t - 1)][TM - 16:TM, ls], U32)
                    w = cat([halo, pltpu.bitcast(kb[0:G, ls], U32)], axis=0)
                if tok is not None:
                    w = w | _rep(pltpu.bitcast(tok, U32), n + 8)
                ke, ko = lo_hi(w[8:])
                ke1, ko1 = lo_hi(pltpu.roll(w, 1, 0)[8:])
                _, ko2 = lo_hi(pltpu.roll(w, 2, 0)[8:])
                s0, s1, s2, s3 = [_rep(sh_ref[a, :, ls], n) for a in range(4)]
                ve, vo = lo_hi(pltpu.bitcast(vb[r0:r0 + G, ls], U32))
                kve = ((ke * s0 + ko1 * s1) + (ke1 * s2 + ko2 * s3)) * ve
                kvo = ((ko * s0 + ke * s1) + (ko1 * s2 + ke1 * s3)) * vo
                kv_ref[r0 // 2:(r0 + G) // 2, ls] = pltpu.bitcast(
                    pltpu.pack_elementwise([kve, kvo], packed_dtype=BF16), U32)
            return run
        return _costed([piece(ls, r0) for b in range(2) for ls in lanes
                        for r0 in range(b * CB, (b + 1) * CB, G)], 2.5 * G + 10)

    def u_fwd(t):
        for b in range(2):
            for ls in lanes:
                kv = lambda: _unpk(kv_ref[b * HB:(b + 1) * HB, ls])
                a = bg.dot(fwd_ref[0:CB, :], kv())
                kv2 = kv()
                kv_live.discard((b, ls.start))
                bb = bg.dot(fwd_ref[CB:2 * CB, :], kv2)
                u_ref[t, b, 0:CB, ls] = a + bb
                u_ref[t, b, CB:2 * CB, ls] = a
                u_ref[t, b, 2 * CB:3 * CB, ls] = bb

    positions = [(slice(r0, r0 + 8), ls) for r0 in range(0, 3 * CB, 8) for ls in lanes]

    def ystatic_pieces(blocks, acc_in, pos=None):
        def piece(rs, ls):
            def run(tok):
                us, ks = {}, {}
                for s, lo, hi in blocks:
                    acc = None
                    for i in range(lo, min(hi, s + 1)):
                        if i not in us:
                            us[i] = _add(u_ref[i // 2, i % 2, rs, ls], tok)
                        if s - i not in ks:
                            ks[s - i] = kk_ref[s - i, rs, ls]
                        p = ks[s - i] * us[i]
                        acc = p if acc is None else acc + p
                    if acc_in:
                        acc = acc + y_ref[s // 2, s % 2, rs, ls]
                    y_ref[s // 2, s % 2, rs, ls] = acc
                return acc
            return run
        return _costed([piece(*p) for p in (positions if pos is None else pos)], 35)

    y_first = [(s, 0, 4) for s in range(NB)]

    def task_pieces(t, delta):
        p = t - delta
        left = p >= T0
        J = jnp.where(left, t, p + NLOOP)
        I = jnp.where(left, p, t)
        kview = kk_ref.at[pl.ds(2 * (J - I) - 1, 3)]

        def piece(rs, ls):
            def run(tok):
                u0 = _add(u_ref[I, 0, rs, ls], tok)
                u1 = _add(u_ref[I, 1, rs, ls], tok)
                kc = kview[1, rs, ls]
                y_ref[J, 0, rs, ls] = (kc * u0 + kview[0, rs, ls] * u1) + y_ref[J, 0, rs, ls]
                y1 = (kview[2, rs, ls] * u0 + kc * u1) + y_ref[J, 1, rs, ls]
                y_ref[J, 1, rs, ls] = y1
                return y1
            return run
        return [piece(*p) for p in positions]

    def diag_pieces(t, I):
        kview = kk_ref.at[pl.ds(2 * (t - I) - 1, 3)]

        def piece(rs, ls):
            def run(tok):
                us = [_add(u_ref[a, b, rs, ls], tok) for a in (t, I) for b in range(2)]
                k0 = kk_ref[0, rs, ls]
                kc = kview[1, rs, ls]
                y_ref[t, 0, rs, ls] = ((k0 * us[0] + y_ref[t, 0, rs, ls])
                                       + (kc * us[2] + kview[0, rs, ls] * us[3]))
                y1 = ((kk_ref[1, rs, ls] * us[0] + k0 * us[1])
                      + (kview[2, rs, ls] * us[2] + kc * us[3]) + y_ref[t, 1, rs, ls])
                y_ref[t, 1, rs, ls] = y1
                return y1
            return run
        return [piece(*p) for p in positions]

    def post_pieces(t):
        def piece(b, r0, ls):
            def run(tok):
                comp = lambda c, off: y_ref[t, b, c * CB + off + r0:c * CB + off + r0 + 16, ls]
                k1l, k1h = _add(comp(0, 0), tok), _add(comp(0, HB), tok)
                rel, reh = k1l - comp(2, 0), k1h - comp(2, HB)
                iml, imh = k1l + comp(1, 0), k1h + comp(1, HB)
                p0 = b * CB + r0 // 2
                yb_ref[p0:p0 + 8, ls] = _pk(rel + reh)
                yb_ref[p0 + HB // 2:p0 + HB // 2 + 8, ls] = _pk(iml + imh)
                yb_ref[p0 + HB:p0 + HB + 8, ls] = _pk(rel - reh)
                oim = iml - imh
                yb_ref[p0 + HB + HB // 2:p0 + HB + HB // 2 + 8, ls] = _pk(oim)
                return oim[8:16]
            return run
        return _costed([piece(b, r0, ls) for b in range(2) for r0 in range(0, HB, 16) for ls in lanes], 45)

    def q_split(t, b, p0, n, ls):
        w = pltpu.bitcast(q_ref.at[rows_of(t)][b * CB + 2 * p0:b * CB + 2 * p0 + 2 * n, ls], U32)
        return lo_hi(w)

    def ln_tiles(xs, tok):
        n = xs[0].shape[0]
        s = _add(xs[0], tok)
        for x in xs[1:]:
            s = s + x
        m = jnp.sum(s, axis=-1, keepdims=True) * (1.0 / D)
        xc = [x - m for x in xs]
        s2 = xc[0] * xc[0]
        for x in xc[1:]:
            s2 = s2 + x * x
        r = lax.rsqrt(jnp.sum(s2, axis=-1, keepdims=True) * (1.0 / D) + EPS)
        return xc, jnp.broadcast_to(r, (n, 128)), jnp.broadcast_to(m, (n, 128))

    def ln1_pieces(t):
        G = 8

        def piece(b, p0):
            def run(tok):
                xc, r, _ = ln_tiles([cat(q_split(t, b, p0, G, ls), axis=0) for ls in lanes], tok)
                for ls, x in zip(lanes, xc):
                    h = (x * r) * _rep(mod_ref[0, :, ls], 2 * G) + _rep(mod_ref[1, :, ls], 2 * G)
                    hp_ref[b * CB + p0:b * CB + p0 + G, ls] = h[:G]
                    hp_ref[b * CB + HB + p0:b * CB + HB + p0 + G, ls] = h[G:]
                return functools.reduce(lambda a, c: a + c, [h[r:r + 8] for r in range(0, 2 * G, 8)])
            return run
        return [piece(b, p0) for b in range(2) for p0 in range(0, HB, G)]

    def y_inv(t, x1_dst):
        yb = opaque(yb_ref)
        hp = opaque(hp_ref)
        for b in range(2):
            ye = bg.dot(inv_ref[0:HB, :], _unpk(yb[b * CB:b * CB + HB, :]))
            yo = bg.dot(inv_ref[HB:CB, :], _unpk(yb[b * CB + HB:(b + 1) * CB, :]))
            for ls in lanes:
                qe, qo = q_split(t, b, 0, HB, ls)
                re, ro = slice(b * CB, b * CB + HB), slice(b * CB + HB, (b + 1) * CB)
                x1_dst[re, ls] = qe + hp[re, ls] * ye[:, ls]
                x1_dst[ro, ls] = qo + hp[ro, ls] * yo[:, ls]

    def ln2_stat_pieces(x1_src, st):
        x1o = opaque(x1_src)

        def piece(r0):
            def run(tok):
                _, r, m = ln_tiles([x1o[r0:r0 + 16, ls] for ls in lanes], tok)
                st[r0:r0 + 16, 0:128] = m
                st[r0:r0 + 16, 128:256] = r
                return r[0:8] + r[8:16]
            return run
        return [piece(h * CB + r0) for r0 in range(0, CB, 16) for h in range(2)]

    tile = lambda j: slice(j * 128, (j + 1) * 128)
    LX, RX = 0, 1
    Lc = lambda i: 2 + 2 * i
    Rc = lambda i: 3 + 2 * i
    others = lambda i: [j for j in range(NL) if j != i]
    edges = [(i, j) for i in range(NL) for j in others(i)]
    pairs = [(i, j) for i, j in edges if i < j]
    a_idx = {k: n for n, k in enumerate(
        [(c, i) for c in "xyw" for i in range(NL)] + [("s",) + e for e in edges]
        + [(c,) + e for c in ("dx", "dy") for e in pairs])}
    b_terms = {}
    for i in range(NL):
        b_terms["D1", i] = [(1, k, Lc(i)) for k in range(NL)]
        b_terms["D2", i] = [(1, i, Lc(i))] + [(-1, i, Rc(j)) for j in others(i)]
        b_terms["D3", i] = [(1, i, Rc(i))] + [(-1, i, Lc(j)) for j in others(i)]
        b_terms["D4", i] = [(1, k, Rc(i)) for k in range(NL)]
    for i, j in edges:
        sg = 1 if i < j else -1
        b_terms["E1", i, j] = [(1, i, Rc(j)), (1, j, Lc(i))]
        b_terms["E2", i, j] = [(sg, j, Lc(i))]
        b_terms["E3", i, j] = [(sg, i, Rc(j))]
    xpairs = [(0, 1), (2, 3)]
    for i, j in xpairs:
        b_terms["d1", i] = [(1, i, LX), (1, j, LX)]
        b_terms["d2", i] = [(1, i, LX), (-1, i, RX)]
        b_terms["d3", j] = [(1, j, RX), (-1, j, LX)]
        b_terms["d4", j] = [(1, j, RX), (1, i, RX)]
        b_terms["e1", i, j] = [(1, i, RX), (1, j, LX)]
        b_terms["e2", i, j] = [(1, j, LX)]
        b_terms["e3", i, j] = [(1, i, RX)]
    b_terms["pl",] = [(1, NL - 1, LX)]
    b_terms["pr",] = [(1, NL - 1, RX)]
    b_idx = {k: n for n, k in enumerate(b_terms)}
    w_refs = ((wg_ref, wgf_ref), (wu_ref, wuf_ref), (wd_ref, wdf_ref))
    done = set()
    check = [True]

    def norm_pieces(x1_src, st, unit, more=True):
        G = 16
        x1o = opaque(x1_src)

        def piece(r0, j):
            def run(tok):
                ls = lanes[j]
                two = lambda ref, c: cat([ref[r0:r0 + G, c], ref[CB + r0:CB + r0 + G, c]], axis=0)
                m, r = _add(two(st, slice(0, 128)), tok), two(st, slice(128, 256))
                h = ((two(x1o, ls) - m) * r) * _rep(mod_ref[2, :, ls], 2 * G) + _rep(mod_ref[3, :, ls], 2 * G)
                put_a(unit, r0, ("x", j), h[:G])
                put_a(unit, r0, ("y", j), h[G:])
                if more:
                    put_a(unit, r0, ("w", j), h[:G] + h[G:])
                    hn_ref[r0:r0 + G, ls] = h[:G]
                    hn_ref[CB + r0:CB + r0 + G, ls] = h[G:]
            return run
        return _costed([piece(r0, j) for r0 in range(0, CB, G) for j in range(NL)], 44)

    def put_a(unit, r0, key, v):
        p0 = a_idx[key] * HB + r0 // 2
        hf_ref[p0:p0 + v.shape[0] // 2, lanes[unit]] = _pk(v)
        done.add(("a", unit, key, r0))

    def pair_pieces(unit):
        G = 16

        def piece(r0, i, j):
            def run(tok):
                assert ("a", unit, ("w", j), r0) in done
                ld = lambda h, k: hn_ref[h * CB + r0:h * CB + r0 + G, lanes[k]]
                xi, yi, xj, yj = _add(ld(0, i), tok), _add(ld(1, i), tok), ld(0, j), ld(1, j)
                put_a(unit, r0, ("s", i, j), xi + yj)
                put_a(unit, r0, ("s", j, i), xj + yi)
                put_a(unit, r0, ("dx", i, j), xj - xi)
                put_a(unit, r0, ("dy", i, j), yi - yj)
            return run
        return _costed([piece(r0, i, j) for r0 in range(0, CB, G) for i, j in pairs], 30)

    def factor_pieces(x1_src, st, unit):
        nrm, prs = norm_pieces(x1_src, st, unit), pair_pieces(unit)
        a, b = len(nrm) // 8, len(prs) // 8
        return [p for g in range(8) for p in nrm[g * a:(g + 1) * a] + prs[g * b:(g + 1) * b]]

    def w_pieces(w, groups):
        src, dst = w_refs[w]

        def piece(keys, r0, G):
            def run(tok):
                blk = {}

                def ld(k, c):
                    if (k, c) not in blk:
                        rt, ct = (k, c) if w < 2 else (c, k)
                        v = src[rt * 128 + r0:rt * 128 + r0 + G, tile(ct)].astype(F32)
                        blk[k, c] = _add(v, tok) if len(blk) < 2 else v
                    return blk[k, c]
                for key in keys:
                    acc = None
                    for sg, k, c in b_terms[key]:
                        v = ld(k, c)
                        acc = (v if sg > 0 else -v) if acc is None else (acc + v if sg > 0 else acc - v)
                    p0 = (b_idx[key] // 2) * HB + r0 // 2
                    dst[p0:p0 + G // 2, tile(b_idx[key] % 2)] = _pk(acc)
                    done.add(("b", w, key, r0 + G))
            return run
        out = []
        for keys in groups:
            G = 32 if len(keys) in (2, 3) else 16
            n = len({t[1:] for k in keys for t in b_terms[k]})
            out += _costed([piece(keys, r0, G) for r0 in range(0, CB, G)], (3 * n + len(keys) + 2) * G / 8)
        return out

    g_edge = lambda i, j: [("E1", i, j), ("E2", i, j), ("E3", i, j)]
    g_left = [[("e1", i, j), ("e2", i, j), ("e3", i, j), ("d1", i), ("d2", i), ("d3", j), ("d4", j)]
              for i, j in xpairs] + [[("pl",), ("pr",)]]
    g_cols = lambda m: ([[("D1", m)], [("D4", m)]] + [g_edge(i, m) for i in range(m)]
                        + [g_edge(m, j) for j in range(m)])
    g_rows = [[(d, i)] for i in range(NL) for d in ("D2", "D3")]

    def rhs(w, key):
        assert not check[0] or ("b", w, key, CB) in done, (w, key)
        return _unpk(w_refs[w][1][(b_idx[key] // 2) * HB:(b_idx[key] // 2 + 1) * HB, tile(b_idx[key] % 2)])

    def lhs(unit, key):
        assert not check[0] or all(("a", unit, key, r) in done for r in range(0, CB, 16)), key
        return _unpk(hf_ref[a_idx[key] * HB:(a_idx[key] + 1) * HB, lanes[unit]])

    def gu_plain(c, unit):
        for h in range(2):
            x = lambda: cat([lhs(unit, ("xy"[h], k)) for k in range(NL)], axis=1)
            p = bg.dot(x(), wg_ref[:, tile(c)]) * bg.dot(x(), wu_ref[:, tile(c)])
            pp_ref[unit * TM + h * CB:unit * TM + (h + 1) * CB, tile(c)] = p

    def gu_finish(w, unit, c, v):
        for h in range(2):
            r = h * CB
            if w == 0:
                gs_ref[r:r + CB, tile(c)] = v[h]
            else:
                pp_ref[unit * TM + r:unit * TM + r + CB, tile(c)] = gs_ref[r:r + CB, tile(c)] * v[h]

    def gu_main(w, unit):
        dot = lambda a, b: bg.dot(lhs(unit, a), rhs(w, b))
        run_ref, off = (gs_ref, 0) if w == 0 else (pp_ref, unit * TM)
        for i in range(NL):
            p = q = None
            for d in range(1, NL):
                j = (i + d) % NL
                lo, hi = min(i, j), max(i, j)
                e1 = dot(("s", i, j), ("E1", i, j))
                e2 = dot(("dx", lo, hi), ("E2", i, j))
                e3 = dot(("dy", lo, hi), ("E3", i, j))
                p = e2 if p is None else p + e2
                q = e1 + e3 if q is None else (q + e1) + e3
                rp, rq = e1 + e2, e3
                if d == 1:
                    x = dot(("x", i), ("D1", i))
                    p, q = p + x, q - x
                elif d == 2:
                    q = q + dot(("w", i), ("D2", i))
                elif d == 3:
                    rp = rp + dot(("w", j), ("D3", j))
                else:
                    x = dot(("y", j), ("D4", j))
                    rp, rq = rp - x, rq + x
                rs = [slice(off + h * CB, off + (h + 1) * CB) for h in range(2)]
                if i != others(j)[0]:
                    rp, rq = rp + run_ref[rs[0], tile(Rc(j))], rq + run_ref[rs[1], tile(Rc(j))]
                if i == others(j)[-1]:
                    gu_finish(w, unit, Rc(j), (rp, rq))
                else:
                    run_ref[rs[0], tile(Rc(j))] = rp
                    run_ref[rs[1], tile(Rc(j))] = rq
            gu_finish(w, unit, Lc(i), (p, q))

    def gu_left(w, unit):
        def dot(f, extra=()):
            ks = [f(i, j) for i, j in xpairs] + list(extra)
            return bg.dot(cat([lhs(unit, a) for a, _ in ks], axis=1), cat([rhs(w, b) for _, b in ks], axis=0))
        one = lambda a, b: bg.dot(lhs(unit, (a, NL - 1)), rhs(w, (b,)))
        e1 = dot(lambda i, j: (("s", i, j), ("e1", i, j)))
        e2 = dot(lambda i, j: (("dx", i, j), ("e2", i, j)))
        e3 = dot(lambda i, j: (("dy", i, j), ("e3", i, j)))
        d1 = dot(lambda i, j: (("x", i), ("d1", i)))
        pl_, ql, pr = e2 + d1, (e1 + e3) - d1, e1 + e2
        ql = ql + dot(lambda i, j: (("w", i), ("d2", i)), [(("y", NL - 1), ("pl",))])
        gu_finish(w, unit, LX, (pl_ + one("x", "pl"), ql))
        d4 = dot(lambda i, j: (("y", j), ("d4", j)))
        pr = (pr - d4) + dot(lambda i, j: (("w", j), ("d3", j)), [(("x", NL - 1), ("pr",))])
        gu_finish(w, unit, RX, (pr, (e3 + d4) + one("y", "pr")))

    def gu_fast(unit):
        gu_main(0, unit)
        gu_left(0, unit)
        gu_left(1, unit)
        gu_main(1, unit)

    def ffn_down(x1_src, t, unit, after=None, e=32):
        ob = o_ref.at[rows_of(t)]
        for r0 in range(0, HB, e):
            rows = lambda ref, base, c: cat([ref[base + o + r0:base + o + r0 + e, c] for o in (0, HB)], axis=0)
            hx = lambda c: rows(pp_ref, unit * TM, tile(c))
            hy = lambda c: rows(pp_ref, unit * TM + CB, tile(c))
            run = lambda h: slice(h * CB + 2 * r0, h * CB + 2 * (r0 + e))

            def left(key):
                kind = key[0]
                if kind[0] in "Ee":
                    l, r = (Lc(key[1]), Rc(key[2])) if kind[0] == "E" else (LX, RX)
                    return (hy if kind[1] == "3" else hx)(r) + (hx if kind[1] == "2" else hy)(l)
                if kind[1] in "12":
                    c = Lc(key[1]) if kind[0] == "D" else LX
                    return hx(c) - hy(c) if kind[1] == "1" else hy(c)
                c = Rc(key[1]) if kind[0] == "D" else RX
                return hx(c) if kind[1] == "3" else hy(c) - hx(c)

            def dot(keys, plain=None):
                keys = [kk for kk in keys if kk in b_terms]
                a = [left(kk) for kk in keys]
                if plain is not None:
                    a, keys = a + [plain(LX), plain(RX)], keys + [("pl",), ("pr",)]
                a, w = cat(a, axis=1), (lambda: cat([rhs(2, kk) for kk in keys], axis=0))
                if plain is not None and e == HB:
                    return cat([bg.dot(a[r:r + HB].astype(BF16), w()) for r in (0, HB)], axis=0)
                return bg.dot(a.astype(BF16), w())

            for i in range(NL):
                ls = lanes[i]
                last = i == NL - 1
                both = dot([("D2", i), ("D3", i), ("d2", i), ("d3", i)])
                p = both + dot([("D1", i), ("d1", i)], hx if last else None)
                q = both + dot([("D4", i), ("d4", i)], hy if last else None)
                if i > 0:
                    p, q = p + gs_ref[run(0), ls], q + gs_ref[run(1), ls]
                for j in range(i + 1, NL):
                    a = dot([("E1", i, j), ("e1", i, j)])
                    c3 = dot([("E3", i, j), ("E3", j, i), ("e3", i, j)])
                    rq = a - c3
                    gs_ref[run(1), lanes[j]] = rq + gs_ref[run(1), lanes[j]] if i > 0 else rq
                    b = dot([("E1", j, i)])
                    c2 = dot([("E2", i, j), ("E2", j, i), ("e2", i, j)])
                    rp = b + c2
                    gs_ref[run(0), lanes[j]] = rp + gs_ref[run(0), lanes[j]] if i > 0 else rp
                    p, q = (p + a) - c2, (q + c3) + b
                assert not check[0] or ('gb', i) in done
                for b, dn in enumerate((p, q)):
                    o = rows(x1_src, b * CB, ls) + _rep(mod_ref[4, :, ls], 2 * e) * dn
                    w = pltpu.pack_elementwise([o[:e], o[e:]], packed_dtype=BF16)
                    ob[run(b), ls] = pltpu.bitcast(w, BF16)
                if after is not None and r0 + e == HB:
                    after(i)

    x1s = [x1_ref.at[r] for r in range(NS)]
    sts = [st_ref.at[r * TM:(r + 1) * TM] for r in range(2)]

    def setup():
        for cp in small:
            cp.wait()
        shk = shk_ref[...].astype(F32)
        for a in range(4):
            sh_ref[a] = jnp.broadcast_to(shk[a:a + 1, :], (8, D))
        zm_ref[...] = pltpu.bitcast(inv_ref[CB:CB + 16, :], I32)
        zs.append(zm_ref[0, 0])

    def prologue():
        ytile = lambda i: ystatic_pieces(y_first, False, [p for p in positions if p[1] == lanes[i]])
        ssm_cp(0).wait()
        k_fwd(0)
        for t in range(2):
            k_cp(t).wait()
            v_cp(t).wait()
            now(kv_pieces(t, 64))
            u_fwd(t)
        bg.flush()
        for i in range(1, NL):
            if i != 3:
                ssm_cp(i).wait()
            if i == 2:
                ssm_cp(3).wait()
            bg.add(ytile(i - 1), 0, 1024)
            k_fwd(i)
            bg.flush()
        q_cp(0).wait()
        now(ytile(NL - 1))
        q_cp(1).wait()
        mod_cp(0).wait()
        mod_chunk(0)
        for t in range(2):
            now(post_pieces(t))
            now(ln1_pieces(t))
            y_inv(t, x1s[t])
        for t in range(2):
            now(ln2_stat_pieces(x1s[t], sts[t]))
        bg.flush()

    def superstep():
        wp = lambda groups: w_pieces(0, groups) + w_pieces(1, groups)

        def wait_gu(*fs):
            for f in fs:
                g_cp(f).wait()
                u_cp(f).wait()

        mod_cp(1).wait()
        mod_chunk(1)
        now(norm_pieces(x1s[0], sts[0], 0, more=False))
        bg.flush()
        wait_gu(0)
        bg.add(norm_pieces(x1s[1], sts[1], 1), 0, 900)
        bg.add(pair_pieces(1) + wp(g_left), 900, 2400)
        for u in range(2):
            gu_plain(0, u)
            gu_plain(1, u)
        bg.flush()
        wait_gu(1, 2)
        bg.add(wp(g_cols(0) + g_cols(1)), 0, 2400)
        for c in range(2, 6):
            gu_plain(c, 0)
        bg.flush()
        k_cp(2).wait()
        v_cp(2).wait()
        wait_gu(3)
        bg.add(kv_pieces(2), 0, 1050)
        bg.add(wp(g_cols(2)[:2]), 1100, 1850)
        gu_plain(6, 0)
        gu_plain(7, 0)
        u_fwd(2)
        bg.flush()
        wait_gu(4, 5)
        ymid = _costed(_group(ystatic_pieces([(s, 4, 6) for s in (4, 5)], True), 2), 17.5 * 2)
        late = g_cols(2)[2:] + g_cols(3) + g_cols(4) + g_rows
        w1 = w_pieces(1, late)
        n1 = len(w1) * 15 // 100
        bg.add(w_pieces(0, late) + w1[:n1], 0, 2450)
        for c in range(8, 12):
            gu_plain(c, 0)
        bg.flush()
        q_cp(2).wait()
        ny = 120 // 2
        bg.add(w1[n1:] + ymid[:ny], 0, 2450)
        gu_main(0, 1)
        bg.flush()
        d_cp.wait()
        order_d = g_left + [g for i in range(NL) for g in (
            [[(d, i)] for d in ("D2", "D3", "D1", "D4")]
            + [g for j in range(i + 1, NL) for g in (g_edge(i, j), g_edge(j, i))])]
        wdp = w_pieces(2, order_d)
        nd = len(wdp) * 89 // 100
        bg.add(wdp[:nd], 0, 2450)
        gu_main(1, 1)
        bg.flush()
        mod_cp(2).wait()
        k_cp(3).wait()
        v_cp(3).wait()
        bg.add(wdp[nd:] + ymid[ny:] + post_pieces(2) + kv_pieces(3, 16), 0, 3300)
        bg.add(linked(ln1_pieces(2), 3), 0, 2500)
        bg.inj = [(100 + 130 * i, gb_tile(i)) for i in range(NL)]
        ffn_down(x1s[0], 0, 0, e=64)
        y_inv(2, x1s[2])
        bg.flush()
        o_cp(0).start()

    def step(t, carry):
        q_cp(t).wait()

        @pl.when(t + 1 < NS)
        def _():
            k_cp(t + 1).wait()
            v_cp(t + 1).wait()

        x1v = x1_ref.at[pl.ds(t - 2, 3)]
        x1 = x1v.at[2]
        bg.add(linked(ln1_pieces(t), 2), 4000, 8500)
        bg.add(ln2_stat_pieces(x1v.at[1], st_ref), 0, 600)
        bg.add(factor_pieces(x1v.at[1], st_ref, 1), 800, 3100)
        kv_live.update((b, ls.start) for b in range(2) for ls in lanes)
        kvp = kv_pieces(jnp.minimum(t + 1, NS - 1), 32)
        nk = len(kvp) * 60 // 100
        bg.add(kvp[:nk], 3136 + 70, 3136 + 700)
        bg.add(kvp[nk:], 9000, 10200)
        ffn_down(x1v.at[0], t - 2, 1)
        u_fwd(t)
        chain(diag_pieces(t, T0 - 1), 2)
        chain(task_pieces(t, 2), 3)
        dep = chain(task_pieces(t, 1), 3)
        chain(post_pieces(t), 1, 3, dep)
        gu_fast(1)
        y_inv(t, x1)
        bg.flush()
        o_cp(t - 2).start()
        return carry

    def epilogue():
        t = NS - 1
        bg.add(ln2_stat_pieces(x1s[t], st_ref), 0, 500)
        bg.add(factor_pieces(x1s[t], st_ref, 1), 700, 2900)
        ffn_down(x1s[t - 1], t - 1, 1)
        o_cp(t - 1).start()
        gu_fast(1)
        cols = [(0 if i == 1 else i * 128, (i + 1) * 128) for i in range(1, NL)]
        last = [pltpu.make_async_copy(o_ref.at[rows_of(t), lo:hi], o_hbm.at[rows_of(t), lo:hi], sem.at[s_o + t + i])
                for i, (lo, hi) in enumerate(cols)]
        ffn_down(x1s[t], t, 1, after=lambda i: i > 0 and last[i - 1].start(), e=HB)
        for i in range(NS - 1):
            o_cp(i).wait()
        for cp in last:
            cp.wait()

    def everything(i, carry):
        prologue()
        superstep()
        lax.fori_loop(T0, NS, step, 0)
        epilogue()
        return carry

    setup()
    lax.fori_loop(0, zs[0] + 1, everything, 0)


@jax.jit
def pallas_adaLN_cond__ssm_conv_h3__glu_gated_bilinear__prompt_kernel(
    A_q, A_k, A_v, A_shift_k, A_ssm_k, A_ssm_D, B_x, B_w_gate, B_w_up, B_w_down, c, w_mod,
):
    B, S, D = A_q.shape
    Fh = B_w_gate.shape[1]
    NB = S // CB
    NS = S // TM
    fwd, inv = _dft_consts()
    anyspec = pl.BlockSpec(memory_space=pl.ANY)
    V = pltpu.VMEM
    out = pl.pallas_call(
        functools.partial(_kernel, S=S, D=D, Fh=Fh),
        in_specs=[anyspec] * 13,
        out_specs=anyspec,
        out_shape=jax.ShapeDtypeStruct((S, D), A_q.dtype),
        scratch_shapes=[
            V((NS, 2, 3 * CB, D), F32),
            V((NB, 3 * CB, D), F32),
            V((NS, 2, 3 * CB, D), F32),
            V((NS, TM, D), F32),
            V((S, D), BF16), V((S, D), BF16), V((S, D), BF16), V((S, D), BF16),
            V((TM, D), F32),
            V((2 * TM, 256), F32),
            V((2 * TM, Fh), F32),
            V((TM, Fh), F32),
            V((TM, D), F32),
            V((55 * HB, 256), U32),
            V((TM // 2, D), U32),
            V((2 * CB, D), U32),
            V((48 * HB, 256), U32), V((48 * HB, 256), U32), V((48 * HB, 256), U32),
            V((D, S), BF16), V((D, 6 * D), BF16), V((D, Fh), BF16), V((D, Fh), BF16), V((Fh, D), BF16),
            V((2 * CB, CB), BF16), V((CB + 16, CB), BF16),
            V((5, 8, D), F32), V((4, 8, D), F32), V((8, 128), I32),
            V((4, D), BF16), V((D,), BF16), V((1, D), BF16),
            pltpu.SemaphoreType.DMA((5 + 4 * NS + D // 128 + 3 + 2 * (Fh // FC) + 4,)),
        ],
        compiler_params=pltpu.CompilerParams(
            internal_scratch_in_bytes=48 * 1024,
            disable_semaphore_checks=True,
            disable_bounds_checks=True,
            vmem_limit_bytes=110 * 1024 * 1024),
        name="adaln_h3_glu",
    )(A_q.reshape(S, D), A_k.reshape(S, D), A_v.reshape(S, D), A_shift_k.T, A_ssm_k,
      A_ssm_D, B_w_gate, B_w_up, B_w_down, c, w_mod, fwd, inv)
    return out.reshape(B, S, D)
```

```python
import functools

import numpy as np
import jax
import jax.numpy as jnp
from jax import lax
import jax.experimental.pallas as pl
import jax.experimental.pallas.tpu as pltpu

F32 = jnp.float32
BF16 = jnp.bfloat16
U32 = jnp.uint32
I32 = jnp.int32

CB = 128
HB = CB // 2
TM = 256
FC = 256
EPS = 1e-5


def _dft_consts():
    k = np.arange(CB, dtype=np.float64)[:, None]
    n = np.arange(CB, dtype=np.float64)[None, :]
    th = np.pi * (4.0 * k + 1.0) * n / (2.0 * CB)
    fwd = np.concatenate([np.cos(th), np.sin(th)], axis=0)
    g = np.concatenate([np.cos(th[:HB]), np.sin(th[:HB])], axis=0).T / CB
    inv = np.concatenate([g[0::2], g[1::2], np.zeros((16, CB))], axis=0)
    return jnp.asarray(fwd, dtype=BF16), jnp.asarray(inv, dtype=BF16)


def _pk(x):
    return pltpu.bitcast(x.astype(BF16), U32)


def _unpk(x):
    return pltpu.bitcast(x, BF16)


def _rep(r, n):
    return r if n == 8 else jnp.concatenate([r] * (n // 8), axis=0)


def _add(x, tok):
    return x if tok is None else x + _rep(tok, x.shape[0])


def _costed(pieces, cost):
    for p in pieces:
        p.cost = cost
    return pieces


def _group(pieces, n):
    def merged(ps):
        def run(tok):
            for p in ps:
                p(tok)
        return run
    return [merged(pieces[i:i + n]) for i in range(0, len(pieces), n)]


class _Sched:
    def __init__(self, token):
        self.token = token
        self.clock = 0.0
        self.q = []
        self.last = None
        self.inj = []

    def add(self, pieces, t0, t1):
        cum = np.cumsum([0.0] + [getattr(p, "cost", 1.0) for p in pieces])
        self.q += [(t0 + (t1 - t0) * cum[i] / cum[-1], i, p) for i, p in enumerate(pieces)]
        self.q.sort(key=lambda e: e[:2])

    def note(self, m, dt):
        rows, cols = m.shape
        tiles = [(slice(r, r + 8), slice(c, c + 128)) for c in range(0, cols, 128) for r in range(0, rows, 8)]
        for i, tl in enumerate(tiles):
            tok = None
            while self.q and self.q[0][0] <= self.clock + dt * (i + 1) / len(tiles):
                if tok is None:
                    tok = self.token(m[tl])
                self.q.pop(0)[2](tok)
        self.clock += dt
        self.last = m[tiles[-1]]
        return m

    def dot(self, a, b):
        if self.inj and self.clock >= self.inj[0][0]:
            self.inj.pop(0)[1]()
        m = jnp.dot(a, b, preferred_element_type=F32)
        return self.note(m, max(a.shape[0], 32) * (a.shape[1] // 128) * (b.shape[1] // 128) / 4)

    def flush(self):
        tok = None if self.last is None or not self.q else self.token(self.last)
        while self.q:
            self.q.pop(0)[2](tok)
        self.clock = 0.0
        self.last = None


def _kernel(q_hbm, k_hbm, v_hbm, shk_hbm, ssmk_hbm, ssmd_hbm, wg_hbm, wu_hbm, wd_hbm,
            c_hbm, wmod_hbm, fwd_hbm, inv_hbm, o_hbm,
            u_ref, kk_ref, y_ref, x1_ref, q_ref, k_ref, v_ref, o_ref,
            hp_ref, st_ref, pp_ref, gs_ref, hn_ref, hf_ref, kv_ref, yb_ref, wgf_ref, wuf_ref, wdf_ref,
            ssmk_ref, wmod_ref, wg_ref, wu_ref, wd_ref, fwd_ref, inv_ref,
            mod_ref, sh_ref, zm_ref, sc_ref, shk_ref, ssmd_ref, c_ref,
            sem, *, S, D, Fh):
    NB = S // CB
    NS = S // TM
    NL = D // 128
    T0 = 3
    NLOOP = NS - T0
    lanes = [slice(i * 128, (i + 1) * 128) for i in range(NL)]
    cat = jnp.concatenate

    offs = [int(o) for o in np.cumsum([0, 5, NS, NS, NS, NL, 3, 3, 2, 1])]
    s_small, s_q, s_k, s_v, s_ssm, s_mod, s_g, s_u, s_d, s_o = offs

    def rows_of(t):
        return pl.ds(t * TM if isinstance(t, int) else pl.multiple_of(t * TM, TM), TM)

    def rows_cp(src, dst, base, t):
        return pltpu.make_async_copy(src.at[rows_of(t), :], dst.at[rows_of(t), :], sem.at[base + t])

    def cols_cp(src, dst, lo, hi, si):
        return pltpu.make_async_copy(src.at[:, lo:hi], dst.at[:, lo:hi], sem.at[si])

    q_cp = lambda t: rows_cp(q_hbm, q_ref, s_q, t)
    k_cp = lambda t: rows_cp(k_hbm, k_ref, s_k, t)
    v_cp = lambda t: rows_cp(v_hbm, v_ref, s_v, t)
    o_cp = lambda t: rows_cp(o_ref, o_hbm, s_o, t)
    small = [pltpu.make_async_copy(s, d, sem.at[s_small + i]) for i, (s, d) in enumerate(
        [(fwd_hbm, fwd_ref), (shk_hbm, shk_ref), (ssmd_hbm, ssmd_ref), (inv_hbm, inv_ref), (c_hbm, c_ref)])]
    ssm_cp = lambda i: pltpu.make_async_copy(ssmk_hbm.at[lanes[i], :], ssmk_ref.at[lanes[i], :],
                                             sem.at[s_ssm + i])
    mod_cols = [(0, 3 * D), (3 * D, 5 * D), (5 * D, 6 * D)]
    mod_cp = lambda i: cols_cp(wmod_hbm, wmod_ref, mod_cols[i][0], mod_cols[i][1], s_mod + i)
    g_cp = lambda f: cols_cp(wg_hbm, wg_ref, f * FC, (f + 1) * FC if f < 2 else Fh, s_g + f)
    u_cp = lambda f: cols_cp(wu_hbm, wu_ref, f * FC, (f + 1) * FC if f < 1 else Fh, s_u + f)
    d_cp = pltpu.make_async_copy(wd_hbm, wd_ref, sem.at[s_d])

    order = small + [ssm_cp(0), k_cp(0), v_cp(0), k_cp(1), v_cp(1),
                     ssm_cp(1), ssm_cp(2), ssm_cp(3), ssm_cp(4), q_cp(0), q_cp(1),
                     mod_cp(0), mod_cp(1)]
    order += [g_cp(0), u_cp(0), g_cp(1), g_cp(2), u_cp(1)]
    order += [k_cp(2), v_cp(2), q_cp(2), d_cp, mod_cp(2), k_cp(3), v_cp(3)]
    for t in range(T0, NS):
        order += [q_cp(t)]
        if t + 1 < NS:
            order += [k_cp(t + 1), v_cp(t + 1)]
    for cp in order:
        cp.start()

    zs = []
    bg = _Sched(lambda x: pltpu.bitcast(pltpu.bitcast(x, I32) & zm_ref[...], F32))

    def opaque(ref):
        return ref.at[pl.ds(pl.multiple_of(zs[0], 32), ref.shape[0])]

    def chain(pieces, dist, extra=0, dep=None):
        hist = [] if dep is None else [dep] * dist
        for p in pieces:
            tok = None
            if len(hist) >= dist:
                tok = bg.token(hist[-dist])
                for _ in range(extra):
                    tok = tok + tok
            hist.append(p(tok))
        return hist[-1]

    def linked(pieces, d):
        res = []

        def wrap(p):
            def run(tok):
                if d and len(res) >= d:
                    tok = tok + bg.token(res[-d])
                res.append(p(tok))
            return run
        return [wrap(p) for p in pieces]

    def now(pieces):
        for p in pieces:
            p(None)

    def mod_chunk(i):
        lo, hi = mod_cols[i]
        m = bg.dot(_unpk(sc_ref[...]), wmod_ref[:, lo:hi])[0:8]
        if i == 0:
            ga = m[:, 2 * D:3 * D]
            mod_ref[0] = (1.0 + m[:, D:2 * D]) * ga
            mod_ref[1] = m[:, 0:D] * ga
        else:
            mod_ref[2] = 1.0 + m[:, D:2 * D]
            mod_ref[3] = m[:, 0:D]

    def gb_tile(i):
        def run():
            w = wmod_ref[:, 5 * D + i * 128:5 * D + (i + 1) * 128]
            mod_ref[4, :, lanes[i]] = jnp.dot(_unpk(sc_ref[...]), w, preferred_element_type=F32)[0:8]
            done.add(('gb', i))
        return run

    def k_fwd(i):
        ls = lanes[i]
        fwd = fwd_ref[...]
        prev = None
        for m in range(NB):
            kf = lax.dot_general(fwd, ssmk_ref[ls, m * CB:(m + 1) * CB], (((1,), (1,)), ((), ())),
                                 preferred_element_type=F32)
            if m == 0:
                c = kf[:CB] + ssmd_ref[...].astype(F32).reshape(1, D)[:, ls]
                d = kf[CB:]
            else:
                c = kf[:CB] + prev[CB:]
                d = kf[CB:] - prev[:CB]
            prev = kf
            kk_ref[m, 0:CB, ls] = c
            kk_ref[m, CB:2 * CB, ls] = d - c
            kk_ref[m, 2 * CB:3 * CB, ls] = c + d
            if m % 4 == 3:
                bg.note(kf, 2 * CB)

    def lo_hi(w):
        return pltpu.bitcast(w << 16, F32), pltpu.bitcast(w & jnp.uint32(0xFFFF0000), F32)

    kv_live = set()

    def kv_pieces(t, G=32):
        n = G // 2
        kb, vb = k_ref.at[rows_of(t)], v_ref.at[rows_of(t)]

        def piece(ls, r0):
            def run(tok):
                assert (r0 // CB, ls.start) not in kv_live
                if r0 > 0:
                    w = pltpu.bitcast(kb[r0 - 16:r0 + G, ls], U32)
                else:
                    if isinstance(t, int) and t == 0:
                        halo = jnp.zeros((8, 128), U32)
                    else:
                        halo = pltpu.bitcast(k_ref.at[rows_of(t - 1)][TM - 16:TM, ls], U32)
                    w = cat([halo, pltpu.bitcast(kb[0:G, ls], U32)], axis=0)
                if tok is not None:
                    w = w | _rep(pltpu.bitcast(tok, U32), n + 8)
                ke, ko = lo_hi(w[8:])
                ke1, ko1 = lo_hi(pltpu.roll(w, 1, 0)[8:])
                _, ko2 = lo_hi(pltpu.roll(w, 2, 0)[8:])
                s0, s1, s2, s3 = [_rep(sh_ref[a, :, ls], n) for a in range(4)]
                ve, vo = lo_hi(pltpu.bitcast(vb[r0:r0 + G, ls], U32))
                kve = ((ke * s0 + ko1 * s1) + (ke1 * s2 + ko2 * s3)) * ve
                kvo = ((ko * s0 + ke * s1) + (ko1 * s2 + ke1 * s3)) * vo
                kv_ref[r0 // 2:(r0 + G) // 2, ls] = pltpu.bitcast(
                    pltpu.pack_elementwise([kve, kvo], packed_dtype=BF16), U32)
            return run
        return _costed([piece(ls, r0) for b in range(2) for ls in lanes
                        for r0 in range(b * CB, (b + 1) * CB, G)], 2.5 * G + 10)

    def u_fwd(t):
        for b in range(2):
            for ls in lanes:
                kv = lambda: _unpk(kv_ref[b * HB:(b + 1) * HB, ls])
                a = bg.dot(fwd_ref[0:CB, :], kv())
                kv2 = kv()
                kv_live.discard((b, ls.start))
                bb = bg.dot(fwd_ref[CB:2 * CB, :], kv2)
                u_ref[t, b, 0:CB, ls] = a + bb
                u_ref[t, b, CB:2 * CB, ls] = a
                u_ref[t, b, 2 * CB:3 * CB, ls] = bb

    positions = [(slice(r0, r0 + 8), ls) for r0 in range(0, 3 * CB, 8) for ls in lanes]

    def ystatic_pieces(blocks, acc_in, pos=None):
        def piece(rs, ls):
            def run(tok):
                us, ks = {}, {}
                for s, lo, hi in blocks:
                    acc = None
                    for i in range(lo, min(hi, s + 1)):
                        if i not in us:
                            us[i] = _add(u_ref[i // 2, i % 2, rs, ls], tok)
                        if s - i not in ks:
                            ks[s - i] = kk_ref[s - i, rs, ls]
                        p = ks[s - i] * us[i]
                        acc = p if acc is None else acc + p
                    if acc_in:
                        acc = acc + y_ref[s // 2, s % 2, rs, ls]
                    y_ref[s // 2, s % 2, rs, ls] = acc
                return acc
            return run
        return _costed([piece(*p) for p in (positions if pos is None else pos)], 35)

    y_first = [(s, 0, 4) for s in range(NB)]

    def task_pieces(t, delta):
        p = t - delta
        left = p >= T0
        J = jnp.where(left, t, p + NLOOP)
        I = jnp.where(left, p, t)
        kview = kk_ref.at[pl.ds(2 * (J - I) - 1, 3)]

        def piece(rs, ls):
            def run(tok):
                u0 = _add(u_ref[I, 0, rs, ls], tok)
                u1 = _add(u_ref[I, 1, rs, ls], tok)
                kc = kview[1, rs, ls]
                y_ref[J, 0, rs, ls] = (kc * u0 + kview[0, rs, ls] * u1) + y_ref[J, 0, rs, ls]
                y1 = (kview[2, rs, ls] * u0 + kc * u1) + y_ref[J, 1, rs, ls]
                y_ref[J, 1, rs, ls] = y1
                return y1
            return run
        return [piece(*p) for p in positions]

    def diag_pieces(t, I):
        kview = kk_ref.at[pl.ds(2 * (t - I) - 1, 3)]

        def piece(rs, ls):
            def run(tok):
                us = [_add(u_ref[a, b, rs, ls], tok) for a in (t, I) for b in range(2)]
                k0 = kk_ref[0, rs, ls]
                kc = kview[1, rs, ls]
                y_ref[t, 0, rs, ls] = ((k0 * us[0] + y_ref[t, 0, rs, ls])
                                       + (kc * us[2] + kview[0, rs, ls] * us[3]))
                y1 = ((kk_ref[1, rs, ls] * us[0] + k0 * us[1])
                      + (kview[2, rs, ls] * us[2] + kc * us[3]) + y_ref[t, 1, rs, ls])
                y_ref[t, 1, rs, ls] = y1
                return y1
            return run
        return [piece(*p) for p in positions]

    def post_pieces(t):
        def piece(b, r0, ls):
            def run(tok):
                comp = lambda c, off: y_ref[t, b, c * CB + off + r0:c * CB + off + r0 + 16, ls]
                k1l, k1h = _add(comp(0, 0), tok), _add(comp(0, HB), tok)
                rel, reh = k1l - comp(2, 0), k1h - comp(2, HB)
                iml, imh = k1l + comp(1, 0), k1h + comp(1, HB)
                p0 = b * CB + r0 // 2
                yb_ref[p0:p0 + 8, ls] = _pk(rel + reh)
                yb_ref[p0 + HB // 2:p0 + HB // 2 + 8, ls] = _pk(iml + imh)
                yb_ref[p0 + HB:p0 + HB + 8, ls] = _pk(rel - reh)
                oim = iml - imh
                yb_ref[p0 + HB + HB // 2:p0 + HB + HB // 2 + 8, ls] = _pk(oim)
                return oim[8:16]
            return run
        return _costed([piece(b, r0, ls) for b in range(2) for r0 in range(0, HB, 16) for ls in lanes], 45)

    def q_split(t, b, p0, n, ls):
        w = pltpu.bitcast(q_ref.at[rows_of(t)][b * CB + 2 * p0:b * CB + 2 * p0 + 2 * n, ls], U32)
        return lo_hi(w)

    def ln_tiles(xs, tok):
        n = xs[0].shape[0]
        s = _add(xs[0], tok)
        for x in xs[1:]:
            s = s + x
        m = jnp.sum(s, axis=-1, keepdims=True) * (1.0 / D)
        xc = [x - m for x in xs]
        s2 = xc[0] * xc[0]
        for x in xc[1:]:
            s2 = s2 + x * x
        r = lax.rsqrt(jnp.sum(s2, axis=-1, keepdims=True) * (1.0 / D) + EPS)
        return xc, jnp.broadcast_to(r, (n, 128)), jnp.broadcast_to(m, (n, 128))

    def ln1_pieces(t):
        G = 8

        def piece(b, p0):
            def run(tok):
                xc, r, _ = ln_tiles([cat(q_split(t, b, p0, G, ls), axis=0) for ls in lanes], tok)
                for ls, x in zip(lanes, xc):
                    h = (x * r) * _rep(mod_ref[0, :, ls], 2 * G) + _rep(mod_ref[1, :, ls], 2 * G)
                    hp_ref[b * CB + p0:b * CB + p0 + G, ls] = h[:G]
                    hp_ref[b * CB + HB + p0:b * CB + HB + p0 + G, ls] = h[G:]
                return functools.reduce(lambda a, c: a + c, [h[r:r + 8] for r in range(0, 2 * G, 8)])
            return run
        return [piece(b, p0) for b in range(2) for p0 in range(0, HB, G)]

    def y_inv(t, x1_dst):
        yb = opaque(yb_ref)
        hp = opaque(hp_ref)
        for b in range(2):
            ye = bg.dot(inv_ref[0:HB, :], _unpk(yb[b * CB:b * CB + HB, :]))
            yo = bg.dot(inv_ref[HB:CB, :], _unpk(yb[b * CB + HB:(b + 1) * CB, :]))
            for ls in lanes:
                qe, qo = q_split(t, b, 0, HB, ls)
                re, ro = slice(b * CB, b * CB + HB), slice(b * CB + HB, (b + 1) * CB)
                x1_dst[re, ls] = qe + hp[re, ls] * ye[:, ls]
                x1_dst[ro, ls] = qo + hp[ro, ls] * yo[:, ls]

    def ln2_stat_pieces(x1_src, st):
        x1o = opaque(x1_src)

        def piece(r0):
            def run(tok):
                _, r, m = ln_tiles([x1o[r0:r0 + 16, ls] for ls in lanes], tok)
                st[r0:r0 + 16, 0:128] = m
                st[r0:r0 + 16, 128:256] = r
                return r[0:8] + r[8:16]
            return run
        return [piece(h * CB + r0) for r0 in range(0, CB, 16) for h in range(2)]

    tile = lambda j: slice(j * 128, (j + 1) * 128)
    LX, RX = 0, 1
    Lc = lambda i: 2 + 2 * i
    RS = 2
    Rc = lambda i: 3 + 2 * ((i - RS) % NL)
    others = lambda i: [j for j in range(NL) if j != i]
    edges = [(i, j) for i in range(NL) for j in others(i)]
    pairs = [(i, j) for i, j in edges if i < j]
    a_idx = {k: n for n, k in enumerate(
        [(c, i) for c in "xyw" for i in range(NL)] + [("s",) + e for e in edges]
        + [(c,) + e for c in ("dx", "dy") for e in pairs])}
    b_terms = {}
    for i in range(NL):
        b_terms["D1", i] = [(1, k, Lc(i)) for k in range(NL)]
        b_terms["D2", i] = [(1, i, Lc(i))] + [(-1, i, Rc(j)) for j in others(i)]
        b_terms["D3", i] = [(1, i, Rc(i))] + [(-1, i, Lc(j)) for j in others(i)]
        b_terms["D4", i] = [(1, k, Rc(i)) for k in range(NL)]
    for i, j in edges:
        sg = 1 if i < j else -1
        b_terms["E1", i, j] = [(1, i, Rc(j)), (1, j, Lc(i))]
        b_terms["E2", i, j] = [(sg, j, Lc(i))]
        b_terms["E3", i, j] = [(sg, i, Rc(j))]
    xpairs = [(0, 1), (2, 3)]
    for i, j in xpairs:
        b_terms["d1", i] = [(1, i, LX), (1, j, LX)]
        b_terms["d2", i] = [(1, i, LX), (-1, i, RX)]
        b_terms["d3", j] = [(1, j, RX), (-1, j, LX)]
        b_terms["d4", j] = [(1, j, RX), (1, i, RX)]
        b_terms["e1", i, j] = [(1, i, RX), (1, j, LX)]
        b_terms["e2", i, j] = [(1, j, LX)]
        b_terms["e3", i, j] = [(1, i, RX)]
    b_terms["pl",] = [(1, NL - 1, LX)]
    b_terms["pr",] = [(1, NL - 1, RX)]
    b_idx = {k: n for n, k in enumerate(b_terms)}
    w_refs = ((wg_ref, wgf_ref), (wu_ref, wuf_ref), (wd_ref, wdf_ref))
    done = set()
    check = [True]

    def norm_pieces(x1_src, st, unit, more=True, base=True):
        G = 16
        x1o = opaque(x1_src)

        def piece(r0, j):
            def run(tok):
                ls = lanes[j]
                two = lambda ref, c: cat([ref[r0:r0 + G, c], ref[CB + r0:CB + r0 + G, c]], axis=0)
                m, r = _add(two(st, slice(0, 128)), tok), two(st, slice(128, 256))
                h = ((two(x1o, ls) - m) * r) * _rep(mod_ref[2, :, ls], 2 * G) + _rep(mod_ref[3, :, ls], 2 * G)
                if base:
                    put_a(unit, r0, ("x", j), h[:G])
                    put_a(unit, r0, ("y", j), h[G:])
                if more:
                    put_a(unit, r0, ("w", j), h[:G] + h[G:])
                    hn_ref[r0:r0 + G, ls] = h[:G]
                    hn_ref[CB + r0:CB + r0 + G, ls] = h[G:]
            return run
        return _costed([piece(r0, j) for r0 in range(0, CB, G) for j in range(NL)], 44)

    def put_a(unit, r0, key, v):
        p0 = a_idx[key] * HB + r0 // 2
        hf_ref[p0:p0 + v.shape[0] // 2, lanes[unit]] = _pk(v)
        done.add(("a", unit, key, r0))

    def pair_pieces(unit):
        G = 16

        def piece(r0, i, j):
            def run(tok):
                assert ("a", unit, ("w", j), r0) in done
                ld = lambda h, k: hn_ref[h * CB + r0:h * CB + r0 + G, lanes[k]]
                xi, yi, xj, yj = _add(ld(0, i), tok), _add(ld(1, i), tok), ld(0, j), ld(1, j)
                put_a(unit, r0, ("s", i, j), xi + yj)
                put_a(unit, r0, ("s", j, i), xj + yi)
                put_a(unit, r0, ("dx", i, j), xj - xi)
                put_a(unit, r0, ("dy", i, j), yi - yj)
            return run
        return _costed([piece(r0, i, j) for r0 in range(0, CB, G) for i, j in pairs], 30)

    def factor_pieces(x1_src, st, unit):
        nrm, prs = norm_pieces(x1_src, st, unit), pair_pieces(unit)
        a, b = len(nrm) // 8, len(prs) // 8
        return [p for g in range(8) for p in nrm[g * a:(g + 1) * a] + prs[g * b:(g + 1) * b]]

    def w_pieces(w, groups):
        src, dst = w_refs[w]

        def piece(keys, r0, G):
            def run(tok):
                blk = {}

                def ld(k, c):
                    if (k, c) not in blk:
                        rt, ct = (k, c) if w < 2 else (c, k)
                        v = src[rt * 128 + r0:rt * 128 + r0 + G, tile(ct)].astype(F32)
                        blk[k, c] = _add(v, tok) if len(blk) < 2 else v
                    return blk[k, c]
                for key in keys:
                    acc = None
                    for sg, k, c in b_terms[key]:
                        v = ld(k, c)
                        acc = (v if sg > 0 else -v) if acc is None else (acc + v if sg > 0 else acc - v)
                    p0 = (b_idx[key] // 2) * HB + r0 // 2
                    dst[p0:p0 + G // 2, tile(b_idx[key] % 2)] = _pk(acc)
                    done.add(("b", w, key, r0 + G))
            return run
        out = []
        for keys in groups:
            G = 32 if len(keys) in (2, 3) else 16
            n = len({t[1:] for k in keys for t in b_terms[k]})
            out += _costed([piece(keys, r0, G) for r0 in range(0, CB, G)], (3 * n + len(keys) + 2) * G / 8)
        return out

    g_edge = lambda i, j: [("E1", i, j), ("E2", i, j), ("E3", i, j)]
    g_left = [[("e1", i, j), ("e2", i, j), ("e3", i, j), ("d1", i), ("d2", i), ("d3", j), ("d4", j)]
              for i, j in xpairs] + [[("pl",), ("pr",)]]
    g_cols = lambda m: ([[("D1", m)], [("D4", (m + RS) % NL)]]
                        + [g_edge(i, j) for i, j in edges if max(Lc(i), Rc(j)) // 2 == m + 1])
    g_rows = [[(d, i)] for i in range(NL) for d in ("D2", "D3")]

    def rhs(w, key):
        assert not check[0] or ("b", w, key, CB) in done, (w, key)
        return _unpk(w_refs[w][1][(b_idx[key] // 2) * HB:(b_idx[key] // 2 + 1) * HB, tile(b_idx[key] % 2)])

    def lhs(unit, key):
        assert not check[0] or all(("a", unit, key, r) in done for r in range(0, CB, 16)), key
        return _unpk(hf_ref[a_idx[key] * HB:(a_idx[key] + 1) * HB, lanes[unit]])

    def gu_finish(w, unit, c, v):
        assert w == 0 or not check[0] or ("g", unit, c) in done
        done.add(("g", unit, c))
        for h in range(2):
            r = slice(unit * TM + h * CB, unit * TM + (h + 1) * CB)
            pp_ref[r, tile(c)] = v[h] if w == 0 else pp_ref[r, tile(c)] * v[h]

    def gu_plain(w, c, unit):
        x = lambda h: cat([lhs(unit, ("xy"[h], k)) for k in range(NL)], axis=1)
        gu_finish(w, unit, c, [bg.dot(x(h), w_refs[w][0][:, tile(c)]) for h in range(2)])

    def gu_main(w, unit, mid=None):
        dot = lambda a, b: bg.dot(lhs(unit, a), rhs(w, b))
        run_ref, off = (pp_ref, unit * TM) if w == 0 else (gs_ref, 0)
        for i in range(NL):
            if mid is not None and mid[0] == i:
                mid[1]()
            p = q = None
            for d in range(1, NL):
                j = (i + d) % NL
                lo, hi = min(i, j), max(i, j)
                e1 = dot(("s", i, j), ("E1", i, j))
                e2 = dot(("dx", lo, hi), ("E2", i, j))
                e3 = dot(("dy", lo, hi), ("E3", i, j))
                p = e2 if p is None else p + e2
                q = e1 + e3 if q is None else (q + e1) + e3
                rp, rq = e1 + e2, e3
                if d == 1:
                    x = dot(("x", i), ("D1", i))
                    p, q = p + x, q - x
                elif d == 2:
                    q = q + dot(("w", i), ("D2", i))
                elif d == 3:
                    rp = rp + dot(("w", j), ("D3", j))
                else:
                    x = dot(("y", j), ("D4", j))
                    rp, rq = rp - x, rq + x
                rs = [slice(off + h * CB, off + (h + 1) * CB) for h in range(2)]
                if i != others(j)[0]:
                    rp, rq = rp + run_ref[rs[0], tile(Rc(j))], rq + run_ref[rs[1], tile(Rc(j))]
                if i == others(j)[-1]:
                    gu_finish(w, unit, Rc(j), (rp, rq))
                else:
                    run_ref[rs[0], tile(Rc(j))] = rp
                    run_ref[rs[1], tile(Rc(j))] = rq
            gu_finish(w, unit, Lc(i), (p, q))

    def gu_left(w, unit):
        def dot(f, extra=()):
            ks = [f(i, j) for i, j in xpairs] + list(extra)
            return bg.dot(cat([lhs(unit, a) for a, _ in ks], axis=1), cat([rhs(w, b) for _, b in ks], axis=0))
        one = lambda a, b: bg.dot(lhs(unit, (a, NL - 1)), rhs(w, (b,)))
        e1 = dot(lambda i, j: (("s", i, j), ("e1", i, j)))
        e2 = dot(lambda i, j: (("dx", i, j), ("e2", i, j)))
        e3 = dot(lambda i, j: (("dy", i, j), ("e3", i, j)))
        d1 = dot(lambda i, j: (("x", i), ("d1", i)))
        pl_, ql, pr = e2 + d1, (e1 + e3) - d1, e1 + e2
        ql = ql + dot(lambda i, j: (("w", i), ("d2", i)), [(("y", NL - 1), ("pl",))])
        gu_finish(w, unit, LX, (pl_ + one("x", "pl"), ql))
        d4 = dot(lambda i, j: (("y", j), ("d4", j)))
        pr = (pr - d4) + dot(lambda i, j: (("w", j), ("d3", j)), [(("x", NL - 1), ("pr",))])
        gu_finish(w, unit, RX, (pr, (e3 + d4) + one("y", "pr")))

    def gu_fast(unit):
        gu_main(0, unit)
        gu_left(0, unit)
        gu_left(1, unit)
        gu_main(1, unit)

    def ffn_down(x1_src, t, unit, after=None, e=32):
        ob = o_ref.at[rows_of(t)]
        for r0 in range(0, HB, e):
            rows = lambda ref, base, c: cat([ref[base + o + r0:base + o + r0 + e, c] for o in (0, HB)], axis=0)
            hx = lambda c: rows(pp_ref, unit * TM, tile(c))
            hy = lambda c: rows(pp_ref, unit * TM + CB, tile(c))
            run = lambda h: slice(h * CB + 2 * r0, h * CB + 2 * (r0 + e))

            def left(key):
                kind = key[0]
                if kind[0] in "Ee":
                    l, r = (Lc(key[1]), Rc(key[2])) if kind[0] == "E" else (LX, RX)
                    return (hy if kind[1] == "3" else hx)(r) + (hx if kind[1] == "2" else hy)(l)
                if kind[1] in "12":
                    c = Lc(key[1]) if kind[0] == "D" else LX
                    return hx(c) - hy(c) if kind[1] == "1" else hy(c)
                c = Rc(key[1]) if kind[0] == "D" else RX
                return hx(c) if kind[1] == "3" else hy(c) - hx(c)

            def dot(keys, plain=None):
                keys = [kk for kk in keys if kk in b_terms]
                a = [left(kk) for kk in keys]
                if plain is not None:
                    a, keys = a + [plain(LX), plain(RX)], keys + [("pl",), ("pr",)]
                a, w = cat(a, axis=1), (lambda: cat([rhs(2, kk) for kk in keys], axis=0))
                if plain is not None and e == HB:
                    return cat([bg.dot(a[r:r + HB].astype(BF16), w()) for r in (0, HB)], axis=0)
                return bg.dot(a.astype(BF16), w())

            for i in range(NL):
                ls = lanes[i]
                last = i == NL - 1
                both = dot([("D2", i), ("D3", i), ("d2", i), ("d3", i)])
                p = both + dot([("D1", i), ("d1", i)], hx if last else None)
                q = both + dot([("D4", i), ("d4", i)], hy if last else None)
                if i > 0:
                    p, q = p + gs_ref[run(0), ls], q + gs_ref[run(1), ls]
                for j in range(i + 1, NL):
                    a = dot([("E1", i, j), ("e1", i, j)])
                    c3 = dot([("E3", i, j), ("E3", j, i), ("e3", i, j)])
                    rq = a - c3
                    gs_ref[run(1), lanes[j]] = rq + gs_ref[run(1), lanes[j]] if i > 0 else rq
                    b = dot([("E1", j, i)])
                    c2 = dot([("E2", i, j), ("E2", j, i), ("e2", i, j)])
                    rp = b + c2
                    gs_ref[run(0), lanes[j]] = rp + gs_ref[run(0), lanes[j]] if i > 0 else rp
                    p, q = (p + a) - c2, (q + c3) + b
                assert not check[0] or ('gb', i) in done
                for b, dn in enumerate((p, q)):
                    o = rows(x1_src, b * CB, ls) + _rep(mod_ref[4, :, ls], 2 * e) * dn
                    w = pltpu.pack_elementwise([o[:e], o[e:]], packed_dtype=BF16)
                    ob[run(b), ls] = pltpu.bitcast(w, BF16)
                if after is not None and r0 + e == HB:
                    after(i)

    x1s = [x1_ref.at[r] for r in range(NS)]
    sts = [st_ref.at[r * TM:(r + 1) * TM] for r in range(2)]

    def setup():
        for cp in small:
            cp.wait()
        shk = shk_ref[...].astype(F32)
        for a in range(4):
            sh_ref[a] = jnp.broadcast_to(shk[a:a + 1, :], (8, D))
        c = c_ref[...].astype(F32)
        sc_ref[...] = _pk(jnp.broadcast_to(c * jax.nn.sigmoid(c), (16, D)))
        zm_ref[...] = pltpu.bitcast(inv_ref[CB:CB + 16, :], I32)
        zs.append(zm_ref[0, 0])

    def prologue():
        ytile = lambda i: ystatic_pieces(y_first, False, [p for p in positions if p[1] == lanes[i]])
        ssm_cp(0).wait()
        k_fwd(0)
        for t in range(2):
            k_cp(t).wait()
            v_cp(t).wait()
            now(kv_pieces(t, 64))
            u_fwd(t)
        bg.flush()
        for i in range(1, NL):
            if i != 3:
                ssm_cp(i).wait()
            if i == 2:
                ssm_cp(3).wait()
            bg.add(ytile(i - 1), 0, 1024)
            k_fwd(i)
            bg.flush()
        q_cp(0).wait()
        now(ytile(NL - 1))
        q_cp(1).wait()
        mod_cp(0).wait()
        mod_chunk(0)
        for t in range(2):
            now(post_pieces(t))
            now(ln1_pieces(t))
            y_inv(t, x1s[t])
        for t in range(2):
            now(ln2_stat_pieces(x1s[t], sts[t]))
        bg.flush()

    def superstep():
        g_main = [g for m in range(NL) for g in g_cols(m)] + g_rows
        mod_cp(1).wait()
        mod_chunk(1)
        now(norm_pieces(x1s[0], sts[0], 0, more=False))
        bg.flush()
        g_cp(0).wait()
        bg.add(norm_pieces(x1s[1], sts[1], 1), 0, 480)
        bg.add(w_pieces(0, g_left), 640, 1150)
        for u in range(2):
            gu_plain(0, LX, u)
            gu_plain(0, RX, u)
        bg.flush()
        u_cp(0).wait()
        g_cp(1).wait()
        prs, np0 = pair_pieces(0), 30
        bg.add(pair_pieces(1) + w_pieces(1, g_left) + w_pieces(0, g_cols(0))
               + norm_pieces(x1s[0], sts[0], 0, base=False) + prs[:np0], 0, 1800)
        for u in range(2):
            gu_plain(1, LX, u)
            gu_plain(1, RX, u)
        gu_plain(0, 2, 0)
        gu_plain(0, 3, 0)
        bg.flush()
        g_cp(2).wait()
        npr = 80
        bg.add(w_pieces(0, g_main[len(g_cols(0)):]) + prs[np0:npr], 0, 2450)
        for c in range(4, 12):
            gu_plain(0, c, 0)
        bg.flush()
        u_cp(1).wait()
        bg.add(prs[npr:] + w_pieces(1, g_main), 0, 2450)
        gu_main(0, 1)
        bg.flush()
        k_cp(2).wait()
        v_cp(2).wait()
        q_cp(2).wait()
        ymid = _costed(_group(ystatic_pieces([(s, 4, 6) for s in (4, 5)], True), 2), 35)
        posts = post_pieces(2)
        fr, ny = 2, 120
        bg.add(kv_pieces(2), 0, fr * 512 - 150)
        bg.add(linked(ln1_pieces(2), 6), 850, 1700)
        bg.add(ymid[:ny], fr * 512 + 750, 3100)
        gu_main(1, 0, (fr, lambda: u_fwd(2)))
        bg.flush()
        d_cp.wait()
        order_d = g_left + [g for i in range(NL) for g in (
            [[(d, i)] for d in ("D2", "D3", "D1", "D4")]
            + [g for j in range(i + 1, NL) for g in (g_edge(i, j), g_edge(j, i))])]
        wdp = w_pieces(2, order_d)
        nd = len(wdp) * 89 // 100
        bg.add(wdp[:nd], 0, 2450)
        gu_main(1, 1)
        bg.flush()
        mod_cp(2).wait()
        k_cp(3).wait()
        v_cp(3).wait()
        bg.add(wdp[nd:] + ymid[ny:] + posts + kv_pieces(3, 16), 0, 3300)
        bg.inj = [(100 + 130 * i, gb_tile(i)) for i in range(NL)]
        ffn_down(x1s[0], 0, 0, e=HB)
        y_inv(2, x1s[2])
        bg.flush()
        o_cp(0).start()

    def step(t, carry):
        q_cp(t).wait()

        @pl.when(t + 1 < NS)
        def _():
            k_cp(t + 1).wait()
            v_cp(t + 1).wait()

        x1v = x1_ref.at[pl.ds(t - 2, 3)]
        x1 = x1v.at[2]
        bg.add(linked(ln1_pieces(t), 2), 4000, 8500)
        bg.add(ln2_stat_pieces(x1v.at[1], st_ref), 0, 600)
        bg.add(factor_pieces(x1v.at[1], st_ref, 1), 800, 3100)
        kv_live.update((b, ls.start) for b in range(2) for ls in lanes)
        kvp = kv_pieces(jnp.minimum(t + 1, NS - 1), 32)
        nk = len(kvp) * 60 // 100
        bg.add(kvp[:nk], 3136 + 70, 3136 + 700)
        bg.add(kvp[nk:], 9000, 10200)
        ffn_down(x1v.at[0], t - 2, 1)
        u_fwd(t)
        chain(diag_pieces(t, T0 - 1), 2)
        chain(task_pieces(t, 2), 3)
        dep = chain(task_pieces(t, 1), 3)
        chain(post_pieces(t), 1, 3, dep)
        gu_fast(1)
        y_inv(t, x1)
        bg.flush()
        o_cp(t - 2).start()
        return carry

    def epilogue():
        t = NS - 1
        bg.add(ln2_stat_pieces(x1s[t], st_ref), 0, 500)
        bg.add(factor_pieces(x1s[t], st_ref, 1), 700, 2900)
        ffn_down(x1s[t - 1], t - 1, 1)
        o_cp(t - 1).start()
        gu_fast(1)
        cols = [(0 if i == 1 else i * 128, (i + 1) * 128) for i in range(1, NL)]
        last = [pltpu.make_async_copy(o_ref.at[rows_of(t), lo:hi], o_hbm.at[rows_of(t), lo:hi], sem.at[s_o + t + i])
                for i, (lo, hi) in enumerate(cols)]
        ffn_down(x1s[t], t, 1, after=lambda i: i > 0 and last[i - 1].start(), e=HB)
        for i in range(NS - 1):
            o_cp(i).wait()
        for cp in last:
            cp.wait()

    def everything(i, carry):
        prologue()
        superstep()
        lax.fori_loop(T0, NS, step, 0)
        epilogue()
        return carry

    setup()
    lax.fori_loop(0, zs[0] + 1, everything, 0)


@jax.jit
def pallas_adaLN_cond__ssm_conv_h3__glu_gated_bilinear__prompt_kernel(
    A_q, A_k, A_v, A_shift_k, A_ssm_k, A_ssm_D, B_x, B_w_gate, B_w_up, B_w_down, c, w_mod,
):
    B, S, D = A_q.shape
    Fh = B_w_gate.shape[1]
    NB = S // CB
    NS = S // TM
    fwd, inv = _dft_consts()
    anyspec = pl.BlockSpec(memory_space=pl.ANY)
    V = pltpu.VMEM
    out = pl.pallas_call(
        functools.partial(_kernel, S=S, D=D, Fh=Fh),
        in_specs=[anyspec] * 13,
        out_specs=anyspec,
        out_shape=jax.ShapeDtypeStruct((S, D), A_q.dtype),
        scratch_shapes=[
            V((NS, 2, 3 * CB, D), F32),
            V((NB, 3 * CB, D), F32),
            V((NS, 2, 3 * CB, D), F32),
            V((NS, TM, D), F32),
            V((S, D), BF16), V((S, D), BF16), V((S, D), BF16), V((S, D), BF16),
            V((TM, D), F32),
            V((2 * TM, 256), F32),
            V((2 * TM, Fh), F32),
            V((TM, Fh), F32),
            V((TM, D), F32),
            V((55 * HB, 256), U32),
            V((TM // 2, D), U32),
            V((2 * CB, D), U32),
            V((48 * HB, 256), U32), V((48 * HB, 256), U32), V((48 * HB, 256), U32),
            V((D, S), BF16), V((D, 6 * D), BF16), V((D, Fh), BF16), V((D, Fh), BF16), V((Fh, D), BF16),
            V((2 * CB, CB), BF16), V((CB + 16, CB), BF16),
            V((5, 8, D), F32), V((4, 8, D), F32), V((8, 128), I32), V((8, D), U32),
            V((4, D), BF16), V((D,), BF16), V((1, D), BF16),
            pltpu.SemaphoreType.DMA((5 + 4 * NS + D // 128 + 3 + 5 + 4,)),
        ],
        compiler_params=pltpu.CompilerParams(
            internal_scratch_in_bytes=48 * 1024,
            disable_semaphore_checks=True,
            disable_bounds_checks=True,
            vmem_limit_bytes=110 * 1024 * 1024),
        name="adaln_h3_glu",
    )(A_q.reshape(S, D), A_k.reshape(S, D), A_v.reshape(S, D), A_shift_k.T, A_ssm_k,
      A_ssm_D, B_w_gate, B_w_up, B_w_down, c, w_mod, fwd, inv)
    return out.reshape(B, S, D)
```

```python
import functools

import numpy as np
import jax
import jax.numpy as jnp
from jax import lax
import jax.experimental.pallas as pl
import jax.experimental.pallas.tpu as pltpu

F32 = jnp.float32
BF16 = jnp.bfloat16
U32 = jnp.uint32
I32 = jnp.int32

CB = 128
HB = CB // 2
TM = 256
FC = 256
EPS = 1e-5


def _dft_consts():
    k = np.arange(CB, dtype=np.float64)[:, None]
    n = np.arange(CB, dtype=np.float64)[None, :]
    th = np.pi * (4.0 * k + 1.0) * n / (2.0 * CB)
    fwd = np.concatenate([np.cos(th), np.sin(th)], axis=0)
    g = np.concatenate([np.cos(th[:HB]), np.sin(th[:HB])], axis=0).T / CB
    inv = np.concatenate([g[0::2], g[1::2], np.zeros((16, CB))], axis=0)
    return jnp.asarray(fwd, dtype=BF16), jnp.asarray(inv, dtype=BF16)


def _pk(x):
    return pltpu.bitcast(x.astype(BF16), U32)


def _unpk(x):
    return pltpu.bitcast(x, BF16)


def _rep(r, n):
    return r if n == 8 else jnp.concatenate([r] * (n // 8), axis=0)


def _add(x, tok):
    return x if tok is None else x + _rep(tok, x.shape[0])


def _costed(pieces, cost):
    for p in pieces:
        p.cost = cost
    return pieces


def _group(pieces, n):
    def merged(ps):
        def run(tok):
            for p in ps:
                p(tok)
        return run
    return [merged(pieces[i:i + n]) for i in range(0, len(pieces), n)]


class _Sched:
    def __init__(self, token):
        self.token = token
        self.clock = 0.0
        self.q = []
        self.last = None
        self.inj = []

    def add(self, pieces, t0, t1):
        cum = np.cumsum([0.0] + [getattr(p, "cost", 1.0) for p in pieces])
        self.q += [(t0 + (t1 - t0) * cum[i] / cum[-1], i, p) for i, p in enumerate(pieces)]
        self.q.sort(key=lambda e: e[:2])

    def note(self, m, dt):
        rows, cols = m.shape
        tiles = [(slice(r, r + 8), slice(c, c + 128)) for c in range(0, cols, 128) for r in range(0, rows, 8)]
        for i, tl in enumerate(tiles):
            tok = None
            while self.q and self.q[0][0] <= self.clock + dt * (i + 1) / len(tiles):
                if tok is None:
                    tok = self.token(m[tl])
                self.q.pop(0)[2](tok)
        self.clock += dt
        self.last = m[tiles[-1]]
        return m

    def dot(self, a, b):
        if self.inj and self.clock >= self.inj[0][0]:
            self.inj.pop(0)[1]()
        m = jnp.dot(a, b, preferred_element_type=F32)
        return self.note(m, max(a.shape[0], 32) * (a.shape[1] // 128) * (b.shape[1] // 128) / 4)

    def flush(self):
        tok = None if self.last is None or not self.q else self.token(self.last)
        while self.q:
            self.q.pop(0)[2](tok)
        self.clock = 0.0
        self.last = None


def _kernel(q_hbm, k_hbm, v_hbm, shk_hbm, ssmk_hbm, ssmd_hbm, wg_hbm, wu_hbm, wd_hbm,
            c_hbm, wmod_hbm, fwd_hbm, inv_hbm, o_hbm,
            u_ref, kk_ref, y_ref, x1_ref, q_ref, k_ref, v_ref, o_ref,
            hp_ref, st_ref, pp_ref, gs_ref, hn_ref, hf_ref, kv_ref, yb_ref, wgf_ref, wuf_ref, wdf_ref,
            ssmk_ref, wmod_ref, wg_ref, wu_ref, wd_ref, fwd_ref, inv_ref,
            mod_ref, sh_ref, zm_ref, sc_ref, fwp_ref, shk_ref, ssmd_ref, c_ref,
            sem, *, S, D, Fh):
    NB = S // CB
    NS = S // TM
    NL = D // 128
    T0 = 3
    NLOOP = NS - T0
    lanes = [slice(i * 128, (i + 1) * 128) for i in range(NL)]
    cat = jnp.concatenate

    offs = [int(o) for o in np.cumsum([0, 5, NS, NS, NS, NL, 3, 3, 2, 1])]
    s_small, s_q, s_k, s_v, s_ssm, s_mod, s_g, s_u, s_d, s_o = offs

    def rows_of(t):
        return pl.ds(t * TM if isinstance(t, int) else pl.multiple_of(t * TM, TM), TM)

    def rows_cp(src, dst, base, t):
        return pltpu.make_async_copy(src.at[rows_of(t), :], dst.at[rows_of(t), :], sem.at[base + t])

    def cols_cp(src, dst, lo, hi, si):
        return pltpu.make_async_copy(src.at[:, lo:hi], dst.at[:, lo:hi], sem.at[si])

    q_cp = lambda t: rows_cp(q_hbm, q_ref, s_q, t)
    k_cp = lambda t: rows_cp(k_hbm, k_ref, s_k, t)
    v_cp = lambda t: rows_cp(v_hbm, v_ref, s_v, t)
    o_cp = lambda t: rows_cp(o_ref, o_hbm, s_o, t)
    small = [pltpu.make_async_copy(s, d, sem.at[s_small + i]) for i, (s, d) in enumerate(
        [(fwd_hbm, fwd_ref), (shk_hbm, shk_ref), (ssmd_hbm, ssmd_ref), (inv_hbm, inv_ref), (c_hbm, c_ref)])]
    ssm_cp = lambda i: pltpu.make_async_copy(ssmk_hbm.at[lanes[i], :], ssmk_ref.at[lanes[i], :],
                                             sem.at[s_ssm + i])
    mod_cols = [(0, 3 * D), (3 * D, 5 * D), (5 * D, 6 * D)]
    mod_cp = lambda i: cols_cp(wmod_hbm, wmod_ref, mod_cols[i][0], mod_cols[i][1], s_mod + i)
    g_cp = lambda f: cols_cp(wg_hbm, wg_ref, f * FC, (f + 1) * FC if f < 2 else Fh, s_g + f)
    u_cp = lambda f: cols_cp(wu_hbm, wu_ref, f * FC, (f + 1) * FC if f < 1 else Fh, s_u + f)
    d_cp = pltpu.make_async_copy(wd_hbm, wd_ref, sem.at[s_d])

    order = small + [ssm_cp(0), k_cp(0), v_cp(0), k_cp(1), v_cp(1),
                     ssm_cp(1), ssm_cp(2), ssm_cp(3), ssm_cp(4), q_cp(0), q_cp(1),
                     mod_cp(0), mod_cp(1)]
    order += [g_cp(0), u_cp(0), g_cp(1), g_cp(2), u_cp(1)]
    order += [k_cp(2), v_cp(2), q_cp(2), d_cp, mod_cp(2), k_cp(3), v_cp(3)]
    for t in range(T0, NS):
        order += [q_cp(t)]
        if t + 1 < NS:
            order += [k_cp(t + 1), v_cp(t + 1)]
    for cp in order:
        cp.start()

    zs = []
    bg = _Sched(lambda x: pltpu.bitcast(pltpu.bitcast(x, I32) & zm_ref[...], F32))

    def opaque(ref):
        return ref.at[pl.ds(pl.multiple_of(zs[0], 32), ref.shape[0])]

    def chain(pieces, dist, extra=0, dep=None):
        hist = [] if dep is None else [dep] * dist
        for p in pieces:
            tok = None
            if len(hist) >= dist:
                tok = bg.token(hist[-dist])
                for _ in range(extra):
                    tok = tok + tok
            hist.append(p(tok))
        return hist[-1]

    def linked(pieces, d):
        res = []

        def wrap(p):
            def run(tok):
                if d and len(res) >= d:
                    tok = tok + bg.token(res[-d])
                res.append(p(tok))
            return run
        return [wrap(p) for p in pieces]

    def now(pieces):
        for p in pieces:
            p(None)

    def mod_chunk(i):
        lo, hi = mod_cols[i]
        m = bg.dot(_unpk(sc_ref[...]), wmod_ref[:, lo:hi])[0:8]
        if i == 0:
            ga = m[:, 2 * D:3 * D]
            mod_ref[0] = (1.0 + m[:, D:2 * D]) * ga
            mod_ref[1] = m[:, 0:D] * ga
        else:
            mod_ref[2] = 1.0 + m[:, D:2 * D]
            mod_ref[3] = m[:, 0:D]

    def gb_tile(i):
        def run():
            w = wmod_ref[:, 5 * D + i * 128:5 * D + (i + 1) * 128]
            mod_ref[4, :, lanes[i]] = jnp.dot(_unpk(sc_ref[...]), w, preferred_element_type=F32)[0:8]
            done.add(('gb', i))
        return run

    def k_fwd(i):
        ls = lanes[i]
        fwd = fwd_ref[...]
        prev = None
        for m in range(NB):
            kf = lax.dot_general(fwd, ssmk_ref[ls, m * CB:(m + 1) * CB], (((1,), (1,)), ((), ())),
                                 preferred_element_type=F32)
            if m == 0:
                c = kf[:CB] + ssmd_ref[...].astype(F32).reshape(1, D)[:, ls]
                d = kf[CB:]
            else:
                c = kf[:CB] + prev[CB:]
                d = kf[CB:] - prev[:CB]
            prev = kf
            kk_ref[m, 0:CB, ls] = c
            kk_ref[m, CB:2 * CB, ls] = d - c
            kk_ref[m, 2 * CB:3 * CB, ls] = c + d
            if m % 4 == 3:
                bg.note(kf, 2 * CB)

    def lo_hi(w):
        return pltpu.bitcast(w << 16, F32), pltpu.bitcast(w & jnp.uint32(0xFFFF0000), F32)

    kv_live = set()

    def kv_pieces(t, G=32):
        n = G // 2
        kb, vb = k_ref.at[rows_of(t)], v_ref.at[rows_of(t)]

        def piece(ls, r0):
            def run(tok):
                assert (r0 // CB, ls.start) not in kv_live
                if r0 > 0:
                    w = pltpu.bitcast(kb[r0 - 16:r0 + G, ls], U32)
                else:
                    if isinstance(t, int) and t == 0:
                        halo = jnp.zeros((8, 128), U32)
                    else:
                        halo = pltpu.bitcast(k_ref.at[rows_of(t - 1)][TM - 16:TM, ls], U32)
                    w = cat([halo, pltpu.bitcast(kb[0:G, ls], U32)], axis=0)
                if tok is not None:
                    w = w | _rep(pltpu.bitcast(tok, U32), n + 8)
                ke, ko = lo_hi(w[8:])
                ke1, ko1 = lo_hi(pltpu.roll(w, 1, 0)[8:])
                _, ko2 = lo_hi(pltpu.roll(w, 2, 0)[8:])
                s0, s1, s2, s3 = [_rep(sh_ref[a, :, ls], n) for a in range(4)]
                ve, vo = lo_hi(pltpu.bitcast(vb[r0:r0 + G, ls], U32))
                kve = ((ke * s0 + ko1 * s1) + (ke1 * s2 + ko2 * s3)) * ve
                kvo = ((ko * s0 + ke * s1) + (ko1 * s2 + ke1 * s3)) * vo
                kv_ref[r0 // 2:(r0 + G) // 2, ls] = _pk(
                    cat([x[r:r + 8] for r in range(0, n, 8) for x in (kve, kvo)], axis=0))
            return run
        return _costed([piece(ls, r0) for b in range(2) for ls in lanes
                        for r0 in range(b * CB, (b + 1) * CB, G)], 2.5 * G + 10)

    def u_fwd(t):
        for b in range(2):
            for ls in lanes:
                kv = lambda: _unpk(kv_ref[b * HB:(b + 1) * HB, ls])
                a = bg.dot(_unpk(fwp_ref[:, 0:CB]), kv())
                kv2 = kv()
                kv_live.discard((b, ls.start))
                bb = bg.dot(_unpk(fwp_ref[:, CB:2 * CB]), kv2)
                u_ref[t, b, 0:CB, ls] = a + bb
                u_ref[t, b, CB:2 * CB, ls] = a
                u_ref[t, b, 2 * CB:3 * CB, ls] = bb

    positions = [(slice(r0, r0 + 8), ls) for r0 in range(0, 3 * CB, 8) for ls in lanes]

    def ystatic_pieces(blocks, acc_in, pos=None):
        def piece(rs, ls):
            def run(tok):
                us, ks = {}, {}
                for s, lo, hi in blocks:
                    acc = None
                    for i in range(lo, min(hi, s + 1)):
                        if i not in us:
                            us[i] = _add(u_ref[i // 2, i % 2, rs, ls], tok)
                        if s - i not in ks:
                            ks[s - i] = kk_ref[s - i, rs, ls]
                        p = ks[s - i] * us[i]
                        acc = p if acc is None else acc + p
                    if acc_in:
                        acc = acc + y_ref[s // 2, s % 2, rs, ls]
                    y_ref[s // 2, s % 2, rs, ls] = acc
                return acc
            return run
        return _costed([piece(*p) for p in (positions if pos is None else pos)], 35)

    y_first = [(s, 0, 4) for s in range(NB)]

    def task_pieces(t, delta):
        p = t - delta
        left = p >= T0
        J = jnp.where(left, t, p + NLOOP)
        I = jnp.where(left, p, t)
        kview = kk_ref.at[pl.ds(2 * (J - I) - 1, 3)]

        def piece(rs, ls):
            def run(tok):
                u0 = _add(u_ref[I, 0, rs, ls], tok)
                u1 = _add(u_ref[I, 1, rs, ls], tok)
                kc = kview[1, rs, ls]
                y_ref[J, 0, rs, ls] = (kc * u0 + kview[0, rs, ls] * u1) + y_ref[J, 0, rs, ls]
                y1 = (kview[2, rs, ls] * u0 + kc * u1) + y_ref[J, 1, rs, ls]
                y_ref[J, 1, rs, ls] = y1
                return y1
            return run
        return [piece(*p) for p in positions]

    def diag_pieces(t, I):
        kview = kk_ref.at[pl.ds(2 * (t - I) - 1, 3)]

        def piece(rs, ls):
            def run(tok):
                us = [_add(u_ref[a, b, rs, ls], tok) for a in (t, I) for b in range(2)]
                k0 = kk_ref[0, rs, ls]
                kc = kview[1, rs, ls]
                y_ref[t, 0, rs, ls] = ((k0 * us[0] + y_ref[t, 0, rs, ls])
                                       + (kc * us[2] + kview[0, rs, ls] * us[3]))
                y1 = ((kk_ref[1, rs, ls] * us[0] + k0 * us[1])
                      + (kview[2, rs, ls] * us[2] + kc * us[3]) + y_ref[t, 1, rs, ls])
                y_ref[t, 1, rs, ls] = y1
                return y1
            return run
        return [piece(*p) for p in positions]

    def post_pieces(t):
        def piece(b, r0, ls):
            def run(tok):
                comp = lambda c, off: y_ref[t, b, c * CB + off + r0:c * CB + off + r0 + 16, ls]
                k1l, k1h = _add(comp(0, 0), tok), _add(comp(0, HB), tok)
                rel, reh = k1l - comp(2, 0), k1h - comp(2, HB)
                iml, imh = k1l + comp(1, 0), k1h + comp(1, HB)
                p0 = b * CB + r0 // 2
                yb_ref[p0:p0 + 8, ls] = _pk(rel + reh)
                yb_ref[p0 + HB // 2:p0 + HB // 2 + 8, ls] = _pk(iml + imh)
                yb_ref[p0 + HB:p0 + HB + 8, ls] = _pk(rel - reh)
                oim = iml - imh
                yb_ref[p0 + HB + HB // 2:p0 + HB + HB // 2 + 8, ls] = _pk(oim)
                return oim[8:16]
            return run
        return _costed([piece(b, r0, ls) for b in range(2) for r0 in range(0, HB, 16) for ls in lanes], 45)

    def q_split(t, b, p0, n, ls):
        w = pltpu.bitcast(q_ref.at[rows_of(t)][b * CB + 2 * p0:b * CB + 2 * p0 + 2 * n, ls], U32)
        return lo_hi(w)

    def ln_tiles(xs, tok):
        n = xs[0].shape[0]
        s = _add(xs[0], tok)
        for x in xs[1:]:
            s = s + x
        m = jnp.sum(s, axis=-1, keepdims=True) * (1.0 / D)
        xc = [x - m for x in xs]
        s2 = xc[0] * xc[0]
        for x in xc[1:]:
            s2 = s2 + x * x
        r = lax.rsqrt(jnp.sum(s2, axis=-1, keepdims=True) * (1.0 / D) + EPS)
        return xc, jnp.broadcast_to(r, (n, 128)), jnp.broadcast_to(m, (n, 128))

    def ln1_pieces(t):
        G = 8

        def piece(b, p0):
            def run(tok):
                xc, r, _ = ln_tiles([cat(q_split(t, b, p0, G, ls), axis=0) for ls in lanes], tok)
                for ls, x in zip(lanes, xc):
                    h = (x * r) * _rep(mod_ref[0, :, ls], 2 * G) + _rep(mod_ref[1, :, ls], 2 * G)
                    hp_ref[b * CB + p0:b * CB + p0 + G, ls] = h[:G]
                    hp_ref[b * CB + HB + p0:b * CB + HB + p0 + G, ls] = h[G:]
                return functools.reduce(lambda a, c: a + c, [h[r:r + 8] for r in range(0, 2 * G, 8)])
            return run
        return [piece(b, p0) for b in range(2) for p0 in range(0, HB, G)]

    def y_inv(t, x1_dst):
        yb = opaque(yb_ref)
        hp = opaque(hp_ref)
        for b in range(2):
            ye = bg.dot(inv_ref[0:HB, :], _unpk(yb[b * CB:b * CB + HB, :]))
            yo = bg.dot(inv_ref[HB:CB, :], _unpk(yb[b * CB + HB:(b + 1) * CB, :]))
            for ls in lanes:
                qe, qo = q_split(t, b, 0, HB, ls)
                re, ro = slice(b * CB, b * CB + HB), slice(b * CB + HB, (b + 1) * CB)
                x1_dst[pl.ds(2 * ls.start + b * CB, HB, stride=2), :] = qe + hp[re, ls] * ye[:, ls]
                x1_dst[pl.ds(2 * ls.start + b * CB + 1, HB, stride=2), :] = qo + hp[ro, ls] * yo[:, ls]

    def ln2_stat_pieces(x1_src, st):
        x1o = opaque(x1_src)

        def piece(r0):
            def run(tok):
                _, r, m = ln_tiles([x1o[j * TM + r0:j * TM + r0 + 16, :] for j in range(NL)], tok)
                st[r0:r0 + 16, 0:128] = m
                st[r0:r0 + 16, 128:256] = r
                return r[0:8] + r[8:16]
            return run
        return [piece(h * CB + r0) for r0 in range(0, CB, 16) for h in range(2)]

    tile = lambda j: slice(j * 128, (j + 1) * 128)
    LX, RX = 0, 1
    Lc = lambda i: 2 + 2 * i
    RS = 2
    Rc = lambda i: 3 + 2 * ((i - RS) % NL)
    others = lambda i: [j for j in range(NL) if j != i]
    edges = [(i, j) for i in range(NL) for j in others(i)]
    pairs = [(i, j) for i, j in edges if i < j]
    a_idx = {k: n for n, k in enumerate(
        [(c, i) for c in "xyw" for i in range(NL)] + [("s",) + e for e in edges]
        + [(c,) + e for c in ("dx", "dy") for e in pairs])}
    b_terms = {}
    for i in range(NL):
        b_terms["D1", i] = [(1, k, Lc(i)) for k in range(NL)]
        b_terms["D2", i] = [(1, i, Lc(i))] + [(-1, i, Rc(j)) for j in others(i)]
        b_terms["D3", i] = [(1, i, Rc(i))] + [(-1, i, Lc(j)) for j in others(i)]
        b_terms["D4", i] = [(1, k, Rc(i)) for k in range(NL)]
    for i, j in edges:
        sg = 1 if i < j else -1
        b_terms["E1", i, j] = [(1, i, Rc(j)), (1, j, Lc(i))]
        b_terms["E2", i, j] = [(sg, j, Lc(i))]
        b_terms["E3", i, j] = [(sg, i, Rc(j))]
    xpairs = [(0, 1), (2, 3)]
    for i, j in xpairs:
        b_terms["d1", i] = [(1, i, LX), (1, j, LX)]
        b_terms["d2", i] = [(1, i, LX), (-1, i, RX)]
        b_terms["d3", j] = [(1, j, RX), (-1, j, LX)]
        b_terms["d4", j] = [(1, j, RX), (1, i, RX)]
        b_terms["e1", i, j] = [(1, i, RX), (1, j, LX)]
        b_terms["e2", i, j] = [(1, j, LX)]
        b_terms["e3", i, j] = [(1, i, RX)]
    b_terms["pl",] = [(1, NL - 1, LX)]
    b_terms["pr",] = [(1, NL - 1, RX)]
    b_idx = {k: n for n, k in enumerate(b_terms)}
    w_refs = ((wg_ref, wgf_ref), (wu_ref, wuf_ref), (wd_ref, wdf_ref))
    done = set()
    check = [True]

    def norm_pieces(x1_src, st, unit, more=True, base=True):
        G = 16
        x1o = opaque(x1_src)

        def piece(r0, j):
            def run(tok):
                ls = lanes[j]
                two = lambda ref, c: cat([ref[r0:r0 + G, c], ref[CB + r0:CB + r0 + G, c]], axis=0)
                m, r = _add(two(st, slice(0, 128)), tok), two(st, slice(128, 256))
                x = cat([x1o[j * TM + o + r0:j * TM + o + r0 + G, :] for o in (0, CB)], axis=0)
                h = ((x - m) * r) * _rep(mod_ref[2, :, ls], 2 * G) + _rep(mod_ref[3, :, ls], 2 * G)
                if base:
                    put_a(unit, r0, ("x", j), h[:G])
                    put_a(unit, r0, ("y", j), h[G:])
                if more:
                    put_a(unit, r0, ("w", j), h[:G] + h[G:])
                    hn_ref[r0:r0 + G, ls] = h[:G]
                    hn_ref[CB + r0:CB + r0 + G, ls] = h[G:]
            return run
        return _costed([piece(r0, j) for r0 in range(0, CB, G) for j in range(NL)], 44)

    def put_a(unit, r0, key, v):
        p0 = a_idx[key] * HB + r0 // 2
        hf_ref[p0:p0 + v.shape[0] // 2, lanes[unit]] = _pk(v)
        done.add(("a", unit, key, r0))

    def pair_pieces(unit):
        G = 16

        def piece(r0, i, j):
            def run(tok):
                assert ("a", unit, ("w", j), r0) in done
                ld = lambda h, k: hn_ref[h * CB + r0:h * CB + r0 + G, lanes[k]]
                xi, yi, xj, yj = _add(ld(0, i), tok), _add(ld(1, i), tok), ld(0, j), ld(1, j)
                put_a(unit, r0, ("s", i, j), xi + yj)
                put_a(unit, r0, ("s", j, i), xj + yi)
                put_a(unit, r0, ("dx", i, j), xj - xi)
                put_a(unit, r0, ("dy", i, j), yi - yj)
            return run
        return _costed([piece(r0, i, j) for r0 in range(0, CB, G) for i, j in pairs], 30)

    def factor_pieces(x1_src, st, unit):
        nrm, prs = norm_pieces(x1_src, st, unit), pair_pieces(unit)
        a, b = len(nrm) // 8, len(prs) // 8
        return [p for g in range(8) for p in nrm[g * a:(g + 1) * a] + prs[g * b:(g + 1) * b]]

    def w_pieces(w, groups):
        src, dst = w_refs[w]

        def piece(keys, r0, G):
            def run(tok):
                blk = {}

                def ld(k, c):
                    if (k, c) not in blk:
                        rt, ct = (k, c) if w < 2 else (c, k)
                        v = src[rt * 128 + r0:rt * 128 + r0 + G, tile(ct)].astype(F32)
                        blk[k, c] = _add(v, tok) if len(blk) < 2 else v
                    return blk[k, c]
                for key in keys:
                    acc = None
                    for sg, k, c in b_terms[key]:
                        v = ld(k, c)
                        acc = (v if sg > 0 else -v) if acc is None else (acc + v if sg > 0 else acc - v)
                    p0 = (b_idx[key] // 2) * HB + r0 // 2
                    dst[p0:p0 + G // 2, tile(b_idx[key] % 2)] = _pk(acc)
                    done.add(("b", w, key, r0 + G))
            return run
        out = []
        for keys in groups:
            G = 32 if len(keys) in (2, 3) else 16
            n = len({t[1:] for k in keys for t in b_terms[k]})
            out += _costed([piece(keys, r0, G) for r0 in range(0, CB, G)], (3 * n + len(keys) + 2) * G / 8)
        return out

    g_edge = lambda i, j: [("E1", i, j), ("E2", i, j), ("E3", i, j)]
    g_left = [[("e1", i, j), ("e2", i, j), ("e3", i, j), ("d1", i), ("d2", i), ("d3", j), ("d4", j)]
              for i, j in xpairs] + [[("pl",), ("pr",)]]
    g_cols = lambda m: ([[("D1", m)], [("D4", (m + RS) % NL)]]
                        + [g_edge(i, j) for i, j in edges if max(Lc(i), Rc(j)) // 2 == m + 1])
    g_rows = [[(d, i)] for i in range(NL) for d in ("D2", "D3")]

    def rhs(w, key):
        assert not check[0] or ("b", w, key, CB) in done, (w, key)
        return _unpk(w_refs[w][1][(b_idx[key] // 2) * HB:(b_idx[key] // 2 + 1) * HB, tile(b_idx[key] % 2)])

    def lhs(unit, key):
        assert not check[0] or all(("a", unit, key, r) in done for r in range(0, CB, 16)), key
        return _unpk(hf_ref[a_idx[key] * HB:(a_idx[key] + 1) * HB, lanes[unit]])

    def gu_finish(w, unit, c, v):
        assert w == 0 or not check[0] or ("g", unit, c) in done
        done.add(("g", unit, c))
        for h in range(2):
            r = slice(unit * TM + h * CB, unit * TM + (h + 1) * CB)
            pp_ref[r, tile(c)] = v[h] if w == 0 else pp_ref[r, tile(c)] * v[h]

    def gu_plain(w, c, unit):
        x = lambda h: cat([lhs(unit, ("xy"[h], k)) for k in range(NL)], axis=1)
        gu_finish(w, unit, c, [bg.dot(x(h), w_refs[w][0][:, tile(c)]) for h in range(2)])

    def gu_main(w, unit, mid=None):
        dot = lambda a, b: bg.dot(lhs(unit, a), rhs(w, b))
        run_ref, off = (pp_ref, unit * TM) if w == 0 else (gs_ref, 0)
        for i in range(NL):
            if mid is not None and mid[0] == i:
                mid[1]()
            p = q = None
            for d in range(1, NL):
                j = (i + d) % NL
                lo, hi = min(i, j), max(i, j)
                e1 = dot(("s", i, j), ("E1", i, j))
                e2 = dot(("dx", lo, hi), ("E2", i, j))
                e3 = dot(("dy", lo, hi), ("E3", i, j))
                p = e2 if p is None else p + e2
                q = e1 + e3 if q is None else (q + e1) + e3
                rp, rq = e1 + e2, e3
                if d == 1:
                    x = dot(("x", i), ("D1", i))
                    p, q = p + x, q - x
                elif d == 2:
                    q = q + dot(("w", i), ("D2", i))
                elif d == 3:
                    rp = rp + dot(("w", j), ("D3", j))
                else:
                    x = dot(("y", j), ("D4", j))
                    rp, rq = rp - x, rq + x
                rs = [slice(off + h * CB, off + (h + 1) * CB) for h in range(2)]
                if i != others(j)[0]:
                    rp, rq = rp + run_ref[rs[0], tile(Rc(j))], rq + run_ref[rs[1], tile(Rc(j))]
                if i == others(j)[-1]:
                    gu_finish(w, unit, Rc(j), (rp, rq))
                else:
                    run_ref[rs[0], tile(Rc(j))] = rp
                    run_ref[rs[1], tile(Rc(j))] = rq
            gu_finish(w, unit, Lc(i), (p, q))

    def gu_left(w, unit):
        def dot(f, extra=()):
            ks = [f(i, j) for i, j in xpairs] + list(extra)
            return bg.dot(cat([lhs(unit, a) for a, _ in ks], axis=1), cat([rhs(w, b) for _, b in ks], axis=0))
        one = lambda a, b: bg.dot(lhs(unit, (a, NL - 1)), rhs(w, (b,)))
        e1 = dot(lambda i, j: (("s", i, j), ("e1", i, j)))
        e2 = dot(lambda i, j: (("dx", i, j), ("e2", i, j)))
        e3 = dot(lambda i, j: (("dy", i, j), ("e3", i, j)))
        d1 = dot(lambda i, j: (("x", i), ("d1", i)))
        pl_, ql, pr = e2 + d1, (e1 + e3) - d1, e1 + e2
        ql = ql + dot(lambda i, j: (("w", i), ("d2", i)), [(("y", NL - 1), ("pl",))])
        gu_finish(w, unit, LX, (pl_ + one("x", "pl"), ql))
        d4 = dot(lambda i, j: (("y", j), ("d4", j)))
        pr = (pr - d4) + dot(lambda i, j: (("w", j), ("d3", j)), [(("x", NL - 1), ("pr",))])
        gu_finish(w, unit, RX, (pr, (e3 + d4) + one("y", "pr")))

    def gu_fast(unit):
        gu_main(0, unit)
        gu_left(0, unit)
        gu_left(1, unit)
        gu_main(1, unit)

    def ffn_down(x1_src, t, unit, after=None, e=128):
        ob = o_ref.at[rows_of(t)]
        for r0 in range(0, CB, e):
            run = lambda h, base=0: slice(base + h * CB + r0, base + h * CB + r0 + e)
            hx = lambda c: pp_ref[run(0, unit * TM), tile(c)]
            hy = lambda c: pp_ref[run(1, unit * TM), tile(c)]

            def left(key):
                kind = key[0]
                if kind[0] in "Ee":
                    l, r = (Lc(key[1]), Rc(key[2])) if kind[0] == "E" else (LX, RX)
                    return (hy if kind[1] == "3" else hx)(r) + (hx if kind[1] == "2" else hy)(l)
                if kind[1] in "12":
                    c = Lc(key[1]) if kind[0] == "D" else LX
                    return hx(c) - hy(c) if kind[1] == "1" else hy(c)
                c = Rc(key[1]) if kind[0] == "D" else RX
                return hx(c) if kind[1] == "3" else hy(c) - hx(c)

            def dot(keys, plain=None):
                keys = [kk for kk in keys if kk in b_terms]
                a = [left(kk) for kk in keys]
                if plain is not None:
                    a, keys = a + [plain(LX), plain(RX)], keys + [("pl",), ("pr",)]
                a, w = cat(a, axis=1), (lambda: cat([rhs(2, kk) for kk in keys], axis=0))
                if plain is not None and e == CB:
                    return cat([bg.dot(a[r:r + HB].astype(BF16), w()) for r in (0, HB)], axis=0)
                return bg.dot(a.astype(BF16), w())

            for i in range(NL):
                ls = lanes[i]
                last = i == NL - 1
                both = dot([("D2", i), ("D3", i), ("d2", i), ("d3", i)])
                p = both + dot([("D1", i), ("d1", i)], hx if last else None)
                q = both + dot([("D4", i), ("d4", i)], hy if last else None)
                if i > 0:
                    p, q = p + gs_ref[run(0), ls], q + gs_ref[run(1), ls]
                for j in range(i + 1, NL):
                    a = dot([("E1", i, j), ("e1", i, j)])
                    c3 = dot([("E3", i, j), ("E3", j, i), ("e3", i, j)])
                    rq = a - c3
                    gs_ref[run(1), lanes[j]] = rq + gs_ref[run(1), lanes[j]] if i > 0 else rq
                    b = dot([("E1", j, i)])
                    c2 = dot([("E2", i, j), ("E2", j, i), ("e2", i, j)])
                    rp = b + c2
                    gs_ref[run(0), lanes[j]] = rp + gs_ref[run(0), lanes[j]] if i > 0 else rp
                    p, q = (p + a) - c2, (q + c3) + b
                assert not check[0] or ('gb', i) in done
                for b, dn in enumerate((p, q)):
                    ob[run(b), ls] = (x1_src[run(b, i * TM), :] + _rep(mod_ref[4, :, ls], e) * dn).astype(BF16)
                if after is not None and r0 + e == CB:
                    after(i)

    x1s = [x1_ref.at[r] for r in range(NS)]
    sts = [st_ref.at[r * TM:(r + 1) * TM] for r in range(2)]

    def setup():
        for cp in small:
            cp.wait()
        shk = shk_ref[...].astype(F32)
        for a in range(4):
            sh_ref[a] = jnp.broadcast_to(shk[a:a + 1, :], (8, D))
        c = c_ref[...].astype(F32)
        sc_ref[...] = _pk(jnp.broadcast_to(c * jax.nn.sigmoid(c), (16, D)))
        src = lax.broadcasted_iota(I32, (CB, CB), 0)
        dst = lax.broadcasted_iota(I32, (CB, CB), 1)
        perm = jnp.where(src == (dst & -16) + 2 * (dst & 7) + ((dst >> 3) & 1), 1.0, 0.0).astype(BF16)
        fwp = jnp.dot(fwd_ref[...], perm, preferred_element_type=F32)
        fwp_ref[:, 0:CB] = _pk(fwp[:CB])
        fwp_ref[:, CB:2 * CB] = _pk(fwp[CB:])
        zm_ref[...] = pltpu.bitcast(inv_ref[CB:CB + 16, :], I32)
        zs.append(zm_ref[0, 0])

    def prologue():
        ytile = lambda i: ystatic_pieces(y_first, False, [p for p in positions if p[1] == lanes[i]])
        ssm_cp(0).wait()
        k_fwd(0)
        for t in range(2):
            k_cp(t).wait()
            v_cp(t).wait()
            now(kv_pieces(t, 64))
            u_fwd(t)
        bg.flush()
        for i in range(1, NL):
            if i != 3:
                ssm_cp(i).wait()
            if i == 2:
                ssm_cp(3).wait()
            bg.add(ytile(i - 1), 0, 1024)
            k_fwd(i)
            bg.flush()
        q_cp(0).wait()
        now(ytile(NL - 1))
        q_cp(1).wait()
        mod_cp(0).wait()
        mod_chunk(0)
        for t in range(2):
            now(post_pieces(t))
            now(ln1_pieces(t))
            y_inv(t, x1s[t])
        for t in range(2):
            now(ln2_stat_pieces(x1s[t], sts[t]))
        bg.flush()

    def superstep():
        g_main = [g for m in range(NL) for g in g_cols(m)] + g_rows
        mod_cp(1).wait()
        mod_chunk(1)
        now(norm_pieces(x1s[0], sts[0], 0, more=False))
        bg.flush()
        g_cp(0).wait()
        bg.add(norm_pieces(x1s[1], sts[1], 1), 0, 480)
        bg.add(w_pieces(0, g_left), 640, 1150)
        for u in range(2):
            gu_plain(0, LX, u)
            gu_plain(0, RX, u)
        bg.flush()
        u_cp(0).wait()
        g_cp(1).wait()
        prs, np0 = pair_pieces(0), 30
        bg.add(pair_pieces(1) + w_pieces(1, g_left) + w_pieces(0, g_cols(0))
               + norm_pieces(x1s[0], sts[0], 0, base=False) + prs[:np0], 0, 1800)
        for u in range(2):
            gu_plain(1, LX, u)
            gu_plain(1, RX, u)
        gu_plain(0, 2, 0)
        gu_plain(0, 3, 0)
        bg.flush()
        g_cp(2).wait()
        npr = 80
        bg.add(w_pieces(0, g_main[len(g_cols(0)):]) + prs[np0:npr], 0, 2450)
        for c in range(4, 12):
            gu_plain(0, c, 0)
        bg.flush()
        u_cp(1).wait()
        bg.add(prs[npr:] + w_pieces(1, g_main), 0, 2450)
        gu_main(0, 1)
        bg.flush()
        k_cp(2).wait()
        v_cp(2).wait()
        q_cp(2).wait()
        ymid = _costed(_group(ystatic_pieces([(s, 4, 6) for s in (4, 5)], True), 2), 35)
        posts = post_pieces(2)
        fr, ny = 2, 120
        bg.add(kv_pieces(2), 0, fr * 512 - 150)
        bg.add(linked(ln1_pieces(2), 6), 850, 1700)
        bg.add(ymid[:ny], fr * 512 + 750, 3100)
        gu_main(1, 0, (fr, lambda: u_fwd(2)))
        bg.flush()
        d_cp.wait()
        order_d = g_left + [g for i in range(NL) for g in (
            [[(d, i)] for d in ("D2", "D3", "D1", "D4")]
            + [g for j in range(i + 1, NL) for g in (g_edge(i, j), g_edge(j, i))])]
        wdp = w_pieces(2, order_d)
        nd = len(wdp) * 89 // 100
        bg.add(wdp[:nd], 0, 2450)
        gu_main(1, 1)
        bg.flush()
        mod_cp(2).wait()
        k_cp(3).wait()
        v_cp(3).wait()
        bg.add(wdp[nd:] + ymid[ny:] + posts + kv_pieces(3, 16), 0, 3300)
        bg.inj = [(100 + 130 * i, gb_tile(i)) for i in range(NL)]
        ffn_down(x1s[0], 0, 0, e=CB)
        y_inv(2, x1s[2])
        bg.flush()
        o_cp(0).start()

    def step(t, carry):
        q_cp(t).wait()

        @pl.when(t + 1 < NS)
        def _():
            k_cp(t + 1).wait()
            v_cp(t + 1).wait()

        x1v = x1_ref.at[pl.ds(t - 2, 3)]
        x1 = x1v.at[2]
        bg.add(linked(ln1_pieces(t), 2), 4000, 8500)
        bg.add(ln2_stat_pieces(x1v.at[1], st_ref), 0, 600)
        bg.add(factor_pieces(x1v.at[1], st_ref, 1), 800, 3100)
        kv_live.update((b, ls.start) for b in range(2) for ls in lanes)
        kvp = kv_pieces(jnp.minimum(t + 1, NS - 1), 32)
        nk = len(kvp) * 60 // 100
        bg.add(kvp[:nk], 3136 + 70, 3136 + 700)
        bg.add(kvp[nk:], 9000, 10200)
        ffn_down(x1v.at[0], t - 2, 1)
        u_fwd(t)
        chain(diag_pieces(t, T0 - 1), 2)
        chain(task_pieces(t, 2), 3)
        dep = chain(task_pieces(t, 1), 3)
        chain(post_pieces(t), 1, 3, dep)
        gu_fast(1)
        y_inv(t, x1)
        bg.flush()
        o_cp(t - 2).start()
        return carry

    def epilogue():
        t = NS - 1
        bg.add(ln2_stat_pieces(x1s[t], st_ref), 0, 500)
        bg.add(factor_pieces(x1s[t], st_ref, 1), 700, 2900)
        ffn_down(x1s[t - 1], t - 1, 1)
        o_cp(t - 1).start()
        gu_fast(1)
        cols = [(0 if i == 1 else i * 128, (i + 1) * 128) for i in range(1, NL)]
        last = [pltpu.make_async_copy(o_ref.at[rows_of(t), lo:hi], o_hbm.at[rows_of(t), lo:hi], sem.at[s_o + t + i])
                for i, (lo, hi) in enumerate(cols)]
        ffn_down(x1s[t], t, 1, after=lambda i: i > 0 and last[i - 1].start(), e=CB)
        for i in range(NS - 1):
            o_cp(i).wait()
        for cp in last:
            cp.wait()

    def everything(i, carry):
        prologue()
        superstep()
        lax.fori_loop(T0, NS, step, 0)
        epilogue()
        return carry

    setup()
    lax.fori_loop(0, zs[0] + 1, everything, 0)


@jax.jit
def pallas_adaLN_cond__ssm_conv_h3__glu_gated_bilinear__prompt_kernel(
    A_q, A_k, A_v, A_shift_k, A_ssm_k, A_ssm_D, B_x, B_w_gate, B_w_up, B_w_down, c, w_mod,
):
    B, S, D = A_q.shape
    Fh = B_w_gate.shape[1]
    NB = S // CB
    NS = S // TM
    fwd, inv = _dft_consts()
    anyspec = pl.BlockSpec(memory_space=pl.ANY)
    V = pltpu.VMEM
    out = pl.pallas_call(
        functools.partial(_kernel, S=S, D=D, Fh=Fh),
        in_specs=[anyspec] * 13,
        out_specs=anyspec,
        out_shape=jax.ShapeDtypeStruct((S, D), A_q.dtype),
        scratch_shapes=[
            V((NS, 2, 3 * CB, D), F32),
            V((NB, 3 * CB, D), F32),
            V((NS, 2, 3 * CB, D), F32),
            V((NS, (D // 128) * TM, 128), F32),
            V((S, D), BF16), V((S, D), BF16), V((S, D), BF16), V((S, D), BF16),
            V((TM, D), F32),
            V((2 * TM, 256), F32),
            V((2 * TM, Fh), F32),
            V((TM, Fh), F32),
            V((TM, D), F32),
            V((55 * HB, 256), U32),
            V((TM // 2, D), U32),
            V((2 * CB, D), U32),
            V((48 * HB, 256), U32), V((48 * HB, 256), U32), V((48 * HB, 256), U32),
            V((D, S), BF16), V((D, 6 * D), BF16), V((D, Fh), BF16), V((D, Fh), BF16), V((Fh, D), BF16),
            V((2 * CB, CB), BF16), V((CB + 16, CB), BF16),
            V((5, 8, D), F32), V((4, 8, D), F32), V((8, 128), I32), V((8, D), U32), V((HB, 2 * CB), U32),
            V((4, D), BF16), V((D,), BF16), V((1, D), BF16),
            pltpu.SemaphoreType.DMA((5 + 4 * NS + D // 128 + 3 + 5 + 4,)),
        ],
        compiler_params=pltpu.CompilerParams(
            internal_scratch_in_bytes=48 * 1024,
            disable_semaphore_checks=True,
            disable_bounds_checks=True,
            vmem_limit_bytes=110 * 1024 * 1024),
        name="adaln_h3_glu",
    )(A_q.reshape(S, D), A_k.reshape(S, D), A_v.reshape(S, D), A_shift_k.T, A_ssm_k,
      A_ssm_D, B_w_gate, B_w_up, B_w_down, c, w_mod, fwd, inv)
    return out.reshape(B, S, D)
```

```python
import functools

import numpy as np
import jax
import jax.numpy as jnp
from jax import lax
import jax.experimental.pallas as pl
import jax.experimental.pallas.tpu as pltpu

F32 = jnp.float32
BF16 = jnp.bfloat16
U32 = jnp.uint32
I32 = jnp.int32

CB = 128
HB = CB // 2
TM = 256
FC = 256
EPS = 1e-5


def _dft_consts():
    k = np.arange(CB, dtype=np.float64)[:, None]
    n = np.arange(CB, dtype=np.float64)[None, :]
    th = np.pi * (4.0 * k + 1.0) * n / (2.0 * CB)
    fwd = np.concatenate([np.cos(th), np.sin(th)], axis=0)
    g = np.concatenate([np.cos(th[:HB]), np.sin(th[:HB])], axis=0).T / CB
    inv = np.concatenate([g[0::2], g[1::2]], axis=0)
    return jnp.asarray(fwd, dtype=BF16), jnp.asarray(inv, dtype=BF16)


def _pk(x):
    return pltpu.bitcast(x.astype(BF16), U32)


def _unpk(x):
    return pltpu.bitcast(x, BF16)


def _rep(r, n):
    return r if n == 8 else jnp.concatenate([r] * (n // 8), axis=0)


def _add(x, tok):
    return x if tok is None else x + _rep(tok, x.shape[0])


def _costed(pieces, cost):
    for p in pieces:
        p.cost = cost
    return pieces


def _group(pieces, n):
    def merged(ps):
        def run(tok):
            for p in ps:
                p(tok)
        return run
    return [merged(pieces[i:i + n]) for i in range(0, len(pieces), n)]


class _Sched:
    def __init__(self, token):
        self.token = token
        self.clock = 0.0
        self.q = []
        self.last = None
        self.inj = []

    def add(self, pieces, t0, t1):
        cum = np.cumsum([0.0] + [getattr(p, "cost", 1.0) for p in pieces])
        self.q += [(t0 + (t1 - t0) * cum[i] / cum[-1], i, p) for i, p in enumerate(pieces)]
        self.q.sort(key=lambda e: e[:2])

    def note(self, m, dt):
        rows, cols = m.shape
        tiles = [(slice(r, r + 8), slice(c, c + 128)) for c in range(0, cols, 128) for r in range(0, rows, 8)]
        for i, tl in enumerate(tiles):
            tok = None
            while self.q and self.q[0][0] <= self.clock + dt * (i + 1) / len(tiles):
                if tok is None:
                    tok = self.token(m[tl])
                self.q.pop(0)[2](tok)
        self.clock += dt
        self.last = m[tiles[-1]]
        return m

    def dot(self, a, b):
        if self.inj and self.clock >= self.inj[0][0]:
            self.inj.pop(0)[1]()
        m = jnp.dot(a, b, preferred_element_type=F32)
        return self.note(m, max(a.shape[0], 32) * (a.shape[1] // 128) * (b.shape[1] // 128) / 4)

    def flush(self):
        tok = None if self.last is None or not self.q else self.token(self.last)
        while self.q:
            self.q.pop(0)[2](tok)
        self.clock = 0.0
        self.last = None


def _kernel(q_hbm, k_hbm, v_hbm, shk_hbm, ssmk_hbm, ssmd_hbm, wg_hbm, wu_hbm, wd_hbm,
            c_hbm, wmod_hbm, fwd_hbm, inv_hbm, o_hbm,
            u_ref, kk_ref, y_ref, x1_ref, q_ref, k_ref, v_ref, o_ref,
            hp_ref, st_ref, pp_ref, gs_ref, hn_ref, hf_ref, kv_ref, yb_ref, wgf_ref, wuf_ref, wdf_ref,
            ssmk_ref, wmod_ref, wg_ref, wu_ref, wd_ref, fwd_ref, inv_ref,
            mod_ref, sh_ref, z0_ref, zm_ref, sc_ref, fwp_ref, shk_ref, ssmd_ref, c_ref,
            sem, *, S, D, Fh):
    NB = S // CB
    NS = S // TM
    NL = D // 128
    T0 = 3
    NLOOP = NS - T0
    lanes = [slice(i * 128, (i + 1) * 128) for i in range(NL)]
    cat = jnp.concatenate

    offs = [int(o) for o in np.cumsum([0, 6, NS, NS, NS, NL, 3, 3, 2, 1])]
    s_small, s_q, s_k, s_v, s_ssm, s_mod, s_g, s_u, s_d, s_o = offs

    def rows_of(t):
        return pl.ds(t * TM if isinstance(t, int) else pl.multiple_of(t * TM, TM), TM)

    def rows_cp(src, dst, base, t):
        return pltpu.make_async_copy(src.at[rows_of(t), :], dst.at[rows_of(t), :], sem.at[base + t])

    def cols_cp(src, dst, lo, hi, si):
        return pltpu.make_async_copy(src.at[:, lo:hi], dst.at[:, lo:hi], sem.at[si])

    q_cp = lambda t: rows_cp(q_hbm, q_ref, s_q, t)
    k_cp = lambda t: rows_cp(k_hbm, k_ref, s_k, t)
    v_cp = lambda t: rows_cp(v_hbm, v_ref, s_v, t)
    o_cp = lambda t: rows_cp(o_ref, o_hbm, s_o, t)
    small = [pltpu.make_async_copy(s, d, sem.at[s_small + i]) for i, (s, d) in enumerate(
        [(z0_ref, zm_ref), (fwd_hbm, fwd_ref), (shk_hbm, shk_ref), (ssmd_hbm, ssmd_ref), (inv_hbm, inv_ref), (c_hbm, c_ref)])]
    ssm_cp = lambda i: pltpu.make_async_copy(ssmk_hbm.at[lanes[i], :], ssmk_ref.at[lanes[i], :],
                                             sem.at[s_ssm + i])
    mod_cols = [(0, 3 * D), (3 * D, 5 * D), (5 * D, 6 * D)]
    mod_cp = lambda i: cols_cp(wmod_hbm, wmod_ref, mod_cols[i][0], mod_cols[i][1], s_mod + i)
    g_cp = lambda f: cols_cp(wg_hbm, wg_ref, f * FC, (f + 1) * FC if f < 2 else Fh, s_g + f)
    u_cp = lambda f: cols_cp(wu_hbm, wu_ref, f * FC, (f + 1) * FC if f < 1 else Fh, s_u + f)
    d_cp = pltpu.make_async_copy(wd_hbm, wd_ref, sem.at[s_d])

    order = small + [ssm_cp(0), k_cp(0), v_cp(0), k_cp(1), v_cp(1),
                     ssm_cp(1), ssm_cp(2), ssm_cp(3), ssm_cp(4), q_cp(0), q_cp(1),
                     mod_cp(0), mod_cp(1)]
    order += [g_cp(0), u_cp(0), g_cp(1), g_cp(2), u_cp(1)]
    order += [k_cp(2), v_cp(2), q_cp(2), d_cp, mod_cp(2), k_cp(3), v_cp(3)]
    for t in range(T0, NS):
        order += [q_cp(t)]
        if t + 1 < NS:
            order += [k_cp(t + 1), v_cp(t + 1)]
    z0_ref[...] = jnp.zeros((8, 128), I32)
    for cp in order:
        cp.start()

    zs = []
    bg = _Sched(lambda x: pltpu.bitcast(pltpu.bitcast(x, I32) & zm_ref[...], F32))

    def opaque(ref):
        return ref.at[pl.ds(pl.multiple_of(zs[0], 32), ref.shape[0])]

    def chain(pieces, dist, extra=0, dep=None):
        hist = [] if dep is None else [dep] * dist
        for p in pieces:
            tok = None
            if len(hist) >= dist:
                tok = bg.token(hist[-dist])
                for _ in range(extra):
                    tok = tok + tok
            hist.append(p(tok))
        return hist[-1]

    def linked(pieces, d):
        res = []

        def wrap(p):
            def run(tok):
                if d and len(res) >= d:
                    tok = tok + bg.token(res[-d])
                res.append(p(tok))
            return run
        return [wrap(p) for p in pieces]

    def now(pieces):
        for p in pieces:
            p(None)

    def mod_chunk(i):
        lo, hi = mod_cols[i]
        m = bg.dot(_unpk(sc_ref[...]), wmod_ref[:, lo:hi])[0:8]
        if i == 0:
            ga = m[:, 2 * D:3 * D]
            mod_ref[0] = (1.0 + m[:, D:2 * D]) * ga
            mod_ref[1] = m[:, 0:D] * ga
        else:
            mod_ref[2] = 1.0 + m[:, D:2 * D]
            mod_ref[3] = m[:, 0:D]

    def gb_tile(i):
        def run():
            w = wmod_ref[:, 5 * D + i * 128:5 * D + (i + 1) * 128]
            mod_ref[4, :, lanes[i]] = jnp.dot(_unpk(sc_ref[...]), w, preferred_element_type=F32)[0:8]
            done.add(('gb', i))
        return run

    def k_fwd(i):
        ls = lanes[i]
        fwd = fwd_ref[...]
        prev = None
        for m in range(NB):
            kf = lax.dot_general(fwd, ssmk_ref[ls, m * CB:(m + 1) * CB], (((1,), (1,)), ((), ())),
                                 preferred_element_type=F32)
            if m == 0:
                c = kf[:CB] + ssmd_ref[...].astype(F32).reshape(1, D)[:, ls]
                d = kf[CB:]
            else:
                c = kf[:CB] + prev[CB:]
                d = kf[CB:] - prev[:CB]
            prev = kf
            kk_ref[m, 0:CB, ls] = c
            kk_ref[m, CB:2 * CB, ls] = d - c
            kk_ref[m, 2 * CB:3 * CB, ls] = c + d
            if m % 4 == 3:
                bg.note(kf, 2 * CB)

    def lo_hi(w):
        return pltpu.bitcast(w << 16, F32), pltpu.bitcast(w & jnp.uint32(0xFFFF0000), F32)

    kv_live = set()

    def kv_pieces(t, G=32):
        n = G // 2
        kb, vb = k_ref.at[rows_of(t)], v_ref.at[rows_of(t)]

        def piece(ls, r0):
            def run(tok):
                assert (r0 // CB, ls.start) not in kv_live
                if r0 > 0:
                    w = pltpu.bitcast(kb[r0 - 16:r0 + G, ls], U32)
                else:
                    if isinstance(t, int) and t == 0:
                        halo = jnp.zeros((8, 128), U32)
                    else:
                        halo = pltpu.bitcast(k_ref.at[rows_of(t - 1)][TM - 16:TM, ls], U32)
                    w = cat([halo, pltpu.bitcast(kb[0:G, ls], U32)], axis=0)
                if tok is not None:
                    w = w | _rep(pltpu.bitcast(tok, U32), n + 8)
                ke, ko = lo_hi(w[8:])
                ke1, ko1 = lo_hi(pltpu.roll(w, 1, 0)[8:])
                _, ko2 = lo_hi(pltpu.roll(w, 2, 0)[8:])
                s0, s1, s2, s3 = [_rep(sh_ref[a, :, ls], n) for a in range(4)]
                ve, vo = lo_hi(pltpu.bitcast(vb[r0:r0 + G, ls], U32))
                kve = ((ke * s0 + ko1 * s1) + (ke1 * s2 + ko2 * s3)) * ve
                kvo = ((ko * s0 + ke * s1) + (ko1 * s2 + ke1 * s3)) * vo
                kv_ref[r0 // 2:(r0 + G) // 2, ls] = _pk(
                    cat([x[r:r + 8] for r in range(0, n, 8) for x in (kve, kvo)], axis=0))
            return run
        return _costed([piece(ls, r0) for b in range(2) for ls in lanes
                        for r0 in range(b * CB, (b + 1) * CB, G)], 2.5 * G + 10)

    def u_fwd(t):
        for b in range(2):
            for ls in lanes:
                kv = lambda: _unpk(kv_ref[b * HB:(b + 1) * HB, ls])
                a = bg.dot(_unpk(fwp_ref[:, 0:CB]), kv())
                kv2 = kv()
                kv_live.discard((b, ls.start))
                bb = bg.dot(_unpk(fwp_ref[:, CB:2 * CB]), kv2)
                u_ref[t, b, 0:CB, ls] = a + bb
                u_ref[t, b, CB:2 * CB, ls] = a
                u_ref[t, b, 2 * CB:3 * CB, ls] = bb

    positions = [(slice(r0, r0 + 8), ls) for r0 in range(0, 3 * CB, 8) for ls in lanes]

    def ystatic_pieces(blocks, acc_in, pos=None):
        def piece(rs, ls):
            def run(tok):
                us, ks = {}, {}
                for s, lo, hi in blocks:
                    acc = None
                    for i in range(lo, min(hi, s + 1)):
                        if i not in us:
                            us[i] = _add(u_ref[i // 2, i % 2, rs, ls], tok)
                        if s - i not in ks:
                            ks[s - i] = kk_ref[s - i, rs, ls]
                        p = ks[s - i] * us[i]
                        acc = p if acc is None else acc + p
                    if acc_in:
                        acc = acc + y_ref[s // 2, s % 2, rs, ls]
                    y_ref[s // 2, s % 2, rs, ls] = acc
                return acc
            return run
        return _costed([piece(*p) for p in (positions if pos is None else pos)], 35)

    y_first = [(s, 0, 4) for s in range(NB)]

    def task_pieces(t, delta):
        p = t - delta
        left = p >= T0
        J = jnp.where(left, t, p + NLOOP)
        I = jnp.where(left, p, t)
        kview = kk_ref.at[pl.ds(2 * (J - I) - 1, 3)]

        def piece(rs, ls):
            def run(tok):
                u0 = _add(u_ref[I, 0, rs, ls], tok)
                u1 = _add(u_ref[I, 1, rs, ls], tok)
                kc = kview[1, rs, ls]
                y_ref[J, 0, rs, ls] = (kc * u0 + kview[0, rs, ls] * u1) + y_ref[J, 0, rs, ls]
                y1 = (kview[2, rs, ls] * u0 + kc * u1) + y_ref[J, 1, rs, ls]
                y_ref[J, 1, rs, ls] = y1
                return y1
            return run
        return [piece(*p) for p in positions]

    def diag_pieces(t, I):
        kview = kk_ref.at[pl.ds(2 * (t - I) - 1, 3)]

        def piece(rs, ls):
            def run(tok):
                us = [_add(u_ref[a, b, rs, ls], tok) for a in (t, I) for b in range(2)]
                k0 = kk_ref[0, rs, ls]
                kc = kview[1, rs, ls]
                y_ref[t, 0, rs, ls] = ((k0 * us[0] + y_ref[t, 0, rs, ls])
                                       + (kc * us[2] + kview[0, rs, ls] * us[3]))
                y1 = ((kk_ref[1, rs, ls] * us[0] + k0 * us[1])
                      + (kview[2, rs, ls] * us[2] + kc * us[3]) + y_ref[t, 1, rs, ls])
                y_ref[t, 1, rs, ls] = y1
                return y1
            return run
        return [piece(*p) for p in positions]

    def post_pieces(t):
        def piece(b, r0, ls):
            def run(tok):
                comp = lambda c, off: y_ref[t, b, c * CB + off + r0:c * CB + off + r0 + 16, ls]
                k1l, k1h = _add(comp(0, 0), tok), _add(comp(0, HB), tok)
                rel, reh = k1l - comp(2, 0), k1h - comp(2, HB)
                iml, imh = k1l + comp(1, 0), k1h + comp(1, HB)
                p0 = b * CB + r0 // 2
                yb_ref[p0:p0 + 8, ls] = _pk(rel + reh)
                yb_ref[p0 + HB // 2:p0 + HB // 2 + 8, ls] = _pk(iml + imh)
                yb_ref[p0 + HB:p0 + HB + 8, ls] = _pk(rel - reh)
                oim = iml - imh
                yb_ref[p0 + HB + HB // 2:p0 + HB + HB // 2 + 8, ls] = _pk(oim)
                return oim[8:16]
            return run
        return _costed([piece(b, r0, ls) for b in range(2) for r0 in range(0, HB, 16) for ls in lanes], 45)

    def q_split(t, b, p0, n, ls):
        w = pltpu.bitcast(q_ref.at[rows_of(t)][b * CB + 2 * p0:b * CB + 2 * p0 + 2 * n, ls], U32)
        return lo_hi(w)

    def ln_tiles(xs, tok):
        n = xs[0].shape[0]
        s = _add(xs[0], tok)
        for x in xs[1:]:
            s = s + x
        m = jnp.sum(s, axis=-1, keepdims=True) * (1.0 / D)
        xc = [x - m for x in xs]
        s2 = xc[0] * xc[0]
        for x in xc[1:]:
            s2 = s2 + x * x
        r = lax.rsqrt(jnp.sum(s2, axis=-1, keepdims=True) * (1.0 / D) + EPS)
        return xc, jnp.broadcast_to(r, (n, 128)), jnp.broadcast_to(m, (n, 128))

    def ln1_pieces(t):
        G = 8

        def piece(b, p0):
            def run(tok):
                xc, r, _ = ln_tiles([cat(q_split(t, b, p0, G, ls), axis=0) for ls in lanes], tok)
                for ls, x in zip(lanes, xc):
                    h = (x * r) * _rep(mod_ref[0, :, ls], 2 * G) + _rep(mod_ref[1, :, ls], 2 * G)
                    hp_ref[b * CB + p0:b * CB + p0 + G, ls] = h[:G]
                    hp_ref[b * CB + HB + p0:b * CB + HB + p0 + G, ls] = h[G:]
                return functools.reduce(lambda a, c: a + c, [h[r:r + 8] for r in range(0, 2 * G, 8)])
            return run
        return [piece(b, p0) for b in range(2) for p0 in range(0, HB, G)]

    def y_inv(t, x1_dst):
        yb = opaque(yb_ref)
        hp = opaque(hp_ref)
        for b in range(2):
            ye = bg.dot(inv_ref[0:HB, :], _unpk(yb[b * CB:b * CB + HB, :]))
            yo = bg.dot(inv_ref[HB:CB, :], _unpk(yb[b * CB + HB:(b + 1) * CB, :]))
            for ls in lanes:
                qe, qo = q_split(t, b, 0, HB, ls)
                re, ro = slice(b * CB, b * CB + HB), slice(b * CB + HB, (b + 1) * CB)
                x1_dst[pl.ds(2 * ls.start + b * CB, HB, stride=2), :] = qe + hp[re, ls] * ye[:, ls]
                x1_dst[pl.ds(2 * ls.start + b * CB + 1, HB, stride=2), :] = qo + hp[ro, ls] * yo[:, ls]

    def ln2_stat_pieces(x1_src, st):
        x1o = opaque(x1_src)

        def piece(r0):
            def run(tok):
                _, r, m = ln_tiles([x1o[j * TM + r0:j * TM + r0 + 16, :] for j in range(NL)], tok)
                st[r0:r0 + 16, 0:128] = m
                st[r0:r0 + 16, 128:256] = r
                return r[0:8] + r[8:16]
            return run
        return [piece(h * CB + r0) for r0 in range(0, CB, 16) for h in range(2)]

    tile = lambda j: slice(j * 128, (j + 1) * 128)
    LX, RX = 0, 1
    Lc = lambda i: 2 + 2 * i
    RS = 2
    Rc = lambda i: 3 + 2 * ((i - RS) % NL)
    others = lambda i: [j for j in range(NL) if j != i]
    edges = [(i, j) for i in range(NL) for j in others(i)]
    pairs = [(i, j) for i, j in edges if i < j]
    a_idx = {k: n for n, k in enumerate(
        [(c, i) for c in "xyw" for i in range(NL)] + [("s",) + e for e in edges]
        + [(c,) + e for c in ("dx", "dy") for e in pairs])}
    b_terms = {}
    for i in range(NL):
        b_terms["D1", i] = [(1, k, Lc(i)) for k in range(NL)]
        b_terms["D2", i] = [(1, i, Lc(i))] + [(-1, i, Rc(j)) for j in others(i)]
        b_terms["D3", i] = [(1, i, Rc(i))] + [(-1, i, Lc(j)) for j in others(i)]
        b_terms["D4", i] = [(1, k, Rc(i)) for k in range(NL)]
    for i, j in edges:
        sg = 1 if i < j else -1
        b_terms["E1", i, j] = [(1, i, Rc(j)), (1, j, Lc(i))]
        b_terms["E2", i, j] = [(sg, j, Lc(i))]
        b_terms["E3", i, j] = [(sg, i, Rc(j))]
    xpairs = [(0, 1), (2, 3)]
    for i, j in xpairs:
        b_terms["d1", i] = [(1, i, LX), (1, j, LX)]
        b_terms["d2", i] = [(1, i, LX), (-1, i, RX)]
        b_terms["d3", j] = [(1, j, RX), (-1, j, LX)]
        b_terms["d4", j] = [(1, j, RX), (1, i, RX)]
        b_terms["e1", i, j] = [(1, i, RX), (1, j, LX)]
        b_terms["e2", i, j] = [(1, j, LX)]
        b_terms["e3", i, j] = [(1, i, RX)]
    b_terms["pl",] = [(1, NL - 1, LX)]
    b_terms["pr",] = [(1, NL - 1, RX)]
    b_idx = {k: n for n, k in enumerate(b_terms)}
    w_refs = ((wg_ref, wgf_ref), (wu_ref, wuf_ref), (wd_ref, wdf_ref))
    done = set()
    check = [True]

    def norm_pieces(x1_src, st, unit, more=True, base=True):
        G = 16
        x1o = opaque(x1_src)

        def piece(r0, j):
            def run(tok):
                ls = lanes[j]
                two = lambda ref, c: cat([ref[r0:r0 + G, c], ref[CB + r0:CB + r0 + G, c]], axis=0)
                m, r = _add(two(st, slice(0, 128)), tok), two(st, slice(128, 256))
                x = cat([x1o[j * TM + o + r0:j * TM + o + r0 + G, :] for o in (0, CB)], axis=0)
                h = ((x - m) * r) * _rep(mod_ref[2, :, ls], 2 * G) + _rep(mod_ref[3, :, ls], 2 * G)
                if base:
                    put_a(unit, r0, ("x", j), h[:G])
                    put_a(unit, r0, ("y", j), h[G:])
                if more:
                    put_a(unit, r0, ("w", j), h[:G] + h[G:])
                    hn_ref[r0:r0 + G, ls] = h[:G]
                    hn_ref[CB + r0:CB + r0 + G, ls] = h[G:]
            return run
        return _costed([piece(r0, j) for r0 in range(0, CB, G) for j in range(NL)], 44)

    def put_a(unit, r0, key, v):
        p0 = a_idx[key] * HB + r0 // 2
        hf_ref[p0:p0 + v.shape[0] // 2, lanes[unit]] = _pk(v)
        done.add(("a", unit, key, r0))

    def pair_pieces(unit):
        G = 16

        def piece(r0, i, j):
            def run(tok):
                assert ("a", unit, ("w", j), r0) in done
                ld = lambda h, k: hn_ref[h * CB + r0:h * CB + r0 + G, lanes[k]]
                xi, yi, xj, yj = _add(ld(0, i), tok), _add(ld(1, i), tok), ld(0, j), ld(1, j)
                put_a(unit, r0, ("s", i, j), xi + yj)
                put_a(unit, r0, ("s", j, i), xj + yi)
                put_a(unit, r0, ("dx", i, j), xj - xi)
                put_a(unit, r0, ("dy", i, j), yi - yj)
            return run
        return _costed([piece(r0, i, j) for r0 in range(0, CB, G) for i, j in pairs], 30)

    def factor_pieces(x1_src, st, unit):
        nrm, prs = norm_pieces(x1_src, st, unit), pair_pieces(unit)
        a, b = len(nrm) // 8, len(prs) // 8
        return [p for g in range(8) for p in nrm[g * a:(g + 1) * a] + prs[g * b:(g + 1) * b]]

    def w_pieces(w, groups):
        src, dst = w_refs[w]

        def piece(keys, r0, G):
            def run(tok):
                blk = {}

                def ld(k, c):
                    if (k, c) not in blk:
                        rt, ct = (k, c) if w < 2 else (c, k)
                        v = src[rt * 128 + r0:rt * 128 + r0 + G, tile(ct)].astype(F32)
                        blk[k, c] = _add(v, tok) if len(blk) < 2 else v
                    return blk[k, c]
                for key in keys:
                    acc = None
                    for sg, k, c in b_terms[key]:
                        v = ld(k, c)
                        acc = (v if sg > 0 else -v) if acc is None else (acc + v if sg > 0 else acc - v)
                    p0 = (b_idx[key] // 2) * HB + r0 // 2
                    dst[p0:p0 + G // 2, tile(b_idx[key] % 2)] = _pk(acc)
                    done.add(("b", w, key, r0 + G))
            return run
        out = []
        for keys in groups:
            G = 32 if len(keys) in (2, 3) else 16
            n = len({t[1:] for k in keys for t in b_terms[k]})
            out += _costed([piece(keys, r0, G) for r0 in range(0, CB, G)], (3 * n + len(keys) + 2) * G / 8)
        return out

    g_edge = lambda i, j: [("E1", i, j), ("E2", i, j), ("E3", i, j)]
    g_left = [[("e1", i, j), ("e2", i, j), ("e3", i, j), ("d1", i), ("d2", i), ("d3", j), ("d4", j)]
              for i, j in xpairs] + [[("pl",), ("pr",)]]
    g_cols = lambda m: ([[("D1", m)], [("D4", (m + RS) % NL)]]
                        + [g_edge(i, j) for i, j in edges if max(Lc(i), Rc(j)) // 2 == m + 1])
    g_rows = [[(d, i)] for i in range(NL) for d in ("D2", "D3")]

    def rhs(w, key):
        assert not check[0] or ("b", w, key, CB) in done, (w, key)
        return _unpk(w_refs[w][1][(b_idx[key] // 2) * HB:(b_idx[key] // 2 + 1) * HB, tile(b_idx[key] % 2)])

    def lhs(unit, key):
        assert not check[0] or all(("a", unit, key, r) in done for r in range(0, CB, 16)), key
        return _unpk(hf_ref[a_idx[key] * HB:(a_idx[key] + 1) * HB, lanes[unit]])

    def gu_finish(w, unit, c, v):
        assert w == 0 or not check[0] or ("g", unit, c) in done
        done.add(("g", unit, c))
        for h in range(2):
            r = slice(unit * TM + h * CB, unit * TM + (h + 1) * CB)
            pp_ref[r, tile(c)] = v[h] if w == 0 else pp_ref[r, tile(c)] * v[h]

    def gu_plain(w, c, unit):
        x = lambda h: cat([lhs(unit, ("xy"[h], k)) for k in range(NL)], axis=1)
        gu_finish(w, unit, c, [bg.dot(x(h), w_refs[w][0][:, tile(c)]) for h in range(2)])

    def gu_main(w, unit, mid=None):
        dot = lambda a, b: bg.dot(lhs(unit, a), rhs(w, b))
        run_ref, off = (pp_ref, unit * TM) if w == 0 else (gs_ref, 0)
        for i in range(NL):
            if mid is not None and mid[0] == i:
                mid[1]()
            p = q = None
            for d in range(1, NL):
                j = (i + d) % NL
                lo, hi = min(i, j), max(i, j)
                e1 = dot(("s", i, j), ("E1", i, j))
                e2 = dot(("dx", lo, hi), ("E2", i, j))
                e3 = dot(("dy", lo, hi), ("E3", i, j))
                p = e2 if p is None else p + e2
                q = e1 + e3 if q is None else (q + e1) + e3
                rp, rq = e1 + e2, e3
                if d == 1:
                    x = dot(("x", i), ("D1", i))
                    p, q = p + x, q - x
                elif d == 2:
                    q = q + dot(("w", i), ("D2", i))
                elif d == 3:
                    rp = rp + dot(("w", j), ("D3", j))
                else:
                    x = dot(("y", j), ("D4", j))
                    rp, rq = rp - x, rq + x
                rs = [slice(off + h * CB, off + (h + 1) * CB) for h in range(2)]
                if i != others(j)[0]:
                    rp, rq = rp + run_ref[rs[0], tile(Rc(j))], rq + run_ref[rs[1], tile(Rc(j))]
                if i == others(j)[-1]:
                    gu_finish(w, unit, Rc(j), (rp, rq))
                else:
                    run_ref[rs[0], tile(Rc(j))] = rp
                    run_ref[rs[1], tile(Rc(j))] = rq
            gu_finish(w, unit, Lc(i), (p, q))

    def gu_left(w, unit):
        def dot(f, extra=()):
            ks = [f(i, j) for i, j in xpairs] + list(extra)
            return bg.dot(cat([lhs(unit, a) for a, _ in ks], axis=1), cat([rhs(w, b) for _, b in ks], axis=0))
        one = lambda a, b: bg.dot(lhs(unit, (a, NL - 1)), rhs(w, (b,)))
        e1 = dot(lambda i, j: (("s", i, j), ("e1", i, j)))
        e2 = dot(lambda i, j: (("dx", i, j), ("e2", i, j)))
        e3 = dot(lambda i, j: (("dy", i, j), ("e3", i, j)))
        d1 = dot(lambda i, j: (("x", i), ("d1", i)))
        pl_, ql, pr = e2 + d1, (e1 + e3) - d1, e1 + e2
        ql = ql + dot(lambda i, j: (("w", i), ("d2", i)), [(("y", NL - 1), ("pl",))])
        gu_finish(w, unit, LX, (pl_ + one("x", "pl"), ql))
        d4 = dot(lambda i, j: (("y", j), ("d4", j)))
        pr = (pr - d4) + dot(lambda i, j: (("w", j), ("d3", j)), [(("x", NL - 1), ("pr",))])
        gu_finish(w, unit, RX, (pr, (e3 + d4) + one("y", "pr")))

    def gu_fast(unit):
        gu_main(0, unit)
        gu_left(0, unit)
        gu_left(1, unit)
        gu_main(1, unit)

    def ffn_down(x1_src, t, unit, after=None, e=128):
        ob = o_ref.at[rows_of(t)]
        for r0 in range(0, CB, e):
            run = lambda h, base=0: slice(base + h * CB + r0, base + h * CB + r0 + e)
            hx = lambda c: pp_ref[run(0, unit * TM), tile(c)]
            hy = lambda c: pp_ref[run(1, unit * TM), tile(c)]

            def left(key):
                kind = key[0]
                if kind[0] in "Ee":
                    l, r = (Lc(key[1]), Rc(key[2])) if kind[0] == "E" else (LX, RX)
                    return (hy if kind[1] == "3" else hx)(r) + (hx if kind[1] == "2" else hy)(l)
                if kind[1] in "12":
                    c = Lc(key[1]) if kind[0] == "D" else LX
                    return hx(c) - hy(c) if kind[1] == "1" else hy(c)
                c = Rc(key[1]) if kind[0] == "D" else RX
                return hx(c) if kind[1] == "3" else hy(c) - hx(c)

            def dot(keys, plain=None):
                keys = [kk for kk in keys if kk in b_terms]
                a = [left(kk) for kk in keys]
                if plain is not None:
                    a, keys = a + [plain(LX), plain(RX)], keys + [("pl",), ("pr",)]
                a, w = cat(a, axis=1), (lambda: cat([rhs(2, kk) for kk in keys], axis=0))
                if plain is not None and e == CB:
                    return cat([bg.dot(a[r:r + HB].astype(BF16), w()) for r in (0, HB)], axis=0)
                return bg.dot(a.astype(BF16), w())

            for i in range(NL):
                ls = lanes[i]
                last = i == NL - 1
                both = dot([("D2", i), ("D3", i), ("d2", i), ("d3", i)])
                p = both + dot([("D1", i), ("d1", i)], hx if last else None)
                q = both + dot([("D4", i), ("d4", i)], hy if last else None)
                if i > 0:
                    p, q = p + gs_ref[run(0), ls], q + gs_ref[run(1), ls]
                for j in range(i + 1, NL):
                    a = dot([("E1", i, j), ("e1", i, j)])
                    c3 = dot([("E3", i, j), ("E3", j, i), ("e3", i, j)])
                    rq = a - c3
                    gs_ref[run(1), lanes[j]] = rq + gs_ref[run(1), lanes[j]] if i > 0 else rq
                    b = dot([("E1", j, i)])
                    c2 = dot([("E2", i, j), ("E2", j, i), ("e2", i, j)])
                    rp = b + c2
                    gs_ref[run(0), lanes[j]] = rp + gs_ref[run(0), lanes[j]] if i > 0 else rp
                    p, q = (p + a) - c2, (q + c3) + b
                assert not check[0] or ('gb', i) in done
                for b, dn in enumerate((p, q)):
                    ob[run(b), ls] = (x1_src[run(b, i * TM), :] + _rep(mod_ref[4, :, ls], e) * dn).astype(BF16)
                if after is not None and r0 + e == CB:
                    after(i)

    x1s = [x1_ref.at[r] for r in range(NS)]
    sts = [st_ref.at[r * TM:(r + 1) * TM] for r in range(2)]

    def setup():
        for cp in small:
            cp.wait()
        shk = shk_ref[...].astype(F32)
        for a in range(4):
            sh_ref[a] = jnp.broadcast_to(shk[a:a + 1, :], (8, D))
        c = c_ref[...].astype(F32)
        sc_ref[...] = _pk(jnp.broadcast_to(c * jax.nn.sigmoid(c), (16, D)))
        src = lax.broadcasted_iota(I32, (CB, CB), 0)
        dst = lax.broadcasted_iota(I32, (CB, CB), 1)
        perm = jnp.where(src == (dst & -16) + 2 * (dst & 7) + ((dst >> 3) & 1), 1.0, 0.0).astype(BF16)
        fwp = jnp.dot(fwd_ref[...], perm, preferred_element_type=F32)
        fwp_ref[:, 0:CB] = _pk(fwp[:CB])
        fwp_ref[:, CB:2 * CB] = _pk(fwp[CB:])
        zs.append(zm_ref[0, 0])

    def prologue():
        ytile = lambda i: ystatic_pieces(y_first, False, [p for p in positions if p[1] == lanes[i]])
        ssm_cp(0).wait()
        k_fwd(0)
        for t in range(2):
            k_cp(t).wait()
            v_cp(t).wait()
            now(kv_pieces(t, 64))
            u_fwd(t)
        bg.flush()
        for i in range(1, NL):
            if i != 3:
                ssm_cp(i).wait()
            if i == 2:
                ssm_cp(3).wait()
            bg.add(ytile(i - 1), 0, 1024)
            k_fwd(i)
            bg.flush()
        q_cp(0).wait()
        now(ytile(NL - 1))
        q_cp(1).wait()
        mod_cp(0).wait()
        mod_chunk(0)
        for t in range(2):
            now(post_pieces(t))
            now(ln1_pieces(t))
            y_inv(t, x1s[t])
        for t in range(2):
            now(ln2_stat_pieces(x1s[t], sts[t]))
        bg.flush()

    def superstep():
        g_main = [g for m in range(NL) for g in g_cols(m)] + g_rows
        mod_cp(1).wait()
        mod_chunk(1)
        now(norm_pieces(x1s[0], sts[0], 0, more=False))
        bg.flush()
        g_cp(0).wait()
        bg.add(norm_pieces(x1s[1], sts[1], 1), 0, 480)
        bg.add(w_pieces(0, g_left), 640, 1150)
        for u in range(2):
            gu_plain(0, LX, u)
            gu_plain(0, RX, u)
        bg.flush()
        u_cp(0).wait()
        g_cp(1).wait()
        prs, np0 = pair_pieces(0), 30
        bg.add(pair_pieces(1) + w_pieces(1, g_left) + w_pieces(0, g_cols(0))
               + norm_pieces(x1s[0], sts[0], 0, base=False) + prs[:np0], 0, 1800)
        for u in range(2):
            gu_plain(1, LX, u)
            gu_plain(1, RX, u)
        gu_plain(0, 2, 0)
        gu_plain(0, 3, 0)
        bg.flush()
        g_cp(2).wait()
        npr = 80
        bg.add(w_pieces(0, g_main[len(g_cols(0)):]) + prs[np0:npr], 0, 2450)
        for c in range(4, 12):
            gu_plain(0, c, 0)
        bg.flush()
        u_cp(1).wait()
        bg.add(prs[npr:] + w_pieces(1, g_main), 0, 2450)
        gu_main(0, 1)
        bg.flush()
        k_cp(2).wait()
        v_cp(2).wait()
        q_cp(2).wait()
        ymid = _costed(_group(ystatic_pieces([(s, 4, 6) for s in (4, 5)], True), 2), 35)
        posts = post_pieces(2)
        fr, ny = 2, 120
        bg.add(kv_pieces(2), 0, fr * 512 - 150)
        bg.add(linked(ln1_pieces(2), 6), 850, 1700)
        bg.add(ymid[:ny], fr * 512 + 750, 3100)
        gu_main(1, 0, (fr, lambda: u_fwd(2)))
        bg.flush()
        d_cp.wait()
        order_d = g_left + [g for i in range(NL) for g in (
            [[(d, i)] for d in ("D2", "D3", "D1", "D4")]
            + [g for j in range(i + 1, NL) for g in (g_edge(i, j), g_edge(j, i))])]
        wdp = w_pieces(2, order_d)
        nd = len(wdp) * 89 // 100
        bg.add(wdp[:nd], 0, 2450)
        gu_main(1, 1)
        bg.flush()
        mod_cp(2).wait()
        k_cp(3).wait()
        v_cp(3).wait()
        bg.add(wdp[nd:] + ymid[ny:] + posts + kv_pieces(3, 16), 0, 3300)
        bg.inj = [(100 + 130 * i, gb_tile(i)) for i in range(NL)]
        ffn_down(x1s[0], 0, 0, e=CB)
        y_inv(2, x1s[2])
        bg.flush()
        o_cp(0).start()

    def step(t, carry):
        q_cp(t).wait()

        @pl.when(t + 1 < NS)
        def _():
            k_cp(t + 1).wait()
            v_cp(t + 1).wait()

        x1v = x1_ref.at[pl.ds(t - 2, 3)]
        x1 = x1v.at[2]
        bg.add(linked(ln1_pieces(t), 2), 4200, 8800)
        bg.add(ln2_stat_pieces(x1v.at[1], st_ref), 0, 600)
        bg.add(factor_pieces(x1v.at[1], st_ref, 1), 800, 3100)
        kv_live.update((b, ls.start) for b in range(2) for ls in lanes)
        kvp = kv_pieces(jnp.minimum(t + 1, NS - 1), 32)
        nk = len(kvp) * 60 // 100
        bg.add(kvp[:nk], 3136 + 70, 3136 + 700)
        bg.add(kvp[nk:], 9000, 10200)
        ffn_down(x1v.at[0], t - 2, 1)
        u_fwd(t)
        chain(diag_pieces(t, T0 - 1), 2)
        chain(task_pieces(t, 2), 3)
        dep = chain(task_pieces(t, 1), 3)
        chain(post_pieces(t), 1, 3, dep)
        gu_fast(1)
        y_inv(t, x1)
        bg.flush()
        o_cp(t - 2).start()
        return carry

    def epilogue():
        t = NS - 1
        bg.add(ln2_stat_pieces(x1s[t], st_ref), 0, 500)
        bg.add(factor_pieces(x1s[t], st_ref, 1), 700, 2900)
        ffn_down(x1s[t - 1], t - 1, 1)
        o_cp(t - 1).start()
        gu_fast(1)
        cols = [(0 if i == 1 else i * 128, (i + 1) * 128) for i in range(1, NL)]
        last = [pltpu.make_async_copy(o_ref.at[rows_of(t), lo:hi], o_hbm.at[rows_of(t), lo:hi], sem.at[s_o + t + i])
                for i, (lo, hi) in enumerate(cols)]
        ffn_down(x1s[t], t, 1, after=lambda i: i > 0 and last[i - 1].start(), e=CB)
        for i in range(NS - 1):
            o_cp(i).wait()
        for cp in last:
            cp.wait()

    def everything(i, carry):
        prologue()
        superstep()
        lax.fori_loop(T0, NS, step, 0)
        epilogue()
        return carry

    setup()
    lax.fori_loop(0, zs[0] + 1, everything, 0)


@jax.jit
def pallas_adaLN_cond__ssm_conv_h3__glu_gated_bilinear__prompt_kernel(
    A_q, A_k, A_v, A_shift_k, A_ssm_k, A_ssm_D, B_x, B_w_gate, B_w_up, B_w_down, c, w_mod,
):
    B, S, D = A_q.shape
    Fh = B_w_gate.shape[1]
    NB = S // CB
    NS = S // TM
    fwd, inv = _dft_consts()
    anyspec = pl.BlockSpec(memory_space=pl.ANY)
    V = pltpu.VMEM
    out = pl.pallas_call(
        functools.partial(_kernel, S=S, D=D, Fh=Fh),
        in_specs=[anyspec] * 13,
        out_specs=anyspec,
        out_shape=jax.ShapeDtypeStruct((S, D), A_q.dtype),
        scratch_shapes=[
            V((NS, 2, 3 * CB, D), F32),
            V((NB, 3 * CB, D), F32),
            V((NS, 2, 3 * CB, D), F32),
            V((NS, (D // 128) * TM, 128), F32),
            V((S, D), BF16), V((S, D), BF16), V((S, D), BF16), V((S, D), BF16),
            V((TM, D), F32),
            V((2 * TM, 256), F32),
            V((2 * TM, Fh), F32),
            V((TM, Fh), F32),
            V((TM, D), F32),
            V((55 * HB, 256), U32),
            V((TM // 2, D), U32),
            V((2 * CB, D), U32),
            V((48 * HB, 256), U32), V((48 * HB, 256), U32), V((48 * HB, 256), U32),
            V((D, S), BF16), V((D, 6 * D), BF16), V((D, Fh), BF16), V((D, Fh), BF16), V((Fh, D), BF16),
            V((2 * CB, CB), BF16), V((CB, CB), BF16),
            V((5, 8, D), F32), V((4, 8, D), F32), V((8, 128), I32), V((8, 128), I32), V((8, D), U32), V((HB, 2 * CB), U32),
            V((4, D), BF16), V((D,), BF16), V((1, D), BF16),
            pltpu.SemaphoreType.DMA((6 + 4 * NS + D // 128 + 3 + 5 + 4,)),
        ],
        compiler_params=pltpu.CompilerParams(
            internal_scratch_in_bytes=48 * 1024,
            disable_semaphore_checks=True,
            disable_bounds_checks=True,
            vmem_limit_bytes=110 * 1024 * 1024),
        name="adaln_h3_glu",
    )(A_q.reshape(S, D), A_k.reshape(S, D), A_v.reshape(S, D), A_shift_k.T, A_ssm_k,
      A_ssm_D, B_w_gate, B_w_up, B_w_down, c, w_mod, fwd, inv)
    return out.reshape(B, S, D)
```

```python
import functools

import numpy as np
import jax
import jax.numpy as jnp
from jax import lax
import jax.experimental.pallas as pl
import jax.experimental.pallas.tpu as pltpu

F32 = jnp.float32
BF16 = jnp.bfloat16
U32 = jnp.uint32
I32 = jnp.int32

CB = 128
HB = CB // 2
TM = 256
FC = 256
EPS = 1e-5


def _dft_consts():
    k = np.arange(CB, dtype=np.float64)[:, None]
    n = np.arange(CB, dtype=np.float64)[None, :]
    th = np.pi * (4.0 * k + 1.0) * n / (2.0 * CB)
    fwd = np.concatenate([np.cos(th), np.sin(th)], axis=0)
    g = np.concatenate([np.cos(th[:HB]), np.sin(th[:HB])], axis=0).T / CB
    inv = np.concatenate([g[0::2], g[1::2]], axis=0)
    return jnp.asarray(fwd, dtype=BF16), jnp.asarray(inv, dtype=BF16)


def _pk(x):
    return pltpu.bitcast(x.astype(BF16), U32)


def _unpk(x):
    return pltpu.bitcast(x, BF16)


def _rep(r, n):
    return r if n == 8 else jnp.concatenate([r] * (n // 8), axis=0)


def _add(x, tok):
    return x if tok is None else x + _rep(tok, x.shape[0])


def _costed(pieces, cost):
    for p in pieces:
        p.cost = cost
    return pieces


class _Sched:
    def __init__(self, token):
        self.token = token
        self.clock = 0.0
        self.q = []
        self.last = None
        self.inj = []

    def add(self, pieces, t0, t1):
        cum = np.cumsum([0.0] + [getattr(p, "cost", 1.0) for p in pieces])
        self.q += [(t0 + (t1 - t0) * cum[i] / cum[-1], i, p) for i, p in enumerate(pieces)]
        self.q.sort(key=lambda e: e[:2])

    def note(self, m, dt):
        rows, cols = m.shape
        tiles = [(slice(r, r + 8), slice(c, c + 128)) for c in range(0, cols, 128) for r in range(0, rows, 8)]
        for i, tl in enumerate(tiles):
            tok = None
            while self.q and self.q[0][0] <= self.clock + dt * (i + 1) / len(tiles):
                if tok is None:
                    tok = self.token(m[tl])
                self.q.pop(0)[2](tok)
        self.clock += dt
        self.last = m[tiles[-1]]
        return m

    def dot(self, a, b):
        if self.inj and self.clock >= self.inj[0][0]:
            self.inj.pop(0)[1]()
        m = jnp.dot(a, b, preferred_element_type=F32)
        return self.note(m, max(a.shape[0], 32) * (a.shape[1] // 128) * (b.shape[1] // 128) / 4)

    def flush(self):
        tok = None if self.last is None or not self.q else self.token(self.last)
        while self.q:
            self.q.pop(0)[2](tok)
        self.clock = 0.0
        self.last = None


def _kernel(q_hbm, k_hbm, v_hbm, shk_hbm, ssmk_hbm, ssmd_hbm, wg_hbm, wu_hbm, wd_hbm,
            c_hbm, wmod_hbm, fwd_hbm, inv_hbm, o_hbm,
            u_ref, kk_ref, y_ref, x1_ref, q_ref, k_ref, v_ref, o_ref,
            hp_ref, st_ref, pp_ref, gs_ref, hn_ref, hf_ref, kv_ref, yb_ref, wgf_ref, wuf_ref, wdf_ref,
            ssmk_ref, wmod_ref, wg_ref, wu_ref, wd_ref, fwd_ref, inv_ref,
            mod_ref, sh_ref, z0_ref, zm_ref, sc_ref, fwp_ref, shk_ref, ssmd_ref, c_ref,
            sem, *, S, D, Fh):
    NB = S // CB
    NS = S // TM
    NL = D // 128
    T0 = 3
    NLOOP = NS - T0
    lanes = [slice(i * 128, (i + 1) * 128) for i in range(NL)]
    cat = jnp.concatenate

    offs = [int(o) for o in np.cumsum([0, 6, NS, NS, NS, NL, 3, 3, 2, 1])]
    s_small, s_q, s_k, s_v, s_ssm, s_mod, s_g, s_u, s_d, s_o = offs

    def rows_of(t):
        return pl.ds(t * TM if isinstance(t, int) else pl.multiple_of(t * TM, TM), TM)

    def rows_cp(src, dst, base, t):
        return pltpu.make_async_copy(src.at[rows_of(t), :], dst.at[rows_of(t), :], sem.at[base + t])

    def cols_cp(src, dst, lo, hi, si):
        return pltpu.make_async_copy(src.at[:, lo:hi], dst.at[:, lo:hi], sem.at[si])

    q_cp = lambda t: rows_cp(q_hbm, q_ref, s_q, t)
    k_cp = lambda t: rows_cp(k_hbm, k_ref, s_k, t)
    v_cp = lambda t: rows_cp(v_hbm, v_ref, s_v, t)
    o_cp = lambda t: rows_cp(o_ref, o_hbm, s_o, t)
    small = [pltpu.make_async_copy(s, d, sem.at[s_small + i]) for i, (s, d) in enumerate(
        [(z0_ref, zm_ref), (fwd_hbm, fwd_ref), (shk_hbm, shk_ref), (ssmd_hbm, ssmd_ref), (inv_hbm, inv_ref), (c_hbm, c_ref)])]
    ssm_cp = lambda i: pltpu.make_async_copy(ssmk_hbm.at[lanes[i], :], ssmk_ref.at[lanes[i], :],
                                             sem.at[s_ssm + i])
    mod_cols = [(0, 3 * D), (3 * D, 5 * D), (5 * D, 6 * D)]
    mod_cp = lambda i: cols_cp(wmod_hbm, wmod_ref, mod_cols[i][0], mod_cols[i][1], s_mod + i)
    g_cp = lambda f: cols_cp(wg_hbm, wg_ref, f * FC, (f + 1) * FC if f < 2 else Fh, s_g + f)
    u_cp = lambda f: cols_cp(wu_hbm, wu_ref, f * FC, (f + 1) * FC if f < 1 else Fh, s_u + f)
    d_cp = pltpu.make_async_copy(wd_hbm, wd_ref, sem.at[s_d])

    order = small + [ssm_cp(0), k_cp(0), v_cp(0), k_cp(1), v_cp(1),
                     ssm_cp(1), ssm_cp(2), ssm_cp(3), ssm_cp(4), q_cp(0), q_cp(1),
                     mod_cp(0), mod_cp(1)]
    order += [g_cp(0), u_cp(0), g_cp(1), g_cp(2), u_cp(1)]
    order += [k_cp(2), v_cp(2), q_cp(2), d_cp, mod_cp(2), k_cp(3), v_cp(3)]
    for t in range(T0, NS):
        order += [q_cp(t)]
        if t + 1 < NS:
            order += [k_cp(t + 1), v_cp(t + 1)]
    z0_ref[...] = jnp.zeros((8, 128), I32)
    for cp in order:
        cp.start()

    zs = []
    bg = _Sched(lambda x: pltpu.bitcast(pltpu.bitcast(x, I32) & zm_ref[...], F32))

    def opaque(ref):
        return ref.at[pl.ds(pl.multiple_of(zs[0], 32), ref.shape[0])]

    def chain(pieces, dist, extra=0, dep=None):
        hist = [] if dep is None else [dep] * dist
        for p in pieces:
            tok = None
            if len(hist) >= dist:
                tok = bg.token(hist[-dist])
                for _ in range(extra):
                    tok = tok + tok
            hist.append(p(tok))
        return hist[-1]

    def chain_rows(piece, dist):
        hist = []
        for ls in lanes:
            hist.append(piece(slice(0, 8), ls)(bg.token(hist[-dist]) if len(hist) >= dist else None))

        def body(g, hist):
            hist = list(hist)
            for ls in lanes:
                hist.append(piece(pl.ds(pl.multiple_of(g * 8, 8), 8), ls)(bg.token(hist[-dist])))
            return tuple(hist[-dist:])
        return lax.fori_loop(1, 3 * CB // 8, body, tuple(hist[-dist:]), unroll=True)[-1]

    def linked(pieces, d):
        res = []

        def wrap(p):
            def run(tok):
                if d and len(res) >= d:
                    tok = tok + bg.token(res[-d])
                res.append(p(tok))
            return run
        return [wrap(p) for p in pieces]

    def now(pieces):
        for p in pieces:
            p(None)

    def mod_chunk(i):
        lo, hi = mod_cols[i]
        m = bg.dot(_unpk(sc_ref[...]), wmod_ref[:, lo:hi])[0:8]
        if i == 0:
            ga = m[:, 2 * D:3 * D]
            mod_ref[0] = (1.0 + m[:, D:2 * D]) * ga
            mod_ref[1] = m[:, 0:D] * ga
        else:
            mod_ref[2] = 1.0 + m[:, D:2 * D]
            mod_ref[3] = m[:, 0:D]

    def gb_tile(i):
        def run():
            w = wmod_ref[:, 5 * D + i * 128:5 * D + (i + 1) * 128]
            mod_ref[4, :, lanes[i]] = jnp.dot(_unpk(sc_ref[...]), w, preferred_element_type=F32)[0:8]
            done.add(('gb', i))
        return run

    def k_fwd(i):
        ls = lanes[i]
        fwd = fwd_ref[...]
        prev = None
        for m in range(NB):
            kf = lax.dot_general(fwd, ssmk_ref[ls, m * CB:(m + 1) * CB], (((1,), (1,)), ((), ())),
                                 preferred_element_type=F32)
            if m == 0:
                c = kf[:CB] + ssmd_ref[...].astype(F32).reshape(1, D)[:, ls]
                d = kf[CB:]
            else:
                c = kf[:CB] + prev[CB:]
                d = kf[CB:] - prev[:CB]
            prev = kf
            kk_ref[m, 0:CB, ls] = c
            kk_ref[m, CB:2 * CB, ls] = d - c
            kk_ref[m, 2 * CB:3 * CB, ls] = c + d
            if m % 4 == 3:
                bg.note(kf, 2 * CB)

    def lo_hi(w):
        return pltpu.bitcast(w << 16, F32), pltpu.bitcast(w & jnp.uint32(0xFFFF0000), F32)

    kv_live = set()

    def kv_pieces(t, G=32):
        n = G // 2
        kb, vb = k_ref.at[rows_of(t)], v_ref.at[rows_of(t)]

        def piece(ls, r0):
            def run(tok):
                assert (r0 // CB, ls.start) not in kv_live
                if r0 > 0:
                    w = pltpu.bitcast(kb[r0 - 16:r0 + G, ls], U32)
                else:
                    if isinstance(t, int) and t == 0:
                        halo = jnp.zeros((8, 128), U32)
                    else:
                        halo = pltpu.bitcast(k_ref.at[rows_of(t - 1)][TM - 16:TM, ls], U32)
                    w = cat([halo, pltpu.bitcast(kb[0:G, ls], U32)], axis=0)
                if tok is not None:
                    w = w | _rep(pltpu.bitcast(tok, U32), n + 8)
                ke, ko = lo_hi(w[8:])
                ke1, ko1 = lo_hi(pltpu.roll(w, 1, 0)[8:])
                _, ko2 = lo_hi(pltpu.roll(w, 2, 0)[8:])
                s0, s1, s2, s3 = [_rep(sh_ref[a, :, ls], n) for a in range(4)]
                ve, vo = lo_hi(pltpu.bitcast(vb[r0:r0 + G, ls], U32))
                kve = ((ke * s0 + ko1 * s1) + (ke1 * s2 + ko2 * s3)) * ve
                kvo = ((ko * s0 + ke * s1) + (ko1 * s2 + ke1 * s3)) * vo
                kv_ref[r0 // 2:(r0 + G) // 2, ls] = _pk(
                    cat([x[r:r + 8] for r in range(0, n, 8) for x in (kve, kvo)], axis=0))
            return run
        return _costed([piece(ls, r0) for b in range(2) for ls in lanes
                        for r0 in range(b * CB, (b + 1) * CB, G)], 2.5 * G + 10)

    def u_fwd(t):
        for b in range(2):
            for ls in lanes:
                kv = lambda: _unpk(kv_ref[b * HB:(b + 1) * HB, ls])
                a = bg.dot(_unpk(fwp_ref[:, 0:CB]), kv())
                kv2 = kv()
                kv_live.discard((b, ls.start))
                bb = bg.dot(_unpk(fwp_ref[:, CB:2 * CB]), kv2)
                u_ref[t, b, 0:CB, ls] = a + bb
                u_ref[t, b, CB:2 * CB, ls] = a
                u_ref[t, b, 2 * CB:3 * CB, ls] = bb

    def yinit_pieces(ls):
        def piece(rs):
            def run(tok):
                n = 4
                k = kk_ref[:, rs, ls]
                u = [_add(u_ref[i // 2, i % 2, rs, ls], tok) for i in range(4)]
                t = [k[:4 - i] * u[i] for i in range(4)]
                a = t[0][1:] + t[1]
                b = a[1:] + t[2]
                y_ref[0:2, :, rs, ls] = cat([t[0][:1], a[:1], b[:1], b[1:] + t[3]], axis=0).reshape(2, 2, 8, 128)
                for s0 in range(4, NB, n):
                    y = k[s0:s0 + n] * u[0]
                    for i in range(1, 4):
                        y = y + k[s0 - i:s0 - i + n] * u[i]
                    y_ref[s0 // 2:(s0 + n) // 2, :, rs, ls] = y.reshape(n // 2, 2, 8, 128)
            return run
        return [piece(slice(r0, r0 + 8)) for r0 in range(0, 3 * CB, 8)]

    def ydiag_pieces(t):
        def piece(rs, ls):
            def run(tok):
                u0, u1 = _add(u_ref[t, 0, rs, ls], tok), _add(u_ref[t, 1, rs, ls], tok)
                k0 = kk_ref[0, rs, ls]
                y_ref[t, 0, rs, ls] = k0 * u0 + y_ref[t, 0, rs, ls]
                y_ref[t, 1, rs, ls] = (kk_ref[1, rs, ls] * u0 + k0 * u1) + y_ref[t, 1, rs, ls]
            return run
        return _costed([piece(slice(r0, r0 + 16), ls) for r0 in range(0, 3 * CB, 16) for ls in lanes], 35)

    def task_pieces(t, delta):
        p = t - delta
        left = p >= T0
        J = jnp.where(left, t, p + NLOOP)
        I = jnp.where(left, p, t)
        kview = kk_ref.at[pl.ds(2 * (J - I) - 1, 3)]

        def piece(rs, ls):
            def run(tok):
                u0 = _add(u_ref[I, 0, rs, ls], tok)
                u1 = _add(u_ref[I, 1, rs, ls], tok)
                kc = kview[1, rs, ls]
                y_ref[J, 0, rs, ls] = (kc * u0 + kview[0, rs, ls] * u1) + y_ref[J, 0, rs, ls]
                y1 = (kview[2, rs, ls] * u0 + kc * u1) + y_ref[J, 1, rs, ls]
                y_ref[J, 1, rs, ls] = y1
                return y1
            return run
        return piece

    def diag_pieces(t, I):
        kview = kk_ref.at[pl.ds(2 * (t - I) - 1, 3)]

        def piece(rs, ls):
            def run(tok):
                us = [_add(u_ref[a, b, rs, ls], tok) for a in (t, I) for b in range(2)]
                k0 = kk_ref[0, rs, ls]
                kc = kview[1, rs, ls]
                y_ref[t, 0, rs, ls] = ((k0 * us[0] + y_ref[t, 0, rs, ls])
                                       + (kc * us[2] + kview[0, rs, ls] * us[3]))
                y1 = ((kk_ref[1, rs, ls] * us[0] + k0 * us[1])
                      + (kview[2, rs, ls] * us[2] + kc * us[3]) + y_ref[t, 1, rs, ls])
                y_ref[t, 1, rs, ls] = y1
                return y1
            return run
        return piece

    def post_pieces(t):
        def piece(b, r0, ls):
            def run(tok):
                comp = lambda c, off: y_ref[t, b, c * CB + off + r0:c * CB + off + r0 + 16, ls]
                k1l, k1h = _add(comp(0, 0), tok), _add(comp(0, HB), tok)
                rel, reh = k1l - comp(2, 0), k1h - comp(2, HB)
                iml, imh = k1l + comp(1, 0), k1h + comp(1, HB)
                p0 = b * CB + r0 // 2
                yb_ref[p0:p0 + 8, ls] = _pk(rel + reh)
                yb_ref[p0 + HB // 2:p0 + HB // 2 + 8, ls] = _pk(iml + imh)
                yb_ref[p0 + HB:p0 + HB + 8, ls] = _pk(rel - reh)
                oim = iml - imh
                yb_ref[p0 + HB + HB // 2:p0 + HB + HB // 2 + 8, ls] = _pk(oim)
                return oim[8:16]
            return run
        return _costed([piece(b, r0, ls) for b in range(2) for r0 in range(0, HB, 16) for ls in lanes], 45)

    def q_split(t, b, p0, n, ls):
        w = pltpu.bitcast(q_ref.at[rows_of(t)][b * CB + 2 * p0:b * CB + 2 * p0 + 2 * n, ls], U32)
        return lo_hi(w)

    def ln_tiles(xs, tok):
        n = xs[0].shape[0]
        s = _add(xs[0], tok)
        for x in xs[1:]:
            s = s + x
        m = jnp.sum(s, axis=-1, keepdims=True) * (1.0 / D)
        xc = [x - m for x in xs]
        s2 = xc[0] * xc[0]
        for x in xc[1:]:
            s2 = s2 + x * x
        r = lax.rsqrt(jnp.sum(s2, axis=-1, keepdims=True) * (1.0 / D) + EPS)
        return xc, jnp.broadcast_to(r, (n, 128)), jnp.broadcast_to(m, (n, 128))

    def ln1_pieces(t):
        G = 8

        def piece(b, p0):
            def run(tok):
                xc, r, _ = ln_tiles([cat(q_split(t, b, p0, G, ls), axis=0) for ls in lanes], tok)
                for ls, x in zip(lanes, xc):
                    h = (x * r) * _rep(mod_ref[0, :, ls], 2 * G) + _rep(mod_ref[1, :, ls], 2 * G)
                    hp_ref[b * CB + p0:b * CB + p0 + G, ls] = h[:G]
                    hp_ref[b * CB + HB + p0:b * CB + HB + p0 + G, ls] = h[G:]
                return functools.reduce(lambda a, c: a + c, [h[r:r + 8] for r in range(0, 2 * G, 8)])
            return run
        return [piece(b, p0) for b in range(2) for p0 in range(0, HB, G)]

    def y_inv(t, x1_dst):
        yb = opaque(yb_ref)
        hp = opaque(hp_ref)
        for b in range(2):
            ye = bg.dot(inv_ref[0:HB, :], _unpk(yb[b * CB:b * CB + HB, :]))
            yo = bg.dot(inv_ref[HB:CB, :], _unpk(yb[b * CB + HB:(b + 1) * CB, :]))
            for ls in lanes:
                qe, qo = q_split(t, b, 0, HB, ls)
                re, ro = slice(b * CB, b * CB + HB), slice(b * CB + HB, (b + 1) * CB)
                x1_dst[pl.ds(2 * ls.start + b * CB, HB, stride=2), :] = qe + hp[re, ls] * ye[:, ls]
                x1_dst[pl.ds(2 * ls.start + b * CB + 1, HB, stride=2), :] = qo + hp[ro, ls] * yo[:, ls]

    def ln2_stat_pieces(x1_src, st):
        x1o = opaque(x1_src)

        def piece(r0):
            def run(tok):
                _, r, m = ln_tiles([x1o[j * TM + r0:j * TM + r0 + 16, :] for j in range(NL)], tok)
                st[r0:r0 + 16, 0:128] = m
                st[r0:r0 + 16, 128:256] = r
                return r[0:8] + r[8:16]
            return run
        return [piece(h * CB + r0) for r0 in range(0, CB, 16) for h in range(2)]

    tile = lambda j: slice(j * 128, (j + 1) * 128)
    LX, RX = 0, 1
    Lc = lambda i: 2 + 2 * i
    RS = 2
    Rc = lambda i: 3 + 2 * ((i - RS) % NL)
    others = lambda i: [j for j in range(NL) if j != i]
    edges = [(i, j) for i in range(NL) for j in others(i)]
    pairs = [(i, j) for i, j in edges if i < j]
    a_idx = {k: n for n, k in enumerate(
        [(c, i) for c in "xyw" for i in range(NL)] + [("s",) + e for e in edges]
        + [(c,) + e for c in ("dx", "dy") for e in pairs])}
    b_terms = {}
    for i in range(NL):
        b_terms["D1", i] = [(1, k, Lc(i)) for k in range(NL)]
        b_terms["D2", i] = [(1, i, Lc(i))] + [(-1, i, Rc(j)) for j in others(i)]
        b_terms["D3", i] = [(1, i, Rc(i))] + [(-1, i, Lc(j)) for j in others(i)]
        b_terms["D4", i] = [(1, k, Rc(i)) for k in range(NL)]
    for i, j in edges:
        sg = 1 if i < j else -1
        b_terms["E1", i, j] = [(1, i, Rc(j)), (1, j, Lc(i))]
        b_terms["E2", i, j] = [(sg, j, Lc(i))]
        b_terms["E3", i, j] = [(sg, i, Rc(j))]
    xpairs = [(0, 1), (2, 3)]
    for i, j in xpairs:
        b_terms["d1", i] = [(1, i, LX), (1, j, LX)]
        b_terms["d2", i] = [(1, i, LX), (-1, i, RX)]
        b_terms["d3", j] = [(1, j, RX), (-1, j, LX)]
        b_terms["d4", j] = [(1, j, RX), (1, i, RX)]
        b_terms["e1", i, j] = [(1, i, RX), (1, j, LX)]
        b_terms["e2", i, j] = [(1, j, LX)]
        b_terms["e3", i, j] = [(1, i, RX)]
    b_terms["pl",] = [(1, NL - 1, LX)]
    b_terms["pr",] = [(1, NL - 1, RX)]
    b_idx = {k: n for n, k in enumerate(b_terms)}
    w_refs = ((wg_ref, wgf_ref), (wu_ref, wuf_ref), (wd_ref, wdf_ref))
    done = set()
    check = [True]

    def norm_pieces(x1_src, st, unit, more=True, base=True):
        G = 16
        x1o = opaque(x1_src)

        def piece(r0, j):
            def run(tok):
                ls = lanes[j]
                two = lambda ref, c: cat([ref[r0:r0 + G, c], ref[CB + r0:CB + r0 + G, c]], axis=0)
                m, r = _add(two(st, slice(0, 128)), tok), two(st, slice(128, 256))
                x = cat([x1o[j * TM + o + r0:j * TM + o + r0 + G, :] for o in (0, CB)], axis=0)
                h = ((x - m) * r) * _rep(mod_ref[2, :, ls], 2 * G) + _rep(mod_ref[3, :, ls], 2 * G)
                if base:
                    put_a(unit, r0, ("x", j), h[:G])
                    put_a(unit, r0, ("y", j), h[G:])
                if more:
                    put_a(unit, r0, ("w", j), h[:G] + h[G:])
                    hn_ref[r0:r0 + G, ls] = h[:G]
                    hn_ref[CB + r0:CB + r0 + G, ls] = h[G:]
            return run
        return _costed([piece(r0, j) for r0 in range(0, CB, G) for j in range(NL)], 44)

    def put_a(unit, r0, key, v):
        p0 = a_idx[key] * HB + r0 // 2
        hf_ref[p0:p0 + v.shape[0] // 2, lanes[unit]] = _pk(v)
        done.add(("a", unit, key, r0))

    def pair_pieces(unit):
        G = 16

        def piece(r0, i, j):
            def run(tok):
                assert ("a", unit, ("w", j), r0) in done
                ld = lambda h, k: hn_ref[h * CB + r0:h * CB + r0 + G, lanes[k]]
                xi, yi, xj, yj = _add(ld(0, i), tok), _add(ld(1, i), tok), ld(0, j), ld(1, j)
                put_a(unit, r0, ("s", i, j), xi + yj)
                put_a(unit, r0, ("s", j, i), xj + yi)
                put_a(unit, r0, ("dx", i, j), xj - xi)
                put_a(unit, r0, ("dy", i, j), yi - yj)
            return run
        return _costed([piece(r0, i, j) for r0 in range(0, CB, G) for i, j in pairs], 30)

    def factor_pieces(x1_src, st, unit):
        nrm, prs = norm_pieces(x1_src, st, unit), pair_pieces(unit)
        a, b = len(nrm) // 8, len(prs) // 8
        return [p for g in range(8) for p in nrm[g * a:(g + 1) * a] + prs[g * b:(g + 1) * b]]

    def w_pieces(w, groups):
        src, dst = w_refs[w]

        def piece(keys, r0, G):
            def run(tok):
                blk = {}

                def ld(k, c):
                    if (k, c) not in blk:
                        rt, ct = (k, c) if w < 2 else (c, k)
                        v = src[rt * 128 + r0:rt * 128 + r0 + G, tile(ct)].astype(F32)
                        blk[k, c] = _add(v, tok) if len(blk) < 2 else v
                    return blk[k, c]
                for key in keys:
                    acc = None
                    for sg, k, c in b_terms[key]:
                        v = ld(k, c)
                        acc = (v if sg > 0 else -v) if acc is None else (acc + v if sg > 0 else acc - v)
                    p0 = (b_idx[key] // 2) * HB + r0 // 2
                    dst[p0:p0 + G // 2, tile(b_idx[key] % 2)] = _pk(acc)
                    done.add(("b", w, key, r0 + G))
            return run
        out = []
        for keys in groups:
            G = 32 if len(keys) in (2, 3) else 16
            n = len({t[1:] for k in keys for t in b_terms[k]})
            out += _costed([piece(keys, r0, G) for r0 in range(0, CB, G)], (3 * n + len(keys) + 2) * G / 8)
        return out

    g_edge = lambda i, j: [("E1", i, j), ("E2", i, j), ("E3", i, j)]
    g_left = [[("e1", i, j), ("e2", i, j), ("e3", i, j), ("d1", i), ("d2", i), ("d3", j), ("d4", j)]
              for i, j in xpairs] + [[("pl",), ("pr",)]]
    g_cols = lambda m: ([[("D1", m)], [("D4", (m + RS) % NL)]]
                        + [g_edge(i, j) for i, j in edges if max(Lc(i), Rc(j)) // 2 == m + 1])
    g_rows = [[(d, i)] for i in range(NL) for d in ("D2", "D3")]

    def rhs(w, key):
        assert not check[0] or ("b", w, key, CB) in done, (w, key)
        return _unpk(w_refs[w][1][(b_idx[key] // 2) * HB:(b_idx[key] // 2 + 1) * HB, tile(b_idx[key] % 2)])

    def lhs(unit, key):
        assert not check[0] or all(("a", unit, key, r) in done for r in range(0, CB, 16)), key
        return _unpk(hf_ref[a_idx[key] * HB:(a_idx[key] + 1) * HB, lanes[unit]])

    def gu_finish(w, unit, c, v):
        assert w == 0 or not check[0] or ("g", unit, c) in done
        done.add(("g", unit, c))
        for h in range(2):
            r = slice(unit * TM + h * CB, unit * TM + (h + 1) * CB)
            pp_ref[r, tile(c)] = v[h] if w == 0 else pp_ref[r, tile(c)] * v[h]

    def gu_plain(w, c, unit):
        x = lambda h: cat([lhs(unit, ("xy"[h], k)) for k in range(NL)], axis=1)
        gu_finish(w, unit, c, [bg.dot(x(h), w_refs[w][0][:, tile(c)]) for h in range(2)])

    def gu_main(w, unit, mid=None):
        dot = lambda a, b: bg.dot(lhs(unit, a), rhs(w, b))
        run_ref, off = (pp_ref, unit * TM) if w == 0 else (gs_ref, 0)
        for i in range(NL):
            if mid is not None and mid[0] == i:
                mid[1]()
            p = q = None
            for d in range(1, NL):
                j = (i + d) % NL
                lo, hi = min(i, j), max(i, j)
                e1 = dot(("s", i, j), ("E1", i, j))
                e2 = dot(("dx", lo, hi), ("E2", i, j))
                e3 = dot(("dy", lo, hi), ("E3", i, j))
                p = e2 if p is None else p + e2
                q = e1 + e3 if q is None else (q + e1) + e3
                rp, rq = e1 + e2, e3
                if d == 1:
                    x = dot(("x", i), ("D1", i))
                    p, q = p + x, q - x
                elif d == 2:
                    q = q + dot(("w", i), ("D2", i))
                elif d == 3:
                    rp = rp + dot(("w", j), ("D3", j))
                else:
                    x = dot(("y", j), ("D4", j))
                    rp, rq = rp - x, rq + x
                rs = [slice(off + h * CB, off + (h + 1) * CB) for h in range(2)]
                if i != others(j)[0]:
                    rp, rq = rp + run_ref[rs[0], tile(Rc(j))], rq + run_ref[rs[1], tile(Rc(j))]
                if i == others(j)[-1]:
                    gu_finish(w, unit, Rc(j), (rp, rq))
                else:
                    run_ref[rs[0], tile(Rc(j))] = rp
                    run_ref[rs[1], tile(Rc(j))] = rq
            gu_finish(w, unit, Lc(i), (p, q))

    def gu_left(w, unit):
        def dot(f, extra=()):
            ks = [f(i, j) for i, j in xpairs] + list(extra)
            return bg.dot(cat([lhs(unit, a) for a, _ in ks], axis=1), cat([rhs(w, b) for _, b in ks], axis=0))
        one = lambda a, b: bg.dot(lhs(unit, (a, NL - 1)), rhs(w, (b,)))
        e1 = dot(lambda i, j: (("s", i, j), ("e1", i, j)))
        e2 = dot(lambda i, j: (("dx", i, j), ("e2", i, j)))
        e3 = dot(lambda i, j: (("dy", i, j), ("e3", i, j)))
        d1 = dot(lambda i, j: (("x", i), ("d1", i)))
        pl_, ql, pr = e2 + d1, (e1 + e3) - d1, e1 + e2
        ql = ql + dot(lambda i, j: (("w", i), ("d2", i)), [(("y", NL - 1), ("pl",))])
        gu_finish(w, unit, LX, (pl_ + one("x", "pl"), ql))
        d4 = dot(lambda i, j: (("y", j), ("d4", j)))
        pr = (pr - d4) + dot(lambda i, j: (("w", j), ("d3", j)), [(("x", NL - 1), ("pr",))])
        gu_finish(w, unit, RX, (pr, (e3 + d4) + one("y", "pr")))

    def gu_fast(unit):
        gu_main(0, unit)
        gu_left(0, unit)
        gu_left(1, unit)
        gu_main(1, unit)

    def ffn_down(x1_src, t, unit, after=None, e=128):
        ob = o_ref.at[rows_of(t)]
        for r0 in range(0, CB, e):
            run = lambda h, base=0: slice(base + h * CB + r0, base + h * CB + r0 + e)
            hx = lambda c: pp_ref[run(0, unit * TM), tile(c)]
            hy = lambda c: pp_ref[run(1, unit * TM), tile(c)]

            def left(key):
                kind = key[0]
                if kind[0] in "Ee":
                    l, r = (Lc(key[1]), Rc(key[2])) if kind[0] == "E" else (LX, RX)
                    return (hy if kind[1] == "3" else hx)(r) + (hx if kind[1] == "2" else hy)(l)
                if kind[1] in "12":
                    c = Lc(key[1]) if kind[0] == "D" else LX
                    return hx(c) - hy(c) if kind[1] == "1" else hy(c)
                c = Rc(key[1]) if kind[0] == "D" else RX
                return hx(c) if kind[1] == "3" else hy(c) - hx(c)

            def dot(keys, plain=None):
                keys = [kk for kk in keys if kk in b_terms]
                a = [left(kk) for kk in keys]
                if plain is not None:
                    a, keys = a + [plain(LX), plain(RX)], keys + [("pl",), ("pr",)]
                a, w = cat(a, axis=1), (lambda: cat([rhs(2, kk) for kk in keys], axis=0))
                if plain is not None and e == CB:
                    return cat([bg.dot(a[r:r + HB].astype(BF16), w()) for r in (0, HB)], axis=0)
                return bg.dot(a.astype(BF16), w())

            for i in range(NL):
                ls = lanes[i]
                last = i == NL - 1
                both = dot([("D2", i), ("D3", i), ("d2", i), ("d3", i)])
                p = both + dot([("D1", i), ("d1", i)], hx if last else None)
                q = both + dot([("D4", i), ("d4", i)], hy if last else None)
                if i > 0:
                    p, q = p + gs_ref[run(0), ls], q + gs_ref[run(1), ls]
                for j in range(i + 1, NL):
                    a = dot([("E1", i, j), ("e1", i, j)])
                    c3 = dot([("E3", i, j), ("E3", j, i), ("e3", i, j)])
                    rq = a - c3
                    gs_ref[run(1), lanes[j]] = rq + gs_ref[run(1), lanes[j]] if i > 0 else rq
                    b = dot([("E1", j, i)])
                    c2 = dot([("E2", i, j), ("E2", j, i), ("e2", i, j)])
                    rp = b + c2
                    gs_ref[run(0), lanes[j]] = rp + gs_ref[run(0), lanes[j]] if i > 0 else rp
                    p, q = (p + a) - c2, (q + c3) + b
                assert not check[0] or ('gb', i) in done
                for b, dn in enumerate((p, q)):
                    ob[run(b), ls] = (x1_src[run(b, i * TM), :] + _rep(mod_ref[4, :, ls], e) * dn).astype(BF16)
                if after is not None and r0 + e == CB:
                    after(i)

    x1s = [x1_ref.at[r] for r in range(NS)]
    sts = [st_ref.at[r * TM:(r + 1) * TM] for r in range(2)]

    def setup():
        for cp in small:
            cp.wait()
        shk = shk_ref[...].astype(F32)
        for a in range(4):
            sh_ref[a] = jnp.broadcast_to(shk[a:a + 1, :], (8, D))
        c = c_ref[...].astype(F32)
        sc_ref[...] = _pk(jnp.broadcast_to(c * jax.nn.sigmoid(c), (16, D)))
        src = lax.broadcasted_iota(I32, (CB, CB), 0)
        dst = lax.broadcasted_iota(I32, (CB, CB), 1)
        perm = jnp.where(src == (dst & -16) + 2 * (dst & 7) + ((dst >> 3) & 1), 1.0, 0.0).astype(BF16)
        fwp = jnp.dot(fwd_ref[...], perm, preferred_element_type=F32)
        fwp_ref[:, 0:CB] = _pk(fwp[:CB])
        fwp_ref[:, CB:2 * CB] = _pk(fwp[CB:])
        zs.append(zm_ref[0, 0])

    def prologue():
        ssm_cp(0).wait()
        k_fwd(0)
        for t in range(2):
            k_cp(t).wait()
            v_cp(t).wait()
            now(kv_pieces(t, 64))
            u_fwd(t)
        bg.flush()
        for i in range(1, NL):
            if i != 3:
                ssm_cp(i).wait()
            if i == 2:
                ssm_cp(3).wait()
            bg.add(yinit_pieces(lanes[i - 1]), 0, 1024)
            k_fwd(i)
            bg.flush()
        q_cp(0).wait()
        now(yinit_pieces(lanes[NL - 1]))
        q_cp(1).wait()
        mod_cp(0).wait()
        mod_chunk(0)
        for t in range(2):
            now(post_pieces(t))
            now(ln1_pieces(t))
            y_inv(t, x1s[t])
        for t in range(2):
            now(ln2_stat_pieces(x1s[t], sts[t]))
        bg.flush()

    def superstep():
        g_main = [g for m in range(NL) for g in g_cols(m)] + g_rows
        mod_cp(1).wait()
        mod_chunk(1)
        now(norm_pieces(x1s[0], sts[0], 0, more=False))
        bg.flush()
        g_cp(0).wait()
        bg.add(norm_pieces(x1s[1], sts[1], 1), 0, 480)
        bg.add(w_pieces(0, g_left), 640, 1150)
        for u in range(2):
            gu_plain(0, LX, u)
            gu_plain(0, RX, u)
        bg.flush()
        u_cp(0).wait()
        g_cp(1).wait()
        prs, np0 = pair_pieces(0), 30
        bg.add(pair_pieces(1) + w_pieces(1, g_left) + w_pieces(0, g_cols(0))
               + norm_pieces(x1s[0], sts[0], 0, base=False) + prs[:np0], 0, 1800)
        for u in range(2):
            gu_plain(1, LX, u)
            gu_plain(1, RX, u)
        gu_plain(0, 2, 0)
        gu_plain(0, 3, 0)
        bg.flush()
        g_cp(2).wait()
        npr = 80
        bg.add(w_pieces(0, g_main[len(g_cols(0)):]) + prs[np0:npr], 0, 2450)
        for c in range(4, 12):
            gu_plain(0, c, 0)
        bg.flush()
        u_cp(1).wait()
        bg.add(prs[npr:] + w_pieces(1, g_main), 0, 2450)
        gu_main(0, 1)
        bg.flush()
        k_cp(2).wait()
        v_cp(2).wait()
        q_cp(2).wait()
        ymid = ydiag_pieces(2)
        posts = post_pieces(2)
        fr, ny = 2, 90
        bg.add(kv_pieces(2, 32), 0, fr * 512 - 150)
        bg.add(linked(ln1_pieces(2), 6), 850, 1700)
        bg.add(ymid[:ny], fr * 512 + 750, 3100)
        gu_main(1, 0, (fr, lambda: u_fwd(2)))
        bg.flush()
        d_cp.wait()
        order_d = g_left + [g for i in range(NL) for g in (
            [[(d, i)] for d in ("D2", "D3", "D1", "D4")]
            + [g for j in range(i + 1, NL) for g in (g_edge(i, j), g_edge(j, i))])]
        wdp = w_pieces(2, order_d)
        nd = len(wdp) * 89 // 100
        bg.add(wdp[:nd], 0, 2450)
        gu_main(1, 1)
        bg.flush()
        mod_cp(2).wait()
        k_cp(3).wait()
        v_cp(3).wait()
        bg.add(wdp[nd:] + ymid[ny:] + posts + kv_pieces(3, 16), 0, 3300)
        bg.inj = [(100 + 130 * i, gb_tile(i)) for i in range(NL)]
        ffn_down(x1s[0], 0, 0, e=CB)
        y_inv(2, x1s[2])
        bg.flush()
        o_cp(0).start()

    def step(t, carry):
        q_cp(t).wait()

        @pl.when(t + 1 < NS)
        def _():
            k_cp(t + 1).wait()
            v_cp(t + 1).wait()

        x1v = x1_ref.at[pl.ds(t - 2, 3)]
        x1 = x1v.at[2]
        bg.add(linked(ln1_pieces(t), 2), 4200, 8800)
        bg.add(ln2_stat_pieces(x1v.at[1], st_ref), 0, 600)
        bg.add(factor_pieces(x1v.at[1], st_ref, 1), 800, 3100)
        kv_live.update((b, ls.start) for b in range(2) for ls in lanes)
        kvp = kv_pieces(jnp.minimum(t + 1, NS - 1), 32)
        nk = len(kvp) * 60 // 100
        bg.add(kvp[:nk], 3136 + 70, 3136 + 700)
        bg.add(kvp[nk:], 9000, 10200)
        ffn_down(x1v.at[0], t - 2, 1)
        u_fwd(t)
        chain_rows(diag_pieces(t, T0 - 1), 2)
        chain_rows(task_pieces(t, 2), 3)
        dep = chain_rows(task_pieces(t, 1), 3)
        chain(post_pieces(t), 1, 3, dep)
        gu_fast(1)
        y_inv(t, x1)
        bg.flush()
        o_cp(t - 2).start()
        return carry

    def epilogue():
        t = NS - 1
        bg.add(ln2_stat_pieces(x1s[t], st_ref), 0, 500)
        bg.add(factor_pieces(x1s[t], st_ref, 1), 700, 2900)
        ffn_down(x1s[t - 1], t - 1, 1)
        o_cp(t - 1).start()
        gu_fast(1)
        cols = [(0 if i == 1 else i * 128, (i + 1) * 128) for i in range(1, NL)]
        last = [pltpu.make_async_copy(o_ref.at[rows_of(t), lo:hi], o_hbm.at[rows_of(t), lo:hi], sem.at[s_o + t + i])
                for i, (lo, hi) in enumerate(cols)]
        ffn_down(x1s[t], t, 1, after=lambda i: i > 0 and last[i - 1].start(), e=CB)
        for i in range(NS - 1):
            o_cp(i).wait()
        for cp in last:
            cp.wait()

    def everything(i, carry):
        prologue()
        superstep()
        lax.fori_loop(T0, NS, step, 0)
        epilogue()
        return carry

    setup()
    lax.fori_loop(0, zs[0] + 1, everything, 0)


@jax.jit
def pallas_adaLN_cond__ssm_conv_h3__glu_gated_bilinear__prompt_kernel(
    A_q, A_k, A_v, A_shift_k, A_ssm_k, A_ssm_D, B_x, B_w_gate, B_w_up, B_w_down, c, w_mod,
):
    B, S, D = A_q.shape
    Fh = B_w_gate.shape[1]
    NB = S // CB
    NS = S // TM
    fwd, inv = _dft_consts()
    anyspec = pl.BlockSpec(memory_space=pl.ANY)
    V = pltpu.VMEM
    out = pl.pallas_call(
        functools.partial(_kernel, S=S, D=D, Fh=Fh),
        in_specs=[anyspec] * 13,
        out_specs=anyspec,
        out_shape=jax.ShapeDtypeStruct((S, D), A_q.dtype),
        scratch_shapes=[
            V((NS, 2, 3 * CB, D), F32),
            V((NB, 3 * CB, D), F32),
            V((NS, 2, 3 * CB, D), F32),
            V((NS, (D // 128) * TM, 128), F32),
            V((S, D), BF16), V((S, D), BF16), V((S, D), BF16), V((S, D), BF16),
            V((TM, D), F32),
            V((2 * TM, 256), F32),
            V((2 * TM, Fh), F32),
            V((TM, Fh), F32),
            V((TM, D), F32),
            V((55 * HB, 256), U32),
            V((TM // 2, D), U32),
            V((2 * CB, D), U32),
            V((48 * HB, 256), U32), V((48 * HB, 256), U32), V((48 * HB, 256), U32),
            V((D, S), BF16), V((D, 6 * D), BF16), V((D, Fh), BF16), V((D, Fh), BF16), V((Fh, D), BF16),
            V((2 * CB, CB), BF16), V((CB, CB), BF16),
            V((5, 8, D), F32), V((4, 8, D), F32), V((8, 128), I32), V((8, 128), I32), V((8, D), U32), V((HB, 2 * CB), U32),
            V((4, D), BF16), V((D,), BF16), V((1, D), BF16),
            pltpu.SemaphoreType.DMA((6 + 4 * NS + D // 128 + 3 + 5 + 4,)),
        ],
        compiler_params=pltpu.CompilerParams(
            internal_scratch_in_bytes=48 * 1024,
            disable_semaphore_checks=True,
            disable_bounds_checks=True,
            vmem_limit_bytes=110 * 1024 * 1024),
        name="adaln_h3_glu",
    )(A_q.reshape(S, D), A_k.reshape(S, D), A_v.reshape(S, D), A_shift_k.T, A_ssm_k,
      A_ssm_D, B_w_gate, B_w_up, B_w_down, c, w_mod, fwd, inv)
    return out.reshape(B, S, D)
```
